```python
import jax
import jax.numpy as jnp

def _softmax(x, axis=-1):
    return jax.nn.softmax(x, axis=axis)
def _gelu(x):
    return jax.nn.gelu(x, approximate=True)
def _silu(x):
    return jax.nn.silu(x)
def _sigmoid(x):
    return jax.nn.sigmoid(x)
def _layernorm(x, axis=-1, eps=1e-5):
    m = jnp.mean(x, axis=axis, keepdims=True)
    v = jnp.var(x, axis=axis, keepdims=True)
    return (x - m) / jnp.sqrt(v + eps)
def _scatter_add(tgt, idx, src, axis=0):
    return tgt.at[idx].add(src)
def _segment_sum(src, seg, n):
    return jax.ops.segment_sum(src, seg, n)
class _Rng:
    def __init__(self, key):
        self._k = key
    def _next(self):
        self._k, sub = jax.random.split(self._k)
        return sub
    def normal(self, shape):
        return jax.random.normal(self._next(), shape, dtype=jnp.bfloat16)
    def randint(self, lo, hi, shape):
        return jax.random.randint(self._next(), shape, lo, hi, dtype=jnp.int32)
    def uniform(self, shape, lo=0.0, hi=1.0):
        return jax.random.uniform(self._next(), shape, jnp.bfloat16, lo, hi)
    def permutation(self, n):
        return jax.random.permutation(self._next(), n)


kernel_name = 'interleave_layers__sliding_block_cached__moe_arch_mod__decode'

def setup_inputs():
    _rng = _Rng(jax.random.key(int.from_bytes(__import__("os").urandom(4), "little")))
    _w = (lambda a: (lambda t: t.astype(jnp.bfloat16) if jnp.issubdtype(t.dtype, jnp.floating) else t)(jnp.asarray(a)))
    def _A_setup():
        B, Sq, D = 4, 1, 640
        Hq, Hkv, Sk, Dh = 32, 32, 4096, 192
        assert Hq % Hkv == 0, (Hq, Hkv)
        return {
            "x": _w((lambda *s: _rng.normal(s) * 0.05)(B, Sq, D)),
            "k_cache": _w((lambda *s: _rng.normal(s) * 0.05)(B, Hkv, Sk, Dh)),
            "v_cache": _w((lambda *s: _rng.normal(s) * 0.05)(B, Hkv, Sk, Dh)),
            "wq": _w((lambda *s: _rng.normal(s) * 0.05)(D, Hq * Dh) * (D ** -0.5)),
            "wo": _w((lambda *s: _rng.normal(s) * 0.05)(Hq * Dh, D) * ((Hq * Dh) ** -0.5)),
        }
    _A_in = _A_setup()

    def _B_setup():
        B, S, D, F, C = 4, 1, 640, 1536, 1
        return {
            "x": _w((lambda *s: _rng.normal(s) * 0.05)(B, S, D)),
            "w_r": _w((lambda *s: _rng.normal(s) * 0.05)(D)),
            "w_gate": _w((lambda *s: _rng.normal(s) * 0.05)(D, F)),
            "w_up": _w((lambda *s: _rng.normal(s) * 0.05)(D, F)),
            "w_down": _w((lambda *s: _rng.normal(s) * 0.05)(F, D)),
        }
    _B_in = _B_setup()

    return {
        "A_x": _A_in["x"],
        "A_k_cache": _A_in["k_cache"],
        "A_v_cache": _A_in["v_cache"],
        "A_wq": _A_in["wq"],
        "A_wo": _A_in["wo"],
        "B_x": _B_in["x"],
        "B_w_r": _B_in["w_r"],
        "B_w_gate": _B_in["w_gate"],
        "B_w_up": _B_in["w_up"],
        "B_w_down": _B_in["w_down"],
    }

def reference(A_x, A_k_cache, A_v_cache, A_wq, A_wo, B_x, B_w_r, B_w_gate, B_w_up, B_w_down):
    def _A_ref(x, k_cache, v_cache, wq, wo):
        B, Sq, D = x.shape
        Hq, Dh = 32, 192
        Hkv, Sk = k_cache.shape[1], k_cache.shape[2]
        W = min(4096, max(256, Sk // 4))
        rep = Hq // Hkv
        q = (lambda x, *d: x.transpose(*d))((x @ wq).reshape(B, Sq, Hq, Dh), 0, 2, 1, 3)
        k = jnp.repeat(k_cache[:, :, Sk - W:, :], rep, axis=1)
        v = jnp.repeat(v_cache[:, :, Sk - W:, :], rep, axis=1)
        scores = jnp.einsum("bhqd,bhkd->bhqk", q, k) * (Dh ** -0.5)
        p = _softmax(scores, axis=-1)
        o = jnp.einsum("bhqk,bhkd->bhqd", p, v)
        return (lambda x, *d: x.transpose(*d))(o, 0, 2, 1, 3).reshape(B, Sq, Hq * Dh) @ wo

    def _B_ref(x, w_r, w_gate, w_up, w_down):
        B, S, D = x.shape
        C = 1
        r = x @ w_r
        idx = jnp.argsort(-r, axis=-1)[:, :C]
        idx_e = jnp.repeat(idx.reshape(B, C, 1), D, axis=2)
        x_sel = jnp.take_along_axis(x, idx_e, axis=1)
        g = _silu(x_sel @ w_gate)
        u = x_sel @ w_up
        y = (g * u) @ w_down
        r_sel = _sigmoid(jnp.take_along_axis(r, idx, axis=1))
        y = y * r_sel.reshape(B, C, 1)
        b_off = (jnp.arange(B) * S).reshape(B, 1)
        flat_idx = (idx + b_off).reshape(B * C)
        zero = (x * 0.0).reshape(B * S, D)
        upd = _scatter_add(zero, flat_idx, y.reshape(B * C, D), axis=0)
        return x + upd.reshape(B, S, D)

    x = A_x
    x = x + _A_ref(_layernorm(x, axis=-1), A_k_cache, A_v_cache, A_wq, A_wo)
    x = x + _B_ref(_layernorm(x, axis=-1), B_w_r, B_w_gate, B_w_up, B_w_down)
    x = x + _A_ref(_layernorm(x, axis=-1), A_k_cache, A_v_cache, A_wq, A_wo)
    x = x + _B_ref(_layernorm(x, axis=-1), B_w_r, B_w_gate, B_w_up, B_w_down)
    return x
```

```python
import jax
import jax.numpy as jnp
from jax import lax
import jax.experimental.pallas as pl
import jax.experimental.pallas.tpu as pltpu

F32 = jnp.float32
BF16 = jnp.bfloat16

B, D, H, DH, SK, F = 4, 640, 32, 192, 4096, 1536
W = min(4096, max(256, SK // 4))
NP = H // 2
PD = 2 * DH
NT = W // 128
CP = 2
NC = NP // CP
NCH = B * NC
LA = 5
EPS = 1e-5
SCALE = DH ** -0.5


def _rowsum_all(x):
    x = x + pltpu.roll(x, 4, 0)
    x = x + pltpu.roll(x, 2, 0)
    return x + pltpu.roll(x, 1, 0)


def _kernel(x_hbm, kt_hbm, vt_hbm, wq_hbm, wo_hbm, wr_hbm, wg_hbm, wu_hbm, wd_hbm,
            o_ref,
            kbuf, vbuf, wqb, wob, wgub, wdb, xb, wrb, state, ksem, vsem, wsem):

    def k_copies(c):
        b = c // NC
        p0 = (c % NC) * CP
        return [pltpu.make_async_copy(
            kt_hbm.at[b, pl.ds(p0, CP), :, pl.ds(SK - W + t * 128, 128)],
            kbuf.at[b, pl.ds(p0, CP), t], ksem.at[c]) for t in range(NT)]

    def v_copy(c):
        b = c // NC
        p0 = (c % NC) * CP
        return pltpu.make_async_copy(
            vt_hbm.at[b, pl.ds(p0, CP), :, pl.ds(SK - W, W)],
            vbuf.at[b, pl.ds(p0, CP)], vsem.at[c])

    def start_chunk(c):
        for cp in k_copies(c):
            cp.start()
        v_copy(c).start()

    def wait_k(c):
        b = c // NC
        p0 = (c % NC) * CP
        view = kbuf.at[b, pl.ds(p0, CP)]
        pltpu.make_async_copy(view, view, ksem.at[c]).wait()

    def col_copies(src, dst, off, n, sem):
        return [pltpu.make_async_copy(src.at[:, pl.ds(t * 128, 128)], dst.at[off + t], sem)
                for t in range(n)]

    def wait_all(buf, sem):
        pltpu.make_async_copy(buf, buf, sem).wait()

    x_cp = pltpu.make_async_copy(x_hbm, xb, wsem.at[0])
    wr_cp = pltpu.make_async_copy(wr_hbm, wrb, wsem.at[1])
    x_cp.start()
    wr_cp.start()
    for cp in col_copies(wq_hbm, wqb, 0, H * DH // 128, wsem.at[2]):
        cp.start()
    for cp in col_copies(wo_hbm, wob, 0, D // 128, wsem.at[3]):
        cp.start()
    for cp in col_copies(wg_hbm, wgub, 0, F // 128, wsem.at[4]):
        cp.start()
    for cp in col_copies(wu_hbm, wgub, F // 128, F // 128, wsem.at[4]):
        cp.start()
    for cp in col_copies(wd_hbm, wdb, 0, D // 128, wsem.at[5]):
        cp.start()
    for c in range(LA):
        start_chunk(c)

    x_cp.wait()
    wr_cp.wait()
    state[...] = jnp.concatenate([xb[...].astype(F32), jnp.zeros((8 - B, D), F32)], axis=0)
    wait_all(wqb, wsem.at[2])
    wait_all(wob, wsem.at[3])
    wait_all(wgub, wsem.at[4])
    wait_all(wdb, wsem.at[5])

    def layernorm_parts(x):
        m = jnp.sum(x, axis=1, keepdims=True) * (1.0 / D)
        xc = x - m
        v = jnp.sum(xc * xc, axis=1, keepdims=True) * (1.0 / D)
        return xc, lax.rsqrt(v + EPS)

    def qproj(xcb, qscale, k):
        w = jnp.concatenate([wqb[3 * k + i] for i in range(3)], axis=1)
        return jnp.dot(xcb, w, preferred_element_type=F32) * qscale

    def scores(q, b, k):
        lane = lax.broadcasted_iota(jnp.int32, (8, 128), 1)
        q0 = q[:, 0:128].astype(BF16)
        qm = q[:, 128:256]
        q2 = q[:, 256:384].astype(BF16)
        mid = jnp.concatenate([jnp.where(lane < 64, qm, 0.0), jnp.where(lane >= 64, qm, 0.0)],
                              axis=0).astype(BF16)
        kk = [jnp.concatenate([kbuf[b, k, t, pl.ds(i * 128, 128), :] for t in range(NT)], axis=1)
              for i in range(3)]
        r0 = jnp.dot(q0, kk[0], preferred_element_type=F32)
        rm = jnp.dot(mid, kk[1], preferred_element_type=F32)
        r2 = jnp.dot(q2, kk[2], preferred_element_type=F32)
        return r0 + rm[0:8], rm[8:16] + r2

    def softmax_num(s):
        m = jnp.max(s, axis=1, keepdims=True)
        p = jnp.exp(s - m)
        return p, jnp.sum(p, axis=1, keepdims=True)

    def pv(b, k, pe, po):
        accs = []
        for g in range(PD // 8):
            p = pe if g < DH // 8 else po
            pr = vbuf[b, k, pl.ds(g * 8, 8), :].astype(F32) * p
            a = pr[:, 0:128]
            for t in range(1, NT):
                a = a + pr[:, t * 128:(t + 1) * 128]
            accs.append(a)
        return jnp.concatenate(accs, axis=0)

    def reduce_o(acc, le, lo):
        at = acc.T
        s = at[0:8]
        for i in range(1, 16):
            s = s + at[8 * i:8 * i + 8]
        lane = lax.broadcasted_iota(jnp.int32, (8, PD), 1)
        inv = jnp.where(lane < DH, 1.0 / le, 1.0 / lo)
        return (s * inv).astype(BF16)

    def oproj(ob, k):
        r0 = pl.multiple_of(k * PD, PD) if not isinstance(k, int) else k * PD
        w = jnp.concatenate([wob[t, pl.ds(r0, PD), :] for t in range(D // 128)], axis=1)
        return jnp.dot(ob, w, preferred_element_type=F32)

    def ffn(x):
        xc, rstd = layernorm_parts(x)
        xcb = xc.astype(BF16)
        wgu = jnp.concatenate([wgub[t] for t in range(2 * F // 128)], axis=1)
        gu = jnp.dot(xcb, wgu, preferred_element_type=F32) * rstd
        g = gu[:, :F]
        u = gu[:, F:]
        hh = (g * jax.nn.sigmoid(g) * u).astype(BF16)
        wd = jnp.concatenate([wdb[t] for t in range(D // 128)], axis=1)
        y = jnp.dot(hh, wd, preferred_element_type=F32)
        wr = wrb[...].astype(F32)
        wr = jnp.concatenate([jnp.broadcast_to(wr[t:t + 1, :], (8, 128)) for t in range(D // 128)], axis=1)
        ln = xc * rstd
        r = jnp.sum(ln * wr, axis=1, keepdims=True)
        return x + ln + y * jax.nn.sigmoid(r)

    def attn1(b, x):
        xc, rstd = layernorm_parts(x)
        xcb = xc.astype(BF16)
        qscale = rstd * SCALE

        def body(j, out):
            c = b * NC + j

            @pl.when(c + LA < NCH)
            def _():
                start_chunk(c + LA)

            wait_k(c)
            ps = []
            for i in range(CP):
                k = j * CP + i
                se, so = scores(qproj(xcb, qscale, k), b, k)
                ps.append(softmax_num(se) + softmax_num(so))
            v_copy(c).wait()
            for i in range(CP):
                k = j * CP + i
                pe, le, po, lo = ps[i]
                out = out + oproj(reduce_o(pv(b, k, pe, po), le, lo), k)
            return out

        out = lax.fori_loop(0, NC, body, jnp.zeros((8, D), F32))
        return x + _rowsum_all(out)

    def attn2(b, x):
        xc, rstd = layernorm_parts(x)
        xcb = xc.astype(BF16)
        qscale = rstd * SCALE
        out = jnp.zeros((8, D), F32)
        for k in range(NP):
            se, so = scores(qproj(xcb, qscale, k), b, k)
            pe, le = softmax_num(se)
            po, lo = softmax_num(so)
            out = out + oproj(reduce_o(pv(b, k, pe, po), le, lo), k)
        return x + _rowsum_all(out)

    def batch_body(b, carry):
        x = jnp.broadcast_to(state[pl.ds(b, 1), :], (8, D))
        x = attn1(b, x)
        x = ffn(x)
        x = attn2(b, x)
        x = ffn(x)
        state[pl.ds(b, 1), :] = x[0:1]
        return carry

    lax.fori_loop(0, B, batch_body, 0)
    o_ref[...] = state[0:B, :].astype(o_ref.dtype)


@jax.jit
def pallas_interleave_layers__sliding_block_cached__moe_arch_mod__decode_kernel(
    A_x: jax.Array,
    A_k_cache: jax.Array,
    A_v_cache: jax.Array,
    A_wq: jax.Array,
    A_wo: jax.Array,
    B_x: jax.Array,
    B_w_r: jax.Array,
    B_w_gate: jax.Array,
    B_w_up: jax.Array,
    B_w_down: jax.Array,
):
    del B_x
    kt = jnp.swapaxes(A_k_cache, 2, 3).reshape(B, NP, PD, SK)
    vt = jnp.swapaxes(A_v_cache, 2, 3).reshape(B, NP, PD, SK)
    out = pl.pallas_call(
        _kernel,
        out_shape=jax.ShapeDtypeStruct((B, D), BF16),
        in_specs=[pl.BlockSpec(memory_space=pl.ANY)] * 9,
        out_specs=pl.BlockSpec(memory_space=pltpu.VMEM),
        scratch_shapes=[
            pltpu.VMEM((B, NP, NT, PD, 128), BF16),
            pltpu.VMEM((B, NP, PD, W), BF16),
            pltpu.VMEM((H * DH // 128, D, 128), BF16),
            pltpu.VMEM((D // 128, H * DH, 128), BF16),
            pltpu.VMEM((2 * F // 128, D, 128), BF16),
            pltpu.VMEM((D // 128, F, 128), BF16),
            pltpu.VMEM((B, D), BF16),
            pltpu.VMEM((D // 128, 128), BF16),
            pltpu.VMEM((8, D), F32),
            pltpu.SemaphoreType.DMA((NCH,)),
            pltpu.SemaphoreType.DMA((NCH,)),
            pltpu.SemaphoreType.DMA((6,)),
        ],
        compiler_params=pltpu.CompilerParams(vmem_limit_bytes=127 * 1024 * 1024),
        name="fused_decode",
    )(A_x.reshape(B, D), kt, vt, A_wq, A_wo, B_w_r.reshape(D // 128, 128), B_w_gate, B_w_up, B_w_down)
    return out.reshape(B, 1, D)
```

```python
import functools

import jax
import jax.numpy as jnp
from jax import lax
import jax.experimental.pallas as pl
import jax.experimental.pallas.tpu as pltpu

F32 = jnp.float32
BF16 = jnp.bfloat16
U32 = jnp.uint32

B, D, H, DH, SK, F = 4, 640, 32, 192, 4096, 1536
W = min(4096, max(256, SK // 4))
NP = H // 2
PD = 2 * DH
NT = W // 128
EPS = 1e-5
SCALE = DH ** -0.5

CFG = dict(
    CP=2,
    LA=4,
    OLAG=8,
    NO_KV_DMA=False,
    NREP=B,
    NO_A1=False,
    REST_UNTIL=B,
    REST_FROM=0,
)


def _rowsum_all(x):
    x = x + pltpu.roll(x, 4, 0)
    x = x + pltpu.roll(x, 2, 0)
    return x + pltpu.roll(x, 1, 0)


def _bf(x):
    return pltpu.bitcast(x, BF16)


def _kernel(x_hbm, kt_hbm, vt_hbm, wq_hbm, wo_hbm, wr_hbm, wg_hbm, wu_hbm, wd_hbm,
            o_ref,
            kbuf, vbuf, wqb, wob, wgb, wub, wdb, xb, wrb, state, ksem, vsem, wsem, *, cfg):
    CP, LA, OLAG = cfg["CP"], cfg["LA"], cfg["OLAG"]
    NC = NP // CP
    NCH = B * NC
    kv_dma = not cfg["NO_KV_DMA"]

    def k_copy(c):
        b = c // NC
        p0 = (c % NC) * CP
        return pltpu.make_async_copy(
            kt_hbm.at[b, pl.ds(p0, CP), :, pl.ds(SK - W, W)],
            kbuf.bitcast(BF16).at[b, pl.ds(p0, CP)], ksem.at[c % LA])

    def v_copy(c):
        b = c // NC
        p0 = (c % NC) * CP
        return pltpu.make_async_copy(
            vt_hbm.at[b, pl.ds(p0, CP), :, pl.ds(SK - W, W)],
            vbuf.at[b, pl.ds(p0, CP)], vsem.at[c % LA])

    w_cps = [pltpu.make_async_copy(src, dst.bitcast(BF16), wsem)
             for src, dst in [(wq_hbm, wqb), (wo_hbm, wob), (wg_hbm, wgb), (wu_hbm, wub), (wd_hbm, wdb)]]
    w_cps += [pltpu.make_async_copy(x_hbm, xb, wsem), pltpu.make_async_copy(wr_hbm, wrb, wsem)]
    for cp in w_cps:
        cp.start()
    if kv_dma:
        for c in range(LA):
            k_copy(c).start()
            v_copy(c).start()
    for cp in w_cps:
        cp.wait()
    state[...] = jnp.concatenate([xb[...].astype(F32), jnp.zeros((8 - B, D), F32)], axis=0)

    def layernorm_parts(x):
        m = jnp.sum(x, axis=1, keepdims=True) * (1.0 / D)
        xc = x - m
        v = jnp.sum(xc * xc, axis=1, keepdims=True) * (1.0 / D)
        return xc, lax.rsqrt(v + EPS)

    def qproj(xcb, qscale, k):
        c0 = pl.multiple_of(k * PD, 128) if not isinstance(k, int) else k * PD
        w = _bf(wqb[:, pl.ds(c0, PD)])
        return jnp.dot(xcb, w, preferred_element_type=F32) * qscale

    def scores(q, b, k):
        lane = lax.broadcasted_iota(jnp.int32, (8, 128), 1)
        q0 = q[:, 0:128].astype(BF16)
        qm = q[:, 128:256]
        q2 = q[:, 256:384].astype(BF16)
        mid = jnp.concatenate([jnp.where(lane < 64, qm, 0.0), jnp.where(lane >= 64, qm, 0.0)],
                              axis=0).astype(BF16)
        kk = [_bf(kbuf[b, k, pl.ds(i * 64, 64), :]) for i in range(3)]
        r0 = jnp.dot(q0, kk[0], preferred_element_type=F32)
        rm = jnp.dot(mid, kk[1], preferred_element_type=F32)
        r2 = jnp.dot(q2, kk[2], preferred_element_type=F32)
        return r0 + rm[0:8], rm[8:16] + r2

    def softmax_num(s):
        m = jnp.max(s, axis=1, keepdims=True)
        p = jnp.exp(s - m)
        return p, jnp.sum(p, axis=1, keepdims=True)

    def pv(b, k, pe, po):
        accs = []
        for g in range(PD // 8):
            p = pe if g < DH // 8 else po
            pr = vbuf[b, k, pl.ds(g * 8, 8), :].astype(F32) * p
            a = pr[:, 0:128]
            for t in range(1, NT):
                a = a + pr[:, t * 128:(t + 1) * 128]
            accs.append(a)
        return jnp.concatenate(accs, axis=0)

    def reduce_o(acc, le, lo):
        at = acc.T
        s = at[0:8]
        for i in range(1, 16):
            s = s + at[8 * i:8 * i + 8]
        lane = lax.broadcasted_iota(jnp.int32, (8, PD), 1)
        inv = jnp.where(lane < DH, 1.0 / le, 1.0 / lo)
        return (s * inv).astype(BF16)

    def oproj(ob, k):
        r0 = pl.multiple_of(k * DH, DH) if not isinstance(k, int) else k * DH
        w = _bf(wob[pl.ds(r0, DH), :])
        return jnp.dot(ob, w, preferred_element_type=F32)

    def ffn(x):
        xc, rstd = layernorm_parts(x)
        xcb = xc.astype(BF16)
        g = jnp.dot(xcb, _bf(wgb[...]), preferred_element_type=F32) * rstd
        u = jnp.dot(xcb, _bf(wub[...]), preferred_element_type=F32) * rstd
        hh = (g * jax.nn.sigmoid(g) * u).astype(BF16)
        y = jnp.dot(hh, _bf(wdb[...]), preferred_element_type=F32)
        wr = wrb[...].astype(F32)
        wr = jnp.concatenate([jnp.broadcast_to(wr[t:t + 1, :], (8, 128)) for t in range(D // 128)], axis=1)
        ln = xc * rstd
        r = jnp.sum(ln * wr, axis=1, keepdims=True)
        return x + ln + y * jax.nn.sigmoid(r)

    def attn1(b, x):
        xc, rstd = layernorm_parts(x)
        xcb = xc.astype(BF16)
        qscale = rstd * SCALE

        def body(j, out):
            c = b * NC + j
            if kv_dma:
                k_copy(c).wait()

                @pl.when(c + LA < NCH)
                def _():
                    k_copy(c + LA).start()

            ps = []
            for i in range(CP if not cfg["NO_A1"] else 0):
                k = j * CP + i
                se, so = scores(qproj(xcb, qscale, k), b, k)
                ps.append(softmax_num(se) + softmax_num(so))
            if kv_dma:
                v_copy(c).wait()

                @pl.when(c + LA < NCH)
                def _():
                    v_copy(c + LA).start()

            for i in range(CP if not cfg["NO_A1"] else 0):
                k = j * CP + i
                pe, le, po, lo = ps[i]
                out = out + oproj(reduce_o(pv(b, k, pe, po), le, lo), k)
            return out

        out = lax.fori_loop(0, NC, body, jnp.zeros((8, D), F32))
        return x + _rowsum_all(out)

    def attn2(b, x):
        xc, rstd = layernorm_parts(x)
        xcb = xc.astype(BF16)
        qscale = rstd * SCALE
        q, sc, ps, os_ = {}, {}, {}, {}
        out = None
        for s in range(-3, NP + OLAG):
            if 0 <= s + 3 < NP:
                q[s + 3] = qproj(xcb, qscale, s + 3)
            if 0 <= s + 2 < NP:
                sc[s + 2] = scores(q.pop(s + 2), b, s + 2)
            if 0 <= s - OLAG < NP:
                y = oproj(os_.pop(s - OLAG), s - OLAG)
                out = y if out is None else out + y
            if 0 <= s + 1 < NP:
                se, so = sc.pop(s + 1)
                ps[s + 1] = softmax_num(se) + softmax_num(so)
            if 0 <= s < NP:
                pe, le, po, lo = ps.pop(s)
                os_[s] = reduce_o(pv(b, s, pe, po), le, lo)
        return x + _rowsum_all(out)

    def batch_body(i, carry):
        b = i % B if cfg["NREP"] != B else i
        x = jnp.broadcast_to(state[pl.ds(b, 1), :], (8, D))
        x = attn1(b, x)
        if cfg["REST_UNTIL"] == B:
            x = ffn(x)
            x = attn2(b, x)
            x = ffn(x)
            state[pl.ds(b, 1), :] = x[0:1]
        else:
            state[pl.ds(b, 1), :] = x[0:1]

            @pl.when(jnp.logical_and(b < cfg["REST_UNTIL"], b >= cfg["REST_FROM"]))
            def _():
                state[pl.ds(b, 1), :] = ffn(attn2(b, ffn(x)))[0:1]
        return carry

    lax.fori_loop(0, cfg["NREP"], batch_body, 0)
    o_ref[...] = state[0:B, :].astype(o_ref.dtype)


def _call(cfg, A_x, A_k_cache, A_v_cache, A_wq, A_wo, B_w_r, B_w_gate, B_w_up, B_w_down):
    kt = jnp.swapaxes(A_k_cache, 2, 3).reshape(B, NP, PD, SK)
    vt = jnp.swapaxes(A_v_cache, 2, 3).reshape(B, NP, PD, SK)
    out = pl.pallas_call(
        functools.partial(_kernel, cfg=cfg),
        out_shape=jax.ShapeDtypeStruct((B, D), BF16),
        in_specs=[pl.BlockSpec(memory_space=pl.ANY)] * 9,
        out_specs=pl.BlockSpec(memory_space=pltpu.VMEM),
        scratch_shapes=[
            pltpu.VMEM((B, NP, PD // 2, W), U32),
            pltpu.VMEM((B, NP, PD, W), BF16),
            pltpu.VMEM((D // 2, H * DH), U32),
            pltpu.VMEM((H * DH // 2, D), U32),
            pltpu.VMEM((D // 2, F), U32),
            pltpu.VMEM((D // 2, F), U32),
            pltpu.VMEM((F // 2, D), U32),
            pltpu.VMEM((B, D), BF16),
            pltpu.VMEM((D // 128, 128), BF16),
            pltpu.VMEM((8, D), F32),
            pltpu.SemaphoreType.DMA((cfg["LA"],)),
            pltpu.SemaphoreType.DMA((cfg["LA"],)),
            pltpu.SemaphoreType.DMA(()),
        ],
        compiler_params=pltpu.CompilerParams(vmem_limit_bytes=127 * 1024 * 1024),
        name="fused_decode",
    )(A_x.reshape(B, D), kt, vt, A_wq, A_wo, B_w_r.reshape(D // 128, 128), B_w_gate, B_w_up, B_w_down)
    return out.reshape(B, 1, D)


@jax.jit
def pallas_interleave_layers__sliding_block_cached__moe_arch_mod__decode_kernel(
    A_x: jax.Array,
    A_k_cache: jax.Array,
    A_v_cache: jax.Array,
    A_wq: jax.Array,
    A_wo: jax.Array,
    B_x: jax.Array,
    B_w_r: jax.Array,
    B_w_gate: jax.Array,
    B_w_up: jax.Array,
    B_w_down: jax.Array,
):
    del B_x
    return _call(CFG, A_x, A_k_cache, A_v_cache, A_wq, A_wo, B_w_r, B_w_gate, B_w_up, B_w_down)
```

```python
import functools

import jax
import jax.numpy as jnp
from jax import lax
import jax.experimental.pallas as pl
import jax.experimental.pallas.tpu as pltpu

F32 = jnp.float32
BF16 = jnp.bfloat16
U32 = jnp.uint32

B, D, H, DH, SK, F = 4, 640, 32, 192, 4096, 1536
W = min(4096, max(256, SK // 4))
NP = H // 2
PD = 2 * DH
NT = W // 128
EPS = 1e-5
SCALE = DH ** -0.5

CFG = dict(
    CP=4,
    LA=3,
    OLAG=8,
    NO_KV_DMA=False,
    NREP=B,
    INJ=0,
    NO_A1=False,
    REST_UNTIL=B,
    REST_FROM=0,
)


def _rowsum_all(x):
    x = x + pltpu.roll(x, 4, 0)
    x = x + pltpu.roll(x, 2, 0)
    return x + pltpu.roll(x, 1, 0)


def _bf(x):
    return pltpu.bitcast(x, BF16)


def _kernel(x_hbm, kt_hbm, vt_hbm, wq_hbm, wo_hbm, wr_hbm, wg_hbm, wu_hbm, wd_hbm,
            o_ref,
            kbuf, vbuf, wqb, wob, wgb, wub, wdb, xb, wrb, state, ksem, vsem, wsem, dummy, isem, *, cfg):
    CP, LA, OLAG = cfg["CP"], cfg["LA"], cfg["OLAG"]
    NC = NP // CP
    NCH = B * NC
    kv_dma = not cfg["NO_KV_DMA"]

    def k_copy(c):
        b = c // NC
        p0 = (c % NC) * CP
        return pltpu.make_async_copy(
            kt_hbm.at[b, pl.ds(p0, CP), :, pl.ds(SK - W, W)],
            kbuf.bitcast(BF16).at[b, pl.ds(p0, CP)], ksem.at[c % LA])

    def v_copy(c):
        b = c // NC
        p0 = (c % NC) * CP
        return pltpu.make_async_copy(
            vt_hbm.at[b, pl.ds(p0, CP), :, pl.ds(SK - W, W)],
            vbuf.at[b, pl.ds(p0, CP)], vsem.at[c % LA])

    w_cps = [pltpu.make_async_copy(src, dst.bitcast(BF16), wsem)
             for src, dst in [(wq_hbm, wqb), (wo_hbm, wob), (wg_hbm, wgb), (wu_hbm, wub), (wd_hbm, wdb)]]
    w_cps += [pltpu.make_async_copy(x_hbm, xb, wsem), pltpu.make_async_copy(wr_hbm, wrb, wsem)]
    for cp in w_cps:
        cp.start()
    if kv_dma:
        for c in range(LA):
            k_copy(c).start()
            v_copy(c).start()
    for cp in w_cps:
        cp.wait()
    state[...] = jnp.concatenate([xb[...].astype(F32), jnp.zeros((8 - B, D), F32)], axis=0)

    def layernorm_parts(x):
        m = jnp.sum(x, axis=1, keepdims=True) * (1.0 / D)
        xc = x - m
        v = jnp.sum(xc * xc, axis=1, keepdims=True) * (1.0 / D)
        return xc, lax.rsqrt(v + EPS)

    def qproj(xcb, qscale, k):
        c0 = pl.multiple_of(k * PD, 128) if not isinstance(k, int) else k * PD
        w = _bf(wqb[:, pl.ds(c0, PD)])
        return jnp.dot(xcb, w, preferred_element_type=F32) * qscale

    def scores(q, b, k):
        lane = lax.broadcasted_iota(jnp.int32, (8, 128), 1)
        q0 = q[:, 0:128].astype(BF16)
        qm = q[:, 128:256]
        q2 = q[:, 256:384].astype(BF16)
        mid = jnp.concatenate([jnp.where(lane < 64, qm, 0.0), jnp.where(lane >= 64, qm, 0.0)],
                              axis=0).astype(BF16)
        kk = [_bf(kbuf[b, k, pl.ds(i * 64, 64), :]) for i in range(3)]
        r0 = jnp.dot(q0, kk[0], preferred_element_type=F32)
        rm = jnp.dot(mid, kk[1], preferred_element_type=F32)
        r2 = jnp.dot(q2, kk[2], preferred_element_type=F32)
        return r0 + rm[0:8], rm[8:16] + r2

    def softmax_num(s):
        m = jnp.max(s, axis=1, keepdims=True)
        p = jnp.exp(s - m)
        return p, jnp.sum(p, axis=1, keepdims=True)

    def pv(b, k, pe, po):
        accs = []
        for g in range(PD // 8):
            p = pe if g < DH // 8 else po
            pr = vbuf[b, k, pl.ds(g * 8, 8), :].astype(F32) * p
            a = pr[:, 0:128]
            for t in range(1, NT):
                a = a + pr[:, t * 128:(t + 1) * 128]
            accs.append(a)
        return jnp.concatenate(accs, axis=0)

    def reduce_o(acc, le, lo):
        at = acc.T
        s = at[0:8]
        for i in range(1, 16):
            s = s + at[8 * i:8 * i + 8]
        lane = lax.broadcasted_iota(jnp.int32, (8, PD), 1)
        inv = jnp.where(lane < DH, 1.0 / le, 1.0 / lo)
        return (s * inv).astype(BF16)

    def oproj(ob, k):
        r0 = pl.multiple_of(k * DH, DH) if not isinstance(k, int) else k * DH
        w = _bf(wob[pl.ds(r0, DH), :])
        return jnp.dot(ob, w, preferred_element_type=F32)

    def ffn(x):
        xc, rstd = layernorm_parts(x)
        xcb = xc.astype(BF16)
        g = jnp.dot(xcb, _bf(wgb[...]), preferred_element_type=F32) * rstd
        u = jnp.dot(xcb, _bf(wub[...]), preferred_element_type=F32) * rstd
        hh = (g * jax.nn.sigmoid(g) * u).astype(BF16)
        y = jnp.dot(hh, _bf(wdb[...]), preferred_element_type=F32)
        wr = wrb[...].astype(F32)
        wr = jnp.concatenate([jnp.broadcast_to(wr[t:t + 1, :], (8, 128)) for t in range(D // 128)], axis=1)
        ln = xc * rstd
        r = jnp.sum(ln * wr, axis=1, keepdims=True)
        return x + ln + y * jax.nn.sigmoid(r)

    def attn1(b, x):
        xc, rstd = layernorm_parts(x)
        xcb = xc.astype(BF16)
        qscale = rstd * SCALE

        def body(j, out):
            c = b * NC + j
            if kv_dma:
                k_copy(c).wait()

                @pl.when(c + LA < NCH)
                def _():
                    k_copy(c + LA).start()

            ps = []
            for i in range(CP if not cfg["NO_A1"] else 0):
                k = j * CP + i
                se, so = scores(qproj(xcb, qscale, k), b, k)
                ps.append(softmax_num(se) + softmax_num(so))
            if kv_dma:
                v_copy(c).wait()

                @pl.when(c + LA < NCH)
                def _():
                    v_copy(c + LA).start()

            for i in range(CP if not cfg["NO_A1"] else 0):
                k = j * CP + i
                pe, le, po, lo = ps[i]
                out = out + oproj(reduce_o(pv(b, k, pe, po), le, lo), k)
            return out

        out = lax.fori_loop(0, NC, body, jnp.zeros((8, D), F32))
        return x + _rowsum_all(out)

    def attn2(b, x):
        xc, rstd = layernorm_parts(x)
        xcb = xc.astype(BF16)
        qscale = rstd * SCALE
        q, sc, ps, os_ = {}, {}, {}, {}
        out = None
        for s in range(-3, NP + OLAG):
            if 0 <= s + 3 < NP:
                q[s + 3] = qproj(xcb, qscale, s + 3)
            if 0 <= s + 2 < NP:
                sc[s + 2] = scores(q.pop(s + 2), b, s + 2)
            if 0 <= s - OLAG < NP:
                y = oproj(os_.pop(s - OLAG), s - OLAG)
                out = y if out is None else out + y
            if 0 <= s + 1 < NP:
                se, so = sc.pop(s + 1)
                ps[s + 1] = softmax_num(se) + softmax_num(so)
            if 0 <= s < NP:
                pe, le, po, lo = ps.pop(s)
                os_[s] = reduce_o(pv(b, s, pe, po), le, lo)
            if cfg["INJ"] and 0 <= s < NP:
                def inj(s=s):
                    bn = (b + 1) % B
                    dst = vbuf.at[bn, s, pl.ds(0, 8)] if cfg["INJ"] in (1, 3) else dummy.at[s]
                    pltpu.make_async_copy(vt_hbm.at[bn, s, pl.ds(0, 8), pl.ds(SK - W, W)], dst, isem).start()
                if cfg["INJ"] >= 3:
                    pl.when(b < B)(inj)
                else:
                    inj()
        if cfg["INJ"]:
            pltpu.make_async_copy(dummy, dummy, isem).wait()
        return x + _rowsum_all(out)

    def batch_body(i, carry):
        b = i % B if cfg["NREP"] != B else i
        x = jnp.broadcast_to(state[pl.ds(b, 1), :], (8, D))
        x = attn1(b, x)
        if cfg["REST_UNTIL"] == B:
            x = ffn(x)
            x = attn2(b, x)
            x = ffn(x)
            state[pl.ds(b, 1), :] = x[0:1]
        else:
            state[pl.ds(b, 1), :] = x[0:1]

            @pl.when(jnp.logical_and(b < cfg["REST_UNTIL"], b >= cfg["REST_FROM"]))
            def _():
                state[pl.ds(b, 1), :] = ffn(attn2(b, ffn(x)))[0:1]
        return carry

    lax.fori_loop(0, cfg["NREP"], batch_body, 0)
    o_ref[...] = state[0:B, :].astype(o_ref.dtype)


def _call(cfg, A_x, A_k_cache, A_v_cache, A_wq, A_wo, B_w_r, B_w_gate, B_w_up, B_w_down):
    kt = jnp.swapaxes(A_k_cache, 2, 3).reshape(B, NP, PD, SK)
    vt = jnp.swapaxes(A_v_cache, 2, 3).reshape(B, NP, PD, SK)
    out = pl.pallas_call(
        functools.partial(_kernel, cfg=cfg),
        out_shape=jax.ShapeDtypeStruct((B, D), BF16),
        in_specs=[pl.BlockSpec(memory_space=pl.ANY)] * 9,
        out_specs=pl.BlockSpec(memory_space=pltpu.VMEM),
        scratch_shapes=[
            pltpu.VMEM((B, NP, PD // 2, W), U32),
            pltpu.VMEM((B, NP, PD, W), BF16),
            pltpu.VMEM((D // 2, H * DH), U32),
            pltpu.VMEM((H * DH // 2, D), U32),
            pltpu.VMEM((D // 2, F), U32),
            pltpu.VMEM((D // 2, F), U32),
            pltpu.VMEM((F // 2, D), U32),
            pltpu.VMEM((B, D), BF16),
            pltpu.VMEM((D // 128, 128), BF16),
            pltpu.VMEM((8, D), F32),
            pltpu.SemaphoreType.DMA((cfg["LA"],)),
            pltpu.SemaphoreType.DMA((cfg["LA"],)),
            pltpu.SemaphoreType.DMA(()),
            pltpu.VMEM((NP, 8, W), BF16),
            pltpu.SemaphoreType.DMA(()),
        ],
        compiler_params=pltpu.CompilerParams(vmem_limit_bytes=127 * 1024 * 1024),
        name="fused_decode",
    )(A_x.reshape(B, D), kt, vt, A_wq, A_wo, B_w_r.reshape(D // 128, 128), B_w_gate, B_w_up, B_w_down)
    return out.reshape(B, 1, D)


@jax.jit
def pallas_interleave_layers__sliding_block_cached__moe_arch_mod__decode_kernel(
    A_x: jax.Array,
    A_k_cache: jax.Array,
    A_v_cache: jax.Array,
    A_wq: jax.Array,
    A_wo: jax.Array,
    B_x: jax.Array,
    B_w_r: jax.Array,
    B_w_gate: jax.Array,
    B_w_up: jax.Array,
    B_w_down: jax.Array,
):
    del B_x
    return _call(CFG, A_x, A_k_cache, A_v_cache, A_wq, A_wo, B_w_r, B_w_gate, B_w_up, B_w_down)
```

```python
import functools

import jax
import jax.numpy as jnp
from jax import lax
import jax.experimental.pallas as pl
import jax.experimental.pallas.tpu as pltpu

F32 = jnp.float32
BF16 = jnp.bfloat16
U32 = jnp.uint32
I32 = jnp.int32

B, D, H, DH, SK, F = 4, 640, 32, 192, 4096, 1536
W = min(4096, max(256, SK // 4))
NP = H // 2
PD = 2 * DH
HD = H * DH
NL = W // 128
EPS = 1e-5
SCALE = DH ** -0.5

RI = 8
RO = PD // (8 * RI)
TPC = RI // 2
TPP = 2 * NP * TPC
NTICK = B * TPP
RING = 32

CFG = dict(
    LA=23,
    LEAD=8,
    OLAG=8,
    SPIN=(1, 50),
    WSPIN=(1, 45),
    NF=6,
    PVMID=30,
    TAIL=True,
    NOCOMP=False,
)


def _rowsum_all(x):
    x = x + pltpu.roll(x, 4, 0)
    x = x + pltpu.roll(x, 2, 0)
    return x + pltpu.roll(x, 1, 0)


def _bf(x):
    return pltpu.bitcast(x, BF16)


def _u32(x):
    return pltpu.bitcast(x, U32)


def _layernorm_parts(x):
    m = jnp.sum(x, axis=1, keepdims=True) * (1.0 / D)
    xc = x - m
    v = jnp.sum(xc * xc, axis=1, keepdims=True) * (1.0 / D)
    return xc, lax.rsqrt(v + EPS)


def _scores(q, kk):
    lane = lax.broadcasted_iota(I32, (8, 128), 1)
    q0 = q[:, 0:128].astype(BF16)
    qm = q[:, 128:256]
    q2 = q[:, 256:384].astype(BF16)
    mid = jnp.concatenate([jnp.where(lane < 64, qm, 0.0), jnp.where(lane >= 64, qm, 0.0)],
                          axis=0).astype(BF16)
    r0 = jnp.dot(q0, kk[0], preferred_element_type=F32)
    rm = jnp.dot(mid, kk[1], preferred_element_type=F32)
    r2 = jnp.dot(q2, kk[2], preferred_element_type=F32)
    return r0 + rm[0:8], rm[8:16] + r2


def _softmax_num(s):
    m = jnp.max(s, axis=1, keepdims=True)
    p = jnp.exp(s - m)
    return p, jnp.sum(p, axis=1, keepdims=True)


def _inv_l(le, lo):
    lane = lax.broadcasted_iota(I32, (8, PD), 1)
    return jnp.where(lane < DH, 1.0 / le, 1.0 / lo)


def _pv(vload, pe, po, hooks=None):
    accs = {}
    order = [16 * blk + i for i in range(16) for blk in range(3)]
    for n, g in enumerate(order):
        if hooks and n in hooks:
            hooks[n]()
        p = pe if g < DH // 8 else po
        pr = vload(g).astype(F32) * p
        a = pr[:, 0:128]
        for t in range(1, NL):
            a = a + pr[:, t * 128:(t + 1) * 128]
        accs[g] = a
    return jnp.concatenate([accs[g] for g in range(PD // 8)], axis=0)


def _reduce_o(acc, inv):
    at = acc.T
    s = at[0:8]
    for i in range(1, 16):
        s = s + at[8 * i:8 * i + 8]
    return (s * inv).astype(BF16)


def _kernel(x_hbm, kt_hbm, vt_hbm, wq_hbm, wo_hbm, wr_hbm, wg_hbm, wu_hbm, wd_hbm,
            o_ref,
            kv, kp, wq_raw, wo_raw, wqp, wop, wgb, wub, wdb, xb, wrb, state, spin_ref,
            sems, wsem, *, cfg):
    LA, LEAD, OLAG = cfg["LA"], cfg["LEAD"], cfg["OLAG"]

    def piece(i, s):
        q, pair, w, b = i & (TPC - 1), (i >> 2) & (NP - 1), (i >> 6) & 1, i >> 7
        r0 = (q + s * TPC) * 8
        if not isinstance(i, int):
            r0 = pl.multiple_of(r0, 8)
        return pair, w, b, b & 1, i & (RING - 1), r0

    def start_piece(i, s):
        pair, w, b, slot, ring, r0 = piece(i, s)

        def go(ww):
            src = vt_hbm if ww else kt_hbm
            pltpu.make_async_copy(src.at[b, pair, :, pl.ds(r0, 8), pl.ds(SK - W, W)],
                                  kv.at[slot, ww, pair, :, pl.ds(r0, 8), :],
                                  sems.at[s, ring]).start(priority=1 - s)

        if isinstance(i, int):
            go(w)
        else:
            for ww in range(2):
                pl.when(jnp.logical_and(w == ww, i < NTICK))(functools.partial(go, ww))

    def wait_tick(i):
        for s in range(2):
            pair, w, b, slot, ring, r0 = piece(i, s)
            view = kv.at[slot, w, pair, :, pl.ds(r0, 8), :]
            pltpu.make_async_copy(view, view, sems.at[s, ring]).wait()

    def spin(n):
        v = spin_ref[...]
        lane = lax.broadcasted_iota(I32, v.shape, 1).astype(F32)
        for _ in range(n[0]):
            v = jnp.max(v, axis=1, keepdims=True) * 0.5 + lane
        for _ in range(n[1] // 2):
            v = v * 0.5
            v = v + lane
        spin_ref[...] = v

    def full_tick(i):
        wait_tick(i)
        start_piece(i + LEAD + 1, 1)
        start_piece(i + LA, 0)

    def burst_tick(i, c):
        full_tick(i)
        return c

    def idle_tick(i, c):
        wait_tick(i)
        start_piece(i + LEAD, 1)
        start_piece(i - 1 + LA, 0)
        pl.when(i + LEAD < NTICK)(lambda: spin(cfg["SPIN"]))
        return c

    def advance(t, need):
        t2 = jnp.maximum(t + 2, need)
        wait_tick(t)
        lax.fori_loop(t + 1, t2 - 1, idle_tick, 0)
        wait_tick(t2 - 1)
        start_piece(t2 - 1 + LEAD, 1)
        return t2

    def mid(t2):
        start_piece(t2 + LEAD, 1)
        start_piece(t2 - 2 + LA, 0)
        start_piece(t2 - 1 + LA, 0)

    small = [pltpu.make_async_copy(x_hbm, xb, wsem.at[0]), pltpu.make_async_copy(wr_hbm, wrb, wsem.at[0])]
    half = D // 2
    big = [pltpu.make_async_copy(wq_hbm, wq_raw, wsem.at[1]),
           pltpu.make_async_copy(wg_hbm, wgb, wsem.at[1]),
           pltpu.make_async_copy(wu_hbm.at[pl.ds(0, half)], wub.at[pl.ds(0, half)], wsem.at[1])]
    for cp in big:
        cp.start(priority=1)
    for cp in small:
        cp.start()
    for i in range(LA):
        start_piece(i, 0)
    spin_ref[...] = jnp.zeros(spin_ref.shape, F32)

    def inject_rows(src, dst, row0, rows, n):
        def body(i, c):
            r = pl.multiple_of(row0 + i * rows, 8)
            pltpu.make_async_copy(src.at[pl.ds(r, rows)], dst.at[pl.ds(r, rows)], wsem.at[2]).start()
            spin(cfg["WSPIN"])
            return c
        lax.fori_loop(0, n, body, 0)

    inject_rows(wo_hbm, wo_raw, 0, 48, HD // 48)
    inject_rows(wd_hbm, wdb, 0, 48, F // 48)
    inject_rows(wu_hbm, wub, half, 16, half // 16)
    for i in range(LEAD + 1):
        start_piece(i, 1)
    for cp in small:
        cp.wait()
    state[...] = jnp.concatenate([xb[...].astype(F32), jnp.zeros((8 - B, D), F32)], axis=0)
    for view in (wo_raw, wdb, wub.at[pl.ds(half, half)]):
        pltpu.make_async_copy(view, view, wsem.at[2]).wait()
    for cp in big:
        cp.wait()

    NRP = 40

    def repack(h, c):
        full_tick(h)
        spin(cfg["SPIN"])
        r = pl.multiple_of(h * 16, 16)
        wqp[pl.ds(pl.multiple_of(h * 8, 8), 8), :] = _u32(wq_raw[pl.ds(r, 16), :])
        n = 160
        r = pl.multiple_of(jnp.minimum(h * n, HD - n), 32)
        wop[pl.ds(pl.multiple_of(r >> 1, 16), n // 2), :] = _u32(wo_raw[pl.ds(r, n), :])
        return c

    lax.fori_loop(0, NRP, repack, 0)
    t0 = jnp.int32(NRP)

    def oproj(ob, k):
        r0 = pl.multiple_of(k * DH, DH) if not isinstance(k, int) else k * DH
        return jnp.dot(ob, _bf(wop[pl.ds(r0, DH), :]), preferred_element_type=F32)

    def ffn(x):
        xc, rstd = _layernorm_parts(x)
        xcb = xc.astype(BF16)
        g = jnp.dot(xcb, wgb[...], preferred_element_type=F32) * rstd
        u = jnp.dot(xcb, wub[...], preferred_element_type=F32) * rstd
        hh = (g * jax.nn.sigmoid(g) * u).astype(BF16)
        y = jnp.dot(hh, wdb[...], preferred_element_type=F32)
        wr = wrb[...].astype(F32)
        wr = jnp.concatenate([jnp.broadcast_to(wr[t:t + 1, :], (8, 128)) for t in range(D // 128)], axis=1)
        ln = xc * rstd
        r = jnp.sum(ln * wr, axis=1, keepdims=True)
        return x + ln + y * jax.nn.sigmoid(r)

    def qproj(xcb, qscale, k):
        c0 = pl.multiple_of(k * PD, 128) if not isinstance(k, int) else k * PD
        return jnp.dot(xcb, _bf(wqp[:, pl.ds(c0, PD)]), preferred_element_type=F32) * qscale

    def half_period(hp, t):
        b = hp >> 1
        slot = b & 1
        vbase = jnp.where((hp & 1) == 0, b * TPP + (NP + 1) * TPC, -TPP)

        x = jnp.broadcast_to(state[pl.ds(b, 1), :], (8, D))
        xc, rstd = _layernorm_parts(x)
        xcb = xc.astype(BF16)
        qscale = rstd * SCALE

        def vload(k):
            return lambda g: kv[slot, 1, k, g // RI, pl.ds((g % RI) * 8, 8), :]

        def step(j, carry):
            t, q, se, so, pe, po, inv, o, out = carry
            kq = jnp.minimum(j, NP - 1)
            ks = jnp.clip(j - 1, 0, NP - 1)
            kv_ = jnp.maximum(j - 3, 0)
            ko = jnp.maximum(j - 4, 0)
            t = advance(t, vbase + kv_ * TPC)
            q_n = qproj(xcb, qscale, kq)
            out = out + oproj(o, ko)
            pe_n, le = _softmax_num(se)
            po_n, lo = _softmax_num(so)
            inv_n = _inv_l(le, lo)
            res = []

            def hook():
                mid(t)
                kall = kv[slot, 0, ks].reshape(PD, W)
                kp[ks] = _u32(kall)
                res.extend(_scores(q, [kall[i * 128:(i + 1) * 128] for i in range(3)]))

            acc = _pv(vload(kv_), pe, po, {cfg["PVMID"]: hook})
            o_n = _reduce_o(acc, jnp.where(j >= 3, inv, 0.0))
            return t, q_n, res[0], res[1], pe_n, po_n, inv_n, o_n, out

        zw = (lax.broadcasted_iota(I32, (8, W), 0) + lax.broadcasted_iota(I32, (8, W), 1)).astype(F32) * (1.0 / W)
        zp = zw[:, :PD]
        init = (t, zp, zw, zw, zw, zw, zp, jnp.zeros((8, PD), BF16), jnp.zeros((8, D), F32))
        t, _, _, _, pe, po, inv, o, out = lax.fori_loop(0, NP + 2, step, init)

        t = advance(t, vbase + (NP - 1) * TPC)
        out = out + oproj(o, NP - 2)
        acc = _pv(vload(NP - 1), pe, po, {45: lambda: mid(t)})
        out = out + oproj(_reduce_o(acc, inv), NP - 1)
        x = ffn(x + _rowsum_all(out))
        state[pl.ds(b, 1), :] = x[0:1]
        t2 = jnp.minimum(t + cfg["NF"], NTICK)
        lax.fori_loop(t, t2, burst_tick, 0)
        return t2

    if cfg["NOCOMP"]:
        advance(t0, NTICK)
    else:
        lax.fori_loop(0, 2 * B - 1, half_period, t0)

    def attn_fast(x):
        slot = (B - 1) % 2
        xc, rstd = _layernorm_parts(x)
        xcb = xc.astype(BF16)
        qscale = rstd * SCALE
        q, sc, ps, os_ = {}, {}, {}, {}
        out = None
        for s in range(-3, NP + OLAG):
            if 0 <= s + 3 < NP:
                k = s + 3
                q[k] = qproj(xcb, qscale, k)
            if 0 <= s + 2 < NP:
                k = s + 2
                sc[k] = _scores(q.pop(k), [_bf(kp[k, i * 64:(i + 1) * 64, :]) for i in range(3)])
            if 0 <= s - OLAG < NP:
                y = oproj(os_.pop(s - OLAG), s - OLAG)
                out = y if out is None else out + y
            if 0 <= s + 1 < NP:
                se, so = sc.pop(s + 1)
                ps[s + 1] = _softmax_num(se) + _softmax_num(so)
            if 0 <= s < NP:
                pe, le, po, lo = ps.pop(s)
                acc = _pv(lambda g: kv[slot, 1, s, g // RI, pl.ds((g % RI) * 8, 8), :], pe, po)
                os_[s] = _reduce_o(acc, _inv_l(le, lo))
        return x + _rowsum_all(out)

    x = jnp.broadcast_to(state[B - 1:B, :], (8, D))
    if cfg["TAIL"]:
        x = ffn(attn_fast(x))
    row = lax.broadcasted_iota(I32, (8, D), 0)
    o_ref[...] = jnp.where(row == B - 1, x, state[...])[0:B].astype(o_ref.dtype)


def _call(cfg, A_x, A_k_cache, A_v_cache, A_wq, A_wo, B_w_r, B_w_gate, B_w_up, B_w_down):
    kt = jnp.swapaxes(A_k_cache, 2, 3).reshape(B, NP, RO, RI * 8, SK)
    vt = jnp.swapaxes(A_v_cache, 2, 3).reshape(B, NP, RO, RI * 8, SK)
    out = pl.pallas_call(
        functools.partial(_kernel, cfg=cfg),
        out_shape=jax.ShapeDtypeStruct((B, D), BF16),
        in_specs=[pl.BlockSpec(memory_space=pl.ANY)] * 9,
        out_specs=pl.BlockSpec(memory_space=pltpu.VMEM),
        scratch_shapes=[
            pltpu.VMEM((2, 2, NP, RO, RI * 8, W), BF16),
            pltpu.VMEM((NP, PD // 2, W), U32),
            pltpu.VMEM((D, HD), BF16),
            pltpu.VMEM((HD, D), BF16),
            pltpu.VMEM((D // 2, HD), U32),
            pltpu.VMEM((HD // 2, D), U32),
            pltpu.VMEM((D, F), BF16),
            pltpu.VMEM((D, F), BF16),
            pltpu.VMEM((F, D), BF16),
            pltpu.VMEM((B, D), BF16),
            pltpu.VMEM((D // 128, 128), BF16),
            pltpu.VMEM((8, D), F32),
            pltpu.VMEM((8, 128), F32),
            pltpu.SemaphoreType.DMA((2, RING)),
            pltpu.SemaphoreType.DMA((3,)),
        ],
        compiler_params=pltpu.CompilerParams(vmem_limit_bytes=120 * 1024 * 1024,
                                             disable_bounds_checks=True,
                                             disable_semaphore_checks=True),
        name="fused_decode",
    )(A_x.reshape(B, D), kt, vt, A_wq, A_wo, B_w_r.reshape(D // 128, 128), B_w_gate, B_w_up, B_w_down)
    return out.reshape(B, 1, D)


@jax.jit
def pallas_interleave_layers__sliding_block_cached__moe_arch_mod__decode_kernel(
    A_x: jax.Array,
    A_k_cache: jax.Array,
    A_v_cache: jax.Array,
    A_wq: jax.Array,
    A_wo: jax.Array,
    B_x: jax.Array,
    B_w_r: jax.Array,
    B_w_gate: jax.Array,
    B_w_up: jax.Array,
    B_w_down: jax.Array,
):
    del B_x
    return _call(CFG, A_x, A_k_cache, A_v_cache, A_wq, A_wo, B_w_r, B_w_gate, B_w_up, B_w_down)
```

```python
import functools

import jax
import jax.numpy as jnp
from jax import lax
import jax.experimental.pallas as pl
import jax.experimental.pallas.tpu as pltpu

F32 = jnp.float32
BF16 = jnp.bfloat16
U32 = jnp.uint32
I32 = jnp.int32

B, D, H, DH, SK, F = 4, 640, 32, 192, 4096, 1536
W = min(4096, max(256, SK // 4))
NP = H // 2
PD = 2 * DH
HD = H * DH
NL = W // 128
NH = F // 128
EPS = 1e-5
SCALE = DH ** -0.5 * 1.4426950408889634

RI = 8
RO = PD // (8 * RI)
TPC = RI // 2
TPP = 2 * NP * TPC
NTICK = B * TPP
RING = 32

CFG = dict(
    LA=23,
    LEAD=8,
    SPIN=(1, 50),
    WSPIN=(1, 45),
    NF=6,
    PVMID=42,
    KRP=50,
    OLAG=1,
    OSKIP=(4, 7, 10),
    NV=6,
    TAIL=2,
)


def _rowsum_all(x):
    x = x + pltpu.roll(x, 4, 0)
    x = x + pltpu.roll(x, 2, 0)
    return x + pltpu.roll(x, 1, 0)


def _bf(x):
    return pltpu.bitcast(x, BF16)


def _u32(x):
    return pltpu.bitcast(x, U32)


def _dot(a, b):
    return jnp.dot(a, b, preferred_element_type=F32)


def _ln_parts(x):
    xb = x.astype(BF16)
    xr = xb.astype(F32)
    m = jnp.sum(xr, axis=1, keepdims=True) * (1.0 / D)
    xc = xr - m
    v = jnp.sum(xc * xc, axis=1, keepdims=True) * (1.0 / D)
    return xb, xr, m, xc, lax.rsqrt(v + EPS)


def _scores(q, kk):
    lane = lax.broadcasted_iota(I32, (8, 128), 1)
    q0 = q[:, 0:128].astype(BF16)
    qm = q[:, 128:256]
    q2 = q[:, 256:384].astype(BF16)
    mid = jnp.concatenate([jnp.where(lane < 64, qm, 0.0), jnp.where(lane >= 64, qm, 0.0)],
                          axis=0).astype(BF16)
    r0 = _dot(q0, kk[0])
    rm = _dot(mid, kk[1])
    r2 = _dot(q2, kk[2])
    return r0 + rm[0:8], rm[8:16] + r2


def _fold(x, op):
    r = x[:, 0:128]
    for t in range(1, x.shape[1] // 128):
        r = op(r, x[:, t * 128:(t + 1) * 128])
    return r


def _tile(x, n):
    return jnp.concatenate([x] * n, axis=1)


def _softmax_pair(se, so):
    top = lax.broadcasted_iota(I32, (8, 128), 0) < 4

    def split(c):
        c = jnp.broadcast_to(c, (8, 128))
        r = pltpu.roll(c, 4, 0)
        return jnp.where(top, c, r), jnp.where(top, r, c)

    m = jnp.max(jnp.where(top, _fold(se, jnp.maximum), _fold(so, jnp.maximum)), axis=1, keepdims=True)
    me, mo = split(m)
    pe = jnp.exp2(se - _tile(me, NL))
    po = jnp.exp2(so - _tile(mo, NL))
    l = jnp.sum(jnp.where(top, _fold(pe, jnp.add), _fold(po, jnp.add)), axis=1, keepdims=True)
    ie, io = split(pl.reciprocal(l, approx=True))
    lane = lax.broadcasted_iota(I32, (8, 128), 1)
    return pe, po, jnp.concatenate([ie, jnp.where(lane < 64, ie, io), io], axis=1)


def _pv(groups, hooks=None):
    nb = len(groups) // 16
    accs = {}
    for n, g in enumerate(16 * blk + i for i in range(16) for blk in range(nb)):
        if hooks and n in hooks:
            hooks[n]()
        vload, p = groups[g]
        accs[g] = _fold(vload() * p, jnp.add)
    return jnp.concatenate([accs[g] for g in range(len(groups))], axis=0)


def _lane_reduce_t(acc):
    at = acc.T
    s = at[0:8]
    for i in range(1, 16):
        s = s + at[8 * i:8 * i + 8]
    return s


def _kernel(x_hbm, kt_hbm, vt_hbm, wq_hbm, wo_hbm, wr_hbm, wg_hbm, wu_hbm, wd_hbm,
            o_ref,
            kv, kp, wq_raw, wo_raw, wg_raw, wu_raw, wd_raw, wxp, wop, wdp, wguf, cs,
            xb_ref, wrb, state, spin_ref, c_s, c_p, c_inv, c_o, c_out,
            sems, wsem, *, cfg):
    LA, LEAD, NV = cfg["LA"], cfg["LEAD"], cfg["NV"]
    NM = NH - NV

    def piece(i, s):
        q, pair, w, b = i & (TPC - 1), (i >> 2) & (NP - 1), (i >> 6) & 1, i >> 7
        r0 = (q + s * TPC) * 8
        if not isinstance(i, int):
            r0 = pl.multiple_of(r0, 8)
        return pair, w, b, b & 1, i & (RING - 1), r0

    def start_piece(i, s):
        pair, w, b, slot, ring, r0 = piece(i, s)

        def go(ww):
            src = vt_hbm if ww else kt_hbm
            pltpu.make_async_copy(src.at[b, pair, :, pl.ds(r0, 8), pl.ds(SK - W, W)],
                                  kv.at[slot, ww, pair, :, pl.ds(r0, 8), :],
                                  sems.at[s, ring]).start(priority=1 - s)

        if isinstance(i, int):
            go(w)
        else:
            for ww in range(2):
                pl.when(jnp.logical_and(w == ww, i < NTICK))(functools.partial(go, ww))

    def wait_piece(i, s):
        pair, w, b, slot, ring, r0 = piece(i, s)
        view = kv.at[slot, w, pair, :, pl.ds(r0, 8), :]
        pltpu.make_async_copy(view, view, sems.at[s, ring]).wait()

    def wait_tick(i):
        wait_piece(i, 0)
        wait_piece(i, 1)

    def spin(n):
        v = spin_ref[...]
        lane = lax.broadcasted_iota(I32, v.shape, 1).astype(F32)
        for _ in range(n[0]):
            v = jnp.max(v, axis=1, keepdims=True) * 0.5 + lane
        for _ in range(n[1] // 2):
            v = v * 0.5
            v = v + lane
        spin_ref[...] = v

    def full_tick(i):
        wait_tick(i)
        start_piece(i + LEAD + 1, 1)
        start_piece(i + LA, 0)

    def burst_tick(i, c):
        full_tick(i)
        return c

    def spin_tick(i, c):
        full_tick(i)
        spin(cfg["SPIN"])
        return c

    def idle_tick(i, c):
        wait_tick(i)
        start_piece(i + LEAD, 1)
        start_piece(i - 1 + LA, 0)
        spin(cfg["SPIN"])
        return c

    def advance(t, need):
        t2 = jnp.maximum(t + 2, need)
        wait_tick(t)
        lax.fori_loop(t + 1, t2 - 1, idle_tick, 0)
        wait_tick(t2 - 1)
        start_piece(t2 - 1 + LEAD, 1)
        return t2

    def mid(t2):
        start_piece(t2 + LEAD, 1)
        start_piece(t2 - 2 + LA, 0)
        start_piece(t2 - 1 + LA, 0)

    half = D // 2
    small = [pltpu.make_async_copy(x_hbm, xb_ref, wsem.at[0]),
             pltpu.make_async_copy(wr_hbm, wrb, wsem.at[1])]
    big = [pltpu.make_async_copy(wq_hbm, wq_raw, wsem.at[2]),
           pltpu.make_async_copy(wg_hbm, wg_raw, wsem.at[3]),
           pltpu.make_async_copy(wu_hbm.at[pl.ds(0, half)], wu_raw.at[pl.ds(0, half)], wsem.at[4])]
    for cp in big:
        cp.start(priority=1)
    for cp in small:
        cp.start()
    for i in range(LA):
        start_piece(i, 0)
    spin_ref[...] = jnp.zeros(spin_ref.shape, F32)

    inject = [(wo_hbm, wo_raw, 0, 48, HD // 48, 5), (wd_hbm, wd_raw, 0, 48, F // 48, 6),
              (wu_hbm, wu_raw, half, 16, half // 16, 7)]
    for src, dst, row0, rows, n, sem in inject:
        def body(i, c, src=src, dst=dst, row0=row0, rows=rows, sem=sem):
            r = pl.multiple_of(row0 + i * rows, 8)
            pltpu.make_async_copy(src.at[pl.ds(r, rows)], dst.at[pl.ds(r, rows)], wsem.at[sem]).start()
            spin(cfg["WSPIN"])
            return c
        lax.fori_loop(0, n, body, 0)

    for i in range(LEAD + 1):
        start_piece(i, 1)
    for cp in small:
        cp.wait()
    state[...] = jnp.concatenate([xb_ref[...].astype(F32), jnp.zeros((8 - B, D), F32)], axis=0)
    for src, dst, row0, rows, n, sem in inject:
        view = dst.at[pl.ds(row0, rows * n)]
        pltpu.make_async_copy(view, view, wsem.at[sem]).wait()
    for cp in big:
        cp.wait()

    NRP = D // 16

    def repack(h, c):
        full_tick(h)
        r = pl.multiple_of(h * 16, 16)
        r2 = pl.multiple_of(h * 8, 8)
        wxp[pl.ds(r2, 8), 0:HD] = _u32(wq_raw[pl.ds(r, 16), :])
        g = wg_raw[pl.ds(r, 16), :]
        u = wu_raw[pl.ds(r, 16), :]
        gu = jnp.concatenate([w[:, i * 128:(i + 1) * 128] for i in range(NH) for w in (g, u)], axis=1)
        wxp[pl.ds(r2, 8), HD:HD + 2 * F] = _u32(gu)
        if NV:
            wguf[pl.ds(r, 16), :] = gu[:, NM * 256:].astype(F32)
        for raw, packed, n in ((wo_raw, wop, 160), (wd_raw, wdp, 48)):
            r = pl.multiple_of(jnp.minimum(h * n, raw.shape[0] - n), 16)
            packed[pl.ds(pl.multiple_of(r >> 1, 8), n // 2), :] = _u32(raw[pl.ds(r, n), :])
        return c

    lax.fori_loop(0, NRP, repack, 0)

    NCS = (HD + 2 * F) // 768

    def colsum(i, c):
        full_tick(NRP + i)
        c0 = pl.multiple_of(i * 768, 128)
        cs[:, pl.ds(c0, 768)] = _dot(jnp.ones((8, D), BF16), _bf(wxp[:, pl.ds(c0, 768)]))
        return c

    lax.fori_loop(0, NCS, colsum, 0)
    t0 = jnp.int32(NRP + NCS)

    def xproj(xb, m, scale, c0, n):
        return (_dot(xb, _bf(wxp[:, pl.ds(c0, n)])) - m * cs[:, pl.ds(c0, n)]) * scale

    def qproj(xb, m, qscale, k):
        return xproj(xb, m, qscale, k * PD if isinstance(k, int) else pl.multiple_of(k * PD, 128), PD)

    def oproj(ob, k):
        r0 = pl.multiple_of(k * DH, DH) if not isinstance(k, int) else k * DH
        return _dot(ob, _bf(wop[pl.ds(r0, DH), :]))

    def kload(k):
        return [_bf(kp[k, i * 64:(i + 1) * 64, :]) for i in range(3)]

    def vgroup(slot, k, o, r):
        return lambda: kv[slot, 1, k, o, pl.ds(r * 8, 8), :].astype(F32)

    def pair_groups(slot, k, pe, po):
        return [(vgroup(slot, k, g // RI, g % RI), pe if g < DH // 8 else po) for g in range(PD // 8)]

    def ffn(x):
        xb, xr, m, xc, rstd = _ln_parts(x)

        def act(gu):
            g = gu[:, 0:128]
            return (g * jax.nn.sigmoid(g) * gu[:, 128:256]).astype(BF16)

        hs = [act(xproj(xb, m, rstd, HD + i * 256, 256)) for i in range(NM)]
        if NV:
            acc = None
            for u in range(D // 128):
                xcol = jnp.concatenate([xr[:, u * 128:(u + 1) * 128]] * 16, axis=0).T
                for i in range(16):
                    y = wguf[u * 128 + i * 8:u * 128 + i * 8 + 8, :] * _tile(xcol[i * 8:i * 8 + 8], 2 * NV)
                    acc = y if acc is None else acc + y
            gu = (_rowsum_all(acc) - m * cs[:, HD + NM * 256:]) * rstd
            hs += [act(gu[:, i * 256:(i + 1) * 256]) for i in range(NV)]
        y = None
        for i in range(NH):
            yi = _dot(hs[i], _bf(wdp[i * 64:(i + 1) * 64, :]))
            y = yi if y is None else y + yi
        wr = wrb[...].astype(F32)
        wr = jnp.concatenate([jnp.broadcast_to(wr[t:t + 1, :], (8, 128)) for t in range(D // 128)], axis=1)
        ln = xc * rstd
        r = jnp.sum(ln * wr, axis=1, keepdims=True)
        return x + ln + y * jax.nn.sigmoid(r)

    NHP = 2 * B - 1

    def half_period(hp, t):
        b = hp >> 1
        slot = b & 1
        first = (hp & 1) == 0
        vbase = jnp.where(first, b * TPP + (NP + 1) * TPC, -TPP)

        tr = jnp.where(first, jnp.maximum(t, b * TPP + cfg["KRP"]), t)
        lax.fori_loop(t, tr, spin_tick, 0)

        def k_repack(i, c):
            full_tick(i)
            kp[i - tr] = _u32(kv[slot, 0, i - tr].reshape(PD, W))
            return c

        t = jnp.where(first, tr + NP, t)
        lax.fori_loop(tr, t, k_repack, 0)

        x = jnp.broadcast_to(state[pl.ds(b, 1), :], (8, D))
        xb, _, m, _, rstd = _ln_parts(x)
        qscale = rstd * SCALE

        def step(j, carry):
            t, q, se, so, pe, po, inv, o, out = carry
            kv_ = jnp.maximum(j - 3, 0)
            t = advance(t, vbase + kv_ * TPC)
            se_n, so_n = _scores(q, kload(jnp.clip(j - 1, 0, NP - 1)))
            q_n = qproj(xb, m, qscale, jnp.minimum(j, NP - 1))
            out = out + oproj(o, jnp.maximum(j - 4, 0))
            pe_n, po_n, inv_n = _softmax_pair(se, so)
            acc = _pv(pair_groups(slot, kv_, pe, po), {cfg["PVMID"]: lambda: mid(t)})
            o_n = (_lane_reduce_t(acc) * jnp.where(j >= 3, inv, 0.0)).astype(BF16)
            return t, q_n, se_n, so_n, pe_n, po_n, inv_n, o_n, out

        zw = (lax.broadcasted_iota(I32, (8, W), 0) + lax.broadcasted_iota(I32, (8, W), 1)).astype(F32) * (1.0 / W)
        zp = zw[:, :PD]
        init = (t, zp, zw, zw, zw, zw, zp, jnp.zeros((8, PD), BF16), jnp.zeros((8, D), F32))
        last = hp == NHP - 1
        t, _, se, so, pe, po, inv, o, out = lax.fori_loop(0, jnp.where(last, NP + 1, NP + 2), step, init)
        t2 = jnp.maximum(t + 2, vbase + (NP - 1) * TPC)

        @pl.when(last)
        def _():
            c_s[0] = se
            c_s[1] = so
            c_p[0] = pe * _tile(inv[:, 0:128], NL)
            c_p[1] = po * _tile(inv[:, 256:384], NL)
            c_o[...] = o.astype(F32)
            c_out[...] = out

        @pl.when(jnp.logical_not(last))
        def _():
            advance(t, t2)
            y = out + oproj(o, NP - 2)
            acc = _pv(pair_groups(slot, NP - 1, pe, po), {45: lambda: mid(t2)})
            y = y + oproj((_lane_reduce_t(acc) * inv).astype(BF16), NP - 1)
            state[pl.ds(b, 1), :] = ffn(x + _rowsum_all(y))[0:1]
            lax.fori_loop(t2, t2 + cfg["NF"], burst_tick, 0)

        return t2 + cfg["NF"]

    lax.fori_loop(0, NHP, half_period, t0)

    slot = (B - 1) % 2
    ka, kb = NP - 2, NP - 1

    def wo_rows(runs):
        return _bf(jnp.concatenate(
            [wop[(k * PD + o * 64 + r * 8) // 2:(k * PD + o * 64 + (r + n) * 8) // 2, :] for k, o, r, n in runs],
            axis=0))

    def run_groups(runs, ps):
        return [(vgroup(slot, k, o, r + i), ps[k][0 if o < RO // 2 else 1]) for k, o, r, n in runs for i in range(n)]

    for i in range(NTICK - 2 * TPC, NTICK):
        wait_piece(i, 1)
    pe, po, inv = _softmax_pair(c_s[0], c_s[1])
    ps = {ka: (c_p[0], c_p[1]), kb: (pe * _tile(inv[:, 0:128], NL), po * _tile(inv[:, 256:384], NL))}
    out = c_out[...] + oproj(c_o[...].astype(BF16), NP - 3)
    runs0 = [(k, o, TPC, TPC) for k in (ka, kb) for o in range(RO)]
    o0 = _lane_reduce_t(_pv(run_groups(runs0, ps))).astype(BF16)

    for i in range(NTICK - 2 * TPC, NTICK - 2):
        wait_piece(i, 0)
    out = out + _dot(o0, wo_rows(runs0))
    runs1 = [(ka, o, 0, TPC) for o in range(RO)] + [(kb, o, 0, 2) for o in range(4)]
    o1 = _lane_reduce_t(_pv(run_groups(runs1, ps))).astype(BF16)

    for i in range(NTICK - 2, NTICK):
        wait_piece(i, 0)
    out = out + _dot(o1, wo_rows(runs1))
    runs2 = [(kb, o, 0, 2) for o in range(4, RO)] + [(kb, o, 2, 2) for o in range(RO)]
    w2 = wo_rows(runs2).astype(F32)
    for i, (vload, p) in enumerate(run_groups(runs2, ps)):
        out = out + w2[i * 8:(i + 1) * 8] * jnp.sum(_fold(vload() * p, jnp.add), axis=1, keepdims=True)
    x = jnp.broadcast_to(state[B - 1:B, :], (8, D)) + _rowsum_all(out)

    def attn_fast(x):
        xb, _, m, _, rstd = _ln_parts(x)
        qscale = rstd * SCALE
        q, sc, ps, os_ = {}, {}, {}, {}
        out = None
        oslot = {}
        sl = cfg["OLAG"]
        for i in range(NP):
            while sl in cfg["OSKIP"]:
                sl += 1
            oslot[sl] = i
            sl += 1
        for s in range(-3, sl):
            if 0 <= s + 3 < NP:
                q[s + 3] = qproj(xb, m, qscale, s + 3)
            if 0 <= s + 2 < NP:
                sc[s + 2] = _scores(q.pop(s + 2), kload(s + 2))
            if s in oslot:
                y = oproj(os_.pop(oslot[s]), oslot[s])
                out = y if out is None else out + y
            if 0 <= s + 1 < NP:
                ps[s + 1] = _softmax_pair(*sc.pop(s + 1))
            if 0 <= s < NP:
                pe, po, inv = ps.pop(s)
                os_[s] = (_lane_reduce_t(_pv(pair_groups(slot, s, pe, po))) * inv).astype(BF16)
        return x + _rowsum_all(out)

    if cfg["TAIL"] >= 1:
        x = ffn(x)
    if cfg["TAIL"] >= 2:
        x = ffn(attn_fast(x))
    row = lax.broadcasted_iota(I32, (8, D), 0)
    o_ref[...] = jnp.where(row == B - 1, x, state[...])[0:B].astype(o_ref.dtype)


def _call(cfg, A_x, A_k_cache, A_v_cache, A_wq, A_wo, B_w_r, B_w_gate, B_w_up, B_w_down):
    kt = jnp.swapaxes(A_k_cache, 2, 3).reshape(B, NP, RO, RI * 8, SK)
    vt = jnp.swapaxes(A_v_cache, 2, 3).reshape(B, NP, RO, RI * 8, SK)
    out = pl.pallas_call(
        functools.partial(_kernel, cfg=cfg),
        out_shape=jax.ShapeDtypeStruct((B, D), BF16),
        in_specs=[pl.BlockSpec(memory_space=pl.ANY)] * 9,
        out_specs=pl.BlockSpec(memory_space=pltpu.VMEM),
        scratch_shapes=[
            pltpu.VMEM((2, 2, NP, RO, RI * 8, W), BF16),
            pltpu.VMEM((NP, PD // 2, W), U32),
            pltpu.VMEM((D, HD), BF16),
            pltpu.VMEM((HD, D), BF16),
            pltpu.VMEM((D, F), BF16),
            pltpu.VMEM((D, F), BF16),
            pltpu.VMEM((F, D), BF16),
            pltpu.VMEM((D // 2, HD + 2 * F), U32),
            pltpu.VMEM((HD // 2, D), U32),
            pltpu.VMEM((F // 2, D), U32),
            pltpu.VMEM((D, max(cfg["NV"], 1) * 256), F32),
            pltpu.VMEM((8, HD + 2 * F), F32),
            pltpu.VMEM((B, D), BF16),
            pltpu.VMEM((D // 128, 128), BF16),
            pltpu.VMEM((8, D), F32),
            pltpu.VMEM((8, 128), F32),
            pltpu.VMEM((2, 8, W), F32),
            pltpu.VMEM((2, 8, W), F32),
            pltpu.VMEM((8, PD), F32),
            pltpu.VMEM((8, PD), F32),
            pltpu.VMEM((8, D), F32),
            pltpu.SemaphoreType.DMA((2, RING)),
            pltpu.SemaphoreType.DMA((8,)),
        ],
        compiler_params=pltpu.CompilerParams(vmem_limit_bytes=120 * 1024 * 1024,
                                             disable_bounds_checks=True,
                                             disable_semaphore_checks=True),
        name="fused_decode",
    )(A_x.reshape(B, D), kt, vt, A_wq, A_wo, B_w_r.reshape(D // 128, 128), B_w_gate, B_w_up, B_w_down)
    return out.reshape(B, 1, D)


@jax.jit
def pallas_interleave_layers__sliding_block_cached__moe_arch_mod__decode_kernel(
    A_x: jax.Array,
    A_k_cache: jax.Array,
    A_v_cache: jax.Array,
    A_wq: jax.Array,
    A_wo: jax.Array,
    B_x: jax.Array,
    B_w_r: jax.Array,
    B_w_gate: jax.Array,
    B_w_up: jax.Array,
    B_w_down: jax.Array,
):
    del B_x
    return _call(CFG, A_x, A_k_cache, A_v_cache, A_wq, A_wo, B_w_r, B_w_gate, B_w_up, B_w_down)
```

```python
import functools

import jax
import jax.numpy as jnp
from jax import lax
import jax.experimental.pallas as pl
import jax.experimental.pallas.tpu as pltpu

F32 = jnp.float32
BF16 = jnp.bfloat16
U32 = jnp.uint32
I32 = jnp.int32

B, D, H, DH, SK, F = 4, 640, 32, 192, 4096, 1536
W = min(4096, max(256, SK // 4))
NP = H // 2
PD = 2 * DH
HD = H * DH
NL = W // 128
NH = F // 128
EPS = 1e-5
SCALE = DH ** -0.5 * 1.4426950408889634

RI = 8
RO = PD // (8 * RI)
TPC = RI // 2
TPP = 2 * NP * TPC
NTICK = B * TPP
RING = 32
VF0, VF1 = 3, 13

CFG = dict(
    LA=23,
    LEAD=8,
    SPIN=(1, 50),
    WSPIN=(1, 45),
    NF=6,
    PVMID=42,
    KRP=50,
    OLAG=3,
    OSKIP=(11,),
    VGRP=(4,),
    VFIRST=False,
    TOK=(1, 1, 0),
    RAWPOS=(4, 6, 7, 9, 10, 12),
    DORD=(),
    TAIL=2,
)


def _rowsum_all(x):
    x = x + pltpu.roll(x, 4, 0)
    x = x + pltpu.roll(x, 2, 0)
    return x + pltpu.roll(x, 1, 0)


def _bf(x):
    return pltpu.bitcast(x, BF16)


def _u32(x):
    return pltpu.bitcast(x, U32)


def _dot(a, b):
    return jnp.dot(a, b, preferred_element_type=F32)


def _sigmoid(x):
    return pl.reciprocal(1.0 + jnp.exp(-x), approx=True)


def _ln_parts(x):
    xb = x.astype(BF16)
    xr = xb.astype(F32)
    m = jnp.sum(xr, axis=1, keepdims=True) * (1.0 / D)
    xc = xr - m
    v = jnp.sum(xc * xc, axis=1, keepdims=True) * (1.0 / D)
    return xb, xr, m, xc, lax.rsqrt(v + EPS)


def _scores(q, kk):
    lane = lax.broadcasted_iota(I32, (8, 128), 1)
    q0 = q[:, 0:128].astype(BF16)
    qm = q[:, 128:256]
    q2 = q[:, 256:384].astype(BF16)
    mid = jnp.concatenate([jnp.where(lane < 64, qm, 0.0), jnp.where(lane >= 64, qm, 0.0)],
                          axis=0).astype(BF16)
    r0 = _dot(q0, kk[0])
    rm = _dot(mid, kk[1])
    r2 = _dot(q2, kk[2])
    return r0 + rm[0:8], rm[8:16] + r2


def _fold(x, op):
    r = x[:, 0:128]
    for t in range(1, x.shape[1] // 128):
        r = op(r, x[:, t * 128:(t + 1) * 128])
    return r


def _tile(x, n):
    return jnp.concatenate([x] * n, axis=1)


def _softmax_pair(se, so):
    top = lax.broadcasted_iota(I32, (8, 128), 0) < 4

    def split(c):
        c = jnp.broadcast_to(c, (8, 128))
        r = pltpu.roll(c, 4, 0)
        return jnp.where(top, c, r), jnp.where(top, r, c)

    m = jnp.max(jnp.where(top, _fold(se, jnp.maximum), _fold(so, jnp.maximum)), axis=1, keepdims=True)
    me, mo = split(m)
    pe = jnp.exp2(se - _tile(me, NL))
    po = jnp.exp2(so - _tile(mo, NL))
    l = jnp.sum(jnp.where(top, _fold(pe, jnp.add), _fold(po, jnp.add)), axis=1, keepdims=True)
    ie, io = split(pl.reciprocal(l, approx=True))
    lane = lax.broadcasted_iota(I32, (8, 128), 1)
    return pe, po, jnp.concatenate([ie, jnp.where(lane < 64, ie, io), io], axis=1)


def _pv(groups, hooks=None):
    nb = len(groups) // 16
    accs = {}
    for n, g in enumerate(16 * blk + i for i in range(16) for blk in range(nb)):
        if hooks and n in hooks:
            hooks[n]()
        vload, p = groups[g]
        accs[g] = _fold(vload() * p, jnp.add)
    return jnp.concatenate([accs[g] for g in range(len(groups))], axis=0)


def _lane_reduce_t(acc):
    at = acc.T
    s = at[0:8]
    for i in range(1, 16):
        s = s + at[8 * i:8 * i + 8]
    return s


def _kernel(x_hbm, kt_hbm, vt_hbm, wq_hbm, wo_hbm, wr_hbm, wg_hbm, wu_hbm, wd_hbm,
            o_ref,
            kv, vf, kp, wq_raw, wo_raw, wg_raw, wu_raw, wd_raw, wxp, wop, wdp, wguf, cs,
            xb_ref, wrb, state, spin_ref, c_s, c_p, c_inv, c_o, c_out,
            sems, wsem, *, cfg):
    LA, LEAD, NV = cfg["LA"], cfg["LEAD"], sum(cfg["VGRP"])
    NM = NH - NV

    def piece(i, s):
        q, pair, w, b = i & (TPC - 1), (i >> 2) & (NP - 1), (i >> 6) & 1, i >> 7
        r0 = (q + s * TPC) * 8
        if not isinstance(i, int):
            r0 = pl.multiple_of(r0, 8)
        return pair, w, b, w * (1 + (b & 1)), i & (RING - 1), r0

    def start_piece(i, s):
        pair, w, b, plane, ring, r0 = piece(i, s)

        def go(ww):
            src = vt_hbm if ww else kt_hbm
            pltpu.make_async_copy(src.at[b, pair, :, pl.ds(r0, 8), pl.ds(SK - W, W)],
                                  kv.at[plane, pair, :, pl.ds(r0, 8), :],
                                  sems.at[s, ring]).start(priority=1 - s)

        if isinstance(i, int):
            go(w)
        else:
            for ww in range(2):
                pl.when(jnp.logical_and(w == ww, i < NTICK))(functools.partial(go, ww))

    def wait_piece(i, s):
        pair, w, b, plane, ring, r0 = piece(i, s)
        view = kv.at[plane, pair, :, pl.ds(r0, 8), :]
        pltpu.make_async_copy(view, view, sems.at[s, ring]).wait()

    def wait_tick(i):
        wait_piece(i, 0)
        wait_piece(i, 1)

    def spin(n):
        v = spin_ref[...]
        lane = lax.broadcasted_iota(I32, v.shape, 1).astype(F32)
        for _ in range(n[0]):
            v = jnp.max(v, axis=1, keepdims=True) * 0.5 + lane
        for _ in range(n[1] // 2):
            v = v * 0.5
            v = v + lane
        spin_ref[...] = v

    def full_tick(i):
        wait_tick(i)
        start_piece(i + LEAD + 1, 1)
        start_piece(i + LA, 0)

    def burst_tick(i, c):
        full_tick(i)
        return c

    def spin_tick(i, c):
        full_tick(i)
        spin(cfg["SPIN"])
        return c

    def idle_tick(i, c):
        wait_tick(i)
        start_piece(i + LEAD, 1)
        start_piece(i - 1 + LA, 0)
        k = ((i >> 2) & (NP - 1)) - 1
        o0 = ((i & 3) - 1) * (RO // 2)
        vf[k - VF0, pl.ds(o0, RO // 2)] = kv[1 + ((i >> 7) & 1), k, pl.ds(o0, RO // 2)].astype(F32)
        return c

    def advance(t, need):
        t2 = jnp.maximum(t + 2, need)
        wait_tick(t)
        lax.fori_loop(t + 1, t2 - 1, idle_tick, 0)
        wait_tick(t2 - 1)
        start_piece(t2 - 1 + LEAD, 1)
        return t2

    def mid(t2):
        start_piece(t2 + LEAD, 1)
        start_piece(t2 - 2 + LA, 0)
        start_piece(t2 - 1 + LA, 0)

    half = D // 2
    small = [pltpu.make_async_copy(x_hbm, xb_ref, wsem.at[0]),
             pltpu.make_async_copy(wr_hbm, wrb, wsem.at[1])]
    big = [pltpu.make_async_copy(wq_hbm, wq_raw, wsem.at[2]),
           pltpu.make_async_copy(wg_hbm, wg_raw, wsem.at[3]),
           pltpu.make_async_copy(wu_hbm.at[pl.ds(0, half)], wu_raw.at[pl.ds(0, half)], wsem.at[4])]
    for cp in big:
        cp.start(priority=1)
    for cp in small:
        cp.start()
    for i in range(LA):
        start_piece(i, 0)
    spin_ref[...] = jnp.zeros(spin_ref.shape, F32)

    inject = [(wo_hbm, wo_raw, 0, 48, HD // 48, 5), (wd_hbm, wd_raw, 0, 48, F // 48, 6),
              (wu_hbm, wu_raw, half, 16, half // 16, 7)]
    for src, dst, row0, rows, n, sem in inject:
        def body(i, c, src=src, dst=dst, row0=row0, rows=rows, sem=sem):
            r = pl.multiple_of(row0 + i * rows, 8)
            pltpu.make_async_copy(src.at[pl.ds(r, rows)], dst.at[pl.ds(r, rows)], wsem.at[sem]).start()
            spin(cfg["WSPIN"])
            return c
        lax.fori_loop(0, n, body, 0)

    for i in range(LEAD + 1):
        start_piece(i, 1)
    for cp in small:
        cp.wait()
    state[...] = jnp.concatenate([xb_ref[...].astype(F32), jnp.zeros((8 - B, D), F32)], axis=0)
    for src, dst, row0, rows, n, sem in inject:
        view = dst.at[pl.ds(row0, rows * n)]
        pltpu.make_async_copy(view, view, wsem.at[sem]).wait()
    for cp in big:
        cp.wait()

    NRP = D // 16

    def repack(h, c):
        full_tick(h)
        r = pl.multiple_of(h * 16, 16)
        r2 = pl.multiple_of(h * 8, 8)
        wxp[pl.ds(r2, 8), 0:HD] = _u32(wq_raw[pl.ds(r, 16), :])
        g = wg_raw[pl.ds(r, 16), :]
        u = wu_raw[pl.ds(r, 16), :]
        gu = jnp.concatenate([w[:, i * 128:(i + 1) * 128] for i in range(NH) for w in (g, u)], axis=1)
        wxp[pl.ds(r2, 8), HD:HD + 2 * F] = _u32(gu)
        if NV:
            wguf[pl.ds(r, 16), :] = gu[:, NM * 256:].astype(F32)
        for raw, packed, n in ((wo_raw, wop, 160), (wd_raw, wdp, 48)):
            r = pl.multiple_of(jnp.minimum(h * n, raw.shape[0] - n), 16)
            packed[pl.ds(pl.multiple_of(r >> 1, 8), n // 2), :] = _u32(raw[pl.ds(r, n), :])
        return c

    lax.fori_loop(0, NRP, repack, 0)

    NCS = (HD + 2 * F) // 768

    def colsum(i, c):
        full_tick(NRP + i)
        c0 = pl.multiple_of(i * 768, 128)
        cs[:, pl.ds(c0, 768)] = _dot(jnp.ones((8, D), BF16), _bf(wxp[:, pl.ds(c0, 768)]))
        return c

    lax.fori_loop(0, NCS, colsum, 0)
    t0 = jnp.int32(NRP + NCS)

    never = spin_ref[...] < -1.0

    def xproj(xb, m, scale, c0, n):
        return (_dot(xb, _bf(wxp[:, pl.ds(c0, n)])) - m * cs[:, pl.ds(c0, n)]) * scale

    def qproj(xb, m, qscale, k):
        return xproj(xb, m, qscale, k * PD if isinstance(k, int) else pl.multiple_of(k * PD, 128), PD)

    def oproj(ob, k):
        r0 = pl.multiple_of(k * DH, DH) if not isinstance(k, int) else k * DH
        return _dot(ob, _bf(wop[pl.ds(r0, DH), :]))

    def kload(k):
        return [_bf(kp[k, i * 64:(i + 1) * 64, :]) for i in range(3)]

    def vgroup(slot, k, o, r):
        return lambda: kv[1 + slot, k, o, pl.ds(r * 8, 8), :].astype(F32)

    def pair_groups(slot, k, pe, po):
        return [(vgroup(slot, k, g // RI, g % RI), pe if g < DH // 8 else po) for g in range(PD // 8)]

    def ffn(x):
        xb, xr, m, xc, rstd = _ln_parts(x)

        def act(gu):
            g = gu[:, 0:128]
            return (g * _sigmoid(g) * gu[:, 128:256]).astype(BF16)

        def vpu_part():
            xcol = [jnp.concatenate([xr[:, u * 128:(u + 1) * 128]] * 16, axis=0).T for u in range(D // 128)]
            res = []
            c0 = 0
            hist = []
            for n in cfg["VGRP"]:
                acc = None
                for us in ((0, 1), (2, 3), (4,)):
                    for i in range(16):
                        for u in us:
                            r = u * 128 + i * 8
                            col = xcol[u][i * 8:i * 8 + 8]
                            lag, nadd, neup = cfg["TOK"]
                            if len(hist) >= lag:
                                tok = hist[-lag]
                                for _ in range(nadd):
                                    tok = tok + 1.0
                                for _ in range(neup):
                                    tok = jnp.exp2(tok)
                                col = jnp.where(never, tok, col)
                            y = wguf[r:r + 8, c0:c0 + n * 256] * _tile(col, 2 * n)
                            acc = y if acc is None else acc + y
                            hist.append(acc[:, 0:128])
                gu = (_rowsum_all(acc) - m * cs[:, HD + NM * 256 + c0:HD + NM * 256 + c0 + n * 256]) * rstd
                res += [act(gu[:, i * 256:(i + 1) * 256]) for i in range(n)]
                c0 += n * 256
            return res

        hv = vpu_part() if cfg["VFIRST"] else None
        hs = [act(xproj(xb, m, rstd, HD + i * 256, 256)) for i in range(NM)]
        hs += hv if cfg["VFIRST"] else vpu_part()
        y = None
        for grp in cfg["DORD"] or [[i] for i in range(NH)]:
            yi = _dot(jnp.concatenate([hs[i] for i in grp], axis=1),
                      _bf(jnp.concatenate([wdp[i * 64:(i + 1) * 64, :] for i in grp], axis=0)))
            y = yi if y is None else y + yi
        wr = wrb[...].astype(F32)
        wr = jnp.concatenate([jnp.broadcast_to(wr[t:t + 1, :], (8, 128)) for t in range(D // 128)], axis=1)
        ln = xc * rstd
        r = jnp.sum(ln * wr, axis=1, keepdims=True)
        return x + ln + y * _sigmoid(r)

    NHP = 2 * B - 1

    def half_period(hp, t):
        b = hp >> 1
        slot = b & 1
        first = (hp & 1) == 0
        vbase = jnp.where(first, b * TPP + (NP + 1) * TPC, -TPP)

        tr = jnp.where(first, jnp.maximum(t, b * TPP + cfg["KRP"]), t)
        lax.fori_loop(t, tr, spin_tick, 0)

        def k_repack(i, c):
            full_tick(i)
            kp[i - tr] = _u32(kv[0, i - tr].reshape(PD, W))
            return c

        t = jnp.where(first, tr + NP, t)
        lax.fori_loop(tr, t, k_repack, 0)

        x = jnp.broadcast_to(state[pl.ds(b, 1), :], (8, D))
        xb, _, m, _, rstd = _ln_parts(x)
        qscale = rstd * SCALE

        def step(j, carry):
            t, q, se, so, pe, po, inv, o, out = carry
            kv_ = jnp.maximum(j - 3, 0)
            t = advance(t, vbase + kv_ * TPC)
            se_n, so_n = _scores(q, kload(jnp.clip(j - 1, 0, NP - 1)))
            q_n = qproj(xb, m, qscale, jnp.minimum(j, NP - 1))
            out = out + oproj(o, jnp.maximum(j - 4, 0))
            pe_n, po_n, inv_n = _softmax_pair(se, so)
            acc = _pv(pair_groups(slot, kv_, pe, po), {cfg["PVMID"]: lambda: mid(t)})
            o_n = (_lane_reduce_t(acc) * jnp.where(j >= 3, inv, 0.0)).astype(BF16)
            return t, q_n, se_n, so_n, pe_n, po_n, inv_n, o_n, out

        zw = (lax.broadcasted_iota(I32, (8, W), 0) + lax.broadcasted_iota(I32, (8, W), 1)).astype(F32) * (1.0 / W)
        zp = zw[:, :PD]
        init = (t, zp, zw, zw, zw, zw, zp, jnp.zeros((8, PD), BF16), jnp.zeros((8, D), F32))
        last = hp == NHP - 1
        t, _, se, so, pe, po, inv, o, out = lax.fori_loop(0, jnp.where(last, NP + 1, NP + 2), step, init)
        t2 = jnp.maximum(t + 2, vbase + (NP - 1) * TPC)

        @pl.when(last)
        def _():
            c_s[0] = se
            c_s[1] = so
            c_p[0] = pe * _tile(inv[:, 0:128], NL)
            c_p[1] = po * _tile(inv[:, 256:384], NL)
            c_o[...] = o.astype(F32)
            c_out[...] = out

        @pl.when(jnp.logical_not(last))
        def _():
            advance(t, t2)
            y = out + oproj(o, NP - 2)
            acc = _pv(pair_groups(slot, NP - 1, pe, po), {45: lambda: mid(t2)})
            y = y + oproj((_lane_reduce_t(acc) * inv).astype(BF16), NP - 1)
            state[pl.ds(b, 1), :] = ffn(x + _rowsum_all(y))[0:1]
            lax.fori_loop(t2, t2 + cfg["NF"], burst_tick, 0)

        return t2 + cfg["NF"]

    lax.fori_loop(0, NHP, half_period, t0)

    slot = (B - 1) % 2
    ka, kb = NP - 2, NP - 1

    def wo_rows(runs):
        return _bf(jnp.concatenate(
            [wop[(k * PD + o * 64 + r * 8) // 2:(k * PD + o * 64 + (r + n) * 8) // 2, :] for k, o, r, n in runs],
            axis=0))

    def run_groups(runs, ps):
        return [(vgroup(slot, k, o, r + i), ps[k][0 if o < RO // 2 else 1]) for k, o, r, n in runs for i in range(n)]

    for i in range(NTICK - 2 * TPC, NTICK):
        wait_piece(i, 1)
    pe, po, inv = _softmax_pair(c_s[0], c_s[1])
    ps = {ka: (c_p[0], c_p[1]), kb: (pe * _tile(inv[:, 0:128], NL), po * _tile(inv[:, 256:384], NL))}
    out = c_out[...] + oproj(c_o[...].astype(BF16), NP - 3)
    runs0 = [(k, o, TPC, TPC) for k in (ka, kb) for o in range(RO)]
    lane = lax.broadcasted_iota(I32, (8, 128), 1)
    sc0 = jnp.concatenate([jnp.ones((8, 128), F32), jnp.where(lane < 64, 1.0, inv[:, 0:128]),
                           jnp.where(lane < 32, inv[:, 0:128], inv[:, 256:384])], axis=1)
    o0 = (_lane_reduce_t(_pv(run_groups(runs0, {ka: ps[ka], kb: (pe, po)}))) * sc0).astype(BF16)

    for i in range(NTICK - 2 * TPC, NTICK - 2):
        wait_piece(i, 0)
    out = out + _dot(o0, wo_rows(runs0))
    runs1 = [(ka, o, 0, TPC) for o in range(RO)] + [(kb, o, 0, 2) for o in range(4)]
    o1 = _lane_reduce_t(_pv(run_groups(runs1, ps))).astype(BF16)

    for i in range(NTICK - 2, NTICK):
        wait_piece(i, 0)
    out = out + _dot(o1, wo_rows(runs1))
    runs2 = [(kb, o, 0, 2) for o in range(4, RO)] + [(kb, o, 2, 2) for o in range(RO)]
    w2 = wo_rows(runs2).astype(F32)
    for i, (vload, p) in enumerate(run_groups(runs2, ps)):
        out = out + w2[i * 8:(i + 1) * 8] * jnp.sum(_fold(vload() * p, jnp.add), axis=1, keepdims=True)
    x = jnp.broadcast_to(state[B - 1:B, :], (8, D)) + _rowsum_all(out)

    def attn_fast(x):
        xb, _, m, _, rstd = _ln_parts(x)
        qscale = rstd * SCALE
        q, sc, ps, os_ = {}, {}, {}, {}
        out = None
        oslot = {}
        sl = cfg["OLAG"]
        for i in range(NP):
            while sl in cfg["OSKIP"]:
                sl += 1
            oslot[sl] = i
            sl += 1
        raw = [k for k in range(NP) if not VF0 <= k < VF1]
        order = list(range(VF0, VF1))
        for pos, k in zip(sorted(cfg["RAWPOS"]), raw):
            order.insert(pos, k)
        for s in range(-3, sl):
            if 0 <= s + 3 < NP:
                q[s + 3] = qproj(xb, m, qscale, order[s + 3])
            if 0 <= s + 2 < NP:
                sc[s + 2] = _scores(q.pop(s + 2), kload(order[s + 2]))
            if s in oslot:
                y = oproj(os_.pop(oslot[s]), order[oslot[s]])
                out = y if out is None else out + y
            if 0 <= s + 1 < NP:
                ps[s + 1] = _softmax_pair(*sc.pop(s + 1))
            if 0 <= s < NP:
                pe, po, inv = ps.pop(s)
                k = order[s]
                groups = pair_groups(slot, k, pe, po)
                if k not in raw:
                    groups = [(functools.partial(lambda g: vf[k - VF0, g // RI, pl.ds((g % RI) * 8, 8), :], g), p)
                              for g, (_, p) in enumerate(groups)]
                os_[s] = (_lane_reduce_t(_pv(groups)) * inv).astype(BF16)
        return x + _rowsum_all(out)

    if cfg["TAIL"] >= 1:
        x = ffn(x)
    if cfg["TAIL"] >= 2:
        x = ffn(attn_fast(x))
    row = lax.broadcasted_iota(I32, (8, D), 0)
    o_ref[...] = jnp.where(row == B - 1, x, state[...])[0:B].astype(o_ref.dtype)


def _call(cfg, A_x, A_k_cache, A_v_cache, A_wq, A_wo, B_w_r, B_w_gate, B_w_up, B_w_down):
    kt = jnp.swapaxes(A_k_cache, 2, 3).reshape(B, NP, RO, RI * 8, SK)
    vt = jnp.swapaxes(A_v_cache, 2, 3).reshape(B, NP, RO, RI * 8, SK)
    out = pl.pallas_call(
        functools.partial(_kernel, cfg=cfg),
        out_shape=jax.ShapeDtypeStruct((B, D), BF16),
        in_specs=[pl.BlockSpec(memory_space=pl.ANY)] * 9,
        out_specs=pl.BlockSpec(memory_space=pltpu.VMEM),
        scratch_shapes=[
            pltpu.VMEM((3, NP, RO, RI * 8, W), BF16),
            pltpu.VMEM((NP - 1 - VF0, RO, RI * 8, W), F32),
            pltpu.VMEM((NP, PD // 2, W), U32),
            pltpu.VMEM((D, HD), BF16),
            pltpu.VMEM((HD, D), BF16),
            pltpu.VMEM((D, F), BF16),
            pltpu.VMEM((D, F), BF16),
            pltpu.VMEM((F, D), BF16),
            pltpu.VMEM((D // 2, HD + 2 * F), U32),
            pltpu.VMEM((HD // 2, D), U32),
            pltpu.VMEM((F // 2, D), U32),
            pltpu.VMEM((D, sum(cfg["VGRP"]) * 256), F32),
            pltpu.VMEM((8, HD + 2 * F), F32),
            pltpu.VMEM((B, D), BF16),
            pltpu.VMEM((D // 128, 128), BF16),
            pltpu.VMEM((8, D), F32),
            pltpu.VMEM((8, 128), F32),
            pltpu.VMEM((2, 8, W), F32),
            pltpu.VMEM((2, 8, W), F32),
            pltpu.VMEM((8, PD), F32),
            pltpu.VMEM((8, PD), F32),
            pltpu.VMEM((8, D), F32),
            pltpu.SemaphoreType.DMA((2, RING)),
            pltpu.SemaphoreType.DMA((8,)),
        ],
        compiler_params=pltpu.CompilerParams(vmem_limit_bytes=120 * 1024 * 1024,
                                             disable_bounds_checks=True,
                                             disable_semaphore_checks=True),
        name="fused_decode",
    )(A_x.reshape(B, D), kt, vt, A_wq, A_wo, B_w_r.reshape(D // 128, 128), B_w_gate, B_w_up, B_w_down)
    return out.reshape(B, 1, D)


@jax.jit
def pallas_interleave_layers__sliding_block_cached__moe_arch_mod__decode_kernel(
    A_x: jax.Array,
    A_k_cache: jax.Array,
    A_v_cache: jax.Array,
    A_wq: jax.Array,
    A_wo: jax.Array,
    B_x: jax.Array,
    B_w_r: jax.Array,
    B_w_gate: jax.Array,
    B_w_up: jax.Array,
    B_w_down: jax.Array,
):
    del B_x
    return _call(CFG, A_x, A_k_cache, A_v_cache, A_wq, A_wo, B_w_r, B_w_gate, B_w_up, B_w_down)
```

```python
import functools

import jax
import jax.numpy as jnp
from jax import lax
import jax.experimental.pallas as pl
import jax.experimental.pallas.tpu as pltpu

F32 = jnp.float32
BF16 = jnp.bfloat16
U32 = jnp.uint32
I32 = jnp.int32

B, D, H, DH, SK, F = 4, 640, 32, 192, 4096, 1536
W = min(4096, max(256, SK // 4))
NP = H // 2
PD = 2 * DH
HD = H * DH
NL = W // 128
NH = F // 128
EPS = 1e-5
SCALE = DH ** -0.5 * 1.4426950408889634

RI = 8
RO = PD // (8 * RI)
TPC = RI // 2
TPP = 2 * NP * TPC
NTICK = B * TPP
RING = 32
VF0, VF1 = 3, 13

CFG = dict(
    LA=23,
    LEAD=8,
    SPIN=(1, 50),
    WSPIN=(1, 45),
    NF=6,
    PVMID=42,
    KRP=50,
    OLAG=3,
    OSKIP=(),
    NV=4,
    TOK=1,
    QTOK=1,
    VQ=(3, 4, 5),
    RAWPOS=(4, 6, 7, 9, 10, 12),
    DORD=(),
    QEARLY=True,
    NLS=2,
    TAIL=2,
)


def _order(cfg):
    raw = [k for k in range(NP) if not VF0 <= k < VF1]
    order = list(range(VF0, VF1))
    for pos, k in zip(sorted(cfg["RAWPOS"]), raw):
        order.insert(pos, k)
    return order, raw


def _rowsum_all(x):
    x = x + pltpu.roll(x, 4, 0)
    x = x + pltpu.roll(x, 2, 0)
    return x + pltpu.roll(x, 1, 0)


def _bf(x):
    return pltpu.bitcast(x, BF16)


def _u32(x):
    return pltpu.bitcast(x, U32)


def _dot(a, b):
    return jnp.dot(a, b, preferred_element_type=F32)


def _sigmoid(x):
    return pl.reciprocal(1.0 + jnp.exp(-x), approx=True)


def _ln_parts(x):
    xb = x.astype(BF16)
    xr = xb.astype(F32)
    m = jnp.sum(xr, axis=1, keepdims=True) * (1.0 / D)
    xc = xr - m
    v = jnp.sum(xc * xc, axis=1, keepdims=True) * (1.0 / D)
    return xb, xr, m, xc, lax.rsqrt(v + EPS)


def _scores(q, kk):
    lane = lax.broadcasted_iota(I32, (8, 128), 1)
    q0 = q[:, 0:128].astype(BF16)
    qm = q[:, 128:256]
    q2 = q[:, 256:384].astype(BF16)
    mid = jnp.concatenate([jnp.where(lane < 64, qm, 0.0), jnp.where(lane >= 64, qm, 0.0)],
                          axis=0).astype(BF16)
    r0 = _dot(q0, kk[0])
    rm = _dot(mid, kk[1])
    r2 = _dot(q2, kk[2])
    return r0 + rm[0:8], rm[8:16] + r2


def _fold(x, op):
    r = x[:, 0:128]
    for t in range(1, x.shape[1] // 128):
        r = op(r, x[:, t * 128:(t + 1) * 128])
    return r


def _tile(x, n):
    return jnp.concatenate([x] * n, axis=1)


def _softmax_pair(se, so, c=None):
    top = lax.broadcasted_iota(I32, (8, 128), 0) < 4

    def split(c):
        c = jnp.broadcast_to(c, (8, 128))
        r = pltpu.roll(c, 4, 0)
        return jnp.where(top, c, r), jnp.where(top, r, c)

    m = jnp.max(jnp.where(top, _fold(se, jnp.maximum), _fold(so, jnp.maximum)), axis=1, keepdims=True)
    me, mo = split(m)
    de, do = se - _tile(me, NL), so - _tile(mo, NL)
    if c is not None:
        de, do = de * c, do * c
    pe, po = jnp.exp2(de), jnp.exp2(do)
    l = jnp.sum(jnp.where(top, _fold(pe, jnp.add), _fold(po, jnp.add)), axis=1, keepdims=True)
    ie, io = split(pl.reciprocal(l, approx=True))
    lane = lax.broadcasted_iota(I32, (8, 128), 1)
    return pe, po, jnp.concatenate([ie, jnp.where(lane < 64, ie, io), io], axis=1)


def _pv(groups, hooks=None):
    nb = len(groups) // 16
    accs = {}
    for n, g in enumerate(16 * blk + i for i in range(16) for blk in range(nb)):
        if hooks and n in hooks:
            hooks[n]()
        vload, p = groups[g]
        accs[g] = _fold(vload() * p, jnp.add)
    return jnp.concatenate([accs[g] for g in range(len(groups))], axis=0)


def _lane_reduce_t(acc):
    at = acc.T
    s = at[0:8]
    for i in range(1, 16):
        s = s + at[8 * i:8 * i + 8]
    return s


def _kernel(x_hbm, kt_hbm, vt_hbm, wq_hbm, wo_hbm, wr_hbm, wg_hbm, wu_hbm, wd_hbm,
            o_ref,
            kv, vf, kp, wq_raw, wo_raw, wg_raw, wu_raw, wd_raw, wxp, wop, wdp, wguf, wqf, cs,
            xb_ref, wrb, state, spin_ref, c_s, c_p, c_inv, c_o, c_out,
            sems, wsem, *, cfg):
    LA, LEAD, NV = cfg["LA"], cfg["LEAD"], cfg["NV"]
    NM = NH - NV
    order, raw = _order(cfg)

    def piece(i, s):
        q, pair, w, b = i & (TPC - 1), (i >> 2) & (NP - 1), (i >> 6) & 1, i >> 7
        r0 = (q + s * TPC) * 8
        if not isinstance(i, int):
            r0 = pl.multiple_of(r0, 8)
        return pair, w, b, w * (1 + (b & 1)), i & (RING - 1), r0

    def start_piece(i, s):
        pair, w, b, plane, ring, r0 = piece(i, s)

        def go(ww):
            src = vt_hbm if ww else kt_hbm
            pltpu.make_async_copy(src.at[b, pair, :, pl.ds(r0, 8), pl.ds(SK - W, W)],
                                  kv.at[plane, pair, :, pl.ds(r0, 8), :],
                                  sems.at[s, ring]).start(priority=1 - s)

        if isinstance(i, int):
            go(w)
        else:
            for ww in range(2):
                pl.when(jnp.logical_and(w == ww, i < NTICK))(functools.partial(go, ww))

    def wait_piece(i, s):
        pair, w, b, plane, ring, r0 = piece(i, s)
        view = kv.at[plane, pair, :, pl.ds(r0, 8), :]
        pltpu.make_async_copy(view, view, sems.at[s, ring]).wait()

    def wait_tick(i):
        wait_piece(i, 0)
        wait_piece(i, 1)

    def spin(n):
        v = spin_ref[...]
        lane = lax.broadcasted_iota(I32, v.shape, 1).astype(F32)
        for _ in range(n[0]):
            v = jnp.max(v, axis=1, keepdims=True) * 0.5 + lane
        for _ in range(n[1] // 2):
            v = v * 0.5
            v = v + lane
        spin_ref[...] = v

    def full_tick(i):
        wait_tick(i)
        start_piece(i + LEAD + 1, 1)
        start_piece(i + LA, 0)

    def burst_tick(i, c):
        full_tick(i)
        return c

    def spin_tick(i, c):
        full_tick(i)
        spin(cfg["SPIN"])
        return c

    def idle_tick(i, c):
        wait_tick(i)
        start_piece(i + LEAD, 1)
        start_piece(i - 1 + LA, 0)
        k = ((i >> 2) & (NP - 1)) - 1
        o0 = ((i & 3) - 1) * (RO // 2)
        vf[k - VF0, pl.ds(o0, RO // 2)] = kv[1 + ((i >> 7) & 1), k, pl.ds(o0, RO // 2)].astype(F32)
        return c

    def advance(t, need):
        t2 = jnp.maximum(t + 2, need)
        wait_tick(t)
        lax.fori_loop(t + 1, t2 - 1, idle_tick, 0)
        wait_tick(t2 - 1)
        start_piece(t2 - 1 + LEAD, 1)
        return t2

    def mid(t2):
        start_piece(t2 + LEAD, 1)
        start_piece(t2 - 2 + LA, 0)
        start_piece(t2 - 1 + LA, 0)

    half = D // 2
    small = [pltpu.make_async_copy(x_hbm, xb_ref, wsem.at[0]),
             pltpu.make_async_copy(wr_hbm, wrb, wsem.at[1])]
    big = [pltpu.make_async_copy(wq_hbm, wq_raw, wsem.at[2]),
           pltpu.make_async_copy(wg_hbm, wg_raw, wsem.at[3]),
           pltpu.make_async_copy(wu_hbm.at[pl.ds(0, half)], wu_raw.at[pl.ds(0, half)], wsem.at[4])]
    for cp in big:
        cp.start(priority=1)
    for cp in small:
        cp.start()
    for i in range(LA):
        start_piece(i, 0)
    spin_ref[...] = jnp.zeros(spin_ref.shape, F32)

    inject = [(wo_hbm, wo_raw, 0, 48, HD // 48, 5), (wd_hbm, wd_raw, 0, 48, F // 48, 6),
              (wu_hbm, wu_raw, half, 16, half // 16, 7)]
    for src, dst, row0, rows, n, sem in inject:
        def body(i, c, src=src, dst=dst, row0=row0, rows=rows, sem=sem):
            r = pl.multiple_of(row0 + i * rows, 8)
            pltpu.make_async_copy(src.at[pl.ds(r, rows)], dst.at[pl.ds(r, rows)], wsem.at[sem]).start()
            spin(cfg["WSPIN"])
            return c
        lax.fori_loop(0, n, body, 0)

    for i in range(LEAD + 1):
        start_piece(i, 1)
    for cp in small:
        cp.wait()
    state[...] = jnp.concatenate([xb_ref[...].astype(F32), jnp.zeros((8 - B, D), F32)], axis=0)
    for src, dst, row0, rows, n, sem in inject:
        view = dst.at[pl.ds(row0, rows * n)]
        pltpu.make_async_copy(view, view, wsem.at[sem]).wait()
    for cp in big:
        cp.wait()

    NRP = D // 16

    def repack(h, c):
        full_tick(h)
        r = pl.multiple_of(h * 16, 16)
        r2 = pl.multiple_of(h * 8, 8)
        wxp[pl.ds(r2, 8), 0:HD] = _u32(wq_raw[pl.ds(r, 16), :])
        for n, pos in enumerate(cfg["VQ"]):
            wqf[pl.ds(r, 16), n * PD:(n + 1) * PD] = (
                wq_raw[pl.ds(r, 16), order[pos] * PD:(order[pos] + 1) * PD].astype(F32))
        g = wg_raw[pl.ds(r, 16), :]
        u = wu_raw[pl.ds(r, 16), :]
        gu = jnp.concatenate([w[:, i * 128:(i + 1) * 128] for i in range(NH) for w in (g, u)], axis=1)
        wxp[pl.ds(r2, 8), HD:HD + 2 * F] = _u32(gu)
        if NV:
            wguf[pl.ds(r, 16), :] = gu[:, NM * 256:].astype(F32)
        for src, packed, n in ((wo_raw, wop, 160), (wd_raw, wdp, 48)):
            r = pl.multiple_of(jnp.minimum(h * n, src.shape[0] - n), 16)
            packed[pl.ds(pl.multiple_of(r >> 1, 8), n // 2), :] = _u32(src[pl.ds(r, n), :])
        return c

    lax.fori_loop(0, NRP, repack, 0)

    NCS = (HD + 2 * F) // 768

    def colsum(i, c):
        full_tick(NRP + i)
        c0 = pl.multiple_of(i * 768, 128)
        cs[:, pl.ds(c0, 768)] = _dot(jnp.ones((8, D), BF16), _bf(wxp[:, pl.ds(c0, 768)]))
        return c

    lax.fori_loop(0, NCS, colsum, 0)
    t0 = jnp.int32(NRP + NCS)

    never = spin_ref[...] < -1.0

    def xproj(xb, m, scale, c0, n):
        y = _dot(xb, _bf(wxp[:, pl.ds(c0, n)])) - m * cs[:, pl.ds(c0, n)]
        return y if scale is None else y * scale

    def qproj(xb, m, qscale, k):
        return xproj(xb, m, qscale, k * PD if isinstance(k, int) else pl.multiple_of(k * PD, 128), PD)

    def oproj(ob, k):
        r0 = pl.multiple_of(k * DH, DH) if not isinstance(k, int) else k * DH
        return _dot(ob, _bf(wop[pl.ds(r0, DH), :]))

    def kload(k):
        return [_bf(kp[k, i * 64:(i + 1) * 64, :]) for i in range(3)]

    def vgroup(slot, k, o, r):
        return lambda: kv[1 + slot, k, o, pl.ds(r * 8, 8), :].astype(F32)

    def pair_groups(slot, k, pe, po):
        return [(vgroup(slot, k, g // RI, g % RI), pe if g < DH // 8 else po) for g in range(PD // 8)]

    def vpu_matvec(xr, w_ref, nadd):
        xcol = [jnp.concatenate([xr[:, u * 128:(u + 1) * 128]] * 16, axis=0).T for u in range(D // 128)]
        acc = None
        for us in ((0, 1), (2, 3), (4,)):
            for i in range(16):
                for u in us:
                    r = u * 128 + i * 8
                    col = xcol[u][i * 8:i * 8 + 8]
                    if acc is not None:
                        tok = acc[:, 0:128]
                        for _ in range(nadd):
                            tok = tok + 1.0
                        col = jnp.where(never, tok, col)
                    y = w_ref[r:r + 8, :] * _tile(col, w_ref.shape[1] // 128)
                    acc = y if acc is None else acc + y
        return _rowsum_all(acc)

    def ffn(x):
        xb, xr, m, xc, rstd = _ln_parts(x)

        def act(gu):
            g = gu[:, 0:128]
            return (g * _sigmoid(g) * gu[:, 128:256]).astype(BF16)

        hs = [act(xproj(xb, m, rstd, HD + i * 256, 256)) for i in range(NM)]
        gu = (vpu_matvec(xr, wguf, cfg["TOK"]) - m * cs[:, HD + NM * 256:]) * rstd
        hs += [act(gu[:, i * 256:(i + 1) * 256]) for i in range(NV)]
        y = None
        for grp in cfg["DORD"] or [[i] for i in range(NH)]:
            yi = _dot(jnp.concatenate([hs[i] for i in grp], axis=1),
                      _bf(jnp.concatenate([wdp[i * 64:(i + 1) * 64, :] for i in grp], axis=0)))
            y = yi if y is None else y + yi
        wr = wrb[...].astype(F32)
        wr = jnp.concatenate([jnp.broadcast_to(wr[t:t + 1, :], (8, 128)) for t in range(D // 128)], axis=1)
        ln = xc * rstd
        r = jnp.sum(ln * wr, axis=1, keepdims=True)
        return x + ln + y * _sigmoid(r)

    NHP = 2 * B - 1

    def half_period(hp, t):
        b = hp >> 1
        slot = b & 1
        first = (hp & 1) == 0
        vbase = jnp.where(first, b * TPP + (NP + 1) * TPC, -TPP)

        tr = jnp.where(first, jnp.maximum(t, b * TPP + cfg["KRP"]), t)
        lax.fori_loop(t, tr, spin_tick, 0)

        def k_repack(i, c):
            full_tick(i)
            kp[i - tr] = _u32(kv[0, i - tr].reshape(PD, W))
            return c

        t = jnp.where(first, tr + NP, t)
        lax.fori_loop(tr, t, k_repack, 0)

        x = jnp.broadcast_to(state[pl.ds(b, 1), :], (8, D))
        xb, _, m, _, rstd = _ln_parts(x)
        qscale = rstd * SCALE

        def step(j, carry):
            t, q, se, so, pe, po, inv, o, out = carry
            kv_ = jnp.maximum(j - 3, 0)
            t = advance(t, vbase + kv_ * TPC)
            se_n, so_n = _scores(q, kload(jnp.clip(j - 1, 0, NP - 1)))
            q_n = qproj(xb, m, qscale, jnp.minimum(j, NP - 1))
            out = out + oproj(o, jnp.maximum(j - 4, 0))
            pe_n, po_n, inv_n = _softmax_pair(se, so)
            acc = _pv(pair_groups(slot, kv_, pe, po), {cfg["PVMID"]: lambda: mid(t)})
            o_n = (_lane_reduce_t(acc) * jnp.where(j >= 3, inv, 0.0)).astype(BF16)
            return t, q_n, se_n, so_n, pe_n, po_n, inv_n, o_n, out

        zw = (lax.broadcasted_iota(I32, (8, W), 0) + lax.broadcasted_iota(I32, (8, W), 1)).astype(F32) * (1.0 / W)
        zp = zw[:, :PD]
        init = (t, zp, zw, zw, zw, zw, zp, jnp.zeros((8, PD), BF16), jnp.zeros((8, D), F32))
        last = hp == NHP - 1
        t, _, se, so, pe, po, inv, o, out = lax.fori_loop(0, jnp.where(last, NP + 1, NP + 2), step, init)
        t2 = jnp.maximum(t + 2, vbase + (NP - 1) * TPC)

        @pl.when(last)
        def _():
            c_s[0] = se
            c_s[1] = so
            c_p[0] = pe * _tile(inv[:, 0:128], NL)
            c_p[1] = po * _tile(inv[:, 256:384], NL)
            c_o[...] = o.astype(F32)
            c_out[...] = out

        @pl.when(jnp.logical_not(last))
        def _():
            advance(t, t2)
            y = out + oproj(o, NP - 2)
            acc = _pv(pair_groups(slot, NP - 1, pe, po), {45: lambda: mid(t2)})
            y = y + oproj((_lane_reduce_t(acc) * inv).astype(BF16), NP - 1)
            state[pl.ds(b, 1), :] = ffn(x + _rowsum_all(y))[0:1]
            lax.fori_loop(t2, t2 + cfg["NF"], burst_tick, 0)

        return t2 + cfg["NF"]

    lax.fori_loop(0, NHP, half_period, t0)

    slot = (B - 1) % 2
    ka, kb = NP - 2, NP - 1

    def wo_rows(runs):
        return _bf(jnp.concatenate(
            [wop[(k * PD + o * 64 + r * 8) // 2:(k * PD + o * 64 + (r + n) * 8) // 2, :] for k, o, r, n in runs],
            axis=0))

    def run_groups(runs, ps):
        return [(vgroup(slot, k, o, r + i), ps[k][0 if o < RO // 2 else 1]) for k, o, r, n in runs for i in range(n)]

    for i in range(NTICK - 2 * TPC, NTICK):
        wait_piece(i, 1)
    pe, po, inv = _softmax_pair(c_s[0], c_s[1])
    ps = {ka: (c_p[0], c_p[1]), kb: (pe * _tile(inv[:, 0:128], NL), po * _tile(inv[:, 256:384], NL))}
    out = c_out[...] + oproj(c_o[...].astype(BF16), NP - 3)
    runs0 = [(k, o, TPC, TPC) for k in (ka, kb) for o in range(RO)]
    lane = lax.broadcasted_iota(I32, (8, 128), 1)
    sc0 = jnp.concatenate([jnp.ones((8, 128), F32), jnp.where(lane < 64, 1.0, inv[:, 0:128]),
                           jnp.where(lane < 32, inv[:, 0:128], inv[:, 256:384])], axis=1)
    o0 = (_lane_reduce_t(_pv(run_groups(runs0, {ka: ps[ka], kb: (pe, po)}))) * sc0).astype(BF16)

    for i in range(NTICK - 2 * TPC, NTICK - 2):
        wait_piece(i, 0)
    out = out + _dot(o0, wo_rows(runs0))
    runs1 = [(ka, o, 0, TPC) for o in range(RO)] + [(kb, o, 0, 2) for o in range(4)]
    o1 = _lane_reduce_t(_pv(run_groups(runs1, ps))).astype(BF16)

    for i in range(NTICK - 2, NTICK):
        wait_piece(i, 0)
    out = out + _dot(o1, wo_rows(runs1))
    runs2 = [(kb, o, 0, 2) for o in range(4, RO)] + [(kb, o, 2, 2) for o in range(RO)]
    w2 = wo_rows(runs2).astype(F32)
    for i, (vload, p) in enumerate(run_groups(runs2, ps)):
        out = out + w2[i * 8:(i + 1) * 8] * jnp.sum(_fold(vload() * p, jnp.add), axis=1, keepdims=True)
    x = jnp.broadcast_to(state[B - 1:B, :], (8, D)) + _rowsum_all(out)

    def attn_fast(x):
        xb, xr, m, _, rstd = _ln_parts(x)
        qscale = rstd * SCALE
        q, sc, ps, os_ = {}, {}, {}, {}
        out = None
        oslot = {}
        sl = cfg["OLAG"]
        for i in range(NP):
            while sl in cfg["OSKIP"]:
                sl += 1
            oslot[sl] = i
            sl += 1
        if cfg["VQ"]:
            qv = vpu_matvec(xr, wqf, cfg["QTOK"])
            for n, pos in enumerate(cfg["VQ"]):
                k = order[pos]
                q[pos] = (qv[:, n * PD:(n + 1) * PD] - m * cs[:, k * PD:(k + 1) * PD]) * qscale
        qm = [pos for pos in range(NP) if pos not in cfg["VQ"]]
        for s in range(-3, sl):
            if cfg["QEARLY"]:
                if 0 <= s + 3 < len(qm):
                    q[qm[s + 3]] = qproj(xb, m, qscale if qm[s + 3] >= cfg["NLS"] else None, order[qm[s + 3]])
            elif s + 3 in qm:
                q[s + 3] = qproj(xb, m, qscale if s + 3 >= cfg["NLS"] else None, order[s + 3])
            if 0 <= s + 2 < NP:
                sc[s + 2] = _scores(q.pop(s + 2), kload(order[s + 2]))
            if s in oslot:
                y = oproj(os_.pop(oslot[s]), order[oslot[s]])
                out = y if out is None else out + y
            if 0 <= s + 1 < NP:
                ps[s + 1] = _softmax_pair(*sc.pop(s + 1), None if s + 1 >= cfg["NLS"] else qscale)
            if 0 <= s < NP:
                pe, po, inv = ps.pop(s)
                k = order[s]
                groups = pair_groups(slot, k, pe, po)
                if k not in raw:
                    groups = [(functools.partial(lambda g: vf[k - VF0, g // RI, pl.ds((g % RI) * 8, 8), :], g), p)
                              for g, (_, p) in enumerate(groups)]
                os_[s] = (_lane_reduce_t(_pv(groups)) * inv).astype(BF16)
        return x + _rowsum_all(out)

    if cfg["TAIL"] >= 1:
        x = ffn(x)
    if cfg["TAIL"] >= 2:
        x = ffn(attn_fast(x))
    row = lax.broadcasted_iota(I32, (8, D), 0)
    o_ref[...] = jnp.where(row == B - 1, x, state[...])[0:B].astype(o_ref.dtype)


def _call(cfg, A_x, A_k_cache, A_v_cache, A_wq, A_wo, B_w_r, B_w_gate, B_w_up, B_w_down):
    kt = jnp.swapaxes(A_k_cache, 2, 3).reshape(B, NP, RO, RI * 8, SK)
    vt = jnp.swapaxes(A_v_cache, 2, 3).reshape(B, NP, RO, RI * 8, SK)
    out = pl.pallas_call(
        functools.partial(_kernel, cfg=cfg),
        out_shape=jax.ShapeDtypeStruct((B, D), BF16),
        in_specs=[pl.BlockSpec(memory_space=pl.ANY)] * 9,
        out_specs=pl.BlockSpec(memory_space=pltpu.VMEM),
        scratch_shapes=[
            pltpu.VMEM((3, NP, RO, RI * 8, W), BF16),
            pltpu.VMEM((NP - 1 - VF0, RO, RI * 8, W), F32),
            pltpu.VMEM((NP, PD // 2, W), U32),
            pltpu.VMEM((D, HD), BF16),
            pltpu.VMEM((HD, D), BF16),
            pltpu.VMEM((D, F), BF16),
            pltpu.VMEM((D, F), BF16),
            pltpu.VMEM((F, D), BF16),
            pltpu.VMEM((D // 2, HD + 2 * F), U32),
            pltpu.VMEM((HD // 2, D), U32),
            pltpu.VMEM((F // 2, D), U32),
            pltpu.VMEM((D, cfg["NV"] * 256), F32),
            pltpu.VMEM((D, max(len(cfg["VQ"]), 1) * PD), F32),
            pltpu.VMEM((8, HD + 2 * F), F32),
            pltpu.VMEM((B, D), BF16),
            pltpu.VMEM((D // 128, 128), BF16),
            pltpu.VMEM((8, D), F32),
            pltpu.VMEM((8, 128), F32),
            pltpu.VMEM((2, 8, W), F32),
            pltpu.VMEM((2, 8, W), F32),
            pltpu.VMEM((8, PD), F32),
            pltpu.VMEM((8, PD), F32),
            pltpu.VMEM((8, D), F32),
            pltpu.SemaphoreType.DMA((2, RING)),
            pltpu.SemaphoreType.DMA((8,)),
        ],
        compiler_params=pltpu.CompilerParams(vmem_limit_bytes=120 * 1024 * 1024,
                                             disable_bounds_checks=True,
                                             disable_semaphore_checks=True),
        name="fused_decode",
    )(A_x.reshape(B, D), kt, vt, A_wq, A_wo, B_w_r.reshape(D // 128, 128), B_w_gate, B_w_up, B_w_down)
    return out.reshape(B, 1, D)


@jax.jit
def pallas_interleave_layers__sliding_block_cached__moe_arch_mod__decode_kernel(
    A_x: jax.Array,
    A_k_cache: jax.Array,
    A_v_cache: jax.Array,
    A_wq: jax.Array,
    A_wo: jax.Array,
    B_x: jax.Array,
    B_w_r: jax.Array,
    B_w_gate: jax.Array,
    B_w_up: jax.Array,
    B_w_down: jax.Array,
):
    del B_x
    return _call(CFG, A_x, A_k_cache, A_v_cache, A_wq, A_wo, B_w_r, B_w_gate, B_w_up, B_w_down)
```

```python
import functools

import jax
import jax.numpy as jnp
from jax import lax
import jax.experimental.pallas as pl
import jax.experimental.pallas.tpu as pltpu

F32 = jnp.float32
BF16 = jnp.bfloat16
U32 = jnp.uint32
I32 = jnp.int32

B, D, H, DH, SK, F = 4, 640, 32, 192, 4096, 1536
W = min(4096, max(256, SK // 4))
NP = H // 2
PD = 2 * DH
HD = H * DH
NL = W // 128
NH = F // 128
EPS = 1e-5
SCALE = DH ** -0.5 * 1.4426950408889634

RI = 8
RO = PD // (8 * RI)
TPC = RI // 2
TPP = 2 * NP * TPC
NTICK = B * TPP
RING = 32
VF0, VF1 = 3, 13

CFG = dict(
    LA=23,
    LEAD=8,
    SPIN=(1, 50),
    WSPIN=(1, 45),
    PVMID=42,
    KRP=54,
    OLAG=3,
    OSKIP=(),
    NV=4,
    TOK=1,
    QTOK=((3, 1),),
    VQ=(3, 4, 5),
    RAWPOS=(4, 6, 7, 9, 10, 12),
    DORD=(),
    QEARLY=True,
    NLS=2,
    TAIL=2,
)


def _order(cfg):
    raw = [k for k in range(NP) if not VF0 <= k < VF1]
    order = list(range(VF0, VF1))
    for pos, k in zip(sorted(cfg["RAWPOS"]), raw):
        order.insert(pos, k)
    return order, raw


def _rowsum_all(x):
    x = x + pltpu.roll(x, 4, 0)
    x = x + pltpu.roll(x, 2, 0)
    return x + pltpu.roll(x, 1, 0)


def _bf(x):
    return pltpu.bitcast(x, BF16)


def _u32(x):
    return pltpu.bitcast(x, U32)


def _dot(a, b):
    return jnp.dot(a, b, preferred_element_type=F32)


def _sigmoid(x):
    return pl.reciprocal(1.0 + jnp.exp(-x), approx=True)


def _ln_parts(x):
    xb = x.astype(BF16)
    xr = xb.astype(F32)
    m = jnp.sum(xr, axis=1, keepdims=True) * (1.0 / D)
    xc = xr - m
    v = jnp.sum(xc * xc, axis=1, keepdims=True) * (1.0 / D)
    return xb, xr, m, xc, lax.rsqrt(v + EPS)


def _scores(q, kk):
    lane = lax.broadcasted_iota(I32, (8, 128), 1)
    q0 = q[:, 0:128].astype(BF16)
    qm = q[:, 128:256]
    q2 = q[:, 256:384].astype(BF16)
    mid = jnp.concatenate([jnp.where(lane < 64, qm, 0.0), jnp.where(lane >= 64, qm, 0.0)],
                          axis=0).astype(BF16)
    r0 = _dot(q0, kk[0])
    rm = _dot(mid, kk[1])
    r2 = _dot(q2, kk[2])
    return r0 + rm[0:8], rm[8:16] + r2


def _fold(x, op):
    r = x[:, 0:128]
    for t in range(1, x.shape[1] // 128):
        r = op(r, x[:, t * 128:(t + 1) * 128])
    return r


def _tile(x, n):
    return jnp.concatenate([x] * n, axis=1)


def _softmax_pair(se, so, c=None):
    top = lax.broadcasted_iota(I32, (8, 128), 0) < 4

    def split(c):
        c = jnp.broadcast_to(c, (8, 128))
        r = pltpu.roll(c, 4, 0)
        return jnp.where(top, c, r), jnp.where(top, r, c)

    m = jnp.max(jnp.where(top, _fold(se, jnp.maximum), _fold(so, jnp.maximum)), axis=1, keepdims=True)
    me, mo = split(m)
    de, do = se - _tile(me, NL), so - _tile(mo, NL)
    if c is not None:
        de, do = de * c, do * c
    pe, po = jnp.exp2(de), jnp.exp2(do)
    l = jnp.sum(jnp.where(top, _fold(pe, jnp.add), _fold(po, jnp.add)), axis=1, keepdims=True)
    ie, io = split(pl.reciprocal(l, approx=True))
    lane = lax.broadcasted_iota(I32, (8, 128), 1)
    return pe, po, jnp.concatenate([ie, jnp.where(lane < 64, ie, io), io], axis=1)


def _pv(groups, hooks=None):
    nb = len(groups) // 16
    accs = {}
    for n, g in enumerate(16 * blk + i for i in range(16) for blk in range(nb)):
        if hooks and n in hooks:
            hooks[n]()
        vload, p = groups[g]
        accs[g] = _fold(vload() * p, jnp.add)
    return jnp.concatenate([accs[g] for g in range(len(groups))], axis=0)


def _lane_reduce_t(acc):
    at = acc.T
    s = at[0:8]
    for i in range(1, 16):
        s = s + at[8 * i:8 * i + 8]
    return s


def _kernel(x_hbm, kt_hbm, vt_hbm, wq_hbm, wo_hbm, wr_hbm, wg_hbm, wu_hbm, wd_hbm,
            o_ref,
            kv, vf, kp, wq_raw, wo_raw, wg_raw, wu_raw, wd_raw, wxp, wop, wdp, wguf, wqf, cs,
            xb_ref, wrb, state, spin_ref, c_s, c_p, c_inv, c_o, c_out,
            sems, wsem, *, cfg):
    LA, LEAD, NV = cfg["LA"], cfg["LEAD"], cfg["NV"]
    NM = NH - NV
    order, raw = _order(cfg)

    def piece(i, s):
        q, pair, w, b = i & (TPC - 1), (i >> 2) & (NP - 1), (i >> 6) & 1, i >> 7
        r0 = (q + s * TPC) * 8
        if not isinstance(i, int):
            r0 = pl.multiple_of(r0, 8)
        return pair, w, b, w * (1 + (b & 1)), i & (RING - 1), r0

    def start_piece(i, s):
        pair, w, b, plane, ring, r0 = piece(i, s)

        def go(ww):
            src = vt_hbm if ww else kt_hbm
            pltpu.make_async_copy(src.at[b, pl.ds(pair * RO, RO), pl.ds(r0, 8), pl.ds(SK - W, W)],
                                  kv.at[plane, pl.ds(pair * RO, RO), pl.ds(r0, 8), :],
                                  sems.at[s, ring]).start(priority=1 - s)

        if isinstance(i, int):
            go(w)
        else:
            for ww in range(2):
                pl.when(jnp.logical_and(w == ww, i < NTICK))(functools.partial(go, ww))

    def wait_piece(i, s):
        pair, w, b, plane, ring, r0 = piece(i, s)
        view = kv.at[plane, pl.ds(pair * RO, RO), pl.ds(r0, 8), :]
        pltpu.make_async_copy(view, view, sems.at[s, ring]).wait()

    def wait_tick(i):
        wait_piece(i, 0)
        wait_piece(i, 1)

    def spin(n):
        v = spin_ref[...]
        lane = lax.broadcasted_iota(I32, v.shape, 1).astype(F32)
        for _ in range(n[0]):
            v = jnp.max(v, axis=1, keepdims=True) * 0.5 + lane
        for _ in range(n[1] // 2):
            v = v * 0.5
            v = v + lane
        spin_ref[...] = v

    def full_tick(i):
        wait_tick(i)
        start_piece(i + LEAD + 1, 1)
        start_piece(i + LA, 0)

    def spin_tick(i, c):
        full_tick(i)
        spin(cfg["SPIN"])
        return c

    def idle_tick(i, c):
        wait_tick(i)
        start_piece(i + LEAD, 1)
        start_piece(i - 1 + LA, 0)
        o0 = (((i >> 2) & (NP - 1)) - 1) * RO + ((i & 3) - 1) * (RO // 2)
        vf[pl.ds(o0 - VF0 * RO, RO // 2)] = kv[1 + ((i >> 7) & 1), pl.ds(o0, RO // 2)].astype(F32)
        return c

    def advance(t, need):
        t2 = jnp.maximum(t + 2, need)
        wait_tick(t)
        lax.fori_loop(t + 1, t2 - 1, idle_tick, 0)
        wait_tick(t2 - 1)
        start_piece(t2 - 1 + LEAD, 1)
        return t2

    def mid(t2):
        start_piece(t2 + LEAD, 1)
        start_piece(t2 - 2 + LA, 0)
        start_piece(t2 - 1 + LA, 0)

    half = D // 2
    small = [pltpu.make_async_copy(x_hbm, xb_ref, wsem.at[0]),
             pltpu.make_async_copy(wr_hbm, wrb, wsem.at[1])]
    big = [pltpu.make_async_copy(wq_hbm, wq_raw, wsem.at[2]),
           pltpu.make_async_copy(wg_hbm, wg_raw, wsem.at[3]),
           pltpu.make_async_copy(wu_hbm.at[pl.ds(0, half)], wu_raw.at[pl.ds(0, half)], wsem.at[4])]
    for cp in big:
        cp.start(priority=1)
    for cp in small:
        cp.start()
    for i in range(LA):
        start_piece(i, 0)
    spin_ref[...] = jnp.zeros(spin_ref.shape, F32)

    inject = [(wo_hbm, wo_raw, 0, 48, HD // 48, 5), (wd_hbm, wd_raw, 0, 48, F // 48, 6),
              (wu_hbm, wu_raw, half, 16, half // 16, 7)]
    for src, dst, row0, rows, n, sem in inject:
        def body(i, c, src=src, dst=dst, row0=row0, rows=rows, sem=sem):
            r = pl.multiple_of(row0 + i * rows, 8)
            pltpu.make_async_copy(src.at[pl.ds(r, rows)], dst.at[pl.ds(r, rows)], wsem.at[sem]).start()
            spin(cfg["WSPIN"])
            return c
        lax.fori_loop(0, n, body, 0)

    for i in range(LEAD + 1):
        start_piece(i, 1)
    for cp in small:
        cp.wait()
    state[...] = jnp.concatenate([xb_ref[...].astype(F32), jnp.zeros((8 - B, D), F32)], axis=0)
    for src, dst, row0, rows, n, sem in inject:
        view = dst.at[pl.ds(row0, rows * n)]
        pltpu.make_async_copy(view, view, wsem.at[sem]).wait()
    for cp in big:
        cp.wait()

    NRP = D // 16

    def repack(h, c):
        full_tick(h)
        r = pl.multiple_of(h * 16, 16)
        r2 = pl.multiple_of(h * 8, 8)
        wxp[pl.ds(r2, 8), 0:HD] = _u32(wq_raw[pl.ds(r, 16), :])
        for n, pos in enumerate(cfg["VQ"]):
            wqf[pl.ds(r, 16), n * PD:(n + 1) * PD] = (
                wq_raw[pl.ds(r, 16), order[pos] * PD:(order[pos] + 1) * PD].astype(F32))
        g = wg_raw[pl.ds(r, 16), :]
        u = wu_raw[pl.ds(r, 16), :]
        gu = jnp.concatenate([w[:, i * 128:(i + 1) * 128] for i in range(NH) for w in (g, u)], axis=1)
        wxp[pl.ds(r2, 8), HD:HD + 2 * F] = _u32(gu)
        if NV:
            wguf[pl.ds(r, 16), :] = gu[:, NM * 256:].astype(F32)
        for src, packed, n in ((wo_raw, wop, 160), (wd_raw, wdp, 48)):
            r = pl.multiple_of(jnp.minimum(h * n, src.shape[0] - n), 16)
            packed[pl.ds(pl.multiple_of(r >> 1, 8), n // 2), :] = _u32(src[pl.ds(r, n), :])
        return c

    lax.fori_loop(0, NRP, repack, 0)

    NCS = (HD + 2 * F) // 768

    def colsum(i, c):
        full_tick(NRP + i)
        c0 = pl.multiple_of(i * 768, 128)
        cs[:, pl.ds(c0, 768)] = _dot(jnp.ones((8, D), BF16), _bf(wxp[:, pl.ds(c0, 768)]))
        return c

    lax.fori_loop(0, NCS, colsum, 0)
    t0 = jnp.int32(NRP + NCS)

    never = spin_ref[...] < -1.0

    def xproj(xb, m, scale, c0, n):
        y = _dot(xb, _bf(wxp[:, pl.ds(c0, n)])) - m * cs[:, pl.ds(c0, n)]
        return y if scale is None else y * scale

    def qproj(xb, m, qscale, k):
        return xproj(xb, m, qscale, k * PD if isinstance(k, int) else pl.multiple_of(k * PD, 128), PD)

    def oproj(ob, k):
        r0 = pl.multiple_of(k * DH, DH) if not isinstance(k, int) else k * DH
        return _dot(ob, _bf(wop[pl.ds(r0, DH), :]))

    def kload(k):
        return [_bf(kp[pl.ds(k * RO + 2 * i, 2)].reshape(64, W)) for i in range(3)]

    def vgroup(slot, k, o, r):
        return lambda: kv[1 + slot, k * RO + o, pl.ds(r * 8, 8), :].astype(F32)

    def pair_groups(slot, k, pe, po):
        return [(vgroup(slot, k, g // RI, g % RI), pe if g < DH // 8 else po) for g in range(PD // 8)]

    def vpu_matvec(xr, w_ref, parts):
        xcol = [jnp.concatenate([xr[:, u * 128:(u + 1) * 128]] * 16, axis=0).T for u in range(D // 128)]
        res = []
        tok = None
        c0 = 0
        for n, nadd in parts:
            acc = None
            for us in ((0, 1), (2, 3), (4,)):
                for i in range(16):
                    for u in us:
                        r = u * 128 + i * 8
                        col = xcol[u][i * 8:i * 8 + 8]
                        if tok is not None:
                            for _ in range(nadd):
                                tok = tok + 1.0
                            col = jnp.where(never, tok, col)
                        y = w_ref[r:r + 8, c0:c0 + n] * _tile(col, n // 128)
                        acc = y if acc is None else acc + y
                        tok = acc[:, 0:128]
            res.append(_rowsum_all(acc))
            c0 += n
        return jnp.concatenate(res, axis=1)

    def act(gu):
        g = gu[:, 0:128]
        return (g * _sigmoid(g) * gu[:, 128:256]).astype(BF16)

    def ffn_res(x, xc, rstd):
        wr = wrb[...].astype(F32)
        wr = jnp.concatenate([jnp.broadcast_to(wr[t:t + 1, :], (8, 128)) for t in range(D // 128)], axis=1)
        ln = xc * rstd
        return x + ln, _sigmoid(jnp.sum(ln * wr, axis=1, keepdims=True))

    def ffn(x):
        xb, xr, m, xc, rstd = _ln_parts(x)

        hs = [act(xproj(xb, m, rstd, HD + i * 256, 256)) for i in range(NM)]
        gu = (vpu_matvec(xr, wguf, [(NV * 256, cfg["TOK"])]) - m * cs[:, HD + NM * 256:]) * rstd
        hs += [act(gu[:, i * 256:(i + 1) * 256]) for i in range(NV)]
        y = None
        for grp in cfg["DORD"] or [[i] for i in range(NH)]:
            yi = _dot(jnp.concatenate([hs[i] for i in grp], axis=1),
                      _bf(jnp.concatenate([wdp[i * 64:(i + 1) * 64, :] for i in grp], axis=0)))
            y = yi if y is None else y + yi
        res, gate = ffn_res(x, xc, rstd)
        return res + y * gate

    NFT = NH // 2 + 1

    def ffn_ticked(x, t):
        xb, _, m, xc, rstd = _ln_parts(x)

        def body(i, carry):
            h, y = carry
            full_tick(t + i)
            c0 = pl.multiple_of(HD + jnp.minimum(i, NFT - 2) * 512, 128)
            gu = xproj(xb, m, rstd, c0, 512)
            r0 = pl.multiple_of(jnp.maximum(i - 1, 0) * 128, 128)
            y = y + _dot(h, _bf(wdp[pl.ds(r0, 128), :]))
            return jnp.concatenate([act(gu[:, 0:256]), act(gu[:, 256:512])], axis=1), y

        _, y = lax.fori_loop(0, NFT, body, (jnp.zeros((8, 256), BF16), jnp.zeros((8, D), F32)))
        res, gate = ffn_res(x, xc, rstd)
        return res + y * gate

    NHP = 2 * B - 1

    def half_period(hp, t):
        b = hp >> 1
        slot = b & 1
        first = (hp & 1) == 0
        vbase = jnp.where(first, b * TPP + (NP + 1) * TPC, -TPP)

        tr = jnp.where(first, jnp.maximum(t, b * TPP + cfg["KRP"]), t)
        lax.fori_loop(t, tr, spin_tick, 0)

        def k_repack(i, c):
            full_tick(i)
            o0 = (i - tr) * 8
            kp[pl.ds(o0, 8)] = _u32(kv[0, pl.ds(o0, 8)].reshape(8 * 64, W)).reshape(8, 32, W)
            return c

        t = jnp.where(first, tr + NP * RO // 8, t)
        lax.fori_loop(tr, t, k_repack, 0)

        x = jnp.broadcast_to(state[pl.ds(b, 1), :], (8, D))
        xb, _, m, _, rstd = _ln_parts(x)
        qscale = rstd * SCALE

        def step(j, carry):
            t, q, se, so, pe, po, inv, o, out = carry
            kv_ = jnp.maximum(j - 3, 0)
            t = advance(t, vbase + kv_ * TPC)
            se_n, so_n = _scores(q, kload(jnp.clip(j - 1, 0, NP - 1)))
            q_n = qproj(xb, m, qscale, jnp.minimum(j, NP - 1))
            out = out + oproj(o, jnp.maximum(j - 4, 0))
            pe_n, po_n, inv_n = _softmax_pair(se, so)
            acc = _pv(pair_groups(slot, kv_, pe, po), {cfg["PVMID"]: lambda: mid(t)})
            o_n = (_lane_reduce_t(acc) * jnp.where(j >= 3, inv, 0.0)).astype(BF16)
            return t, q_n, se_n, so_n, pe_n, po_n, inv_n, o_n, out

        zw = (lax.broadcasted_iota(I32, (8, W), 0) + lax.broadcasted_iota(I32, (8, W), 1)).astype(F32) * (1.0 / W)
        zp = zw[:, :PD]
        init = (t, zp, zw, zw, zw, zw, zp, jnp.zeros((8, PD), BF16), jnp.zeros((8, D), F32))
        last = hp == NHP - 1
        t, _, se, so, pe, po, inv, o, out = lax.fori_loop(0, jnp.where(last, NP + 1, NP + 2), step, init)
        t2 = jnp.maximum(t + 2, vbase + (NP - 1) * TPC)

        @pl.when(last)
        def _():
            c_s[0] = se
            c_s[1] = so
            c_p[0] = pe * _tile(inv[:, 0:128], NL)
            c_p[1] = po * _tile(inv[:, 256:384], NL)
            c_o[...] = o.astype(F32)
            c_out[...] = out

        @pl.when(jnp.logical_not(last))
        def _():
            advance(t, t2)
            y = out + oproj(o, NP - 2)
            acc = _pv(pair_groups(slot, NP - 1, pe, po), {45: lambda: mid(t2)})
            olast = (_lane_reduce_t(acc) * inv).astype(BF16)
            full_tick(t2)
            y = y + oproj(olast, NP - 1)
            state[pl.ds(b, 1), :] = ffn_ticked(x + _rowsum_all(y), t2 + 1)[0:1]

        return t2 + 1 + NFT

    lax.fori_loop(0, NHP, half_period, t0)

    slot = (B - 1) % 2
    ka, kb = NP - 2, NP - 1

    def wo_rows(runs):
        return _bf(jnp.concatenate(
            [wop[(k * PD + o * 64 + r * 8) // 2:(k * PD + o * 64 + (r + n) * 8) // 2, :] for k, o, r, n in runs],
            axis=0))

    def run_groups(runs, ps):
        return [(vgroup(slot, k, o, r + i), ps[k][0 if o < RO // 2 else 1]) for k, o, r, n in runs for i in range(n)]

    for i in range(NTICK - 2 * TPC, NTICK):
        wait_piece(i, 1)
    pe, po, inv = _softmax_pair(c_s[0], c_s[1])
    ps = {ka: (c_p[0], c_p[1]), kb: (pe * _tile(inv[:, 0:128], NL), po * _tile(inv[:, 256:384], NL))}
    out = c_out[...] + oproj(c_o[...].astype(BF16), NP - 3)
    runs0 = [(k, o, TPC, TPC) for k in (ka, kb) for o in range(RO)]
    lane = lax.broadcasted_iota(I32, (8, 128), 1)
    sc0 = jnp.concatenate([jnp.ones((8, 128), F32), jnp.where(lane < 64, 1.0, inv[:, 0:128]),
                           jnp.where(lane < 32, inv[:, 0:128], inv[:, 256:384])], axis=1)
    o0 = (_lane_reduce_t(_pv(run_groups(runs0, {ka: ps[ka], kb: (pe, po)}))) * sc0).astype(BF16)

    for i in range(NTICK - 2 * TPC, NTICK - 2):
        wait_piece(i, 0)
    out = out + _dot(o0, wo_rows(runs0))
    runs1 = [(ka, o, 0, TPC) for o in range(RO)] + [(kb, o, 0, 2) for o in range(4)]
    o1 = _lane_reduce_t(_pv(run_groups(runs1, ps))).astype(BF16)

    for i in range(NTICK - 2, NTICK):
        wait_piece(i, 0)
    out = out + _dot(o1, wo_rows(runs1))
    runs2 = [(kb, o, 0, 2) for o in range(4, RO)] + [(kb, o, 2, 2) for o in range(RO)]
    w2 = wo_rows(runs2).astype(F32)
    for i, (vload, p) in enumerate(run_groups(runs2, ps)):
        out = out + w2[i * 8:(i + 1) * 8] * jnp.sum(_fold(vload() * p, jnp.add), axis=1, keepdims=True)
    x = jnp.broadcast_to(state[B - 1:B, :], (8, D)) + _rowsum_all(out)

    def attn_fast(x):
        xb, xr, m, _, rstd = _ln_parts(x)
        qscale = rstd * SCALE
        q, sc, ps, os_ = {}, {}, {}, {}
        out = None
        oslot = {}
        sl = cfg["OLAG"]
        for i in range(NP):
            while sl in cfg["OSKIP"]:
                sl += 1
            oslot[sl] = i
            sl += 1
        if cfg["VQ"]:
            qv = vpu_matvec(xr, wqf, [(n * PD, d) for n, d in cfg["QTOK"]])
            for n, pos in enumerate(cfg["VQ"]):
                k = order[pos]
                q[pos] = (qv[:, n * PD:(n + 1) * PD] - m * cs[:, k * PD:(k + 1) * PD]) * qscale
        qm = [pos for pos in range(NP) if pos not in cfg["VQ"]]
        for s in range(-3, sl):
            if cfg["QEARLY"]:
                if 0 <= s + 3 < len(qm):
                    q[qm[s + 3]] = qproj(xb, m, qscale if qm[s + 3] >= cfg["NLS"] else None, order[qm[s + 3]])
            elif s + 3 in qm:
                q[s + 3] = qproj(xb, m, qscale if s + 3 >= cfg["NLS"] else None, order[s + 3])
            if 0 <= s + 2 < NP:
                sc[s + 2] = _scores(q.pop(s + 2), kload(order[s + 2]))
            if s in oslot:
                y = oproj(os_.pop(oslot[s]), order[oslot[s]])
                out = y if out is None else out + y
            if 0 <= s + 1 < NP:
                ps[s + 1] = _softmax_pair(*sc.pop(s + 1), None if s + 1 >= cfg["NLS"] else qscale)
            if 0 <= s < NP:
                pe, po, inv = ps.pop(s)
                k = order[s]
                groups = pair_groups(slot, k, pe, po)
                if k not in raw:
                    groups = [(functools.partial(lambda g: vf[(k - VF0) * RO + g // RI, pl.ds((g % RI) * 8, 8), :], g), p)
                              for g, (_, p) in enumerate(groups)]
                os_[s] = (_lane_reduce_t(_pv(groups)) * inv).astype(BF16)
        return x + _rowsum_all(out)

    if cfg["TAIL"] >= 1:
        x = ffn(x)
    if cfg["TAIL"] >= 2:
        x = ffn(attn_fast(x))
    row = lax.broadcasted_iota(I32, (8, D), 0)
    o_ref[...] = jnp.where(row == B - 1, x, state[...])[0:B].astype(o_ref.dtype)


def _call(cfg, A_x, A_k_cache, A_v_cache, A_wq, A_wo, B_w_r, B_w_gate, B_w_up, B_w_down):
    kt = jnp.swapaxes(A_k_cache, 2, 3).reshape(B, NP * RO, RI * 8, SK)
    vt = jnp.swapaxes(A_v_cache, 2, 3).reshape(B, NP * RO, RI * 8, SK)
    out = pl.pallas_call(
        functools.partial(_kernel, cfg=cfg),
        out_shape=jax.ShapeDtypeStruct((B, D), BF16),
        in_specs=[pl.BlockSpec(memory_space=pl.ANY)] * 9,
        out_specs=pl.BlockSpec(memory_space=pltpu.VMEM),
        scratch_shapes=[
            pltpu.VMEM((3, NP * RO, RI * 8, W), BF16),
            pltpu.VMEM(((NP - 1 - VF0) * RO, RI * 8, W), F32),
            pltpu.VMEM((NP * RO, RI * 4, W), U32),
            pltpu.VMEM((D, HD), BF16),
            pltpu.VMEM((HD, D), BF16),
            pltpu.VMEM((D, F), BF16),
            pltpu.VMEM((D, F), BF16),
            pltpu.VMEM((F, D), BF16),
            pltpu.VMEM((D // 2, HD + 2 * F), U32),
            pltpu.VMEM((HD // 2, D), U32),
            pltpu.VMEM((F // 2, D), U32),
            pltpu.VMEM((D, cfg["NV"] * 256), F32),
            pltpu.VMEM((D, max(len(cfg["VQ"]), 1) * PD), F32),
            pltpu.VMEM((8, HD + 2 * F), F32),
            pltpu.VMEM((B, D), BF16),
            pltpu.VMEM((D // 128, 128), BF16),
            pltpu.VMEM((8, D), F32),
            pltpu.VMEM((8, 128), F32),
            pltpu.VMEM((2, 8, W), F32),
            pltpu.VMEM((2, 8, W), F32),
            pltpu.VMEM((8, PD), F32),
            pltpu.VMEM((8, PD), F32),
            pltpu.VMEM((8, D), F32),
            pltpu.SemaphoreType.DMA((2, RING)),
            pltpu.SemaphoreType.DMA((8,)),
        ],
        compiler_params=pltpu.CompilerParams(vmem_limit_bytes=120 * 1024 * 1024,
                                             disable_bounds_checks=True,
                                             disable_semaphore_checks=True),
        name="fused_decode",
    )(A_x.reshape(B, D), kt, vt, A_wq, A_wo, B_w_r.reshape(D // 128, 128), B_w_gate, B_w_up, B_w_down)
    return out.reshape(B, 1, D)


@jax.jit
def pallas_interleave_layers__sliding_block_cached__moe_arch_mod__decode_kernel(
    A_x: jax.Array,
    A_k_cache: jax.Array,
    A_v_cache: jax.Array,
    A_wq: jax.Array,
    A_wo: jax.Array,
    B_x: jax.Array,
    B_w_r: jax.Array,
    B_w_gate: jax.Array,
    B_w_up: jax.Array,
    B_w_down: jax.Array,
):
    del B_x
    return _call(CFG, A_x, A_k_cache, A_v_cache, A_wq, A_wo, B_w_r, B_w_gate, B_w_up, B_w_down)
```

```python
import functools

import jax
import jax.numpy as jnp
from jax import lax
import jax.experimental.pallas as pl
import jax.experimental.pallas.tpu as pltpu

F32 = jnp.float32
BF16 = jnp.bfloat16
U32 = jnp.uint32
I32 = jnp.int32

B, D, H, DH, SK, F = 4, 640, 32, 192, 4096, 1536
W = min(4096, max(256, SK // 4))
NP = H // 2
PD = 2 * DH
HD = H * DH
NL = W // 128
NH = F // 128
EPS = 1e-5
SCALE = DH ** -0.5 * 1.4426950408889634

RI = 8
RO = PD // (8 * RI)
TPC = RI // 2
TPP = 2 * NP * TPC
NTICK = B * TPP
RING = 32
VF0, VF1 = 3, 13

CFG = dict(
    LA=23,
    LEAD=11,
    SPIN=(1, 50),
    WSPIN=(1, 45),
    HALF=2,
    HSPIN=(),
    KSPIN=(1, 20),
    PVMID=(21, 45),
    KRP=54,
    OLAG=3,
    OSKIP=(),
    NV=4,
    TOK=1,
    QTOK=((3, 1),),
    VQ=(3, 4, 5),
    RAWPOS=(4, 6, 7, 9, 10, 12),
    DORD=(),
    QEARLY=True,
    NLS=2,
    TAIL=2,
)


def _order(cfg):
    raw = [k for k in range(NP) if not VF0 <= k < VF1]
    order = list(range(VF0, VF1))
    for pos, k in zip(sorted(cfg["RAWPOS"]), raw):
        order.insert(pos, k)
    return order, raw


def _rowsum_all(x):
    x = x + pltpu.roll(x, 4, 0)
    x = x + pltpu.roll(x, 2, 0)
    return x + pltpu.roll(x, 1, 0)


def _bf(x):
    return pltpu.bitcast(x, BF16)


def _u32(x):
    return pltpu.bitcast(x, U32)


def _dot(a, b):
    return jnp.dot(a, b, preferred_element_type=F32)


def _sigmoid(x):
    return pl.reciprocal(1.0 + jnp.exp(-x), approx=True)


def _ln_parts(x):
    xb = x.astype(BF16)
    xr = xb.astype(F32)
    m = jnp.sum(xr, axis=1, keepdims=True) * (1.0 / D)
    xc = xr - m
    v = jnp.sum(xc * xc, axis=1, keepdims=True) * (1.0 / D)
    return xb, xr, m, xc, lax.rsqrt(v + EPS)


def _scores(q, kk):
    lane = lax.broadcasted_iota(I32, (8, 128), 1)
    q0 = q[:, 0:128].astype(BF16)
    qm = q[:, 128:256]
    q2 = q[:, 256:384].astype(BF16)
    mid = jnp.concatenate([jnp.where(lane < 64, qm, 0.0), jnp.where(lane >= 64, qm, 0.0)],
                          axis=0).astype(BF16)
    r0 = _dot(q0, kk[0])
    rm = _dot(mid, kk[1])
    r2 = _dot(q2, kk[2])
    return r0 + rm[0:8], rm[8:16] + r2


def _fold(x, op):
    r = x[:, 0:128]
    for t in range(1, x.shape[1] // 128):
        r = op(r, x[:, t * 128:(t + 1) * 128])
    return r


def _tile(x, n):
    return jnp.concatenate([x] * n, axis=1)


def _softmax_pair(se, so, c=None):
    top = lax.broadcasted_iota(I32, (8, 128), 0) < 4

    def split(c):
        c = jnp.broadcast_to(c, (8, 128))
        r = pltpu.roll(c, 4, 0)
        return jnp.where(top, c, r), jnp.where(top, r, c)

    m = jnp.max(jnp.where(top, _fold(se, jnp.maximum), _fold(so, jnp.maximum)), axis=1, keepdims=True)
    me, mo = split(m)
    de, do = se - _tile(me, NL), so - _tile(mo, NL)
    if c is not None:
        de, do = de * c, do * c
    pe, po = jnp.exp2(de), jnp.exp2(do)
    l = jnp.sum(jnp.where(top, _fold(pe, jnp.add), _fold(po, jnp.add)), axis=1, keepdims=True)
    ie, io = split(pl.reciprocal(l, approx=True))
    lane = lax.broadcasted_iota(I32, (8, 128), 1)
    return pe, po, jnp.concatenate([ie, jnp.where(lane < 64, ie, io), io], axis=1)


def _pv(groups, hooks=None):
    nb = len(groups) // 16
    accs = {}
    for n, g in enumerate(16 * blk + i for i in range(16) for blk in range(nb)):
        if hooks and n in hooks:
            hooks[n]()
        vload, p = groups[g]
        accs[g] = _fold(vload() * p, jnp.add)
    return jnp.concatenate([accs[g] for g in range(len(groups))], axis=0)


def _lane_reduce_t(acc):
    at = acc.T
    s = at[0:8]
    for i in range(1, 16):
        s = s + at[8 * i:8 * i + 8]
    return s


def _kernel(x_hbm, kt_hbm, vt_hbm, wq_hbm, wo_hbm, wr_hbm, wg_hbm, wu_hbm, wd_hbm,
            o_ref,
            kv, vf, kp, wq_raw, wo_raw, wg_raw, wu_raw, wd_raw, wxp, wop, wdp, wguf, wqf, cs,
            xb_ref, wrb, state, spin_ref, c_s, c_p, c_inv, c_o, c_out,
            sems, wsem, *, cfg):
    LA, LEAD, NV = cfg["LA"], cfg["LEAD"], cfg["NV"]
    NM = NH - NV
    HALF = cfg["HALF"]
    order, raw = _order(cfg)

    def piece(i, s):
        q, pair, w, b = i & (TPC - 1), (i >> 2) & (NP - 1), (i >> 6) & 1, i >> 7
        r0 = (q + s * TPC) * 8
        if not isinstance(i, int):
            r0 = pl.multiple_of(r0, 8)
        return pair, w, b, w * (1 + (b & 1)), i & (RING - 1), r0

    def start_piece(i, s, hf=None):
        pair, w, b, plane, ring, r0 = piece(i, s)
        osl = pl.ds(pair * RO, RO) if hf is None else pl.ds(pair * RO + hf * (RO // 2), RO // 2)

        def go(ww):
            src = vt_hbm if ww else kt_hbm
            pltpu.make_async_copy(src.at[b, osl, pl.ds(r0, 8), pl.ds(SK - W, W)],
                                  kv.at[plane, osl, pl.ds(r0, 8), :],
                                  sems.at[s, ring]).start(priority=1 - s)

        if isinstance(i, int):
            go(w)
        else:
            for ww in range(2):
                pl.when(jnp.logical_and(w == ww, i < NTICK))(functools.partial(go, ww))

    def wait_piece(i, s):
        pair, w, b, plane, ring, r0 = piece(i, s)
        view = kv.at[plane, pl.ds(pair * RO, RO), pl.ds(r0, 8), :]
        pltpu.make_async_copy(view, view, sems.at[s, ring]).wait()

    def wait_tick(i):
        wait_piece(i, 0)
        wait_piece(i, 1)

    def spin(n):
        v = spin_ref[...]
        lane = lax.broadcasted_iota(I32, v.shape, 1).astype(F32)
        for _ in range(n[0]):
            v = jnp.max(v, axis=1, keepdims=True) * 0.5 + lane
        for _ in range(n[1] // 2):
            v = v * 0.5
            v = v + lane
        spin_ref[...] = v

    def full_tick(i):
        wait_tick(i)
        start_piece(i + LEAD + 1, 1)
        start_piece(i + LA, 0)

    def spin_tick(i, c):
        full_tick(i)
        spin(cfg["SPIN"])
        return c

    def half_tick(h, lead, la, work):
        i = h >> 1
        pl.when((h & 1) == 0)(lambda: wait_tick(i))
        start_piece(i + lead, 1, h & 1)
        work()
        start_piece(jnp.where((h & 1) == 1, i + la, NTICK), 0)

    def idle_half(h, c):
        def work():
            o0 = (((h >> 3) & (NP - 1)) - 1) * RO + (((h >> 1) & 3) - 1) * 3
            r = pl.ds(pl.multiple_of((h & 1) * 32, 32), 32)
            vf[pl.ds(o0 - VF0 * RO, 3), r, :] = kv[1 + ((h >> 8) & 1), pl.ds(o0, 3), r, :].astype(F32)
            if cfg["HSPIN"]:
                spin(cfg["HSPIN"])

        half_tick(h, LEAD, LA - 1, work)
        return c

    def advance(t, need):
        t2 = jnp.maximum(t + 2, need)
        wait_tick(t)
        lax.fori_loop(2 * t + 2, 2 * t2 - 2, idle_half, 0)
        wait_tick(t2 - 1)
        start_piece(t2 - 1 + LEAD, 1, 0 if HALF else None)
        return t2

    def mid(t2, n, after=None):
        if n == 0 and HALF:
            start_piece(t2 - 1 + LEAD, 1, 1)
        if n == 1:
            start_piece(t2 + LEAD, 1, 0 if HALF > 1 else None)
            start_piece(t2 - 2 + LA, 0)
            start_piece(t2 - 1 + LA, 0)
        if n == 2 and HALF > 1:
            kv[0, NP * RO, 0:16, 0:128] = jnp.concatenate([after, after], axis=0).astype(BF16)
            start_piece(t2 + LEAD, 1, 1)

    half = D // 2
    small = [pltpu.make_async_copy(x_hbm, xb_ref, wsem.at[0]),
             pltpu.make_async_copy(wr_hbm, wrb, wsem.at[1])]
    big = [pltpu.make_async_copy(wq_hbm, wq_raw, wsem.at[2]),
           pltpu.make_async_copy(wg_hbm, wg_raw, wsem.at[3]),
           pltpu.make_async_copy(wu_hbm.at[pl.ds(0, half)], wu_raw.at[pl.ds(0, half)], wsem.at[4])]
    for cp in big:
        cp.start(priority=1)
    for cp in small:
        cp.start()
    for i in range(LA):
        start_piece(i, 0)
    spin_ref[...] = jnp.zeros(spin_ref.shape, F32)

    inject = [(wo_hbm, wo_raw, 0, 48, HD // 48, 5), (wd_hbm, wd_raw, 0, 48, F // 48, 6),
              (wu_hbm, wu_raw, half, 16, half // 16, 7)]
    for src, dst, row0, rows, n, sem in inject:
        def body(i, c, src=src, dst=dst, row0=row0, rows=rows, sem=sem):
            r = pl.multiple_of(row0 + i * rows, 8)
            pltpu.make_async_copy(src.at[pl.ds(r, rows)], dst.at[pl.ds(r, rows)], wsem.at[sem]).start()
            spin(cfg["WSPIN"])
            return c
        lax.fori_loop(0, n, body, 0)

    for i in range(LEAD + 1):
        start_piece(i, 1)
    for cp in small:
        cp.wait()
    state[...] = jnp.concatenate([xb_ref[...].astype(F32), jnp.zeros((8 - B, D), F32)], axis=0)
    for src, dst, row0, rows, n, sem in inject:
        view = dst.at[pl.ds(row0, rows * n)]
        pltpu.make_async_copy(view, view, wsem.at[sem]).wait()
    for cp in big:
        cp.wait()

    NRP = D // 16

    def repack(h, c):
        full_tick(h)
        r = pl.multiple_of(h * 16, 16)
        r2 = pl.multiple_of(h * 8, 8)
        wxp[pl.ds(r2, 8), 0:HD] = _u32(wq_raw[pl.ds(r, 16), :])
        for n, pos in enumerate(cfg["VQ"]):
            wqf[pl.ds(r, 16), n * PD:(n + 1) * PD] = (
                wq_raw[pl.ds(r, 16), order[pos] * PD:(order[pos] + 1) * PD].astype(F32))
        g = wg_raw[pl.ds(r, 16), :]
        u = wu_raw[pl.ds(r, 16), :]
        gu = jnp.concatenate([w[:, i * 128:(i + 1) * 128] for i in range(NH) for w in (g, u)], axis=1)
        wxp[pl.ds(r2, 8), HD:HD + 2 * F] = _u32(gu)
        if NV:
            wguf[pl.ds(r, 16), :] = gu[:, NM * 256:].astype(F32)
        for src, packed, n in ((wo_raw, wop, 160), (wd_raw, wdp, 48)):
            r = pl.multiple_of(jnp.minimum(h * n, src.shape[0] - n), 16)
            packed[pl.ds(pl.multiple_of(r >> 1, 8), n // 2), :] = _u32(src[pl.ds(r, n), :])
        return c

    lax.fori_loop(0, NRP, repack, 0)

    NCS = (HD + 2 * F) // 768

    def colsum(i, c):
        full_tick(NRP + i)
        c0 = pl.multiple_of(i * 768, 128)
        cs[:, pl.ds(c0, 768)] = _dot(jnp.ones((8, D), BF16), _bf(wxp[:, pl.ds(c0, 768)]))
        return c

    lax.fori_loop(0, NCS, colsum, 0)
    t0 = jnp.int32(NRP + NCS)

    never = spin_ref[...] < -1.0

    def xproj(xb, m, scale, c0, n):
        y = _dot(xb, _bf(wxp[:, pl.ds(c0, n)])) - m * cs[:, pl.ds(c0, n)]
        return y if scale is None else y * scale

    def qproj(xb, m, qscale, k):
        return xproj(xb, m, qscale, k * PD if isinstance(k, int) else pl.multiple_of(k * PD, 128), PD)

    def oproj(ob, k):
        r0 = pl.multiple_of(k * DH, DH) if not isinstance(k, int) else k * DH
        return _dot(ob, _bf(wop[pl.ds(r0, DH), :]))

    def kload(k):
        return [_bf(kp[pl.ds(k * RO + 2 * i, 2)].reshape(64, W)) for i in range(3)]

    def vgroup(slot, k, o, r):
        return lambda: kv[1 + slot, k * RO + o, pl.ds(r * 8, 8), :].astype(F32)

    def pair_groups(slot, k, pe, po):
        return [(vgroup(slot, k, g // RI, g % RI), pe if g < DH // 8 else po) for g in range(PD // 8)]

    def vpu_matvec(xr, w_ref, parts):
        xcol = [jnp.concatenate([xr[:, u * 128:(u + 1) * 128]] * 16, axis=0).T for u in range(D // 128)]
        res = []
        tok = None
        c0 = 0
        for n, nadd in parts:
            acc = None
            for us in ((0, 1), (2, 3), (4,)):
                for i in range(16):
                    for u in us:
                        r = u * 128 + i * 8
                        col = xcol[u][i * 8:i * 8 + 8]
                        if tok is not None:
                            for _ in range(nadd):
                                tok = tok + 1.0
                            col = jnp.where(never, tok, col)
                        y = w_ref[r:r + 8, c0:c0 + n] * _tile(col, n // 128)
                        acc = y if acc is None else acc + y
                        tok = acc[:, 0:128]
            res.append(_rowsum_all(acc))
            c0 += n
        return jnp.concatenate(res, axis=1)

    def act(gu):
        g = gu[:, 0:128]
        return (g * _sigmoid(g) * gu[:, 128:256]).astype(BF16)

    def ffn_res(x, xc, rstd):
        wr = wrb[...].astype(F32)
        wr = jnp.concatenate([jnp.broadcast_to(wr[t:t + 1, :], (8, 128)) for t in range(D // 128)], axis=1)
        return x + xc * rstd, _sigmoid(jnp.sum(xc * wr, axis=1, keepdims=True) * rstd)

    def ffn(x):
        xb, xr, m, xc, rstd = _ln_parts(x)

        hs = [act(xproj(xb, m, rstd, HD + i * 256, 256)) for i in range(NM)]
        gu = (vpu_matvec(xr, wguf, [(NV * 256, cfg["TOK"])]) - m * cs[:, HD + NM * 256:]) * rstd
        hs += [act(gu[:, i * 256:(i + 1) * 256]) for i in range(NV)]
        y = None
        for grp in cfg["DORD"] or [[i] for i in range(NH)]:
            yi = _dot(jnp.concatenate([hs[i] for i in grp], axis=1),
                      _bf(jnp.concatenate([wdp[i * 64:(i + 1) * 64, :] for i in grp], axis=0)))
            y = yi if y is None else y + yi
        res, gate = ffn_res(x, xc, rstd)
        return res + y * gate

    NFT = NH // 2 + 1

    def ffn_ticked(x, t):
        def body(i, carry):
            h, y, _ = carry
            full_tick(t + i)
            xb, _, m, xc, rstd = _ln_parts(x)
            c0 = pl.multiple_of(HD + jnp.minimum(i, NFT - 2) * 512, 128)
            gu = xproj(xb, m, rstd, c0, 512)
            r0 = pl.multiple_of(jnp.maximum(i - 1, 0) * 128, 128)
            y = y + _dot(h, _bf(wdp[pl.ds(r0, 128), :]))
            res, gate = ffn_res(x, xc, rstd)
            return jnp.concatenate([act(gu[:, 0:256]), act(gu[:, 256:512])], axis=1), y, res + y * gate

        return lax.fori_loop(0, NFT, body, (jnp.zeros((8, 256), BF16), jnp.zeros((8, D), F32), x))[2]

    NHP = 2 * B - 1

    def half_period(hp, t):
        b = hp >> 1
        slot = b & 1
        first = (hp & 1) == 0
        vbase = jnp.where(first, b * TPP + (NP + 1) * TPC, -TPP)

        tr = jnp.where(first, jnp.maximum(t, b * TPP + cfg["KRP"]), t)
        lax.fori_loop(t, tr, spin_tick, 0)

        def k_repack(h, c):
            def work():
                o0 = (h - 2 * tr) * 4
                kp[pl.ds(o0, 4)] = _u32(kv[0, pl.ds(o0, 4)].reshape(4 * 64, W)).reshape(4, 32, W)
                spin(cfg["KSPIN"])

            half_tick(h, LEAD + 1, LA, work)
            return c

        t = jnp.where(first, tr + NP * RO // 8, t)
        lax.fori_loop(2 * tr, 2 * t, k_repack, 0)

        x = jnp.broadcast_to(state[pl.ds(b, 1), :], (8, D))
        xb, _, m, _, rstd = _ln_parts(x)
        qscale = rstd * SCALE

        def step(j, carry):
            t, q, se, so, pe, po, inv, o, out = carry
            kv_ = jnp.maximum(j - 3, 0)
            t = advance(t, vbase + kv_ * TPC)
            se_n, so_n = _scores(q, kload(jnp.clip(j - 1, 0, NP - 1)))
            q_n = qproj(xb, m, qscale, jnp.minimum(j, NP - 1))
            out = out + oproj(o, jnp.maximum(j - 4, 0))
            pe_n, po_n, inv_n = _softmax_pair(se, so)
            acc = _pv(pair_groups(slot, kv_, pe, po),
                      {cfg["PVMID"][0]: lambda: mid(t, 0), cfg["PVMID"][1]: lambda: mid(t, 1)})
            mid(t, 2, q_n[:, 256:384])
            o_n = (_lane_reduce_t(acc) * jnp.where(j >= 3, inv, 0.0)).astype(BF16)
            return t, q_n, se_n, so_n, pe_n, po_n, inv_n, o_n, out

        zw = (lax.broadcasted_iota(I32, (8, W), 0) + lax.broadcasted_iota(I32, (8, W), 1)).astype(F32) * (1.0 / W)
        zp = zw[:, :PD]
        init = (t, zp, zw, zw, zw, zw, zp, jnp.zeros((8, PD), BF16), jnp.zeros((8, D), F32))
        last = hp == NHP - 1
        t, _, se, so, pe, po, inv, o, out = lax.fori_loop(0, jnp.where(last, NP + 1, NP + 2), step, init)
        t2 = jnp.maximum(t + 2, vbase + (NP - 1) * TPC)

        @pl.when(last)
        def _():
            c_s[0] = se
            c_s[1] = so
            c_p[0] = pe * _tile(inv[:, 0:128], NL)
            c_p[1] = po * _tile(inv[:, 256:384], NL)
            c_o[...] = o.astype(F32)
            c_out[...] = out

        @pl.when(jnp.logical_not(last))
        def _():
            advance(t, t2)
            y = out + oproj(o, NP - 2)
            acc = _pv(pair_groups(slot, NP - 1, pe, po), {24: lambda: mid(t2, 0), 45: lambda: mid(t2, 1)})
            olast = _lane_reduce_t(acc) * inv
            mid(t2, 2, olast[:, 0:128])
            olast = olast.astype(BF16)
            full_tick(t2)
            y = y + oproj(olast, NP - 1)
            state[pl.ds(b, 1), :] = ffn_ticked(x + _rowsum_all(y), t2 + 1)[0:1]

        return t2 + 1 + NFT

    lax.fori_loop(0, NHP, half_period, t0)

    slot = (B - 1) % 2
    ka, kb = NP - 2, NP - 1

    def wo_rows(runs):
        return _bf(jnp.concatenate(
            [wop[(k * PD + o * 64 + r * 8) // 2:(k * PD + o * 64 + (r + n) * 8) // 2, :] for k, o, r, n in runs],
            axis=0))

    def run_groups(runs, ps):
        return [(vgroup(slot, k, o, r + i), ps[k][0 if o < RO // 2 else 1]) for k, o, r, n in runs for i in range(n)]

    for i in range(NTICK - 2 * TPC, NTICK):
        wait_piece(i, 1)
    pe, po, inv = _softmax_pair(c_s[0], c_s[1])
    ps = {ka: (c_p[0], c_p[1]), kb: (pe * _tile(inv[:, 0:128], NL), po * _tile(inv[:, 256:384], NL))}
    out = c_out[...] + oproj(c_o[...].astype(BF16), NP - 3)
    runs0 = [(k, o, TPC, TPC) for k in (ka, kb) for o in range(RO)]
    lane = lax.broadcasted_iota(I32, (8, 128), 1)
    sc0 = jnp.concatenate([jnp.ones((8, 128), F32), jnp.where(lane < 64, 1.0, inv[:, 0:128]),
                           jnp.where(lane < 32, inv[:, 0:128], inv[:, 256:384])], axis=1)
    o0 = (_lane_reduce_t(_pv(run_groups(runs0, {ka: ps[ka], kb: (pe, po)}))) * sc0).astype(BF16)

    for i in range(NTICK - 2 * TPC, NTICK - 2):
        wait_piece(i, 0)
    out = out + _dot(o0, wo_rows(runs0))
    runs1 = [(ka, o, 0, TPC) for o in range(RO)] + [(kb, o, 0, 2) for o in range(4)]
    o1 = _lane_reduce_t(_pv(run_groups(runs1, ps))).astype(BF16)

    for i in range(NTICK - 2, NTICK):
        wait_piece(i, 0)
    out = out + _dot(o1, wo_rows(runs1))
    runs2 = [(kb, o, 0, 2) for o in range(4, RO)] + [(kb, o, 2, 2) for o in range(RO)]
    w2 = wo_rows(runs2).astype(F32)
    for i, (vload, p) in enumerate(run_groups(runs2, ps)):
        out = out + w2[i * 8:(i + 1) * 8] * jnp.sum(_fold(vload() * p, jnp.add), axis=1, keepdims=True)
    x = jnp.broadcast_to(state[B - 1:B, :], (8, D)) + _rowsum_all(out)

    def attn_fast(x):
        xb, xr, m, _, rstd = _ln_parts(x)
        qscale = rstd * SCALE
        q, sc, ps, os_ = {}, {}, {}, {}
        out = None
        oslot = {}
        sl = cfg["OLAG"]
        for i in range(NP):
            while sl in cfg["OSKIP"]:
                sl += 1
            oslot[sl] = i
            sl += 1
        if cfg["VQ"]:
            qv = vpu_matvec(xr, wqf, [(n * PD, d) for n, d in cfg["QTOK"]])
            for n, pos in enumerate(cfg["VQ"]):
                k = order[pos]
                q[pos] = (qv[:, n * PD:(n + 1) * PD] - m * cs[:, k * PD:(k + 1) * PD]) * qscale
        qm = [pos for pos in range(NP) if pos not in cfg["VQ"]]
        for s in range(-3, sl):
            if cfg["QEARLY"]:
                if 0 <= s + 3 < len(qm):
                    q[qm[s + 3]] = qproj(xb, m, qscale if qm[s + 3] >= cfg["NLS"] else None, order[qm[s + 3]])
            elif s + 3 in qm:
                q[s + 3] = qproj(xb, m, qscale if s + 3 >= cfg["NLS"] else None, order[s + 3])
            if 0 <= s + 2 < NP:
                sc[s + 2] = _scores(q.pop(s + 2), kload(order[s + 2]))
            if s in oslot:
                y = oproj(os_.pop(oslot[s]), order[oslot[s]])
                out = y if out is None else out + y
            if 0 <= s + 1 < NP:
                ps[s + 1] = _softmax_pair(*sc.pop(s + 1), None if s + 1 >= cfg["NLS"] else qscale)
            if 0 <= s < NP:
                pe, po, inv = ps.pop(s)
                k = order[s]
                groups = pair_groups(slot, k, pe, po)
                if k not in raw:
                    groups = [(functools.partial(lambda g: vf[(k - VF0) * RO + g // RI, pl.ds((g % RI) * 8, 8), :], g), p)
                              for g, (_, p) in enumerate(groups)]
                os_[s] = (_lane_reduce_t(_pv(groups)) * inv).astype(BF16)
        return x + _rowsum_all(out)

    if cfg["TAIL"] >= 1:
        x = ffn(x)
    if cfg["TAIL"] >= 2:
        x = ffn(attn_fast(x))
    row = lax.broadcasted_iota(I32, (8, D), 0)
    o_ref[...] = jnp.where(row == B - 1, x, state[...])[0:B].astype(o_ref.dtype)


def _call(cfg, A_x, A_k_cache, A_v_cache, A_wq, A_wo, B_w_r, B_w_gate, B_w_up, B_w_down):
    kt = jnp.swapaxes(A_k_cache, 2, 3).reshape(B, NP * RO, RI * 8, SK)
    vt = jnp.swapaxes(A_v_cache, 2, 3).reshape(B, NP * RO, RI * 8, SK)
    out = pl.pallas_call(
        functools.partial(_kernel, cfg=cfg),
        out_shape=jax.ShapeDtypeStruct((B, D), BF16),
        in_specs=[pl.BlockSpec(memory_space=pl.ANY)] * 9,
        out_specs=pl.BlockSpec(memory_space=pltpu.VMEM),
        scratch_shapes=[
            pltpu.VMEM((3, NP * RO + 1, RI * 8, W), BF16),
            pltpu.VMEM(((NP - 1 - VF0) * RO, RI * 8, W), F32),
            pltpu.VMEM((NP * RO, RI * 4, W), U32),
            pltpu.VMEM((D, HD), BF16),
            pltpu.VMEM((HD, D), BF16),
            pltpu.VMEM((D, F), BF16),
            pltpu.VMEM((D, F), BF16),
            pltpu.VMEM((F, D), BF16),
            pltpu.VMEM((D // 2, HD + 2 * F), U32),
            pltpu.VMEM((HD // 2, D), U32),
            pltpu.VMEM((F // 2, D), U32),
            pltpu.VMEM((D, cfg["NV"] * 256), F32),
            pltpu.VMEM((D, max(len(cfg["VQ"]), 1) * PD), F32),
            pltpu.VMEM((8, HD + 2 * F), F32),
            pltpu.VMEM((B, D), BF16),
            pltpu.VMEM((D // 128, 128), BF16),
            pltpu.VMEM((8, D), F32),
            pltpu.VMEM((8, 128), F32),
            pltpu.VMEM((2, 8, W), F32),
            pltpu.VMEM((2, 8, W), F32),
            pltpu.VMEM((8, PD), F32),
            pltpu.VMEM((8, PD), F32),
            pltpu.VMEM((8, D), F32),
            pltpu.SemaphoreType.DMA((2, RING)),
            pltpu.SemaphoreType.DMA((8,)),
        ],
        compiler_params=pltpu.CompilerParams(vmem_limit_bytes=120 * 1024 * 1024,
                                             disable_bounds_checks=True,
                                             disable_semaphore_checks=True),
        name="fused_decode",
    )(A_x.reshape(B, D), kt, vt, A_wq, A_wo, B_w_r.reshape(D // 128, 128), B_w_gate, B_w_up, B_w_down)
    return out.reshape(B, 1, D)


@jax.jit
def pallas_interleave_layers__sliding_block_cached__moe_arch_mod__decode_kernel(
    A_x: jax.Array,
    A_k_cache: jax.Array,
    A_v_cache: jax.Array,
    A_wq: jax.Array,
    A_wo: jax.Array,
    B_x: jax.Array,
    B_w_r: jax.Array,
    B_w_gate: jax.Array,
    B_w_up: jax.Array,
    B_w_down: jax.Array,
):
    del B_x
    return _call(CFG, A_x, A_k_cache, A_v_cache, A_wq, A_wo, B_w_r, B_w_gate, B_w_up, B_w_down)
```

```python
import functools

import jax
import jax.numpy as jnp
from jax import lax
import jax.experimental.pallas as pl
import jax.experimental.pallas.tpu as pltpu

F32 = jnp.float32
BF16 = jnp.bfloat16
U32 = jnp.uint32
I32 = jnp.int32

B, D, H, DH, SK, F = 4, 640, 32, 192, 4096, 1536
W = min(4096, max(256, SK // 4))
NP = H // 2
PD = 2 * DH
HD = H * DH
NL = W // 128
NH = F // 128
EPS = 1e-5
SCALE = DH ** -0.5 * 1.4426950408889634

RI = 8
RO = PD // (8 * RI)
TPC = RI // 2
TPP = 2 * NP * TPC
NTICK = B * TPP
RING = 32
VF0, VF1 = 3, 12

CFG = dict(
    LA=23,
    LEAD=11,
    SPIN=(1, 50),
    WSPIN=(1, 45),
    HALF=2,
    HSPIN=(),
    KSPIN=(1, 20),
    PVMID=(21, 45),
    KRP=54,
    OLAG=4,
    OSKIP=(6,),
    NV=4,
    TOK=0,
    QTOK=1,
    ND=4,
    DTOK=1,
    VO=(1,),
    VOT=(15, 32),
    OTOK=0,
    VQ=(3, 4, 5),
    RAWPOS=(2, 6, 7, 8, 10, 11, 12),
    QEARLY=True,
    NLS=3,
    TAIL=2,
)


def _order(cfg):
    raw = [k for k in range(NP) if not VF0 <= k < VF1]
    order = list(range(VF0, VF1))
    for pos, k in zip(sorted(cfg["RAWPOS"]), raw):
        order.insert(pos, k)
    return order, raw


def _rowsum_all(x):
    x = x + pltpu.roll(x, 4, 0)
    x = x + pltpu.roll(x, 2, 0)
    return x + pltpu.roll(x, 1, 0)


def _bf(x):
    return pltpu.bitcast(x, BF16)


def _u32(x):
    return pltpu.bitcast(x, U32)


def _dot(a, b):
    return jnp.dot(a, b, preferred_element_type=F32)


def _sigmoid(x):
    return pl.reciprocal(1.0 + jnp.exp(-x), approx=True)


def _ln_parts(x):
    xb = x.astype(BF16)
    xr = xb.astype(F32)
    m = jnp.sum(xr, axis=1, keepdims=True) * (1.0 / D)
    xc = xr - m
    v = jnp.sum(xc * xc, axis=1, keepdims=True) * (1.0 / D)
    return xb, xr, m, xc, lax.rsqrt(v + EPS)


def _scores(q, kk):
    lane = lax.broadcasted_iota(I32, (8, 128), 1)
    q0 = q[:, 0:128].astype(BF16)
    qm = q[:, 128:256]
    q2 = q[:, 256:384].astype(BF16)
    mid = jnp.concatenate([jnp.where(lane < 64, qm, 0.0), jnp.where(lane >= 64, qm, 0.0)],
                          axis=0).astype(BF16)
    r0 = _dot(q0, kk[0])
    rm = _dot(mid, kk[1])
    r2 = _dot(q2, kk[2])
    return r0 + rm[0:8], rm[8:16] + r2


def _fold(x, op):
    r = x[:, 0:128]
    for t in range(1, x.shape[1] // 128):
        r = op(r, x[:, t * 128:(t + 1) * 128])
    return r


def _tile(x, n):
    return jnp.concatenate([x] * n, axis=1)


def _softmax_pair(se, so, c=None):
    top = lax.broadcasted_iota(I32, (8, 128), 0) < 4

    def split(c):
        c = jnp.broadcast_to(c, (8, 128))
        r = pltpu.roll(c, 4, 0)
        return jnp.where(top, c, r), jnp.where(top, r, c)

    m = jnp.max(jnp.where(top, _fold(se, jnp.maximum), _fold(so, jnp.maximum)), axis=1, keepdims=True)
    me, mo = split(m)
    de, do = se - _tile(me, NL), so - _tile(mo, NL)
    if c is not None:
        de, do = de * c, do * c
    pe, po = jnp.exp2(de), jnp.exp2(do)
    l = jnp.sum(jnp.where(top, _fold(pe, jnp.add), _fold(po, jnp.add)), axis=1, keepdims=True)
    ie, io = split(pl.reciprocal(l, approx=True))
    lane = lax.broadcasted_iota(I32, (8, 128), 1)
    return pe, po, jnp.concatenate([ie, jnp.where(lane < 64, ie, io), io], axis=1)


def _pv(groups, hooks=None):
    nb = len(groups) // 16
    accs = {}
    for n, g in enumerate(16 * blk + i for i in range(16) for blk in range(nb)):
        if hooks and n in hooks:
            hooks[n]()
        vload, p = groups[g]
        accs[g] = _fold(vload() * p, jnp.add)
    return jnp.concatenate([accs[g] for g in range(len(groups))], axis=0)


def _lane_reduce_t(acc):
    at = acc.T
    s = at[0:8]
    for i in range(1, 16):
        s = s + at[8 * i:8 * i + 8]
    return s


def _kernel(x_hbm, kt_hbm, vt_hbm, wq_hbm, wo_hbm, wr_hbm, wg_hbm, wu_hbm, wd_hbm,
            o_ref,
            kv, vf, kp, wq_raw, wo_raw, wg_raw, wu_raw, wd_raw, wxp, wop, wdp, wguf, wqf, wdf, wof, cs,
            xb_ref, wrb, state, spin_ref, c_s, c_p, c_o, c_out,
            sems, wsem, *, cfg):
    LA, LEAD, NV = cfg["LA"], cfg["LEAD"], cfg["NV"]
    NM = NH - NV
    ND = cfg["ND"]
    HALF = cfg["HALF"]
    order, raw = _order(cfg)

    def piece(i, s):
        q, pair, w, b = i & (TPC - 1), (i >> 2) & (NP - 1), (i >> 6) & 1, i >> 7
        r0 = (q + s * TPC) * 8
        if not isinstance(i, int):
            r0 = pl.multiple_of(r0, 8)
        return pair, w, b, w * (1 + (b & 1)), i & (RING - 1), r0

    def start_piece(i, s, hf=None):
        pair, w, b, plane, ring, r0 = piece(i, s)
        osl = pl.ds(pair * RO, RO) if hf is None else pl.ds(pair * RO + hf * (RO // 2), RO // 2)

        def go(ww):
            src = vt_hbm if ww else kt_hbm
            pltpu.make_async_copy(src.at[b, osl, pl.ds(r0, 8), pl.ds(SK - W, W)],
                                  kv.at[plane, osl, pl.ds(r0, 8), :],
                                  sems.at[s, ring]).start(priority=1 - s)

        if isinstance(i, int):
            go(w)
        else:
            for ww in range(2):
                pl.when(jnp.logical_and(w == ww, i < NTICK))(functools.partial(go, ww))

    def wait_piece(i, s):
        pair, w, b, plane, ring, r0 = piece(i, s)
        view = kv.at[plane, pl.ds(pair * RO, RO), pl.ds(r0, 8), :]
        pltpu.make_async_copy(view, view, sems.at[s, ring]).wait()

    def wait_tick(i):
        wait_piece(i, 0)
        wait_piece(i, 1)

    def spin(n):
        v = spin_ref[...]
        lane = lax.broadcasted_iota(I32, v.shape, 1).astype(F32)
        for _ in range(n[0]):
            v = jnp.max(v, axis=1, keepdims=True) * 0.5 + lane
        for _ in range(n[1] // 2):
            v = v * 0.5
            v = v + lane
        spin_ref[...] = v

    def full_tick(i):
        wait_tick(i)
        start_piece(i + LEAD + 1, 1)
        start_piece(i + LA, 0)

    def spin_tick(i, c):
        full_tick(i)
        spin(cfg["SPIN"])
        return c

    def half_tick(h, lead, la, work):
        i = h >> 1
        pl.when((h & 1) == 0)(lambda: wait_tick(i))
        start_piece(i + lead, 1, h & 1)
        work()
        start_piece(jnp.where((h & 1) == 1, i + la, NTICK), 0)

    def idle_half(h, c):
        def work():
            o0 = (((h >> 3) & (NP - 1)) - 1) * RO + (((h >> 1) & 3) - 1) * 3
            r = pl.ds(pl.multiple_of((h & 1) * 32, 32), 32)
            vf[pl.ds(o0 - VF0 * RO, 3), r, :] = kv[1 + ((h >> 8) & 1), pl.ds(o0, 3), r, :].astype(F32)
            if cfg["HSPIN"]:
                spin(cfg["HSPIN"])

        half_tick(h, LEAD, LA - 1, work)
        return c

    def advance(t, need):
        t2 = jnp.maximum(t + 2, need)
        wait_tick(t)
        lax.fori_loop(2 * t + 2, 2 * t2 - 2, idle_half, 0)
        wait_tick(t2 - 1)
        start_piece(t2 - 1 + LEAD, 1, 0 if HALF else None)
        return t2

    def mid(t2, n, after=None):
        if n == 0 and HALF:
            start_piece(t2 - 1 + LEAD, 1, 1)
        if n == 1:
            start_piece(t2 + LEAD, 1, 0 if HALF > 1 else None)
            start_piece(t2 - 2 + LA, 0)
            start_piece(t2 - 1 + LA, 0)
        if n == 2 and HALF > 1:
            kv[0, NP * RO, 0:16, 0:128] = jnp.concatenate([after, after], axis=0).astype(BF16)
            start_piece(t2 + LEAD, 1, 1)

    half = D // 2
    small = [pltpu.make_async_copy(x_hbm, xb_ref, wsem.at[0]),
             pltpu.make_async_copy(wr_hbm, wrb, wsem.at[1])]
    big = [pltpu.make_async_copy(wq_hbm, wq_raw, wsem.at[2]),
           pltpu.make_async_copy(wg_hbm, wg_raw, wsem.at[3]),
           pltpu.make_async_copy(wu_hbm.at[pl.ds(0, half)], wu_raw.at[pl.ds(0, half)], wsem.at[4])]
    for cp in big:
        cp.start(priority=1)
    for cp in small:
        cp.start()
    for i in range(LA):
        start_piece(i, 0)
    spin_ref[...] = jnp.zeros(spin_ref.shape, F32)

    inject = [(wo_hbm, wo_raw, 0, 48, HD // 48, 5), (wd_hbm, wd_raw, 0, 48, F // 48, 6),
              (wu_hbm, wu_raw, half, 16, half // 16, 7)]
    for src, dst, row0, rows, n, sem in inject:
        def body(i, c, src=src, dst=dst, row0=row0, rows=rows, sem=sem):
            r = pl.multiple_of(row0 + i * rows, 8)
            pltpu.make_async_copy(src.at[pl.ds(r, rows)], dst.at[pl.ds(r, rows)], wsem.at[sem]).start()
            spin(cfg["WSPIN"])
            return c
        lax.fori_loop(0, n, body, 0)

    for i in range(LEAD + 1):
        start_piece(i, 1)
    for cp in small:
        cp.wait()
    state[...] = jnp.concatenate([xb_ref[...].astype(F32), jnp.zeros((8 - B, D), F32)], axis=0)
    for src, dst, row0, rows, n, sem in inject:
        view = dst.at[pl.ds(row0, rows * n)]
        pltpu.make_async_copy(view, view, wsem.at[sem]).wait()
    for cp in big:
        cp.wait()

    NRP = D // 16

    def repack(h, c):
        full_tick(h)
        r = pl.multiple_of(h * 16, 16)
        r2 = pl.multiple_of(h * 8, 8)
        wxp[pl.ds(r2, 8), 0:HD] = _u32(wq_raw[pl.ds(r, 16), :])
        for n, pos in enumerate(cfg["VQ"]):
            wqf[pl.ds(r, 16), n * PD:(n + 1) * PD] = (
                wq_raw[pl.ds(r, 16), order[pos] * PD:(order[pos] + 1) * PD].astype(F32))
        g = wg_raw[pl.ds(r, 16), :]
        u = wu_raw[pl.ds(r, 16), :]
        gu = jnp.concatenate([w[:, i * 128:(i + 1) * 128] for i in range(NH) for w in (g, u)], axis=1)
        wxp[pl.ds(r2, 8), HD:HD + 2 * F] = _u32(gu)
        if NV:
            wguf[pl.ds(r, 16), :] = gu[:, NM * 256:].astype(F32)
        for n, pos in enumerate(cfg["VO"]):
            ro = pl.multiple_of(jnp.minimum(r, PD - 16), 16)
            wof[pl.ds(n * PD + ro, 16), :] = wo_raw[pl.ds(order[pos] * PD + ro, 16), :].astype(F32)
        if ND:
            rd = pl.multiple_of(jnp.minimum(r, ND * 128 - 16), 16)
            wdf[pl.ds(rd, 16), :] = wd_raw[pl.ds(rd, 16), :].astype(F32)
        for src, packed, n in ((wo_raw, wop, 160), (wd_raw, wdp, 48)):
            r = pl.multiple_of(jnp.minimum(h * n, src.shape[0] - n), 16)
            packed[pl.ds(pl.multiple_of(r >> 1, 8), n // 2), :] = _u32(src[pl.ds(r, n), :])
        return c

    lax.fori_loop(0, NRP, repack, 0)

    NCS = (HD + 2 * F) // 768

    def colsum(i, c):
        full_tick(NRP + i)
        c0 = pl.multiple_of(i * 768, 128)
        cs[:, pl.ds(c0, 768)] = _dot(jnp.ones((8, D), BF16), _bf(wxp[:, pl.ds(c0, 768)]))
        return c

    lax.fori_loop(0, NCS, colsum, 0)
    t0 = jnp.int32(NRP + NCS)

    never = spin_ref[...] < -1.0

    def xproj(xb, m, scale, c0, n):
        y = _dot(xb, _bf(wxp[:, pl.ds(c0, n)])) - m * cs[:, pl.ds(c0, n)]
        return y if scale is None else y * scale

    def qproj(xb, m, qscale, k):
        return xproj(xb, m, qscale, k * PD if isinstance(k, int) else pl.multiple_of(k * PD, 128), PD)

    def oproj(ob, k):
        r0 = pl.multiple_of(k * DH, DH) if not isinstance(k, int) else k * DH
        return _dot(ob, _bf(wop[pl.ds(r0, DH), :]))

    def kload(k):
        return [_bf(kp[pl.ds(k * RO + 2 * i, 2)].reshape(64, W)) for i in range(3)]

    def vgroup(slot, k, o, r):
        return lambda: kv[1 + slot, k * RO + o, pl.ds(r * 8, 8), :].astype(F32)

    def pair_groups(slot, k, pe, po):
        return [(vgroup(slot, k, g // RI, g % RI), pe if g < DH // 8 else po) for g in range(PD // 8)]

    def vpu_matvec(xr, w_ref, nadd, per_step=1, tok=None):
        nu = xr.shape[1] // 128
        xcol = [jnp.concatenate([xr[:, u * 128:(u + 1) * 128]] * 16, axis=0).T for u in range(nu)]
        seq = [(u, i) for u0 in range(0, nu, 2) for i in range(16) for u in range(u0, min(u0 + 2, nu))]
        accs = [None] * per_step
        for n in range(0, len(seq), per_step):
            if tok is not None:
                for _ in range(nadd):
                    tok = tok + 1.0
            for a, (u, i) in enumerate(seq[n:n + per_step]):
                col = xcol[u][i * 8:i * 8 + 8]
                if tok is not None:
                    col = jnp.where(never, tok, col)
                y = w_ref[u * 128 + i * 8:u * 128 + i * 8 + 8, :] * _tile(col, w_ref.shape[1] // 128)
                accs[a] = y if accs[a] is None else accs[a] + y
            tok = accs[0][:, 0:128]
        return functools.reduce(jnp.add, accs), tok

    def act(gu):
        g = gu[:, 0:128]
        return (g * _sigmoid(g) * gu[:, 128:256]).astype(BF16)

    def ffn_res(x, xc, rstd):
        wr = wrb[...].astype(F32)
        wr = jnp.concatenate([jnp.broadcast_to(wr[t:t + 1, :], (8, 128)) for t in range(D // 128)], axis=1)
        return x + xc * rstd, _sigmoid(jnp.sum(xc * wr, axis=1, keepdims=True) * rstd)

    def ffn(x):
        xb, xr, m, xc, rstd = _ln_parts(x)

        hs = [act(xproj(xb, m, rstd, HD + i * 256, 256)) for i in range(NM)]
        gu, tok = vpu_matvec(xr, wguf, cfg["TOK"])
        gu = (_rowsum_all(gu) - m * cs[:, HD + NM * 256:]) * rstd
        hs += [act(gu[:, i * 256:(i + 1) * 256]) for i in range(NV)]
        y = None
        for i in range(ND, NH):
            yi = _dot(hs[i], _bf(wdp[i * 64:(i + 1) * 64, :]))
            y = yi if y is None else y + yi
        if ND:
            yv, _ = vpu_matvec(jnp.concatenate(hs[:ND], axis=1).astype(F32), wdf, cfg["DTOK"], 2, tok)
            y = y + _rowsum_all(yv)
        res, gate = ffn_res(x, xc, rstd)
        return res + y * gate

    NFT = NH // 2 + 1

    def ffn_ticked(x, t):
        def body(i, carry):
            h, y, _ = carry
            full_tick(t + i)
            xb, _, m, xc, rstd = _ln_parts(x)
            c0 = pl.multiple_of(HD + jnp.minimum(i, NFT - 2) * 512, 128)
            gu = xproj(xb, m, rstd, c0, 512)
            r0 = pl.multiple_of(jnp.maximum(i - 1, 0) * 128, 128)
            y = y + _dot(h, _bf(wdp[pl.ds(r0, 128), :]))
            res, gate = ffn_res(x, xc, rstd)
            return jnp.concatenate([act(gu[:, 0:256]), act(gu[:, 256:512])], axis=1), y, res + y * gate

        return lax.fori_loop(0, NFT, body, (jnp.zeros((8, 256), BF16), jnp.zeros((8, D), F32), x))[2]

    NHP = 2 * B - 1

    def half_period(hp, t):
        b = hp >> 1
        slot = b & 1
        first = (hp & 1) == 0
        vbase = jnp.where(first, b * TPP + (NP + 1) * TPC, -TPP)

        tr = jnp.where(first, jnp.maximum(t, b * TPP + cfg["KRP"]), t)
        lax.fori_loop(t, tr, spin_tick, 0)

        def k_repack(h, c):
            def work():
                o0 = (h - 2 * tr) * 4
                kp[pl.ds(o0, 4)] = _u32(kv[0, pl.ds(o0, 4)].reshape(4 * 64, W)).reshape(4, 32, W)
                spin(cfg["KSPIN"])

            half_tick(h, LEAD + 1, LA, work)
            return c

        t = jnp.where(first, tr + NP * RO // 8, t)
        lax.fori_loop(2 * tr, 2 * t, k_repack, 0)

        x = jnp.broadcast_to(state[pl.ds(b, 1), :], (8, D))
        xb, _, m, _, rstd = _ln_parts(x)
        qscale = rstd * SCALE

        def step(j, carry):
            t, q, se, so, pe, po, inv, o, out = carry
            kv_ = jnp.maximum(j - 3, 0)
            t = advance(t, vbase + kv_ * TPC)
            se_n, so_n = _scores(q, kload(jnp.clip(j - 1, 0, NP - 1)))
            q_n = qproj(xb, m, qscale, jnp.minimum(j, NP - 1))
            out = out + oproj(o, jnp.maximum(j - 4, 0))
            pe_n, po_n, inv_n = _softmax_pair(se, so)
            acc = _pv(pair_groups(slot, kv_, pe, po),
                      {cfg["PVMID"][0]: lambda: mid(t, 0), cfg["PVMID"][1]: lambda: mid(t, 1)})
            mid(t, 2, q_n[:, 256:384])
            o_n = (_lane_reduce_t(acc) * jnp.where(j >= 3, inv, 0.0)).astype(BF16)
            return t, q_n, se_n, so_n, pe_n, po_n, inv_n, o_n, out

        zw = (lax.broadcasted_iota(I32, (8, W), 0) + lax.broadcasted_iota(I32, (8, W), 1)).astype(F32) * (1.0 / W)
        zp = zw[:, :PD]
        init = (t, zp, zw, zw, zw, zw, zp, jnp.zeros((8, PD), BF16), jnp.zeros((8, D), F32))
        last = hp == NHP - 1
        t, q, se, so, pe, po, inv, o, out = lax.fori_loop(0, jnp.where(last, NP, NP + 2), step, init)
        t2 = jnp.maximum(t + 2, vbase + (NP - 1) * TPC)

        @pl.when(last)
        def _():
            c_s[0] = se
            c_s[1] = so
            c_p[0] = pe
            c_p[1] = po
            c_o[0] = q
            c_o[1] = inv
            c_o[2] = o.astype(F32)
            c_out[...] = out

        @pl.when(jnp.logical_not(last))
        def _():
            advance(t, t2)
            y = out + oproj(o, NP - 2)
            acc = _pv(pair_groups(slot, NP - 1, pe, po), {24: lambda: mid(t2, 0), 45: lambda: mid(t2, 1)})
            olast = _lane_reduce_t(acc) * inv
            mid(t2, 2, olast[:, 0:128])
            olast = olast.astype(BF16)
            full_tick(t2)
            y = y + oproj(olast, NP - 1)
            state[pl.ds(b, 1), :] = ffn_ticked(x + _rowsum_all(y), t2 + 1)[0:1]

        return t2 + 1 + NFT

    lax.fori_loop(0, NHP, half_period, t0)

    slot = (B - 1) % 2
    ka, kb = NP - 2, NP - 1

    def wo_rows(runs):
        return _bf(jnp.concatenate(
            [wop[(k * PD + o * 64 + r * 8) // 2:(k * PD + o * 64 + (r + n) * 8) // 2, :] for k, o, r, n in runs],
            axis=0))

    def run_groups(runs, ps):
        return [(vgroup(slot, k, o, r + i), ps[k][0 if o < RO // 2 else 1]) for k, o, r, n in runs for i in range(n)]

    def normalised(pe, po, inv):
        return pe * _tile(inv[:, 0:128], NL), po * _tile(inv[:, 256:384], NL)

    for i in range(NTICK - 3 * TPC, NTICK - 2 * TPC):
        wait_tick(i)
    se, so = _scores(c_o[0], kload(kb))
    out = c_out[...] + oproj(c_o[2].astype(BF16), NP - 4)
    pa = normalised(*_softmax_pair(c_s[0], c_s[1]))
    o = (_lane_reduce_t(_pv(pair_groups(slot, NP - 3, c_p[0], c_p[1]))) * c_o[1]).astype(BF16)

    for i in range(NTICK - 2 * TPC, NTICK):
        wait_piece(i, 1)
    pe, po, inv = _softmax_pair(se, so)
    ps = {ka: pa, kb: normalised(pe, po, inv)}
    out = out + oproj(o, NP - 3)
    runs0 = [(k, o, TPC, TPC) for k in (ka, kb) for o in range(RO)]
    lane = lax.broadcasted_iota(I32, (8, 128), 1)
    sc0 = jnp.concatenate([jnp.ones((8, 128), F32), jnp.where(lane < 64, 1.0, inv[:, 0:128]),
                           jnp.where(lane < 32, inv[:, 0:128], inv[:, 256:384])], axis=1)
    o0 = (_lane_reduce_t(_pv(run_groups(runs0, {ka: ps[ka], kb: (pe, po)}))) * sc0).astype(BF16)

    for i in range(NTICK - 2 * TPC, NTICK - 2):
        wait_piece(i, 0)
    out = out + _dot(o0, wo_rows(runs0))
    runs1 = [(ka, o, 0, TPC) for o in range(RO)] + [(kb, o, 0, 2) for o in range(4)]
    o1 = _lane_reduce_t(_pv(run_groups(runs1, ps))).astype(BF16)

    for i in range(NTICK - 2, NTICK):
        wait_piece(i, 0)
    out = out + _dot(o1, wo_rows(runs1))
    runs2 = [(kb, o, 0, 2) for o in range(4, RO)] + [(kb, o, 2, 2) for o in range(RO)]
    w2 = wo_rows(runs2).astype(F32)
    for i, (vload, p) in enumerate(run_groups(runs2, ps)):
        out = out + w2[i * 8:(i + 1) * 8] * jnp.sum(_fold(vload() * p, jnp.add), axis=1, keepdims=True)
    x = jnp.broadcast_to(state[B - 1:B, :], (8, D)) + _rowsum_all(out)

    def attn_fast(x):
        xb, xr, m, _, rstd = _ln_parts(x)
        qscale = rstd * SCALE
        q, sc, ps, os_ = {}, {}, {}, {}
        out = None
        oslot = {}
        sl = cfg["OLAG"]
        for i in range(NP):
            while sl in cfg["OSKIP"]:
                sl += 1
            if i not in cfg["VO"]:
                oslot[sl] = i
            sl += 1
        if cfg["VQ"]:
            qv = _rowsum_all(vpu_matvec(xr, wqf, cfg["QTOK"])[0])
            for n, pos in enumerate(cfg["VQ"]):
                k = order[pos]
                q[pos] = (qv[:, n * PD:(n + 1) * PD] - m * cs[:, k * PD:(k + 1) * PD]) * qscale
        qm = [pos for pos in range(NP) if pos not in cfg["VQ"]]
        for s in range(-3, sl):
            if cfg["QEARLY"]:
                if 0 <= s + 3 < len(qm):
                    q[qm[s + 3]] = qproj(xb, m, qscale if qm[s + 3] >= cfg["NLS"] else None, order[qm[s + 3]])
            elif s + 3 in qm:
                q[s + 3] = qproj(xb, m, qscale if s + 3 >= cfg["NLS"] else None, order[s + 3])
            if 0 <= s + 2 < NP:
                sc[s + 2] = _scores(q.pop(s + 2), kload(order[s + 2]))
            if s in oslot:
                y = oproj(os_.pop(oslot[s]), order[oslot[s]])
                out = y if out is None else out + y
            if 0 <= s + 1 < NP:
                ps[s + 1] = _softmax_pair(*sc.pop(s + 1), None if s + 1 >= cfg["NLS"] else qscale)
            if 0 <= s < NP:
                pe, po, inv = ps.pop(s)
                k = order[s]
                groups = pair_groups(slot, k, pe, po)
                if k not in raw:
                    groups = [(functools.partial(lambda g: vf[(k - VF0) * RO + g // RI, pl.ds((g % RI) * 8, 8), :], g), p)
                              for g, (_, p) in enumerate(groups)]
                acc = _pv(groups)
                if s == cfg["VOT"][0]:
                    tok = acc[cfg["VOT"][1] * 8:cfg["VOT"][1] * 8 + 8]
                o = _lane_reduce_t(acc) * inv
                os_[s] = (_rowsum_all(o) if s in cfg["VO"] else o).astype(BF16)
        if cfg["VO"]:
            ov = jnp.concatenate([os_.pop(i) for i in cfg["VO"]], axis=1).astype(F32)
            out = out + vpu_matvec(ov, wof, cfg["OTOK"], 2, tok)[0]
        return x + _rowsum_all(out)

    if cfg["TAIL"] >= 1:
        x = ffn(x)
    if cfg["TAIL"] >= 2:
        x = ffn(attn_fast(x))
    row = lax.broadcasted_iota(I32, (8, D), 0)
    o_ref[...] = jnp.where(row == B - 1, x, state[...])[0:B].astype(o_ref.dtype)


def _call(cfg, A_x, A_k_cache, A_v_cache, A_wq, A_wo, B_w_r, B_w_gate, B_w_up, B_w_down):
    kt = jnp.swapaxes(A_k_cache, 2, 3).reshape(B, NP * RO, RI * 8, SK)
    vt = jnp.swapaxes(A_v_cache, 2, 3).reshape(B, NP * RO, RI * 8, SK)
    out = pl.pallas_call(
        functools.partial(_kernel, cfg=cfg),
        out_shape=jax.ShapeDtypeStruct((B, D), BF16),
        in_specs=[pl.BlockSpec(memory_space=pl.ANY)] * 9,
        out_specs=pl.BlockSpec(memory_space=pltpu.VMEM),
        scratch_shapes=[
            pltpu.VMEM((3, NP * RO + 1, RI * 8, W), BF16),
            pltpu.VMEM(((NP - 1 - VF0) * RO, RI * 8, W), F32),
            pltpu.VMEM((NP * RO, RI * 4, W), U32),
            pltpu.VMEM((D, HD), BF16),
            pltpu.VMEM((HD, D), BF16),
            pltpu.VMEM((D, F), BF16),
            pltpu.VMEM((D, F), BF16),
            pltpu.VMEM((F, D), BF16),
            pltpu.VMEM((D // 2, HD + 2 * F), U32),
            pltpu.VMEM((HD // 2, D), U32),
            pltpu.VMEM((F // 2, D), U32),
            pltpu.VMEM((D, cfg["NV"] * 256), F32),
            pltpu.VMEM((D, max(len(cfg["VQ"]), 1) * PD), F32),
            pltpu.VMEM((max(cfg["ND"], 1) * 128, D), F32),
            pltpu.VMEM((max(len(cfg["VO"]), 1) * PD, D), F32),
            pltpu.VMEM((8, HD + 2 * F), F32),
            pltpu.VMEM((B, D), BF16),
            pltpu.VMEM((D // 128, 128), BF16),
            pltpu.VMEM((8, D), F32),
            pltpu.VMEM((8, 128), F32),
            pltpu.VMEM((2, 8, W), F32),
            pltpu.VMEM((2, 8, W), F32),
            pltpu.VMEM((3, 8, PD), F32),
            pltpu.VMEM((8, D), F32),
            pltpu.SemaphoreType.DMA((2, RING)),
            pltpu.SemaphoreType.DMA((8,)),
        ],
        compiler_params=pltpu.CompilerParams(vmem_limit_bytes=120 * 1024 * 1024,
                                             disable_bounds_checks=True,
                                             disable_semaphore_checks=True),
        name="fused_decode",
    )(A_x.reshape(B, D), kt, vt, A_wq, A_wo, B_w_r.reshape(D // 128, 128), B_w_gate, B_w_up, B_w_down)
    return out.reshape(B, 1, D)


@jax.jit
def pallas_interleave_layers__sliding_block_cached__moe_arch_mod__decode_kernel(
    A_x: jax.Array,
    A_k_cache: jax.Array,
    A_v_cache: jax.Array,
    A_wq: jax.Array,
    A_wo: jax.Array,
    B_x: jax.Array,
    B_w_r: jax.Array,
    B_w_gate: jax.Array,
    B_w_up: jax.Array,
    B_w_down: jax.Array,
):
    del B_x
    return _call(CFG, A_x, A_k_cache, A_v_cache, A_wq, A_wo, B_w_r, B_w_gate, B_w_up, B_w_down)
```

```python
import functools

import jax
import jax.numpy as jnp
from jax import lax
import jax.experimental.pallas as pl
import jax.experimental.pallas.tpu as pltpu

F32 = jnp.float32
BF16 = jnp.bfloat16
U32 = jnp.uint32
I32 = jnp.int32

B, D, H, DH, SK, F = 4, 640, 32, 192, 4096, 1536
W = min(4096, max(256, SK // 4))
NP = H // 2
PD = 2 * DH
HD = H * DH
NL = W // 128
NH = F // 128
EPS = 1e-5
SCALE = DH ** -0.5 * 1.4426950408889634

RI = 8
RO = PD // (8 * RI)
TPC = RI // 2
TPP = 2 * NP * TPC
NTICK = B * TPP
RING = 32
VF0, VF1 = 3, 12

CFG = dict(
    LA=23,
    LEAD=11,
    SPIN=(1, 50),
    WSPIN=(1, 45),
    HALF=2,
    HSPIN=(),
    KSPIN=(1, 20),
    PVMID=(21, 45),
    KRP=54,
    OLAG=4,
    OSKIP=(6,),
    NV=4,
    TOK=0,
    QTOK=1,
    ND=4,
    DTOK=1,
    VO=(1,),
    VOT=(15, 32),
    OTOK=0,
    VQ=(3, 4, 5),
    RAWPOS=(2, 6, 7, 8, 10, 11, 12),
    QEARLY=True,
    NLS=3,
    TAIL=2,
)


def _order(cfg):
    raw = [k for k in range(NP) if not VF0 <= k < VF1]
    order = list(range(VF0, VF1))
    for pos, k in zip(sorted(cfg["RAWPOS"]), raw):
        order.insert(pos, k)
    return order, raw


def _rowsum_all(x):
    x = x + pltpu.roll(x, 4, 0)
    x = x + pltpu.roll(x, 2, 0)
    return x + pltpu.roll(x, 1, 0)


def _bf(x):
    return pltpu.bitcast(x, BF16)


def _u32(x):
    return pltpu.bitcast(x, U32)


def _dot(a, b):
    return jnp.dot(a, b, preferred_element_type=F32)


def _sigmoid(x):
    return pl.reciprocal(1.0 + jnp.exp(-x), approx=True)


def _round(x):
    return x.astype(BF16).astype(F32)


def _ln_parts(x):
    xb = x.astype(BF16)
    xr = xb.astype(F32)
    m = jnp.sum(xr, axis=1, keepdims=True) * (1.0 / D)
    xc = xr - m
    v = jnp.sum(xc * xc, axis=1, keepdims=True) * (1.0 / D)
    m = _round(m)
    v = _round(_round(v) + EPS)
    return xb, xr, m, xr - m, pl.reciprocal(_round(v * lax.rsqrt(v)), approx=True)


def _scores(q, kk):
    lane = lax.broadcasted_iota(I32, (8, 128), 1)
    q0 = q[:, 0:128].astype(BF16)
    qm = q[:, 128:256]
    q2 = q[:, 256:384].astype(BF16)
    mid = jnp.concatenate([jnp.where(lane < 64, qm, 0.0), jnp.where(lane >= 64, qm, 0.0)],
                          axis=0).astype(BF16)
    r0 = _dot(q0, kk[0])
    rm = _dot(mid, kk[1])
    r2 = _dot(q2, kk[2])
    return r0 + rm[0:8], rm[8:16] + r2


def _fold(x, op):
    r = x[:, 0:128]
    for t in range(1, x.shape[1] // 128):
        r = op(r, x[:, t * 128:(t + 1) * 128])
    return r


def _tile(x, n):
    return jnp.concatenate([x] * n, axis=1)


def _softmax_pair(se, so, c=None):
    top = lax.broadcasted_iota(I32, (8, 128), 0) < 4

    def split(c):
        c = jnp.broadcast_to(c, (8, 128))
        r = pltpu.roll(c, 4, 0)
        return jnp.where(top, c, r), jnp.where(top, r, c)

    m = jnp.max(jnp.where(top, _fold(se, jnp.maximum), _fold(so, jnp.maximum)), axis=1, keepdims=True)
    me, mo = split(m)
    de, do = se - _tile(me, NL), so - _tile(mo, NL)
    if c is not None:
        de, do = de * c, do * c
    pe, po = jnp.exp2(de), jnp.exp2(do)
    l = jnp.sum(jnp.where(top, _fold(pe, jnp.add), _fold(po, jnp.add)), axis=1, keepdims=True)
    ie, io = split(pl.reciprocal(l, approx=True))
    lane = lax.broadcasted_iota(I32, (8, 128), 1)
    return pe, po, jnp.concatenate([ie, jnp.where(lane < 64, ie, io), io], axis=1)


def _pv(groups, hooks=None):
    nb = len(groups) // 16
    accs = {}
    for n, g in enumerate(16 * blk + i for i in range(16) for blk in range(nb)):
        if hooks and n in hooks:
            hooks[n]()
        vload, p = groups[g]
        accs[g] = _fold(vload() * p, jnp.add)
    return jnp.concatenate([accs[g] for g in range(len(groups))], axis=0)


def _lane_reduce_t(acc):
    at = acc.T
    s = at[0:8]
    for i in range(1, 16):
        s = s + at[8 * i:8 * i + 8]
    return s


def _kernel(x_hbm, kt_hbm, vt_hbm, wq_hbm, wo_hbm, wr_hbm, wg_hbm, wu_hbm, wd_hbm,
            o_ref,
            kv, vf, kp, wq_raw, wo_raw, wg_raw, wu_raw, wd_raw, wxp, wop, wdp, wguf, wqf, wdf, wof, cs,
            xb_ref, wrb, state, spin_ref, c_s, c_p, c_o, c_out,
            sems, wsem, *, cfg):
    LA, LEAD, NV = cfg["LA"], cfg["LEAD"], cfg["NV"]
    NM = NH - NV
    ND = cfg["ND"]
    HALF = cfg["HALF"]
    order, raw = _order(cfg)

    def piece(i, s):
        q, pair, w, b = i & (TPC - 1), (i >> 2) & (NP - 1), (i >> 6) & 1, i >> 7
        r0 = (q + s * TPC) * 8
        if not isinstance(i, int):
            r0 = pl.multiple_of(r0, 8)
        return pair, w, b, w * (1 + (b & 1)), i & (RING - 1), r0

    def start_piece(i, s, hf=None):
        pair, w, b, plane, ring, r0 = piece(i, s)
        osl = pl.ds(pair * RO, RO) if hf is None else pl.ds(pair * RO + hf * (RO // 2), RO // 2)

        def go(ww):
            src = vt_hbm if ww else kt_hbm
            pltpu.make_async_copy(src.at[b, osl, pl.ds(r0, 8), pl.ds(SK - W, W)],
                                  kv.at[plane, osl, pl.ds(r0, 8), :],
                                  sems.at[s, ring]).start(priority=1 - s)

        if isinstance(i, int):
            go(w)
        else:
            for ww in range(2):
                pl.when(jnp.logical_and(w == ww, i < NTICK))(functools.partial(go, ww))

    def wait_piece(i, s):
        pair, w, b, plane, ring, r0 = piece(i, s)
        view = kv.at[plane, pl.ds(pair * RO, RO), pl.ds(r0, 8), :]
        pltpu.make_async_copy(view, view, sems.at[s, ring]).wait()

    def wait_tick(i):
        wait_piece(i, 0)
        wait_piece(i, 1)

    def spin(n):
        v = spin_ref[...]
        lane = lax.broadcasted_iota(I32, v.shape, 1).astype(F32)
        for _ in range(n[0]):
            v = jnp.max(v, axis=1, keepdims=True) * 0.5 + lane
        for _ in range(n[1] // 2):
            v = v * 0.5
            v = v + lane
        spin_ref[...] = v

    def full_tick(i):
        wait_tick(i)
        start_piece(i + LEAD + 1, 1)
        start_piece(i + LA, 0)

    def spin_tick(i, c):
        full_tick(i)
        spin(cfg["SPIN"])
        return c

    def half_tick(h, lead, la, work):
        i = h >> 1
        pl.when((h & 1) == 0)(lambda: wait_tick(i))
        start_piece(i + lead, 1, h & 1)
        work()
        start_piece(jnp.where((h & 1) == 1, i + la, NTICK), 0)

    def idle_half(h, c):
        def work():
            o0 = (((h >> 3) & (NP - 1)) - 1) * RO + (((h >> 1) & 3) - 1) * 3
            r = pl.ds(pl.multiple_of((h & 1) * 32, 32), 32)
            vf[pl.ds(o0 - VF0 * RO, 3), r, :] = kv[1 + ((h >> 8) & 1), pl.ds(o0, 3), r, :].astype(F32)
            if cfg["HSPIN"]:
                spin(cfg["HSPIN"])

        half_tick(h, LEAD, LA - 1, work)
        return c

    def advance(t, need):
        t2 = jnp.maximum(t + 2, need)
        wait_tick(t)
        lax.fori_loop(2 * t + 2, 2 * t2 - 2, idle_half, 0)
        wait_tick(t2 - 1)
        start_piece(t2 - 1 + LEAD, 1, 0 if HALF else None)
        return t2

    def mid(t2, n, after=None):
        if n == 0 and HALF:
            start_piece(t2 - 1 + LEAD, 1, 1)
        if n == 1:
            start_piece(t2 + LEAD, 1, 0 if HALF > 1 else None)
            start_piece(t2 - 2 + LA, 0)
            start_piece(t2 - 1 + LA, 0)
        if n == 2 and HALF > 1:
            kv[0, NP * RO, 0:16, 0:128] = jnp.concatenate([after, after], axis=0).astype(BF16)
            start_piece(t2 + LEAD, 1, 1)

    half = D // 2
    small = [pltpu.make_async_copy(x_hbm, xb_ref, wsem.at[0]),
             pltpu.make_async_copy(wr_hbm, wrb, wsem.at[1])]
    big = [pltpu.make_async_copy(wq_hbm, wq_raw, wsem.at[2]),
           pltpu.make_async_copy(wg_hbm, wg_raw, wsem.at[3]),
           pltpu.make_async_copy(wu_hbm.at[pl.ds(0, half)], wu_raw.at[pl.ds(0, half)], wsem.at[4])]
    for cp in big:
        cp.start(priority=1)
    for cp in small:
        cp.start()
    for i in range(LA):
        start_piece(i, 0)
    spin_ref[...] = jnp.zeros(spin_ref.shape, F32)

    inject = [(wo_hbm, wo_raw, 0, 48, HD // 48, 5), (wd_hbm, wd_raw, 0, 48, F // 48, 6),
              (wu_hbm, wu_raw, half, 16, half // 16, 7)]
    for src, dst, row0, rows, n, sem in inject:
        def body(i, c, src=src, dst=dst, row0=row0, rows=rows, sem=sem):
            r = pl.multiple_of(row0 + i * rows, 8)
            pltpu.make_async_copy(src.at[pl.ds(r, rows)], dst.at[pl.ds(r, rows)], wsem.at[sem]).start()
            spin(cfg["WSPIN"])
            return c
        lax.fori_loop(0, n, body, 0)

    for i in range(LEAD + 1):
        start_piece(i, 1)
    for cp in small:
        cp.wait()
    state[...] = jnp.concatenate([xb_ref[...].astype(F32), jnp.zeros((8 - B, D), F32)], axis=0)
    for src, dst, row0, rows, n, sem in inject:
        view = dst.at[pl.ds(row0, rows * n)]
        pltpu.make_async_copy(view, view, wsem.at[sem]).wait()
    for cp in big:
        cp.wait()

    NRP = D // 16

    def repack(h, c):
        full_tick(h)
        r = pl.multiple_of(h * 16, 16)
        r2 = pl.multiple_of(h * 8, 8)
        wxp[pl.ds(r2, 8), 0:HD] = _u32(wq_raw[pl.ds(r, 16), :])
        for n, pos in enumerate(cfg["VQ"]):
            wqf[pl.ds(r, 16), n * PD:(n + 1) * PD] = (
                wq_raw[pl.ds(r, 16), order[pos] * PD:(order[pos] + 1) * PD].astype(F32))
        g = wg_raw[pl.ds(r, 16), :]
        u = wu_raw[pl.ds(r, 16), :]
        gu = jnp.concatenate([w[:, i * 128:(i + 1) * 128] for i in range(NH) for w in (g, u)], axis=1)
        wxp[pl.ds(r2, 8), HD:HD + 2 * F] = _u32(gu)
        if NV:
            wguf[pl.ds(r, 16), :] = gu[:, NM * 256:].astype(F32)
        for n, pos in enumerate(cfg["VO"]):
            ro = pl.multiple_of(jnp.minimum(r, PD - 16), 16)
            wof[pl.ds(n * PD + ro, 16), :] = wo_raw[pl.ds(order[pos] * PD + ro, 16), :].astype(F32)
        if ND:
            rd = pl.multiple_of(jnp.minimum(r, ND * 128 - 16), 16)
            wdf[pl.ds(rd, 16), :] = wd_raw[pl.ds(rd, 16), :].astype(F32)
        for src, packed, n in ((wo_raw, wop, 160), (wd_raw, wdp, 48)):
            r = pl.multiple_of(jnp.minimum(h * n, src.shape[0] - n), 16)
            packed[pl.ds(pl.multiple_of(r >> 1, 8), n // 2), :] = _u32(src[pl.ds(r, n), :])
        return c

    lax.fori_loop(0, NRP, repack, 0)

    NCS = (HD + 2 * F) // 768

    def colsum(i, c):
        full_tick(NRP + i)
        c0 = pl.multiple_of(i * 768, 128)
        cs[:, pl.ds(c0, 768)] = _dot(jnp.ones((8, D), BF16), _bf(wxp[:, pl.ds(c0, 768)]))
        return c

    lax.fori_loop(0, NCS, colsum, 0)
    t0 = jnp.int32(NRP + NCS)

    never = spin_ref[...] < -1.0

    def xproj(xb, m, scale, c0, n):
        y = _dot(xb, _bf(wxp[:, pl.ds(c0, n)])) - m * cs[:, pl.ds(c0, n)]
        return y if scale is None else y * scale

    def qproj(xb, m, qscale, k):
        return xproj(xb, m, qscale, k * PD if isinstance(k, int) else pl.multiple_of(k * PD, 128), PD)

    def oproj(ob, k):
        r0 = pl.multiple_of(k * DH, DH) if not isinstance(k, int) else k * DH
        return _dot(ob, _bf(wop[pl.ds(r0, DH), :]))

    def kload(k):
        return [_bf(kp[pl.ds(k * RO + 2 * i, 2)].reshape(64, W)) for i in range(3)]

    def vgroup(slot, k, o, r):
        return lambda: kv[1 + slot, k * RO + o, pl.ds(r * 8, 8), :].astype(F32)

    def pair_groups(slot, k, pe, po):
        return [(vgroup(slot, k, g // RI, g % RI), pe if g < DH // 8 else po) for g in range(PD // 8)]

    def vpu_matvec(xr, w_ref, nadd, per_step=1, tok=None):
        nu = xr.shape[1] // 128
        xcol = [jnp.concatenate([xr[:, u * 128:(u + 1) * 128]] * 16, axis=0).T for u in range(nu)]
        seq = [(u, i) for u0 in range(0, nu, 2) for i in range(16) for u in range(u0, min(u0 + 2, nu))]
        accs = [None] * per_step
        for n in range(0, len(seq), per_step):
            if tok is not None:
                for _ in range(nadd):
                    tok = tok + 1.0
            for a, (u, i) in enumerate(seq[n:n + per_step]):
                col = xcol[u][i * 8:i * 8 + 8]
                if tok is not None:
                    col = jnp.where(never, tok, col)
                y = w_ref[u * 128 + i * 8:u * 128 + i * 8 + 8, :] * _tile(col, w_ref.shape[1] // 128)
                accs[a] = y if accs[a] is None else accs[a] + y
            tok = accs[0][:, 0:128]
        return functools.reduce(jnp.add, accs), tok

    def act(gu):
        g = gu[:, 0:128]
        return (g * _sigmoid(g) * gu[:, 128:256]).astype(BF16)

    def ffn_res(x, xc, rstd):
        wr = wrb[...].astype(F32)
        wr = jnp.concatenate([jnp.broadcast_to(wr[t:t + 1, :], (8, 128)) for t in range(D // 128)], axis=1)
        return x + xc * rstd, _round(_sigmoid(_round(jnp.sum(xc * wr, axis=1, keepdims=True) * rstd)))

    def ffn(x):
        xb, xr, m, xc, rstd = _ln_parts(x)

        hs = [act(xproj(xb, m, rstd, HD + i * 256, 256)) for i in range(NM)]
        gu, tok = vpu_matvec(xr, wguf, cfg["TOK"])
        gu = (_rowsum_all(gu) - m * cs[:, HD + NM * 256:]) * rstd
        hs += [act(gu[:, i * 256:(i + 1) * 256]) for i in range(NV)]
        y = None
        for i in range(ND, NH):
            yi = _dot(hs[i], _bf(wdp[i * 64:(i + 1) * 64, :]))
            y = yi if y is None else y + yi
        if ND:
            yv, _ = vpu_matvec(jnp.concatenate(hs[:ND], axis=1).astype(F32), wdf, cfg["DTOK"], 2, tok)
            y = y + _rowsum_all(yv)
        res, gate = ffn_res(xr, xc, rstd)
        return res + y * gate

    NFT = NH // 2 + 1

    def ffn_ticked(x, t):
        def body(i, carry):
            h, y, _ = carry
            full_tick(t + i)
            xb, xr, m, xc, rstd = _ln_parts(x)
            c0 = pl.multiple_of(HD + jnp.minimum(i, NFT - 2) * 512, 128)
            gu = xproj(xb, m, rstd, c0, 512)
            r0 = pl.multiple_of(jnp.maximum(i - 1, 0) * 128, 128)
            y = y + _dot(h, _bf(wdp[pl.ds(r0, 128), :]))
            res, gate = ffn_res(xr, xc, rstd)
            return jnp.concatenate([act(gu[:, 0:256]), act(gu[:, 256:512])], axis=1), y, res + y * gate

        return lax.fori_loop(0, NFT, body, (jnp.zeros((8, 256), BF16), jnp.zeros((8, D), F32), x))[2]

    NHP = 2 * B - 1

    def half_period(hp, t):
        b = hp >> 1
        slot = b & 1
        first = (hp & 1) == 0
        vbase = jnp.where(first, b * TPP + (NP + 1) * TPC, -TPP)

        tr = jnp.where(first, jnp.maximum(t, b * TPP + cfg["KRP"]), t)
        lax.fori_loop(t, tr, spin_tick, 0)

        def k_repack(h, c):
            def work():
                o0 = (h - 2 * tr) * 4
                kp[pl.ds(o0, 4)] = _u32(kv[0, pl.ds(o0, 4)].reshape(4 * 64, W)).reshape(4, 32, W)
                spin(cfg["KSPIN"])

            half_tick(h, LEAD + 1, LA, work)
            return c

        t = jnp.where(first, tr + NP * RO // 8, t)
        lax.fori_loop(2 * tr, 2 * t, k_repack, 0)

        xb, x, m, _, rstd = _ln_parts(jnp.broadcast_to(state[pl.ds(b, 1), :], (8, D)))
        qscale = rstd * SCALE

        def step(j, carry):
            t, q, se, so, pe, po, inv, o, out = carry
            kv_ = jnp.maximum(j - 3, 0)
            t = advance(t, vbase + kv_ * TPC)
            se_n, so_n = _scores(q, kload(jnp.clip(j - 1, 0, NP - 1)))
            q_n = qproj(xb, m, qscale, jnp.minimum(j, NP - 1))
            out = out + oproj(o, jnp.maximum(j - 4, 0))
            pe_n, po_n, inv_n = _softmax_pair(se, so)
            acc = _pv(pair_groups(slot, kv_, pe, po),
                      {cfg["PVMID"][0]: lambda: mid(t, 0), cfg["PVMID"][1]: lambda: mid(t, 1)})
            mid(t, 2, q_n[:, 256:384])
            o_n = (_lane_reduce_t(acc) * jnp.where(j >= 3, inv, 0.0)).astype(BF16)
            return t, q_n, se_n, so_n, pe_n, po_n, inv_n, o_n, out

        zw = (lax.broadcasted_iota(I32, (8, W), 0) + lax.broadcasted_iota(I32, (8, W), 1)).astype(F32) * (1.0 / W)
        zp = zw[:, :PD]
        init = (t, zp, zw, zw, zw, zw, zp, jnp.zeros((8, PD), BF16), jnp.zeros((8, D), F32))
        last = hp == NHP - 1
        t, q, se, so, pe, po, inv, o, out = lax.fori_loop(0, jnp.where(last, NP, NP + 2), step, init)
        t2 = jnp.maximum(t + 2, vbase + (NP - 1) * TPC)

        @pl.when(last)
        def _():
            c_s[0] = se
            c_s[1] = so
            c_p[0] = pe
            c_p[1] = po
            c_o[0] = q
            c_o[1] = inv
            c_o[2] = o.astype(F32)
            c_out[...] = out

        @pl.when(jnp.logical_not(last))
        def _():
            advance(t, t2)
            y = out + oproj(o, NP - 2)
            acc = _pv(pair_groups(slot, NP - 1, pe, po), {24: lambda: mid(t2, 0), 45: lambda: mid(t2, 1)})
            olast = _lane_reduce_t(acc) * inv
            mid(t2, 2, olast[:, 0:128])
            olast = olast.astype(BF16)
            full_tick(t2)
            y = y + oproj(olast, NP - 1)
            state[pl.ds(b, 1), :] = ffn_ticked(x + _rowsum_all(y), t2 + 1)[0:1]

        return t2 + 1 + NFT

    lax.fori_loop(0, NHP, half_period, t0)

    slot = (B - 1) % 2
    ka, kb = NP - 2, NP - 1

    def wo_rows(runs):
        return _bf(jnp.concatenate(
            [wop[(k * PD + o * 64 + r * 8) // 2:(k * PD + o * 64 + (r + n) * 8) // 2, :] for k, o, r, n in runs],
            axis=0))

    def run_groups(runs, ps):
        return [(vgroup(slot, k, o, r + i), ps[k][0 if o < RO // 2 else 1]) for k, o, r, n in runs for i in range(n)]

    def normalised(pe, po, inv):
        return pe * _tile(inv[:, 0:128], NL), po * _tile(inv[:, 256:384], NL)

    for i in range(NTICK - 3 * TPC, NTICK - 2 * TPC):
        wait_tick(i)
    se, so = _scores(c_o[0], kload(kb))
    out = c_out[...] + oproj(c_o[2].astype(BF16), NP - 4)
    pa = normalised(*_softmax_pair(c_s[0], c_s[1]))
    o = (_lane_reduce_t(_pv(pair_groups(slot, NP - 3, c_p[0], c_p[1]))) * c_o[1]).astype(BF16)

    for i in range(NTICK - 2 * TPC, NTICK):
        wait_piece(i, 1)
    pe, po, inv = _softmax_pair(se, so)
    ps = {ka: pa, kb: normalised(pe, po, inv)}
    out = out + oproj(o, NP - 3)
    runs0 = [(k, o, TPC, TPC) for k in (ka, kb) for o in range(RO)]
    lane = lax.broadcasted_iota(I32, (8, 128), 1)
    sc0 = jnp.concatenate([jnp.ones((8, 128), F32), jnp.where(lane < 64, 1.0, inv[:, 0:128]),
                           jnp.where(lane < 32, inv[:, 0:128], inv[:, 256:384])], axis=1)
    o0 = (_lane_reduce_t(_pv(run_groups(runs0, {ka: ps[ka], kb: (pe, po)}))) * sc0).astype(BF16)

    for i in range(NTICK - 2 * TPC, NTICK - 2):
        wait_piece(i, 0)
    out = out + _dot(o0, wo_rows(runs0))
    runs1 = [(ka, o, 0, TPC) for o in range(RO)] + [(kb, o, 0, 2) for o in range(4)]
    o1 = _lane_reduce_t(_pv(run_groups(runs1, ps))).astype(BF16)

    for i in range(NTICK - 2, NTICK):
        wait_piece(i, 0)
    out = out + _dot(o1, wo_rows(runs1))
    runs2 = [(kb, o, 0, 2) for o in range(4, RO)] + [(kb, o, 2, 2) for o in range(RO)]
    w2 = wo_rows(runs2).astype(F32)
    for i, (vload, p) in enumerate(run_groups(runs2, ps)):
        out = out + w2[i * 8:(i + 1) * 8] * jnp.sum(_fold(vload() * p, jnp.add), axis=1, keepdims=True)
    x = jnp.broadcast_to(state[B - 1:B, :], (8, D)) + _rowsum_all(out)

    def attn_fast(x):
        xb, xr, m, _, rstd = _ln_parts(x)
        qscale = rstd * SCALE
        q, sc, ps, os_ = {}, {}, {}, {}
        out = None
        oslot = {}
        sl = cfg["OLAG"]
        for i in range(NP):
            while sl in cfg["OSKIP"]:
                sl += 1
            if i not in cfg["VO"]:
                oslot[sl] = i
            sl += 1
        if cfg["VQ"]:
            qv = _rowsum_all(vpu_matvec(xr, wqf, cfg["QTOK"])[0])
            for n, pos in enumerate(cfg["VQ"]):
                k = order[pos]
                q[pos] = (qv[:, n * PD:(n + 1) * PD] - m * cs[:, k * PD:(k + 1) * PD]) * qscale
        qm = [pos for pos in range(NP) if pos not in cfg["VQ"]]
        for s in range(-3, sl):
            if cfg["QEARLY"]:
                if 0 <= s + 3 < len(qm):
                    q[qm[s + 3]] = qproj(xb, m, qscale if qm[s + 3] >= cfg["NLS"] else None, order[qm[s + 3]])
            elif s + 3 in qm:
                q[s + 3] = qproj(xb, m, qscale if s + 3 >= cfg["NLS"] else None, order[s + 3])
            if 0 <= s + 2 < NP:
                sc[s + 2] = _scores(q.pop(s + 2), kload(order[s + 2]))
            if s in oslot:
                y = oproj(os_.pop(oslot[s]), order[oslot[s]])
                out = y if out is None else out + y
            if 0 <= s + 1 < NP:
                ps[s + 1] = _softmax_pair(*sc.pop(s + 1), None if s + 1 >= cfg["NLS"] else qscale)
            if 0 <= s < NP:
                pe, po, inv = ps.pop(s)
                k = order[s]
                groups = pair_groups(slot, k, pe, po)
                if k not in raw:
                    groups = [(functools.partial(lambda g: vf[(k - VF0) * RO + g // RI, pl.ds((g % RI) * 8, 8), :], g), p)
                              for g, (_, p) in enumerate(groups)]
                acc = _pv(groups)
                if s == cfg["VOT"][0]:
                    tok = acc[cfg["VOT"][1] * 8:cfg["VOT"][1] * 8 + 8]
                o = _lane_reduce_t(acc) * inv
                os_[s] = (_rowsum_all(o) if s in cfg["VO"] else o).astype(BF16)
        if cfg["VO"]:
            ov = jnp.concatenate([os_.pop(i) for i in cfg["VO"]], axis=1).astype(F32)
            out = out + vpu_matvec(ov, wof, cfg["OTOK"], 2, tok)[0]
        return xr + _rowsum_all(out)

    if cfg["TAIL"] >= 1:
        x = ffn(x)
    if cfg["TAIL"] >= 2:
        x = ffn(attn_fast(x))
    row = lax.broadcasted_iota(I32, (8, D), 0)
    o_ref[...] = jnp.where(row == B - 1, x, state[...])[0:B].astype(o_ref.dtype)


def _call(cfg, A_x, A_k_cache, A_v_cache, A_wq, A_wo, B_w_r, B_w_gate, B_w_up, B_w_down):
    kt = jnp.swapaxes(A_k_cache, 2, 3).reshape(B, NP * RO, RI * 8, SK)
    vt = jnp.swapaxes(A_v_cache, 2, 3).reshape(B, NP * RO, RI * 8, SK)
    out = pl.pallas_call(
        functools.partial(_kernel, cfg=cfg),
        out_shape=jax.ShapeDtypeStruct((B, D), BF16),
        in_specs=[pl.BlockSpec(memory_space=pl.ANY)] * 9,
        out_specs=pl.BlockSpec(memory_space=pltpu.VMEM),
        scratch_shapes=[
            pltpu.VMEM((3, NP * RO + 1, RI * 8, W), BF16),
            pltpu.VMEM(((NP - 1 - VF0) * RO, RI * 8, W), F32),
            pltpu.VMEM((NP * RO, RI * 4, W), U32),
            pltpu.VMEM((D, HD), BF16),
            pltpu.VMEM((HD, D), BF16),
            pltpu.VMEM((D, F), BF16),
            pltpu.VMEM((D, F), BF16),
            pltpu.VMEM((F, D), BF16),
            pltpu.VMEM((D // 2, HD + 2 * F), U32),
            pltpu.VMEM((HD // 2, D), U32),
            pltpu.VMEM((F // 2, D), U32),
            pltpu.VMEM((D, cfg["NV"] * 256), F32),
            pltpu.VMEM((D, max(len(cfg["VQ"]), 1) * PD), F32),
            pltpu.VMEM((max(cfg["ND"], 1) * 128, D), F32),
            pltpu.VMEM((max(len(cfg["VO"]), 1) * PD, D), F32),
            pltpu.VMEM((8, HD + 2 * F), F32),
            pltpu.VMEM((B, D), BF16),
            pltpu.VMEM((D // 128, 128), BF16),
            pltpu.VMEM((8, D), F32),
            pltpu.VMEM((8, 128), F32),
            pltpu.VMEM((2, 8, W), F32),
            pltpu.VMEM((2, 8, W), F32),
            pltpu.VMEM((3, 8, PD), F32),
            pltpu.VMEM((8, D), F32),
            pltpu.SemaphoreType.DMA((2, RING)),
            pltpu.SemaphoreType.DMA((8,)),
        ],
        compiler_params=pltpu.CompilerParams(vmem_limit_bytes=120 * 1024 * 1024,
                                             disable_bounds_checks=True,
                                             disable_semaphore_checks=True),
        name="fused_decode",
    )(A_x.reshape(B, D), kt, vt, A_wq, A_wo, B_w_r.reshape(D // 128, 128), B_w_gate, B_w_up, B_w_down)
    return out.reshape(B, 1, D)


@jax.jit
def pallas_interleave_layers__sliding_block_cached__moe_arch_mod__decode_kernel(
    A_x: jax.Array,
    A_k_cache: jax.Array,
    A_v_cache: jax.Array,
    A_wq: jax.Array,
    A_wo: jax.Array,
    B_x: jax.Array,
    B_w_r: jax.Array,
    B_w_gate: jax.Array,
    B_w_up: jax.Array,
    B_w_down: jax.Array,
):
    del B_x
    return _call(CFG, A_x, A_k_cache, A_v_cache, A_wq, A_wo, B_w_r, B_w_gate, B_w_up, B_w_down)
```

```python
import functools

import jax
import jax.numpy as jnp
from jax import lax
import jax.experimental.pallas as pl
import jax.experimental.pallas.tpu as pltpu

F32 = jnp.float32
BF16 = jnp.bfloat16
U32 = jnp.uint32
I32 = jnp.int32

B, D, H, DH, SK, F = 4, 640, 32, 192, 4096, 1536
W = min(4096, max(256, SK // 4))
NP = H // 2
PD = 2 * DH
HD = H * DH
NL = W // 128
NH = F // 128
EPS = 1e-5
SCALE = DH ** -0.5 * 1.4426950408889634

RI = 8
RO = PD // (8 * RI)
TPC = RI // 2
TPP = 2 * NP * TPC
NTICK = B * TPP
RING = 32
VF0, VF1 = 0, 12

CFG = dict(
    LA=23,
    LEAD=11,
    SPIN=(1, 50),
    WSPIN=(1, 45),
    HALF=2,
    LSPIN=(1, 20),
    KSPIN=(1, 20),
    HSPIN=(1, 8),
    HTOP=False,
    KTOP=True,
    PVMID=(21, 45),
    KRP=54,
    OLAG=3,
    OSKIP=(4, 5),
    NV=4,
    TOK=0,
    QTOK=1,
    ND=4,
    DTOK=1,
    VO=(2, 0, 8),
    VOT=((15, 0, 0, 2, 0), (4, 32, 0, 2, 0), (11, 32, 0, 2, 2)),
    VQ=(3, 4, 5),
    RAWPOS=(5, 7, 9, 11),
    QEARLY=True,
    NLS=2,
    TAIL=2,
)


def _order(cfg):
    raw = [k for k in range(NP) if not VF0 <= k < VF1]
    order = list(range(VF0, VF1))
    for pos, k in zip(sorted(cfg["RAWPOS"]), raw):
        order.insert(pos, k)
    return order, raw


def _rowsum_all(x):
    x = x + pltpu.roll(x, 4, 0)
    x = x + pltpu.roll(x, 2, 0)
    return x + pltpu.roll(x, 1, 0)


def _bf(x):
    return pltpu.bitcast(x, BF16)


def _u32(x):
    return pltpu.bitcast(x, U32)


def _dot(a, b):
    return jnp.dot(a, b, preferred_element_type=F32)


def _sigmoid(x):
    return pl.reciprocal(1.0 + jnp.exp(-x), approx=True)


def _round(x):
    return x.astype(BF16).astype(F32)


def _ln_parts(x):
    xb = x.astype(BF16)
    xr = xb.astype(F32)
    m = jnp.sum(xr, axis=1, keepdims=True) * (1.0 / D)
    xc = xr - m
    v = jnp.sum(xc * xc, axis=1, keepdims=True) * (1.0 / D)
    m = _round(m)
    v = _round(_round(v) + EPS)
    return xb, xr, m, xr - m, pl.reciprocal(_round(v * lax.rsqrt(v)), approx=True)


def _scores(q, kk):
    lane = lax.broadcasted_iota(I32, (8, 128), 1)
    q0 = q[:, 0:128].astype(BF16)
    qm = q[:, 128:256]
    q2 = q[:, 256:384].astype(BF16)
    mid = jnp.concatenate([jnp.where(lane < 64, qm, 0.0), jnp.where(lane >= 64, qm, 0.0)],
                          axis=0).astype(BF16)
    r0 = _dot(q0, kk[0])
    rm = _dot(mid, kk[1])
    r2 = _dot(q2, kk[2])
    return r0 + rm[0:8], rm[8:16] + r2


def _fold(x, op):
    r = x[:, 0:128]
    for t in range(1, x.shape[1] // 128):
        r = op(r, x[:, t * 128:(t + 1) * 128])
    return r


def _tile(x, n):
    return jnp.concatenate([x] * n, axis=1)


def _softmax_pair(se, so, c=None):
    top = lax.broadcasted_iota(I32, (8, 128), 0) < 4

    def split(c):
        c = jnp.broadcast_to(c, (8, 128))
        r = pltpu.roll(c, 4, 0)
        return jnp.where(top, c, r), jnp.where(top, r, c)

    m = jnp.max(jnp.where(top, _fold(se, jnp.maximum), _fold(so, jnp.maximum)), axis=1, keepdims=True)
    me, mo = split(m)
    de, do = se - _tile(me, NL), so - _tile(mo, NL)
    if c is not None:
        de, do = de * c, do * c
    pe, po = jnp.exp2(de), jnp.exp2(do)
    l = jnp.sum(jnp.where(top, _fold(pe, jnp.add), _fold(po, jnp.add)), axis=1, keepdims=True)
    ie, io = split(pl.reciprocal(l, approx=True))
    lane = lax.broadcasted_iota(I32, (8, 128), 1)
    return pe, po, jnp.concatenate([ie, jnp.where(lane < 64, ie, io), io], axis=1)


def _pv(groups, hooks=None):
    nb = len(groups) // 16
    accs = {}
    for n, g in enumerate(16 * blk + i for i in range(16) for blk in range(nb)):
        if hooks and n in hooks:
            hooks[n]()
        vload, p = groups[g]
        accs[g] = _fold(vload() * p, jnp.add)
    return jnp.concatenate([accs[g] for g in range(len(groups))], axis=0)


def _lane_reduce_t(acc):
    at = acc.T
    s = at[0:8]
    for i in range(1, 16):
        s = s + at[8 * i:8 * i + 8]
    return s


def _kernel(x_hbm, kt_hbm, vt_hbm, wq_hbm, wo_hbm, wr_hbm, wg_hbm, wu_hbm, wd_hbm,
            o_ref,
            kv, vf, kp, wq_raw, wo_raw, wg_raw, wu_raw, wd_raw, wxp, wop, wdp, wguf, wqf, wdf, wof, cs,
            xb_ref, wrb, state, spin_ref, c_s, c_p, c_o, c_out,
            sems, wsem, *, cfg):
    LA, LEAD, NV = cfg["LA"], cfg["LEAD"], cfg["NV"]
    NM = NH - NV
    ND = cfg["ND"]
    HALF = cfg["HALF"]
    order, raw = _order(cfg)

    def piece(i, s):
        q, pair, w, b = i & (TPC - 1), (i >> 2) & (NP - 1), (i >> 6) & 1, i >> 7
        r0 = (q + s * TPC) * 8
        if not isinstance(i, int):
            r0 = pl.multiple_of(r0, 8)
        return pair, w, b, w * (1 + (b & 1)), i & (RING - 1), r0

    def start_piece(i, s, hf=None):
        pair, w, b, plane, ring, r0 = piece(i, s)
        osl = pl.ds(pair * RO, RO) if hf is None else pl.ds(pair * RO + hf * (RO // 2), RO // 2)

        def go(ww):
            src = vt_hbm if ww else kt_hbm
            pltpu.make_async_copy(src.at[b, osl, pl.ds(r0, 8), pl.ds(SK - W, W)],
                                  kv.at[plane, osl, pl.ds(r0, 8), :],
                                  sems.at[s, ring]).start(priority=1 - s)

        if isinstance(i, int):
            go(w)
        else:
            for ww in range(2):
                pl.when(jnp.logical_and(w == ww, i < NTICK))(functools.partial(go, ww))

    def wait_piece(i, s):
        pair, w, b, plane, ring, r0 = piece(i, s)
        view = kv.at[plane, pl.ds(pair * RO, RO), pl.ds(r0, 8), :]
        pltpu.make_async_copy(view, view, sems.at[s, ring]).wait()

    def wait_tick(i):
        wait_piece(i, 0)
        wait_piece(i, 1)

    def spin(n):
        v = spin_ref[...]
        lane = lax.broadcasted_iota(I32, v.shape, 1).astype(F32)
        for _ in range(n[0]):
            v = jnp.max(v, axis=1, keepdims=True) * 0.5 + lane
        for _ in range(n[1] // 2):
            v = v * 0.5
            v = v + lane
        spin_ref[...] = v

    def full_tick(i):
        wait_tick(i)
        start_piece(i + LEAD + 1, 1)
        start_piece(i + LA, 0)

    def spin_tick(i, c):
        full_tick(i)
        spin(cfg["SPIN"])
        return c

    def half_tick(h, lead, la, work, sp, top):
        i = h >> 1
        pl.when((h & 1) == 0)(lambda: wait_tick(i))
        if top:
            start_piece(i + lead, 1, h & 1)
        work()
        spin(sp)
        if not top:
            start_piece(i + lead, 1, h & 1)
        start_piece(jnp.where((h & 1) == 1, i + la, NTICK), 0)

    def idle_half(h, c):
        def work():
            n = (((h >> 3) & (NP - 1)) - 4) * 4 + (h & 7) - 2
            o0 = jnp.minimum(n * 2, VF1 * RO - 2)
            vf[pl.ds(o0, 2)] = kv[1 + ((h >> 8) & 1), pl.ds(o0, 2)].astype(F32)

        half_tick(h, LEAD, LA - 1, work, cfg["HSPIN"], cfg["HTOP"])
        return c

    def advance(t, need):
        t2 = jnp.maximum(t + 2, need)
        wait_tick(t)
        lax.fori_loop(2 * t + 2, 2 * t2 - 2, idle_half, 0)
        wait_tick(t2 - 1)
        start_piece(t2 - 1 + LEAD, 1, 0 if HALF else None)
        return t2

    def mid(t2, n, after=None):
        if n == 0 and HALF:
            start_piece(t2 - 1 + LEAD, 1, 1)
        if n == 1:
            start_piece(t2 + LEAD, 1, 0 if HALF > 1 else None)
            start_piece(t2 - 2 + LA, 0)
            start_piece(t2 - 1 + LA, 0)
        if n == 2 and HALF > 1:
            kv[0, NP * RO, 0:16, 0:128] = jnp.concatenate([after, after], axis=0).astype(BF16)
            start_piece(t2 + LEAD, 1, 1)

    half = D // 2
    small = [pltpu.make_async_copy(x_hbm, xb_ref, wsem.at[0]),
             pltpu.make_async_copy(wr_hbm, wrb, wsem.at[1])]
    big = [pltpu.make_async_copy(wq_hbm, wq_raw, wsem.at[2]),
           pltpu.make_async_copy(wg_hbm, wg_raw, wsem.at[3]),
           pltpu.make_async_copy(wu_hbm.at[pl.ds(0, half)], wu_raw.at[pl.ds(0, half)], wsem.at[4])]
    for cp in big:
        cp.start(priority=1)
    for cp in small:
        cp.start()
    spin_ref[...] = jnp.zeros(spin_ref.shape, F32)

    inject = [(wo_hbm, wo_raw, 0, 48, HD // 48, 5), (wd_hbm, wd_raw, 0, 48, F // 48, 6),
              (wu_hbm, wu_raw, half, 16, half // 16, 7)]
    for src, dst, row0, rows, n, sem in inject:
        def body(i, c, src=src, dst=dst, row0=row0, rows=rows, sem=sem):
            r = pl.multiple_of(row0 + i * rows, 8)
            pltpu.make_async_copy(src.at[pl.ds(r, rows)], dst.at[pl.ds(r, rows)], wsem.at[sem]).start()
            spin(cfg["WSPIN"])
            return c
        lax.fori_loop(0, n, body, 0)
        if dst is wo_raw:
            for i in range(LA):
                start_piece(i, 0)

    def lead_in(h, c):
        start_piece(h >> 1, 1, h & 1)
        spin(cfg["LSPIN"])
        return c

    lax.fori_loop(0, 2 * (LEAD + 1), lead_in, 0)
    for cp in small:
        cp.wait()
    state[...] = jnp.concatenate([xb_ref[...].astype(F32), jnp.zeros((8 - B, D), F32)], axis=0)
    for src, dst, row0, rows, n, sem in inject:
        view = dst.at[pl.ds(row0, rows * n)]
        pltpu.make_async_copy(view, view, wsem.at[sem]).wait()
    for cp in big:
        cp.wait()

    NRP = D // 16

    def repack(h, c):
        full_tick(h)
        r = pl.multiple_of(h * 16, 16)
        r2 = pl.multiple_of(h * 8, 8)
        wxp[pl.ds(r2, 8), 0:HD] = _u32(wq_raw[pl.ds(r, 16), :])
        for n, pos in enumerate(cfg["VQ"]):
            wqf[pl.ds(r, 16), n * PD:(n + 1) * PD] = (
                wq_raw[pl.ds(r, 16), order[pos] * PD:(order[pos] + 1) * PD].astype(F32))
        g = wg_raw[pl.ds(r, 16), :]
        u = wu_raw[pl.ds(r, 16), :]
        gu = jnp.concatenate([w[:, i * 128:(i + 1) * 128] for i in range(NH) for w in (g, u)], axis=1)
        wxp[pl.ds(r2, 8), HD:HD + 2 * F] = _u32(gu)
        if NV:
            wguf[pl.ds(r, 16), :] = gu[:, NM * 256:].astype(F32)
        for n, pos in enumerate(cfg["VO"]):
            ro = pl.multiple_of(jnp.minimum(r, PD - 16), 16)
            wof[pl.ds(n * PD + ro, 16), :] = wo_raw[pl.ds(order[pos] * PD + ro, 16), :].astype(F32)
        if ND:
            rd = pl.multiple_of(jnp.minimum(r, ND * 128 - 16), 16)
            wdf[pl.ds(rd, 16), :] = wd_raw[pl.ds(rd, 16), :].astype(F32)
        for src, packed, n in ((wo_raw, wop, 160), (wd_raw, wdp, 48)):
            r = pl.multiple_of(jnp.minimum(h * n, src.shape[0] - n), 16)
            packed[pl.ds(pl.multiple_of(r >> 1, 8), n // 2), :] = _u32(src[pl.ds(r, n), :])
        return c

    lax.fori_loop(0, NRP, repack, 0)

    NCS = (HD + 2 * F) // 768

    def colsum(i, c):
        full_tick(NRP + i)
        c0 = pl.multiple_of(i * 768, 128)
        cs[:, pl.ds(c0, 768)] = _dot(jnp.ones((8, D), BF16), _bf(wxp[:, pl.ds(c0, 768)]))
        return c

    lax.fori_loop(0, NCS, colsum, 0)
    t0 = jnp.int32(NRP + NCS)

    never = spin_ref[...] < -1.0

    def xproj(xb, m, scale, c0, n):
        y = _dot(xb, _bf(wxp[:, pl.ds(c0, n)])) - m * cs[:, pl.ds(c0, n)]
        return y if scale is None else y * scale

    def qproj(xb, m, qscale, k):
        return xproj(xb, m, qscale, k * PD if isinstance(k, int) else pl.multiple_of(k * PD, 128), PD)

    def oproj(ob, k):
        r0 = pl.multiple_of(k * DH, DH) if not isinstance(k, int) else k * DH
        return _dot(ob, _bf(wop[pl.ds(r0, DH), :]))

    def kload(k):
        return [_bf(kp[pl.ds(k * RO + 2 * i, 2)].reshape(64, W)) for i in range(3)]

    def vgroup(slot, k, o, r):
        return lambda: kv[1 + slot, k * RO + o, pl.ds(r * 8, 8), :].astype(F32)

    def pair_groups(slot, k, pe, po):
        return [(vgroup(slot, k, g // RI, g % RI), pe if g < DH // 8 else po) for g in range(PD // 8)]

    def vpu_matvec(xr, w_ref, nadd, per_step=1, tok=None):
        nu = xr.shape[1] // 128
        xcol = [jnp.concatenate([xr[:, u * 128:(u + 1) * 128]] * 16, axis=0).T for u in range(nu)]
        seq = [(u, i) for u0 in range(0, nu, 2) for i in range(16) for u in range(u0, min(u0 + 2, nu))]
        accs = [None] * per_step
        for n in range(0, len(seq), per_step):
            if tok is not None:
                for _ in range(nadd):
                    tok = tok + 1.0
            for a, (u, i) in enumerate(seq[n:n + per_step]):
                col = xcol[u][i * 8:i * 8 + 8]
                if tok is not None:
                    col = jnp.where(never, tok, col)
                y = w_ref[u * 128 + i * 8:u * 128 + i * 8 + 8, :] * _tile(col, w_ref.shape[1] // 128)
                accs[a] = y if accs[a] is None else accs[a] + y
            tok = accs[0][:, 0:128]
        return functools.reduce(jnp.add, accs), tok

    def act(gu):
        g = gu[:, 0:128]
        return (g * _sigmoid(g) * gu[:, 128:256]).astype(BF16)

    def ffn_res(x, xc, rstd):
        wr = wrb[...].astype(F32)
        wr = jnp.concatenate([jnp.broadcast_to(wr[t:t + 1, :], (8, 128)) for t in range(D // 128)], axis=1)
        return x + xc * rstd, _round(_sigmoid(_round(jnp.sum(xc * wr, axis=1, keepdims=True) * rstd)))

    def ffn(x):
        xb, xr, m, xc, rstd = _ln_parts(x)

        hs = [act(xproj(xb, m, rstd, HD + i * 256, 256)) for i in range(NM)]
        gu, tok = vpu_matvec(xr, wguf, cfg["TOK"])
        gu = (_rowsum_all(gu) - m * cs[:, HD + NM * 256:]) * rstd
        hs += [act(gu[:, i * 256:(i + 1) * 256]) for i in range(NV)]
        y = None
        for i in range(ND, NH):
            yi = _dot(hs[i], _bf(wdp[i * 64:(i + 1) * 64, :]))
            y = yi if y is None else y + yi
        if ND:
            yv, _ = vpu_matvec(jnp.concatenate(hs[:ND], axis=1).astype(F32), wdf, cfg["DTOK"], 2, tok)
            y = y + _rowsum_all(yv)
        res, gate = ffn_res(xr, xc, rstd)
        return res + y * gate

    NFT = NH // 2 + 1

    def ffn_ticked(x, t):
        def body(i, carry):
            h, y, _ = carry
            full_tick(t + i)
            xb, xr, m, xc, rstd = _ln_parts(x)
            c0 = pl.multiple_of(HD + jnp.minimum(i, NFT - 2) * 512, 128)
            gu = xproj(xb, m, rstd, c0, 512)
            r0 = pl.multiple_of(jnp.maximum(i - 1, 0) * 128, 128)
            y = y + _dot(h, _bf(wdp[pl.ds(r0, 128), :]))
            res, gate = ffn_res(xr, xc, rstd)
            return jnp.concatenate([act(gu[:, 0:256]), act(gu[:, 256:512])], axis=1), y, res + y * gate

        return lax.fori_loop(0, NFT, body, (jnp.zeros((8, 256), BF16), jnp.zeros((8, D), F32), x))[2]

    NHP = 2 * B - 1

    def half_period(hp, t):
        b = hp >> 1
        slot = b & 1
        first = (hp & 1) == 0
        vbase = jnp.where(first, b * TPP + (NP + 1) * TPC, -TPP)

        tr = jnp.where(first, jnp.maximum(t, b * TPP + cfg["KRP"]), t)
        lax.fori_loop(t, tr, spin_tick, 0)

        def k_repack(h, c):
            def work():
                o0 = (h - 2 * tr) * 4
                kp[pl.ds(o0, 4)] = _u32(kv[0, pl.ds(o0, 4)].reshape(4 * 64, W)).reshape(4, 32, W)

            half_tick(h, LEAD + 1, LA, work, cfg["KSPIN"], cfg["KTOP"])
            return c

        t = jnp.where(first, tr + NP * RO // 8, t)
        lax.fori_loop(2 * tr, 2 * t, k_repack, 0)

        xb, x, m, _, rstd = _ln_parts(jnp.broadcast_to(state[pl.ds(b, 1), :], (8, D)))
        qscale = rstd * SCALE

        def step(j, carry):
            t, q, se, so, pe, po, inv, o, out = carry
            kv_ = jnp.maximum(j - 3, 0)
            t = advance(t, vbase + kv_ * TPC)
            se_n, so_n = _scores(q, kload(jnp.clip(j - 1, 0, NP - 1)))
            q_n = qproj(xb, m, qscale, jnp.minimum(j, NP - 1))
            out = out + oproj(o, jnp.maximum(j - 4, 0))
            pe_n, po_n, inv_n = _softmax_pair(se, so)
            acc = _pv(pair_groups(slot, kv_, pe, po),
                      {cfg["PVMID"][0]: lambda: mid(t, 0), cfg["PVMID"][1]: lambda: mid(t, 1)})
            mid(t, 2, q_n[:, 256:384])
            o_n = (_lane_reduce_t(acc) * jnp.where(j >= 3, inv, 0.0)).astype(BF16)
            return t, q_n, se_n, so_n, pe_n, po_n, inv_n, o_n, out

        zw = (lax.broadcasted_iota(I32, (8, W), 0) + lax.broadcasted_iota(I32, (8, W), 1)).astype(F32) * (1.0 / W)
        zp = zw[:, :PD]
        init = (t, zp, zw, zw, zw, zw, zp, jnp.zeros((8, PD), BF16), jnp.zeros((8, D), F32))
        last = hp == NHP - 1
        t, q, se, so, pe, po, inv, o, out = lax.fori_loop(0, jnp.where(last, NP, NP + 2), step, init)
        t2 = jnp.maximum(t + 2, vbase + (NP - 1) * TPC)

        @pl.when(last)
        def _():
            c_s[0] = se
            c_s[1] = so
            c_p[0] = pe
            c_p[1] = po
            c_o[0] = q
            c_o[1] = inv
            c_o[2] = o.astype(F32)
            c_out[...] = out

        @pl.when(jnp.logical_not(last))
        def _():
            advance(t, t2)
            y = out + oproj(o, NP - 2)
            acc = _pv(pair_groups(slot, NP - 1, pe, po), {24: lambda: mid(t2, 0), 45: lambda: mid(t2, 1)})
            olast = _lane_reduce_t(acc) * inv
            mid(t2, 2, olast[:, 0:128])
            olast = olast.astype(BF16)
            full_tick(t2)
            y = y + oproj(olast, NP - 1)
            state[pl.ds(b, 1), :] = ffn_ticked(x + _rowsum_all(y), t2 + 1)[0:1]

        return t2 + 1 + NFT

    lax.fori_loop(0, NHP, half_period, t0)

    slot = (B - 1) % 2
    ka, kb = NP - 2, NP - 1

    def wo_rows(runs):
        return _bf(jnp.concatenate(
            [wop[(k * PD + o * 64 + r * 8) // 2:(k * PD + o * 64 + (r + n) * 8) // 2, :] for k, o, r, n in runs],
            axis=0))

    def run_groups(runs, ps):
        return [(vgroup(slot, k, o, r + i), ps[k][0 if o < RO // 2 else 1]) for k, o, r, n in runs for i in range(n)]

    def normalised(pe, po, inv):
        return pe * _tile(inv[:, 0:128], NL), po * _tile(inv[:, 256:384], NL)

    def pv_o_vpu(runs):
        w = wo_rows(runs).astype(F32)
        return functools.reduce(jnp.add, [
            w[i * 8:(i + 1) * 8] * jnp.sum(_fold(vload() * p, jnp.add), axis=1, keepdims=True)
            for i, (vload, p) in enumerate(run_groups(runs, ps))])

    kc = NP - 3
    for i in range(NTICK - 3 * TPC, NTICK - TPC):
        wait_piece(i, 1)
    se, so = _scores(c_o[0], kload(kb))
    out = c_out[...] + oproj(c_o[2].astype(BF16), NP - 4)
    ps = {kc: normalised(c_p[0], c_p[1], c_o[1]), ka: normalised(*_softmax_pair(c_s[0], c_s[1]))}
    runs = [(k, o, TPC, TPC) for k in (kc, ka) for o in range(RO)]
    o = _lane_reduce_t(_pv(run_groups(runs, ps))).astype(BF16)
    ps[kb] = normalised(*_softmax_pair(se, so))

    for i in range(NTICK - 3 * TPC, NTICK - 2 * TPC):
        wait_piece(i, 0)
    for i in range(NTICK - TPC, NTICK):
        wait_piece(i, 1)
    out = out + _dot(o, wo_rows(runs))
    runs0 = [(kc, o, 0, TPC) for o in range(RO)] + [(kb, o, TPC, TPC) for o in range(RO)]
    o0 = _lane_reduce_t(_pv(run_groups(runs0, ps))).astype(BF16)

    for i in range(NTICK - 2 * TPC, NTICK - TPC):
        wait_piece(i, 0)
    out = out + _dot(o0, wo_rows(runs0))
    runs1 = [(ka, o, 0, TPC) for o in range(RO)]
    acc = [_fold(vload() * p, jnp.add) for vload, p in run_groups(runs1, ps)]
    zero = [jnp.zeros((8, 128), F32)] * 4
    o1 = _lane_reduce_t(jnp.concatenate(acc[:12] + zero + acc[12:] + zero, axis=0)).astype(BF16)

    for i in range(NTICK - TPC, NTICK - 2):
        wait_piece(i, 0)
    out = out + _dot(o1, wo_rows(runs1[:3] + runs1[:1] + runs1[3:] + runs1[:1]))
    out = out + pv_o_vpu([(kb, o, 0, 2) for o in range(RO)])

    for i in range(NTICK - 2, NTICK):
        wait_piece(i, 0)
    out = out + pv_o_vpu([(kb, o, 2, 2) for o in range(RO)])
    x = jnp.broadcast_to(state[B - 1:B, :], (8, D)) + _rowsum_all(out)

    def attn_fast(x):
        xb, xr, m, _, rstd = _ln_parts(x)
        qscale = rstd * SCALE
        q, sc, ps, os_, deadline, outv = {}, {}, {}, {}, {}, []
        out = None
        oslot = {}
        sl = cfg["OLAG"]
        for i in range(NP):
            while sl in cfg["OSKIP"]:
                sl += 1
            if i not in cfg["VO"]:
                oslot[sl] = i
            sl += 1
        if cfg["VQ"]:
            qv = _rowsum_all(vpu_matvec(xr, wqf, cfg["QTOK"])[0])
            for n, pos in enumerate(cfg["VQ"]):
                k = order[pos]
                q[pos] = (qv[:, n * PD:(n + 1) * PD] - m * cs[:, k * PD:(k + 1) * PD]) * qscale
        qm = [pos for pos in range(NP) if pos not in cfg["VQ"]]
        for s in range(-3, sl):
            if cfg["QEARLY"]:
                if 0 <= s + 3 < len(qm):
                    q[qm[s + 3]] = qproj(xb, m, qscale if qm[s + 3] >= cfg["NLS"] else None, order[qm[s + 3]])
            elif s + 3 in qm:
                q[s + 3] = qproj(xb, m, qscale if s + 3 >= cfg["NLS"] else None, order[s + 3])
            if 0 <= s + 2 < NP:
                qq = q.pop(s + 2)
                if s in deadline:
                    qq = jnp.concatenate([jnp.where(never, deadline.pop(s), qq[:, 0:128]), qq[:, 128:]], axis=1)
                sc[s + 2] = _scores(qq, kload(order[s + 2]))
            if s in oslot:
                y = oproj(os_.pop(oslot[s]), order[oslot[s]])
                out = y if out is None else out + y
            if 0 <= s + 1 < NP:
                ps[s + 1] = _softmax_pair(*sc.pop(s + 1), None if s + 1 >= cfg["NLS"] else qscale)
            if 0 <= s < NP:
                pe, po, inv = ps.pop(s)
                k = order[s]
                groups = pair_groups(slot, k, pe, po)
                if k not in raw:
                    groups = [(functools.partial(lambda g: vf[(k - VF0) * RO + g // RI, pl.ds((g % RI) * 8, 8), :], g), p)
                              for g, (_, p) in enumerate(groups)]
                acc = _pv(groups)
                o = _lane_reduce_t(acc) * inv
                os_[s] = (_rowsum_all(o) if s in cfg["VO"] else o).astype(BF16)
                for n, (tpos, tg, nadd, per, dl) in enumerate(cfg["VOT"]):
                    if tpos == s:
                        y, tok = vpu_matvec(os_.pop(cfg["VO"][n]).astype(F32), wof.at[n * PD:(n + 1) * PD], nadd, per,
                                            acc[tg * 8:tg * 8 + 8])
                        outv.append(y)
                        if dl:
                            deadline[s + dl] = tok
        out = functools.reduce(jnp.add, [out] + outv)
        return xr + _rowsum_all(out)

    if cfg["TAIL"] >= 1:
        x = ffn(x)
    if cfg["TAIL"] >= 2:
        x = ffn(attn_fast(x))
    row = lax.broadcasted_iota(I32, (8, D), 0)
    o_ref[...] = jnp.where(row == B - 1, x, state[...])[0:B].astype(o_ref.dtype)


def _call(cfg, A_x, A_k_cache, A_v_cache, A_wq, A_wo, B_w_r, B_w_gate, B_w_up, B_w_down):
    kt = jnp.swapaxes(A_k_cache, 2, 3).reshape(B, NP * RO, RI * 8, SK)
    vt = jnp.swapaxes(A_v_cache, 2, 3).reshape(B, NP * RO, RI * 8, SK)
    out = pl.pallas_call(
        functools.partial(_kernel, cfg=cfg),
        out_shape=jax.ShapeDtypeStruct((B, D), BF16),
        in_specs=[pl.BlockSpec(memory_space=pl.ANY)] * 9,
        out_specs=pl.BlockSpec(memory_space=pltpu.VMEM),
        scratch_shapes=[
            pltpu.VMEM((3, NP * RO + 1, RI * 8, W), BF16),
            pltpu.VMEM((VF1 * RO, RI * 8, W), F32),
            pltpu.VMEM((NP * RO, RI * 4, W), U32),
            pltpu.VMEM((D, HD), BF16),
            pltpu.VMEM((HD, D), BF16),
            pltpu.VMEM((D, F), BF16),
            pltpu.VMEM((D, F), BF16),
            pltpu.VMEM((F, D), BF16),
            pltpu.VMEM((D // 2, HD + 2 * F), U32),
            pltpu.VMEM((HD // 2, D), U32),
            pltpu.VMEM((F // 2, D), U32),
            pltpu.VMEM((D, cfg["NV"] * 256), F32),
            pltpu.VMEM((D, max(len(cfg["VQ"]), 1) * PD), F32),
            pltpu.VMEM((max(cfg["ND"], 1) * 128, D), F32),
            pltpu.VMEM((max(len(cfg["VO"]), 1) * PD, D), F32),
            pltpu.VMEM((8, HD + 2 * F), F32),
            pltpu.VMEM((B, D), BF16),
            pltpu.VMEM((D // 128, 128), BF16),
            pltpu.VMEM((8, D), F32),
            pltpu.VMEM((8, 128), F32),
            pltpu.VMEM((2, 8, W), F32),
            pltpu.VMEM((2, 8, W), F32),
            pltpu.VMEM((3, 8, PD), F32),
            pltpu.VMEM((8, D), F32),
            pltpu.SemaphoreType.DMA((2, RING)),
            pltpu.SemaphoreType.DMA((8,)),
        ],
        compiler_params=pltpu.CompilerParams(vmem_limit_bytes=126 * 1024 * 1024,
                                             disable_bounds_checks=True,
                                             disable_semaphore_checks=True),
        name="fused_decode",
    )(A_x.reshape(B, D), kt, vt, A_wq, A_wo, B_w_r.reshape(D // 128, 128), B_w_gate, B_w_up, B_w_down)
    return out.reshape(B, 1, D)


@jax.jit
def pallas_interleave_layers__sliding_block_cached__moe_arch_mod__decode_kernel(
    A_x: jax.Array,
    A_k_cache: jax.Array,
    A_v_cache: jax.Array,
    A_wq: jax.Array,
    A_wo: jax.Array,
    B_x: jax.Array,
    B_w_r: jax.Array,
    B_w_gate: jax.Array,
    B_w_up: jax.Array,
    B_w_down: jax.Array,
):
    del B_x
    return _call(CFG, A_x, A_k_cache, A_v_cache, A_wq, A_wo, B_w_r, B_w_gate, B_w_up, B_w_down)
```

```python
import functools

import jax
import jax.numpy as jnp
from jax import lax
import jax.experimental.pallas as pl
import jax.experimental.pallas.tpu as pltpu

F32 = jnp.float32
BF16 = jnp.bfloat16
U32 = jnp.uint32
I32 = jnp.int32

B, D, H, DH, SK, F = 4, 640, 32, 192, 4096, 1536
W = min(4096, max(256, SK // 4))
NP = H // 2
PD = 2 * DH
HD = H * DH
NL = W // 128
NH = F // 128
EPS = 1e-5
SCALE = DH ** -0.5 * 1.4426950408889634

RI = 8
RO = PD // (8 * RI)
TPC = RI // 2
TPP = 2 * NP * TPC
NTICK = B * TPP
RING = 32
VF0, VF1 = 0, 12

CFG = dict(
    LA=23,
    LEAD=11,
    SPIN=(1, 50),
    WSPIN=(1, 45),
    HALF=2,
    LSPIN=(1, 20),
    KSPIN=(1, 20),
    HSPIN=(1, 8),
    HTOP=False,
    KTOP=True,
    PVMID=(21, 45),
    KRP=54,
    OLAG=3,
    OSKIP=(4, 5),
    NV=4,
    TOK=0,
    QTOK=0,
    ND=4,
    DTOK=1,
    DLATE=2,
    VO=(2, 0, 8),
    VOT=((15, 0, 0, 2, 0), (4, 32, 0, 2, 0), (11, 32, 0, 2, 2)),
    VQ=(2, 3, 4),
    RAWPOS=(7, 9, 10, 12),
    QEARLY=True,
    NLS=1,
    TAIL=2,
)


def _order(cfg):
    raw = [k for k in range(NP) if not VF0 <= k < VF1]
    order = list(range(VF0, VF1))
    for pos, k in zip(sorted(cfg["RAWPOS"]), raw):
        order.insert(pos, k)
    return order, raw


def _rowsum_all(x):
    x = x + pltpu.roll(x, 4, 0)
    x = x + pltpu.roll(x, 2, 0)
    return x + pltpu.roll(x, 1, 0)


def _bf(x):
    return pltpu.bitcast(x, BF16)


def _u32(x):
    return pltpu.bitcast(x, U32)


def _dot(a, b):
    return jnp.dot(a, b, preferred_element_type=F32)


def _sigmoid(x):
    return pl.reciprocal(1.0 + jnp.exp(-x), approx=True)


def _round(x):
    return x.astype(BF16).astype(F32)


def _ln_parts(x):
    xb = x.astype(BF16)
    xr = xb.astype(F32)
    m = jnp.sum(xr, axis=1, keepdims=True) * (1.0 / D)
    xc = xr - m
    v = jnp.sum(xc * xc, axis=1, keepdims=True) * (1.0 / D)
    m = _round(m)
    v = _round(_round(v) + EPS)
    return xb, xr, m, xr - m, pl.reciprocal(_round(v * lax.rsqrt(v)), approx=True)


def _scores(q, kk):
    lane = lax.broadcasted_iota(I32, (8, 128), 1)
    q0 = q[:, 0:128].astype(BF16)
    qm = q[:, 128:256]
    q2 = q[:, 256:384].astype(BF16)
    mid = jnp.concatenate([jnp.where(lane < 64, qm, 0.0), jnp.where(lane >= 64, qm, 0.0)],
                          axis=0).astype(BF16)
    r0 = _dot(q0, kk[0])
    rm = _dot(mid, kk[1])
    r2 = _dot(q2, kk[2])
    return r0 + rm[0:8], rm[8:16] + r2


def _fold(x, op):
    r = x[:, 0:128]
    for t in range(1, x.shape[1] // 128):
        r = op(r, x[:, t * 128:(t + 1) * 128])
    return r


def _tile(x, n):
    return jnp.concatenate([x] * n, axis=1)


def _softmax_pair(se, so, c=None):
    top = lax.broadcasted_iota(I32, (8, 128), 0) < 4

    def split(c):
        c = jnp.broadcast_to(c, (8, 128))
        r = pltpu.roll(c, 4, 0)
        return jnp.where(top, c, r), jnp.where(top, r, c)

    m = jnp.max(jnp.where(top, _fold(se, jnp.maximum), _fold(so, jnp.maximum)), axis=1, keepdims=True)
    me, mo = split(m)
    de, do = se - _tile(me, NL), so - _tile(mo, NL)
    if c is not None:
        de, do = de * c, do * c
    pe, po = jnp.exp2(de), jnp.exp2(do)
    l = jnp.sum(jnp.where(top, _fold(pe, jnp.add), _fold(po, jnp.add)), axis=1, keepdims=True)
    ie, io = split(pl.reciprocal(l, approx=True))
    lane = lax.broadcasted_iota(I32, (8, 128), 1)
    return pe, po, jnp.concatenate([ie, jnp.where(lane < 64, ie, io), io], axis=1)


def _pv(groups, hooks=None):
    nb = len(groups) // 16
    accs = {}
    for n, g in enumerate(16 * blk + i for i in range(16) for blk in range(nb)):
        if hooks and n in hooks:
            hooks[n]()
        vload, p = groups[g]
        accs[g] = _fold(vload() * p, jnp.add)
    return jnp.concatenate([accs[g] for g in range(len(groups))], axis=0)


def _lane_reduce_t(acc):
    at = acc.T
    s = at[0:8]
    for i in range(1, 16):
        s = s + at[8 * i:8 * i + 8]
    return s


def _kernel(x_hbm, kt_hbm, vt_hbm, wq_hbm, wo_hbm, wr_hbm, wg_hbm, wu_hbm, wd_hbm,
            o_ref,
            kv, vf, kp, wq_raw, wo_raw, wg_raw, wu_raw, wd_raw, wxp, wop, wdp, wguf, wqf, wdf, wof, cs,
            xb_ref, wrb, state, spin_ref, c_s, c_p, c_o, c_out,
            sems, wsem, *, cfg):
    LA, LEAD, NV = cfg["LA"], cfg["LEAD"], cfg["NV"]
    NM = NH - NV
    ND = cfg["ND"]
    HALF = cfg["HALF"]
    order, raw = _order(cfg)

    def piece(i, s):
        q, pair, w, b = i & (TPC - 1), (i >> 2) & (NP - 1), (i >> 6) & 1, i >> 7
        r0 = (q + s * TPC) * 8
        if not isinstance(i, int):
            r0 = pl.multiple_of(r0, 8)
        return pair, w, b, w * (1 + (b & 1)), i & (RING - 1), r0

    def start_piece(i, s, hf=None):
        pair, w, b, plane, ring, r0 = piece(i, s)
        osl = pl.ds(pair * RO, RO) if hf is None else pl.ds(pair * RO + hf * (RO // 2), RO // 2)

        def go(ww):
            src = vt_hbm if ww else kt_hbm
            pltpu.make_async_copy(src.at[b, osl, pl.ds(r0, 8), pl.ds(SK - W, W)],
                                  kv.at[plane, osl, pl.ds(r0, 8), :],
                                  sems.at[s, ring]).start(priority=1 - s)

        if isinstance(i, int):
            go(w)
        else:
            for ww in range(2):
                pl.when(jnp.logical_and(w == ww, i < NTICK))(functools.partial(go, ww))

    def wait_piece(i, s):
        pair, w, b, plane, ring, r0 = piece(i, s)
        view = kv.at[plane, pl.ds(pair * RO, RO), pl.ds(r0, 8), :]
        pltpu.make_async_copy(view, view, sems.at[s, ring]).wait()

    def wait_tick(i):
        wait_piece(i, 0)
        wait_piece(i, 1)

    def spin(n):
        v = spin_ref[...]
        lane = lax.broadcasted_iota(I32, v.shape, 1).astype(F32)
        for _ in range(n[0]):
            v = jnp.max(v, axis=1, keepdims=True) * 0.5 + lane
        for _ in range(n[1] // 2):
            v = v * 0.5
            v = v + lane
        spin_ref[...] = v

    def full_tick(i):
        wait_tick(i)
        start_piece(i + LEAD + 1, 1)
        start_piece(i + LA, 0)

    def spin_tick(i, c):
        full_tick(i)
        spin(cfg["SPIN"])
        return c

    def half_tick(h, lead, la, work, sp, top):
        i = h >> 1
        pl.when((h & 1) == 0)(lambda: wait_tick(i))
        if top:
            start_piece(i + lead, 1, h & 1)
        work()
        spin(sp)
        if not top:
            start_piece(i + lead, 1, h & 1)
        start_piece(jnp.where((h & 1) == 1, i + la, NTICK), 0)

    def idle_half(h, c):
        def work():
            n = (((h >> 3) & (NP - 1)) - 4) * 4 + (h & 7) - 2
            o0 = jnp.minimum(n * 2, VF1 * RO - 2)
            vf[pl.ds(o0, 2)] = kv[1 + ((h >> 8) & 1), pl.ds(o0, 2)].astype(F32)

        half_tick(h, LEAD, LA - 1, work, cfg["HSPIN"], cfg["HTOP"])
        return c

    def advance(t, need):
        t2 = jnp.maximum(t + 2, need)
        wait_tick(t)
        lax.fori_loop(2 * t + 2, 2 * t2 - 2, idle_half, 0)
        wait_tick(t2 - 1)
        start_piece(t2 - 1 + LEAD, 1, 0 if HALF else None)
        return t2

    def mid(t2, n, after=None):
        if n == 0 and HALF:
            start_piece(t2 - 1 + LEAD, 1, 1)
        if n == 1:
            start_piece(t2 + LEAD, 1, 0 if HALF > 1 else None)
            start_piece(t2 - 2 + LA, 0)
            start_piece(t2 - 1 + LA, 0)
        if n == 2 and HALF > 1:
            kv[0, NP * RO, 0:16, 0:128] = jnp.concatenate([after, after], axis=0).astype(BF16)
            start_piece(t2 + LEAD, 1, 1)

    half = D // 2
    small = [pltpu.make_async_copy(x_hbm, xb_ref, wsem.at[0]),
             pltpu.make_async_copy(wr_hbm, wrb, wsem.at[1])]
    big = [pltpu.make_async_copy(wq_hbm, wq_raw, wsem.at[2]),
           pltpu.make_async_copy(wg_hbm, wg_raw, wsem.at[3]),
           pltpu.make_async_copy(wu_hbm.at[pl.ds(0, half)], wu_raw.at[pl.ds(0, half)], wsem.at[4])]
    for cp in big:
        cp.start(priority=1)
    for cp in small:
        cp.start()
    spin_ref[...] = jnp.zeros(spin_ref.shape, F32)

    inject = [(wo_hbm, wo_raw, 0, 48, HD // 48, 5), (wd_hbm, wd_raw, 0, 48, F // 48, 6),
              (wu_hbm, wu_raw, half, 16, half // 16, 7)]
    for src, dst, row0, rows, n, sem in inject:
        def body(i, c, src=src, dst=dst, row0=row0, rows=rows, sem=sem):
            r = pl.multiple_of(row0 + i * rows, 8)
            pltpu.make_async_copy(src.at[pl.ds(r, rows)], dst.at[pl.ds(r, rows)], wsem.at[sem]).start()
            spin(cfg["WSPIN"])
            return c
        lax.fori_loop(0, n, body, 0)
        if dst is wo_raw:
            for i in range(LA):
                start_piece(i, 0)

    def lead_in(h, c):
        start_piece(h >> 1, 1, h & 1)
        spin(cfg["LSPIN"])
        return c

    lax.fori_loop(0, 2 * (LEAD + 1), lead_in, 0)
    for cp in small:
        cp.wait()
    state[...] = jnp.concatenate([xb_ref[...].astype(F32), jnp.zeros((8 - B, D), F32)], axis=0)
    for src, dst, row0, rows, n, sem in inject:
        view = dst.at[pl.ds(row0, rows * n)]
        pltpu.make_async_copy(view, view, wsem.at[sem]).wait()
    for cp in big:
        cp.wait()

    NRP = D // 16

    def repack(h, c):
        full_tick(h)
        r = pl.multiple_of(h * 16, 16)
        r2 = pl.multiple_of(h * 8, 8)
        wxp[pl.ds(r2, 8), 0:HD] = _u32(wq_raw[pl.ds(r, 16), :])
        for n, pos in enumerate(cfg["VQ"]):
            wqf[pl.ds(r, 16), n * PD:(n + 1) * PD] = (
                wq_raw[pl.ds(r, 16), order[pos] * PD:(order[pos] + 1) * PD].astype(F32))
        g = wg_raw[pl.ds(r, 16), :]
        u = wu_raw[pl.ds(r, 16), :]
        gu = jnp.concatenate([w[:, i * 128:(i + 1) * 128] for i in range(NH) for w in (g, u)], axis=1)
        wxp[pl.ds(r2, 8), HD:HD + 2 * F] = _u32(gu)
        if NV:
            wguf[pl.ds(r, 16), :] = gu[:, NM * 256:].astype(F32)
        for n, pos in enumerate(cfg["VO"]):
            ro = pl.multiple_of(jnp.minimum(r, PD - 16), 16)
            wof[pl.ds(n * PD + ro, 16), :] = wo_raw[pl.ds(order[pos] * PD + ro, 16), :].astype(F32)
        if ND:
            nd = 16 if ND * 128 <= D else 32
            rd = pl.multiple_of(jnp.minimum(h * nd, ND * 128 - nd), 16)
            wdf[pl.ds(rd, nd), :] = wd_raw[pl.ds(rd, nd), :].astype(F32)
        for src, packed, n in ((wo_raw, wop, 160), (wd_raw, wdp, 48)):
            r = pl.multiple_of(jnp.minimum(h * n, src.shape[0] - n), 16)
            packed[pl.ds(pl.multiple_of(r >> 1, 8), n // 2), :] = _u32(src[pl.ds(r, n), :])
        return c

    lax.fori_loop(0, NRP, repack, 0)

    NCS = (HD + 2 * F) // 768

    def colsum(i, c):
        full_tick(NRP + i)
        c0 = pl.multiple_of(i * 768, 128)
        cs[:, pl.ds(c0, 768)] = _dot(jnp.ones((8, D), BF16), _bf(wxp[:, pl.ds(c0, 768)]))
        return c

    lax.fori_loop(0, NCS, colsum, 0)
    t0 = jnp.int32(NRP + NCS)

    never = spin_ref[...] < -1.0

    def xproj(xb, m, scale, c0, n):
        y = _dot(xb, _bf(wxp[:, pl.ds(c0, n)])) - m * cs[:, pl.ds(c0, n)]
        return y if scale is None else y * scale

    def qproj(xb, m, qscale, k):
        return xproj(xb, m, qscale, k * PD if isinstance(k, int) else pl.multiple_of(k * PD, 128), PD)

    def oproj(ob, k):
        r0 = pl.multiple_of(k * DH, DH) if not isinstance(k, int) else k * DH
        return _dot(ob, _bf(wop[pl.ds(r0, DH), :]))

    def kload(k):
        return [_bf(kp[pl.ds(k * RO + 2 * i, 2)].reshape(64, W)) for i in range(3)]

    def vgroup(slot, k, o, r):
        return lambda: kv[1 + slot, k * RO + o, pl.ds(r * 8, 8), :].astype(F32)

    def pair_groups(slot, k, pe, po):
        return [(vgroup(slot, k, g // RI, g % RI), pe if g < DH // 8 else po) for g in range(PD // 8)]

    def vpu_matvec(xr, w_ref, nadd, per_step=1, tok=None):
        nu = xr.shape[1] // 128
        xcol = [jnp.concatenate([xr[:, u * 128:(u + 1) * 128]] * 16, axis=0).T for u in range(nu)]
        seq = [(u, i) for u0 in range(0, nu, 2) for i in range(16) for u in range(u0, min(u0 + 2, nu))]
        accs = [None] * per_step
        for n in range(0, len(seq), per_step):
            if tok is not None:
                for _ in range(nadd):
                    tok = tok + 1.0
            for a, (u, i) in enumerate(seq[n:n + per_step]):
                col = xcol[u][i * 8:i * 8 + 8]
                if tok is not None:
                    col = jnp.where(never, tok, col)
                y = w_ref[u * 128 + i * 8:u * 128 + i * 8 + 8, :] * _tile(col, w_ref.shape[1] // 128)
                accs[a] = y if accs[a] is None else accs[a] + y
            tok = accs[0][:, 0:128]
        return functools.reduce(jnp.add, accs), tok

    def act(gu):
        g = gu[:, 0:128]
        return (g * _sigmoid(g) * gu[:, 128:256]).astype(BF16)

    def ffn_res(x, xc, rstd):
        wr = wrb[...].astype(F32)
        wr = jnp.concatenate([jnp.broadcast_to(wr[t:t + 1, :], (8, 128)) for t in range(D // 128)], axis=1)
        return x + xc * rstd, _round(_sigmoid(_round(jnp.sum(xc * wr, axis=1, keepdims=True) * rstd)))

    def ffn(x):
        xb, xr, m, xc, rstd = _ln_parts(x)

        hs = [act(xproj(xb, m, rstd, HD + i * 256, 256)) for i in range(NM)]
        gu, tok = vpu_matvec(xr, wguf, cfg["TOK"])
        gu = (_rowsum_all(gu) - m * cs[:, HD + NM * 256:]) * rstd
        hs += [act(gu[:, i * 256:(i + 1) * 256]) for i in range(NV)]
        y = None
        late = list(range(NM - cfg["DLATE"], NM))
        for i in [i for i in range(ND, NH) if i not in late] + late:
            yi = _dot(hs[i], _bf(wdp[i * 64:(i + 1) * 64, :]))
            y = yi if y is None else y + yi
        if ND:
            yv, _ = vpu_matvec(jnp.concatenate(hs[:ND], axis=1).astype(F32), wdf, cfg["DTOK"], 2, tok)
            y = y + _rowsum_all(yv)
        res, gate = ffn_res(xr, xc, rstd)
        return res + y * gate

    NFT = NH // 2 + 1

    def ffn_ticked(x, t):
        def body(i, carry):
            h, y, _ = carry
            full_tick(t + i)
            xb, xr, m, xc, rstd = _ln_parts(x)
            c0 = pl.multiple_of(HD + jnp.minimum(i, NFT - 2) * 512, 128)
            gu = xproj(xb, m, rstd, c0, 512)
            r0 = pl.multiple_of(jnp.maximum(i - 1, 0) * 128, 128)
            y = y + _dot(h, _bf(wdp[pl.ds(r0, 128), :]))
            res, gate = ffn_res(xr, xc, rstd)
            return jnp.concatenate([act(gu[:, 0:256]), act(gu[:, 256:512])], axis=1), y, res + y * gate

        return lax.fori_loop(0, NFT, body, (jnp.zeros((8, 256), BF16), jnp.zeros((8, D), F32), x))[2]

    NHP = 2 * B - 1

    def half_period(hp, t):
        b = hp >> 1
        slot = b & 1
        first = (hp & 1) == 0
        vbase = jnp.where(first, b * TPP + (NP + 1) * TPC, -TPP)

        tr = jnp.where(first, jnp.maximum(t, b * TPP + cfg["KRP"]), t)
        lax.fori_loop(t, tr, spin_tick, 0)

        def k_repack(h, c):
            def work():
                o0 = (h - 2 * tr) * 4
                kp[pl.ds(o0, 4)] = _u32(kv[0, pl.ds(o0, 4)].reshape(4 * 64, W)).reshape(4, 32, W)

            half_tick(h, LEAD + 1, LA, work, cfg["KSPIN"], cfg["KTOP"])
            return c

        t = jnp.where(first, tr + NP * RO // 8, t)
        lax.fori_loop(2 * tr, 2 * t, k_repack, 0)

        xb, x, m, _, rstd = _ln_parts(jnp.broadcast_to(state[pl.ds(b, 1), :], (8, D)))
        qscale = rstd * SCALE

        def step(j, carry):
            t, q, se, so, pe, po, inv, o, out = carry
            kv_ = jnp.maximum(j - 3, 0)
            t = advance(t, vbase + kv_ * TPC)
            se_n, so_n = _scores(q, kload(jnp.clip(j - 1, 0, NP - 1)))
            q_n = qproj(xb, m, qscale, jnp.minimum(j, NP - 1))
            out = out + oproj(o, jnp.maximum(j - 4, 0))
            pe_n, po_n, inv_n = _softmax_pair(se, so)
            acc = _pv(pair_groups(slot, kv_, pe, po),
                      {cfg["PVMID"][0]: lambda: mid(t, 0), cfg["PVMID"][1]: lambda: mid(t, 1)})
            mid(t, 2, q_n[:, 256:384])
            o_n = (_lane_reduce_t(acc) * jnp.where(j >= 3, inv, 0.0)).astype(BF16)
            return t, q_n, se_n, so_n, pe_n, po_n, inv_n, o_n, out

        zw = (lax.broadcasted_iota(I32, (8, W), 0) + lax.broadcasted_iota(I32, (8, W), 1)).astype(F32) * (1.0 / W)
        zp = zw[:, :PD]
        init = (t, zp, zw, zw, zw, zw, zp, jnp.zeros((8, PD), BF16), jnp.zeros((8, D), F32))
        last = hp == NHP - 1
        t, q, se, so, pe, po, inv, o, out = lax.fori_loop(0, jnp.where(last, NP, NP + 2), step, init)
        t2 = jnp.maximum(t + 2, vbase + (NP - 1) * TPC)

        @pl.when(last)
        def _():
            c_s[0] = se
            c_s[1] = so
            c_p[0] = pe
            c_p[1] = po
            c_o[0] = q
            c_o[1] = inv
            c_o[2] = o.astype(F32)
            c_out[...] = out

        @pl.when(jnp.logical_not(last))
        def _():
            advance(t, t2)
            y = out + oproj(o, NP - 2)
            acc = _pv(pair_groups(slot, NP - 1, pe, po), {24: lambda: mid(t2, 0), 45: lambda: mid(t2, 1)})
            olast = _lane_reduce_t(acc) * inv
            mid(t2, 2, olast[:, 0:128])
            olast = olast.astype(BF16)
            full_tick(t2)
            y = y + oproj(olast, NP - 1)
            state[pl.ds(b, 1), :] = ffn_ticked(x + _rowsum_all(y), t2 + 1)[0:1]

        return t2 + 1 + NFT

    lax.fori_loop(0, NHP, half_period, t0)

    slot = (B - 1) % 2
    ka, kb = NP - 2, NP - 1

    def wo_rows(runs):
        return _bf(jnp.concatenate(
            [wop[(k * PD + o * 64 + r * 8) // 2:(k * PD + o * 64 + (r + n) * 8) // 2, :] for k, o, r, n in runs],
            axis=0))

    def run_groups(runs, ps):
        return [(vgroup(slot, k, o, r + i), ps[k][0 if o < RO // 2 else 1]) for k, o, r, n in runs for i in range(n)]

    def normalised(pe, po, inv):
        return pe * _tile(inv[:, 0:128], NL), po * _tile(inv[:, 256:384], NL)

    def pv_o_vpu(runs):
        w = wo_rows(runs).astype(F32)
        return functools.reduce(jnp.add, [
            w[i * 8:(i + 1) * 8] * jnp.sum(_fold(vload() * p, jnp.add), axis=1, keepdims=True)
            for i, (vload, p) in enumerate(run_groups(runs, ps))])

    kc = NP - 3
    for i in range(NTICK - 3 * TPC, NTICK - TPC):
        wait_piece(i, 1)
    se, so = _scores(c_o[0], kload(kb))
    out = c_out[...] + oproj(c_o[2].astype(BF16), NP - 4)
    ps = {kc: normalised(c_p[0], c_p[1], c_o[1]), ka: normalised(*_softmax_pair(c_s[0], c_s[1]))}
    runs = [(k, o, TPC, TPC) for k in (kc, ka) for o in range(RO)]
    o = _lane_reduce_t(_pv(run_groups(runs, ps))).astype(BF16)
    ps[kb] = normalised(*_softmax_pair(se, so))

    for i in range(NTICK - 3 * TPC, NTICK - 2 * TPC):
        wait_piece(i, 0)
    for i in range(NTICK - TPC, NTICK):
        wait_piece(i, 1)
    out = out + _dot(o, wo_rows(runs))
    runs0 = [(kc, o, 0, TPC) for o in range(RO)] + [(kb, o, TPC, TPC) for o in range(RO)]
    o0 = _lane_reduce_t(_pv(run_groups(runs0, ps))).astype(BF16)

    for i in range(NTICK - 2 * TPC, NTICK - TPC):
        wait_piece(i, 0)
    out = out + _dot(o0, wo_rows(runs0))
    runs1 = [(ka, o, 0, TPC) for o in range(RO)]
    acc = [_fold(vload() * p, jnp.add) for vload, p in run_groups(runs1, ps)]
    zero = [jnp.zeros((8, 128), F32)] * 4
    o1 = _lane_reduce_t(jnp.concatenate(acc[:12] + zero + acc[12:] + zero, axis=0)).astype(BF16)

    for i in range(NTICK - TPC, NTICK - 2):
        wait_piece(i, 0)
    out = out + _dot(o1, wo_rows(runs1[:3] + runs1[:1] + runs1[3:] + runs1[:1]))
    out = out + pv_o_vpu([(kb, o, 0, 2) for o in range(RO)])

    for i in range(NTICK - 2, NTICK):
        wait_piece(i, 0)
    out = out + pv_o_vpu([(kb, o, 2, 2) for o in range(RO)])
    x = jnp.broadcast_to(state[B - 1:B, :], (8, D)) + _rowsum_all(out)

    def attn_fast(x):
        xb, xr, m, _, rstd = _ln_parts(x)
        qscale = rstd * SCALE
        q, sc, ps, os_, deadline, outv = {}, {}, {}, {}, {}, []
        out = None
        oslot = {}
        sl = cfg["OLAG"]
        for i in range(NP):
            while sl in cfg["OSKIP"]:
                sl += 1
            if i not in cfg["VO"]:
                oslot[sl] = i
            sl += 1
        if cfg["VQ"]:
            qv = _rowsum_all(vpu_matvec(xr, wqf, cfg["QTOK"])[0])
            for n, pos in enumerate(cfg["VQ"]):
                k = order[pos]
                q[pos] = (qv[:, n * PD:(n + 1) * PD] - m * cs[:, k * PD:(k + 1) * PD]) * qscale
        qm = [pos for pos in range(NP) if pos not in cfg["VQ"]]
        for s in range(-3, sl):
            if cfg["QEARLY"]:
                if 0 <= s + 3 < len(qm):
                    q[qm[s + 3]] = qproj(xb, m, qscale if qm[s + 3] >= cfg["NLS"] else None, order[qm[s + 3]])
            elif s + 3 in qm:
                q[s + 3] = qproj(xb, m, qscale if s + 3 >= cfg["NLS"] else None, order[s + 3])
            if 0 <= s + 2 < NP:
                qq = q.pop(s + 2)
                if s in deadline:
                    qq = jnp.concatenate([jnp.where(never, deadline.pop(s), qq[:, 0:128]), qq[:, 128:]], axis=1)
                sc[s + 2] = _scores(qq, kload(order[s + 2]))
            if s in oslot:
                y = oproj(os_.pop(oslot[s]), order[oslot[s]])
                out = y if out is None else out + y
            if 0 <= s + 1 < NP:
                ps[s + 1] = _softmax_pair(*sc.pop(s + 1), None if s + 1 >= cfg["NLS"] else qscale)
            if 0 <= s < NP:
                pe, po, inv = ps.pop(s)
                k = order[s]
                groups = pair_groups(slot, k, pe, po)
                if k not in raw:
                    groups = [(functools.partial(lambda g: vf[(k - VF0) * RO + g // RI, pl.ds((g % RI) * 8, 8), :], g), p)
                              for g, (_, p) in enumerate(groups)]
                acc = _pv(groups)
                o = _lane_reduce_t(acc) * inv
                os_[s] = (_rowsum_all(o) if s in cfg["VO"] else o).astype(BF16)
                for n, (tpos, tg, nadd, per, dl) in enumerate(cfg["VOT"]):
                    if tpos == s:
                        y, tok = vpu_matvec(os_.pop(cfg["VO"][n]).astype(F32), wof.at[n * PD:(n + 1) * PD], nadd, per,
                                            acc[tg * 8:tg * 8 + 8])
                        outv.append(y)
                        if dl:
                            deadline[s + dl] = tok
        out = functools.reduce(jnp.add, [out] + outv)
        return xr + _rowsum_all(out)

    if cfg["TAIL"] >= 1:
        x = ffn(x)
    if cfg["TAIL"] >= 2:
        x = ffn(attn_fast(x))
    row = lax.broadcasted_iota(I32, (8, D), 0)
    o_ref[...] = jnp.where(row == B - 1, x, state[...])[0:B].astype(o_ref.dtype)


def _call(cfg, A_x, A_k_cache, A_v_cache, A_wq, A_wo, B_w_r, B_w_gate, B_w_up, B_w_down):
    kt = jnp.swapaxes(A_k_cache, 2, 3).reshape(B, NP * RO, RI * 8, SK)
    vt = jnp.swapaxes(A_v_cache, 2, 3).reshape(B, NP * RO, RI * 8, SK)
    out = pl.pallas_call(
        functools.partial(_kernel, cfg=cfg),
        out_shape=jax.ShapeDtypeStruct((B, D), BF16),
        in_specs=[pl.BlockSpec(memory_space=pl.ANY)] * 9,
        out_specs=pl.BlockSpec(memory_space=pltpu.VMEM),
        scratch_shapes=[
            pltpu.VMEM((3, NP * RO + 1, RI * 8, W), BF16),
            pltpu.VMEM((VF1 * RO, RI * 8, W), F32),
            pltpu.VMEM((NP * RO, RI * 4, W), U32),
            pltpu.VMEM((D, HD), BF16),
            pltpu.VMEM((HD, D), BF16),
            pltpu.VMEM((D, F), BF16),
            pltpu.VMEM((D, F), BF16),
            pltpu.VMEM((F, D), BF16),
            pltpu.VMEM((D // 2, HD + 2 * F), U32),
            pltpu.VMEM((HD // 2, D), U32),
            pltpu.VMEM((F // 2, D), U32),
            pltpu.VMEM((D, cfg["NV"] * 256), F32),
            pltpu.VMEM((D, max(len(cfg["VQ"]), 1) * PD), F32),
            pltpu.VMEM((max(cfg["ND"], 1) * 128, D), F32),
            pltpu.VMEM((max(len(cfg["VO"]), 1) * PD, D), F32),
            pltpu.VMEM((8, HD + 2 * F), F32),
            pltpu.VMEM((B, D), BF16),
            pltpu.VMEM((D // 128, 128), BF16),
            pltpu.VMEM((8, D), F32),
            pltpu.VMEM((8, 128), F32),
            pltpu.VMEM((2, 8, W), F32),
            pltpu.VMEM((2, 8, W), F32),
            pltpu.VMEM((3, 8, PD), F32),
            pltpu.VMEM((8, D), F32),
            pltpu.SemaphoreType.DMA((2, RING)),
            pltpu.SemaphoreType.DMA((8,)),
        ],
        compiler_params=pltpu.CompilerParams(vmem_limit_bytes=126 * 1024 * 1024,
                                             disable_bounds_checks=True,
                                             disable_semaphore_checks=True),
        name="fused_decode",
    )(A_x.reshape(B, D), kt, vt, A_wq, A_wo, B_w_r.reshape(D // 128, 128), B_w_gate, B_w_up, B_w_down)
    return out.reshape(B, 1, D)


@jax.jit
def pallas_interleave_layers__sliding_block_cached__moe_arch_mod__decode_kernel(
    A_x: jax.Array,
    A_k_cache: jax.Array,
    A_v_cache: jax.Array,
    A_wq: jax.Array,
    A_wo: jax.Array,
    B_x: jax.Array,
    B_w_r: jax.Array,
    B_w_gate: jax.Array,
    B_w_up: jax.Array,
    B_w_down: jax.Array,
):
    del B_x
    return _call(CFG, A_x, A_k_cache, A_v_cache, A_wq, A_wo, B_w_r, B_w_gate, B_w_up, B_w_down)
```

```python
import functools

import jax
import jax.numpy as jnp
from jax import lax
import jax.experimental.pallas as pl
import jax.experimental.pallas.tpu as pltpu

F32 = jnp.float32
BF16 = jnp.bfloat16
U32 = jnp.uint32
I32 = jnp.int32

B, D, H, DH, SK, F = 4, 640, 32, 192, 4096, 1536
W = min(4096, max(256, SK // 4))
NP = H // 2
PD = 2 * DH
HD = H * DH
NL = W // 128
NH = F // 128
EPS = 1e-5
SCALE = DH ** -0.5 * 1.4426950408889634

RI = 8
RO = PD // (8 * RI)
TPC = RI // 2
TPP = 2 * NP * TPC
NTICK = B * TPP
RING = 32
VF0, VF1 = 0, 12

CFG = dict(
    LA=23,
    LEAD=11,
    SPIN=(1, 50),
    WSPIN=(1, 45),
    HALF=2,
    LSPIN=(1, 20),
    KSPIN=(1, 20),
    HSPIN=(1, 8),
    HTOP=False,
    KTOP=True,
    PVMID=(21, 45),
    KRP=54,
    OLAG=3,
    OSKIP=(4, 5),
    NV=4,
    TOK=0,
    QTOK=0,
    ND=4,
    DTOK=1,
    DLATE=2,
    SUMAT=(0, 1, 2, 3, 4, 5, 6, 7, 8, 9, 10, 11, 12, 13, 14),
    VO=(2, 0, 8),
    VOT=((15, 0, 0, 2, 0), (4, 47, 0, 2, 0), (11, 32, 0, 2, 2)),
    VQ=(2, 3, 4),
    RAWPOS=(2, 7, 10, 14),
    QEARLY=True,
    NLS=2,
    TAIL=2,
)


def _order(cfg):
    raw = [k for k in range(NP) if not VF0 <= k < VF1]
    order = list(range(VF0, VF1))
    for pos, k in zip(sorted(cfg["RAWPOS"]), raw):
        order.insert(pos, k)
    return order, raw


def _rowsum_all(x):
    x = x + pltpu.roll(x, 4, 0)
    x = x + pltpu.roll(x, 2, 0)
    return x + pltpu.roll(x, 1, 0)


def _bf(x):
    return pltpu.bitcast(x, BF16)


def _u32(x):
    return pltpu.bitcast(x, U32)


def _dot(a, b):
    return jnp.dot(a, b, preferred_element_type=F32)


def _sigmoid(x):
    return pl.reciprocal(1.0 + jnp.exp(-x), approx=True)


def _round(x):
    return x.astype(BF16).astype(F32)


def _ln_parts(x):
    xb = x.astype(BF16)
    xr = xb.astype(F32)
    m = jnp.sum(xr, axis=1, keepdims=True) * (1.0 / D)
    xc = xr - m
    v = jnp.sum(xc * xc, axis=1, keepdims=True) * (1.0 / D)
    m = _round(m)
    v = _round(_round(v) + EPS)
    return xb, xr, m, xr - m, pl.reciprocal(_round(v * lax.rsqrt(v)), approx=True)


def _scores(q, kk):
    lane = lax.broadcasted_iota(I32, (8, 128), 1)
    q0 = q[:, 0:128].astype(BF16)
    qm = q[:, 128:256]
    q2 = q[:, 256:384].astype(BF16)
    mid = jnp.concatenate([jnp.where(lane < 64, qm, 0.0), jnp.where(lane >= 64, qm, 0.0)],
                          axis=0).astype(BF16)
    r0 = _dot(q0, kk[0])
    rm = _dot(mid, kk[1])
    r2 = _dot(q2, kk[2])
    return r0 + rm[0:8], rm[8:16] + r2


def _fold(x, op):
    r = x[:, 0:128]
    for t in range(1, x.shape[1] // 128):
        r = op(r, x[:, t * 128:(t + 1) * 128])
    return r


def _tile(x, n):
    return jnp.concatenate([x] * n, axis=1)


def _inv_sums(parts):
    row = lax.broadcasted_iota(I32, (8, 128), 0)
    c = parts[0]
    for i in range(1, len(parts)):
        c = jnp.where(row >= i, parts[i], c)
    r = jnp.broadcast_to(pl.reciprocal(jnp.sum(c, axis=1, keepdims=True), approx=True), (8, 128))
    inv = [jnp.broadcast_to(r[i:i + 1], (8, 128)) for i in range(len(parts))]
    lane = lax.broadcasted_iota(I32, (8, 128), 1)
    return [jnp.concatenate([ie, jnp.where(lane < 64, ie, io), io], axis=1) for ie, io in zip(inv[0::2], inv[1::2])]


def _softmax_pair(se, so, c=None, sums=True):
    top = lax.broadcasted_iota(I32, (8, 128), 0) < 4

    def split(c):
        c = jnp.broadcast_to(c, (8, 128))
        r = pltpu.roll(c, 4, 0)
        return jnp.where(top, c, r), jnp.where(top, r, c)

    m = jnp.max(jnp.where(top, _fold(se, jnp.maximum), _fold(so, jnp.maximum)), axis=1, keepdims=True)
    me, mo = split(m)
    de, do = se - _tile(me, NL), so - _tile(mo, NL)
    if c is not None:
        de, do = de * c, do * c
    pe, po = jnp.exp2(de), jnp.exp2(do)
    if not sums:
        return pe, po, [_fold(pe, jnp.add), _fold(po, jnp.add)]
    l = jnp.sum(jnp.where(top, _fold(pe, jnp.add), _fold(po, jnp.add)), axis=1, keepdims=True)
    ie, io = split(pl.reciprocal(l, approx=True))
    lane = lax.broadcasted_iota(I32, (8, 128), 1)
    return pe, po, jnp.concatenate([ie, jnp.where(lane < 64, ie, io), io], axis=1)


def _pv(groups, hooks=None):
    nb = len(groups) // 16
    accs = {}
    for n, g in enumerate(16 * blk + i for i in range(16) for blk in range(nb)):
        if hooks and n in hooks:
            hooks[n]()
        vload, p = groups[g]
        accs[g] = _fold(vload() * p, jnp.add)
    return jnp.concatenate([accs[g] for g in range(len(groups))], axis=0)


def _lane_reduce_t(acc):
    at = acc.T
    s = at[0:8]
    for i in range(1, 16):
        s = s + at[8 * i:8 * i + 8]
    return s


def _kernel(x_hbm, kt_hbm, vt_hbm, wq_hbm, wo_hbm, wr_hbm, wg_hbm, wu_hbm, wd_hbm,
            o_ref,
            kv, vf, kp, wq_raw, wo_raw, wg_raw, wu_raw, wd_raw, wxp, wop, wdp, wguf, wqf, wdf, wof, cs,
            xb_ref, wrb, state, spin_ref, c_s, c_p, c_o, c_out,
            sems, wsem, *, cfg):
    LA, LEAD, NV = cfg["LA"], cfg["LEAD"], cfg["NV"]
    NM = NH - NV
    ND = cfg["ND"]
    HALF = cfg["HALF"]
    order, raw = _order(cfg)

    def piece(i, s):
        q, pair, w, b = i & (TPC - 1), (i >> 2) & (NP - 1), (i >> 6) & 1, i >> 7
        r0 = (q + s * TPC) * 8
        if not isinstance(i, int):
            r0 = pl.multiple_of(r0, 8)
        return pair, w, b, w * (1 + (b & 1)), i & (RING - 1), r0

    def start_piece(i, s, hf=None):
        pair, w, b, plane, ring, r0 = piece(i, s)
        osl = pl.ds(pair * RO, RO) if hf is None else pl.ds(pair * RO + hf * (RO // 2), RO // 2)

        def go(ww):
            src = vt_hbm if ww else kt_hbm
            pltpu.make_async_copy(src.at[b, osl, pl.ds(r0, 8), pl.ds(SK - W, W)],
                                  kv.at[plane, osl, pl.ds(r0, 8), :],
                                  sems.at[s, ring]).start(priority=1 - s)

        if isinstance(i, int):
            go(w)
        else:
            for ww in range(2):
                pl.when(jnp.logical_and(w == ww, i < NTICK))(functools.partial(go, ww))

    def wait_piece(i, s):
        pair, w, b, plane, ring, r0 = piece(i, s)
        view = kv.at[plane, pl.ds(pair * RO, RO), pl.ds(r0, 8), :]
        pltpu.make_async_copy(view, view, sems.at[s, ring]).wait()

    def wait_tick(i):
        wait_piece(i, 0)
        wait_piece(i, 1)

    def spin(n):
        v = spin_ref[...]
        lane = lax.broadcasted_iota(I32, v.shape, 1).astype(F32)
        for _ in range(n[0]):
            v = jnp.max(v, axis=1, keepdims=True) * 0.5 + lane
        for _ in range(n[1] // 2):
            v = v * 0.5
            v = v + lane
        spin_ref[...] = v

    def full_tick(i):
        wait_tick(i)
        start_piece(i + LEAD + 1, 1)
        start_piece(i + LA, 0)

    def spin_tick(i, c):
        full_tick(i)
        spin(cfg["SPIN"])
        return c

    def half_tick(h, lead, la, work, sp, top):
        i = h >> 1
        pl.when((h & 1) == 0)(lambda: wait_tick(i))
        if top:
            start_piece(i + lead, 1, h & 1)
        work()
        spin(sp)
        if not top:
            start_piece(i + lead, 1, h & 1)
        start_piece(jnp.where((h & 1) == 1, i + la, NTICK), 0)

    def idle_half(h, c):
        def work():
            n = (((h >> 3) & (NP - 1)) - 4) * 4 + (h & 7) - 2
            o0 = jnp.minimum(n * 2, VF1 * RO - 2)
            vf[pl.ds(o0, 2)] = kv[1 + ((h >> 8) & 1), pl.ds(o0, 2)].astype(F32)

        half_tick(h, LEAD, LA - 1, work, cfg["HSPIN"], cfg["HTOP"])
        return c

    def advance(t, need):
        t2 = jnp.maximum(t + 2, need)
        wait_tick(t)
        lax.fori_loop(2 * t + 2, 2 * t2 - 2, idle_half, 0)
        wait_tick(t2 - 1)
        start_piece(t2 - 1 + LEAD, 1, 0 if HALF else None)
        return t2

    def mid(t2, n, after=None):
        if n == 0 and HALF:
            start_piece(t2 - 1 + LEAD, 1, 1)
        if n == 1:
            start_piece(t2 + LEAD, 1, 0 if HALF > 1 else None)
            start_piece(t2 - 2 + LA, 0)
            start_piece(t2 - 1 + LA, 0)
        if n == 2 and HALF > 1:
            kv[0, NP * RO, 0:16, 0:128] = jnp.concatenate([after, after], axis=0).astype(BF16)
            start_piece(t2 + LEAD, 1, 1)

    half = D // 2
    small = [pltpu.make_async_copy(x_hbm, xb_ref, wsem.at[0]),
             pltpu.make_async_copy(wr_hbm, wrb, wsem.at[1])]
    big = [pltpu.make_async_copy(wq_hbm, wq_raw, wsem.at[2]),
           pltpu.make_async_copy(wg_hbm, wg_raw, wsem.at[3]),
           pltpu.make_async_copy(wu_hbm.at[pl.ds(0, half)], wu_raw.at[pl.ds(0, half)], wsem.at[4])]
    for cp in big:
        cp.start(priority=1)
    for cp in small:
        cp.start()
    spin_ref[...] = jnp.zeros(spin_ref.shape, F32)

    inject = [(wo_hbm, wo_raw, 0, 48, HD // 48, 5), (wd_hbm, wd_raw, 0, 48, F // 48, 6),
              (wu_hbm, wu_raw, half, 16, half // 16, 7)]
    for src, dst, row0, rows, n, sem in inject:
        def body(i, c, src=src, dst=dst, row0=row0, rows=rows, sem=sem):
            r = pl.multiple_of(row0 + i * rows, 8)
            pltpu.make_async_copy(src.at[pl.ds(r, rows)], dst.at[pl.ds(r, rows)], wsem.at[sem]).start()
            spin(cfg["WSPIN"])
            return c
        lax.fori_loop(0, n, body, 0)
        if dst is wo_raw:
            for i in range(LA):
                start_piece(i, 0)

    def lead_in(h, c):
        start_piece(h >> 1, 1, h & 1)
        spin(cfg["LSPIN"])
        return c

    lax.fori_loop(0, 2 * (LEAD + 1), lead_in, 0)
    for cp in small:
        cp.wait()
    state[...] = jnp.concatenate([xb_ref[...].astype(F32), jnp.zeros((8 - B, D), F32)], axis=0)
    for src, dst, row0, rows, n, sem in inject:
        view = dst.at[pl.ds(row0, rows * n)]
        pltpu.make_async_copy(view, view, wsem.at[sem]).wait()
    for cp in big:
        cp.wait()

    NRP = D // 16

    def repack(h, c):
        full_tick(h)
        r = pl.multiple_of(h * 16, 16)
        r2 = pl.multiple_of(h * 8, 8)
        wxp[pl.ds(r2, 8), 0:HD] = _u32(wq_raw[pl.ds(r, 16), :])
        for n, pos in enumerate(cfg["VQ"]):
            wqf[pl.ds(r, 16), n * PD:(n + 1) * PD] = (
                wq_raw[pl.ds(r, 16), order[pos] * PD:(order[pos] + 1) * PD].astype(F32))
        g = wg_raw[pl.ds(r, 16), :]
        u = wu_raw[pl.ds(r, 16), :]
        gu = jnp.concatenate([w[:, i * 128:(i + 1) * 128] for i in range(NH) for w in (g, u)], axis=1)
        wxp[pl.ds(r2, 8), HD:HD + 2 * F] = _u32(gu)
        if NV:
            wguf[pl.ds(r, 16), :] = gu[:, NM * 256:].astype(F32)
        for n, pos in enumerate(cfg["VO"]):
            ro = pl.multiple_of(jnp.minimum(r, PD - 16), 16)
            wof[pl.ds(n * PD + ro, 16), :] = wo_raw[pl.ds(order[pos] * PD + ro, 16), :].astype(F32)
        if ND:
            nd = 16 if ND * 128 <= D else 32
            rd = pl.multiple_of(jnp.minimum(h * nd, ND * 128 - nd), 16)
            wdf[pl.ds(rd, nd), :] = wd_raw[pl.ds(rd, nd), :].astype(F32)
        for src, packed, n in ((wo_raw, wop, 160), (wd_raw, wdp, 48)):
            r = pl.multiple_of(jnp.minimum(h * n, src.shape[0] - n), 16)
            packed[pl.ds(pl.multiple_of(r >> 1, 8), n // 2), :] = _u32(src[pl.ds(r, n), :])
        return c

    lax.fori_loop(0, NRP, repack, 0)

    NCS = (HD + 2 * F) // 768

    def colsum(i, c):
        full_tick(NRP + i)
        c0 = pl.multiple_of(i * 768, 128)
        cs[:, pl.ds(c0, 768)] = _dot(jnp.ones((8, D), BF16), _bf(wxp[:, pl.ds(c0, 768)]))
        return c

    lax.fori_loop(0, NCS, colsum, 0)
    t0 = jnp.int32(NRP + NCS)

    never = spin_ref[...] < -1.0

    def xproj(xb, m, scale, c0, n):
        y = _dot(xb, _bf(wxp[:, pl.ds(c0, n)])) - m * cs[:, pl.ds(c0, n)]
        return y if scale is None else y * scale

    def qproj(xb, m, qscale, k):
        return xproj(xb, m, qscale, k * PD if isinstance(k, int) else pl.multiple_of(k * PD, 128), PD)

    def oproj(ob, k):
        r0 = pl.multiple_of(k * DH, DH) if not isinstance(k, int) else k * DH
        return _dot(ob, _bf(wop[pl.ds(r0, DH), :]))

    def kload(k):
        return [_bf(kp[pl.ds(k * RO + 2 * i, 2)].reshape(64, W)) for i in range(3)]

    def vgroup(slot, k, o, r):
        return lambda: kv[1 + slot, k * RO + o, pl.ds(r * 8, 8), :].astype(F32)

    def pair_groups(slot, k, pe, po):
        return [(vgroup(slot, k, g // RI, g % RI), pe if g < DH // 8 else po) for g in range(PD // 8)]

    def vpu_matvec(xr, w_ref, nadd, per_step=1, tok=None):
        nu = xr.shape[1] // 128
        xcol = [jnp.concatenate([xr[:, u * 128:(u + 1) * 128]] * 16, axis=0).T for u in range(nu)]
        seq = [(u, i) for u0 in range(0, nu, 2) for i in range(16) for u in range(u0, min(u0 + 2, nu))]
        accs = [None] * per_step
        for n in range(0, len(seq), per_step):
            if tok is not None:
                for _ in range(nadd):
                    tok = tok + 1.0
            for a, (u, i) in enumerate(seq[n:n + per_step]):
                col = xcol[u][i * 8:i * 8 + 8]
                if tok is not None:
                    col = jnp.where(never, tok, col)
                y = w_ref[u * 128 + i * 8:u * 128 + i * 8 + 8, :] * _tile(col, w_ref.shape[1] // 128)
                accs[a] = y if accs[a] is None else accs[a] + y
            tok = accs[0][:, 0:128]
        return functools.reduce(jnp.add, accs), tok

    def act(gu):
        g = gu[:, 0:128]
        return (g * _sigmoid(g) * gu[:, 128:256]).astype(BF16)

    def ffn_res(x, xc, rstd):
        wr = wrb[...].astype(F32)
        wr = jnp.concatenate([jnp.broadcast_to(wr[t:t + 1, :], (8, 128)) for t in range(D // 128)], axis=1)
        return x + xc * rstd, _round(_sigmoid(_round(jnp.sum(xc * wr, axis=1, keepdims=True) * rstd)))

    def ffn(x):
        xb, xr, m, xc, rstd = _ln_parts(x)

        hs = [act(xproj(xb, m, rstd, HD + i * 256, 256)) for i in range(NM)]
        gu, tok = vpu_matvec(xr, wguf, cfg["TOK"])
        gu = (_rowsum_all(gu) - m * cs[:, HD + NM * 256:]) * rstd
        hs += [act(gu[:, i * 256:(i + 1) * 256]) for i in range(NV)]
        y = None
        late = list(range(NM - cfg["DLATE"], NM))
        for i in [i for i in range(ND, NH) if i not in late] + late:
            yi = _dot(hs[i], _bf(wdp[i * 64:(i + 1) * 64, :]))
            y = yi if y is None else y + yi
        if ND:
            yv, _ = vpu_matvec(jnp.concatenate(hs[:ND], axis=1).astype(F32), wdf, cfg["DTOK"], 2, tok)
            y = y + _rowsum_all(yv)
        res, gate = ffn_res(xr, xc, rstd)
        return res + y * gate

    NFT = NH // 2 + 1

    def ffn_ticked(x, t):
        def body(i, carry):
            h, y, _ = carry
            full_tick(t + i)
            xb, xr, m, xc, rstd = _ln_parts(x)
            c0 = pl.multiple_of(HD + jnp.minimum(i, NFT - 2) * 512, 128)
            gu = xproj(xb, m, rstd, c0, 512)
            r0 = pl.multiple_of(jnp.maximum(i - 1, 0) * 128, 128)
            y = y + _dot(h, _bf(wdp[pl.ds(r0, 128), :]))
            res, gate = ffn_res(xr, xc, rstd)
            return jnp.concatenate([act(gu[:, 0:256]), act(gu[:, 256:512])], axis=1), y, res + y * gate

        return lax.fori_loop(0, NFT, body, (jnp.zeros((8, 256), BF16), jnp.zeros((8, D), F32), x))[2]

    NHP = 2 * B - 1

    def half_period(hp, t):
        b = hp >> 1
        slot = b & 1
        first = (hp & 1) == 0
        vbase = jnp.where(first, b * TPP + (NP + 1) * TPC, -TPP)

        tr = jnp.where(first, jnp.maximum(t, b * TPP + cfg["KRP"]), t)
        lax.fori_loop(t, tr, spin_tick, 0)

        def k_repack(h, c):
            def work():
                o0 = (h - 2 * tr) * 4
                kp[pl.ds(o0, 4)] = _u32(kv[0, pl.ds(o0, 4)].reshape(4 * 64, W)).reshape(4, 32, W)

            half_tick(h, LEAD + 1, LA, work, cfg["KSPIN"], cfg["KTOP"])
            return c

        t = jnp.where(first, tr + NP * RO // 8, t)
        lax.fori_loop(2 * tr, 2 * t, k_repack, 0)

        xb, x, m, _, rstd = _ln_parts(jnp.broadcast_to(state[pl.ds(b, 1), :], (8, D)))
        qscale = rstd * SCALE

        def step(j, carry):
            t, q, se, so, pe, po, inv, o, out = carry
            kv_ = jnp.maximum(j - 3, 0)
            t = advance(t, vbase + kv_ * TPC)
            se_n, so_n = _scores(q, kload(jnp.clip(j - 1, 0, NP - 1)))
            q_n = qproj(xb, m, qscale, jnp.minimum(j, NP - 1))
            out = out + oproj(o, jnp.maximum(j - 4, 0))
            pe_n, po_n, inv_n = _softmax_pair(se, so)
            acc = _pv(pair_groups(slot, kv_, pe, po),
                      {cfg["PVMID"][0]: lambda: mid(t, 0), cfg["PVMID"][1]: lambda: mid(t, 1)})
            mid(t, 2, q_n[:, 256:384])
            o_n = (_lane_reduce_t(acc) * jnp.where(j >= 3, inv, 0.0)).astype(BF16)
            return t, q_n, se_n, so_n, pe_n, po_n, inv_n, o_n, out

        zw = (lax.broadcasted_iota(I32, (8, W), 0) + lax.broadcasted_iota(I32, (8, W), 1)).astype(F32) * (1.0 / W)
        zp = zw[:, :PD]
        init = (t, zp, zw, zw, zw, zw, zp, jnp.zeros((8, PD), BF16), jnp.zeros((8, D), F32))
        last = hp == NHP - 1
        t, q, se, so, pe, po, inv, o, out = lax.fori_loop(0, jnp.where(last, NP, NP + 2), step, init)
        t2 = jnp.maximum(t + 2, vbase + (NP - 1) * TPC)

        @pl.when(last)
        def _():
            c_s[0] = se
            c_s[1] = so
            c_p[0] = pe
            c_p[1] = po
            c_o[0] = q
            c_o[1] = inv
            c_o[2] = o.astype(F32)
            c_out[...] = out

        @pl.when(jnp.logical_not(last))
        def _():
            advance(t, t2)
            y = out + oproj(o, NP - 2)
            acc = _pv(pair_groups(slot, NP - 1, pe, po), {24: lambda: mid(t2, 0), 45: lambda: mid(t2, 1)})
            olast = _lane_reduce_t(acc) * inv
            mid(t2, 2, olast[:, 0:128])
            olast = olast.astype(BF16)
            full_tick(t2)
            y = y + oproj(olast, NP - 1)
            state[pl.ds(b, 1), :] = ffn_ticked(x + _rowsum_all(y), t2 + 1)[0:1]

        return t2 + 1 + NFT

    lax.fori_loop(0, NHP, half_period, t0)

    slot = (B - 1) % 2
    ka, kb = NP - 2, NP - 1

    def wo_rows(runs):
        return _bf(jnp.concatenate(
            [wop[(k * PD + o * 64 + r * 8) // 2:(k * PD + o * 64 + (r + n) * 8) // 2, :] for k, o, r, n in runs],
            axis=0))

    def run_groups(runs, ps):
        return [(vgroup(slot, k, o, r + i), ps[k][0 if o < RO // 2 else 1]) for k, o, r, n in runs for i in range(n)]

    def normalised(pe, po, inv):
        return pe * _tile(inv[:, 0:128], NL), po * _tile(inv[:, 256:384], NL)

    def pv_o_vpu(runs):
        w = wo_rows(runs).astype(F32)
        return functools.reduce(jnp.add, [
            w[i * 8:(i + 1) * 8] * jnp.sum(_fold(vload() * p, jnp.add), axis=1, keepdims=True)
            for i, (vload, p) in enumerate(run_groups(runs, ps))])

    kc = NP - 3
    for i in range(NTICK - 3 * TPC, NTICK - TPC):
        wait_piece(i, 1)
    se, so = _scores(c_o[0], kload(kb))
    out = c_out[...] + oproj(c_o[2].astype(BF16), NP - 4)
    ps = {kc: normalised(c_p[0], c_p[1], c_o[1]), ka: normalised(*_softmax_pair(c_s[0], c_s[1]))}
    runs = [(k, o, TPC, TPC) for k in (kc, ka) for o in range(RO)]
    o = _lane_reduce_t(_pv(run_groups(runs, ps))).astype(BF16)
    ps[kb] = normalised(*_softmax_pair(se, so))

    for i in range(NTICK - 3 * TPC, NTICK - 2 * TPC):
        wait_piece(i, 0)
    for i in range(NTICK - TPC, NTICK):
        wait_piece(i, 1)
    out = out + _dot(o, wo_rows(runs))
    runs0 = [(kc, o, 0, TPC) for o in range(RO)] + [(kb, o, TPC, TPC) for o in range(RO)]
    o0 = _lane_reduce_t(_pv(run_groups(runs0, ps))).astype(BF16)

    for i in range(NTICK - 2 * TPC, NTICK - TPC):
        wait_piece(i, 0)
    out = out + _dot(o0, wo_rows(runs0))
    runs1 = [(ka, o, 0, TPC) for o in range(RO)]
    acc = [_fold(vload() * p, jnp.add) for vload, p in run_groups(runs1, ps)]
    zero = [jnp.zeros((8, 128), F32)] * 4
    o1 = _lane_reduce_t(jnp.concatenate(acc[:12] + zero + acc[12:] + zero, axis=0)).astype(BF16)

    for i in range(NTICK - TPC, NTICK - 2):
        wait_piece(i, 0)
    out = out + _dot(o1, wo_rows(runs1[:3] + runs1[:1] + runs1[3:] + runs1[:1]))
    out = out + pv_o_vpu([(kb, o, 0, 2) for o in range(RO)])

    for i in range(NTICK - 2, NTICK):
        wait_piece(i, 0)
    out = out + pv_o_vpu([(kb, o, 2, 2) for o in range(RO)])
    x = jnp.broadcast_to(state[B - 1:B, :], (8, D)) + _rowsum_all(out)

    def attn_fast(x):
        xb, xr, m, _, rstd = _ln_parts(x)
        qscale = rstd * SCALE
        q, sc, ps, os_, deadline, outv = {}, {}, {}, {}, {}, []
        invs, pend, parts = {}, [], []

        def get_o(pos):
            o = os_.pop(pos) * invs.pop(pos)
            return (_rowsum_all(o) if pos in cfg["VO"] else o).astype(BF16)

        out = None
        oslot = {}
        sl = cfg["OLAG"]
        for i in range(NP):
            while sl in cfg["OSKIP"]:
                sl += 1
            if i not in cfg["VO"]:
                oslot[sl] = i
            sl += 1
        if cfg["VQ"]:
            qv = _rowsum_all(vpu_matvec(xr, wqf, cfg["QTOK"])[0])
            for n, pos in enumerate(cfg["VQ"]):
                k = order[pos]
                q[pos] = (qv[:, n * PD:(n + 1) * PD] - m * cs[:, k * PD:(k + 1) * PD]) * qscale
        qm = [pos for pos in range(NP) if pos not in cfg["VQ"]]
        for s in range(-3, sl):
            if cfg["QEARLY"]:
                if 0 <= s + 3 < len(qm):
                    q[qm[s + 3]] = qproj(xb, m, qscale if qm[s + 3] >= cfg["NLS"] else None, order[qm[s + 3]])
            elif s + 3 in qm:
                q[s + 3] = qproj(xb, m, qscale if s + 3 >= cfg["NLS"] else None, order[s + 3])
            if 0 <= s + 2 < NP:
                qq = q.pop(s + 2)
                if s in deadline:
                    qq = jnp.concatenate([jnp.where(never, deadline.pop(s), qq[:, 0:128]), qq[:, 128:]], axis=1)
                sc[s + 2] = _scores(qq, kload(order[s + 2]))
            if s in oslot:
                y = oproj(get_o(oslot[s]), order[oslot[s]])
                out = y if out is None else out + y
            if 0 <= s + 1 < NP:
                ps[s + 1] = _softmax_pair(*sc.pop(s + 1), None if s + 1 >= cfg["NLS"] else qscale, sums=False)
                pend.append(s + 1)
                parts += ps[s + 1][2]
                if s + 1 in cfg["SUMAT"] or s + 1 == NP - 1 or len(pend) == 4:
                    invs.update(zip(pend, _inv_sums(parts)))
                    pend, parts = [], []
            if 0 <= s < NP:
                pe, po, _ = ps.pop(s)
                k = order[s]
                groups = pair_groups(slot, k, pe, po)
                if k not in raw:
                    groups = [(functools.partial(lambda g: vf[(k - VF0) * RO + g // RI, pl.ds((g % RI) * 8, 8), :], g), p)
                              for g, (_, p) in enumerate(groups)]
                acc = _pv(groups)
                os_[s] = _lane_reduce_t(acc)
                for n, (tpos, tg, nadd, per, dl) in enumerate(cfg["VOT"]):
                    if tpos == s:
                        y, tok = vpu_matvec(get_o(cfg["VO"][n]).astype(F32), wof.at[n * PD:(n + 1) * PD], nadd, per,
                                            acc[tg * 8:tg * 8 + 8])
                        outv.append(y)
                        if dl:
                            deadline[s + dl] = tok
        out = functools.reduce(jnp.add, [out] + outv)
        return xr + _rowsum_all(out)

    if cfg["TAIL"] >= 1:
        x = ffn(x)
    if cfg["TAIL"] >= 2:
        x = ffn(attn_fast(x))
    row = lax.broadcasted_iota(I32, (8, D), 0)
    o_ref[...] = jnp.where(row == B - 1, x, state[...])[0:B].astype(o_ref.dtype)


def _call(cfg, A_x, A_k_cache, A_v_cache, A_wq, A_wo, B_w_r, B_w_gate, B_w_up, B_w_down):
    kt = jnp.swapaxes(A_k_cache, 2, 3).reshape(B, NP * RO, RI * 8, SK)
    vt = jnp.swapaxes(A_v_cache, 2, 3).reshape(B, NP * RO, RI * 8, SK)
    out = pl.pallas_call(
        functools.partial(_kernel, cfg=cfg),
        out_shape=jax.ShapeDtypeStruct((B, D), BF16),
        in_specs=[pl.BlockSpec(memory_space=pl.ANY)] * 9,
        out_specs=pl.BlockSpec(memory_space=pltpu.VMEM),
        scratch_shapes=[
            pltpu.VMEM((3, NP * RO + 1, RI * 8, W), BF16),
            pltpu.VMEM((VF1 * RO, RI * 8, W), F32),
            pltpu.VMEM((NP * RO, RI * 4, W), U32),
            pltpu.VMEM((D, HD), BF16),
            pltpu.VMEM((HD, D), BF16),
            pltpu.VMEM((D, F), BF16),
            pltpu.VMEM((D, F), BF16),
            pltpu.VMEM((F, D), BF16),
            pltpu.VMEM((D // 2, HD + 2 * F), U32),
            pltpu.VMEM((HD // 2, D), U32),
            pltpu.VMEM((F // 2, D), U32),
            pltpu.VMEM((D, cfg["NV"] * 256), F32),
            pltpu.VMEM((D, max(len(cfg["VQ"]), 1) * PD), F32),
            pltpu.VMEM((max(cfg["ND"], 1) * 128, D), F32),
            pltpu.VMEM((max(len(cfg["VO"]), 1) * PD, D), F32),
            pltpu.VMEM((8, HD + 2 * F), F32),
            pltpu.VMEM((B, D), BF16),
            pltpu.VMEM((D // 128, 128), BF16),
            pltpu.VMEM((8, D), F32),
            pltpu.VMEM((8, 128), F32),
            pltpu.VMEM((2, 8, W), F32),
            pltpu.VMEM((2, 8, W), F32),
            pltpu.VMEM((3, 8, PD), F32),
            pltpu.VMEM((8, D), F32),
            pltpu.SemaphoreType.DMA((2, RING)),
            pltpu.SemaphoreType.DMA((8,)),
        ],
        compiler_params=pltpu.CompilerParams(vmem_limit_bytes=126 * 1024 * 1024,
                                             disable_bounds_checks=True,
                                             disable_semaphore_checks=True),
        name="fused_decode",
    )(A_x.reshape(B, D), kt, vt, A_wq, A_wo, B_w_r.reshape(D // 128, 128), B_w_gate, B_w_up, B_w_down)
    return out.reshape(B, 1, D)


@jax.jit
def pallas_interleave_layers__sliding_block_cached__moe_arch_mod__decode_kernel(
    A_x: jax.Array,
    A_k_cache: jax.Array,
    A_v_cache: jax.Array,
    A_wq: jax.Array,
    A_wo: jax.Array,
    B_x: jax.Array,
    B_w_r: jax.Array,
    B_w_gate: jax.Array,
    B_w_up: jax.Array,
    B_w_down: jax.Array,
):
    del B_x
    return _call(CFG, A_x, A_k_cache, A_v_cache, A_wq, A_wo, B_w_r, B_w_gate, B_w_up, B_w_down)
```

```python
import functools

import jax
import jax.numpy as jnp
from jax import lax
import jax.experimental.pallas as pl
import jax.experimental.pallas.tpu as pltpu

F32 = jnp.float32
BF16 = jnp.bfloat16
U32 = jnp.uint32
I32 = jnp.int32

B, D, H, DH, SK, F = 4, 640, 32, 192, 4096, 1536
W = min(4096, max(256, SK // 4))
NP = H // 2
PD = 2 * DH
HD = H * DH
NL = W // 128
NH = F // 128
EPS = 1e-5
SCALE = DH ** -0.5 * 1.4426950408889634

RI = 8
RO = PD // (8 * RI)
TPC = RI // 2
TPP = 2 * NP * TPC
NTICK = B * TPP
RING = 32
VF = 12

CFG = dict(
    LA=23,
    LEAD=11,
    KRP=54,
    PVMID=(21, 45),
    SPIN=(1, 50),
    WSPIN=(1, 45),
    LSPIN=(1, 20),
    KSPIN=(1, 20),
    HSPIN=(1, 8),
    NV=4,
    ND=4,
    DLATE=2,
    TOK=0,
    DTOK=1,
    QTOK=0,
    RAWPOS=(2, 7, 10, 14),
    OLAG=3,
    OSKIP=(4, 5),
    NLS=2,
    VQ=(2, 3, 4),
    VO=(2, 0, 8),
    VOT=((15, 0, 0, 2, 0), (4, 47, 0, 2, 0), (11, 32, 0, 2, 2)),
)


def _order(cfg):
    order = list(range(VF))
    for pos, k in zip(sorted(cfg["RAWPOS"]), range(VF, NP)):
        order.insert(pos, k)
    return order


def _rowsum_all(x):
    x = x + pltpu.roll(x, 4, 0)
    x = x + pltpu.roll(x, 2, 0)
    return x + pltpu.roll(x, 1, 0)


def _bf(x):
    return pltpu.bitcast(x, BF16)


def _u32(x):
    return pltpu.bitcast(x, U32)


def _dot(a, b):
    return jnp.dot(a, b, preferred_element_type=F32)


def _sigmoid(x):
    return pl.reciprocal(1.0 + jnp.exp(-x), approx=True)


def _round(x):
    return x.astype(BF16).astype(F32)


def _ln_parts(x):
    xb = x.astype(BF16)
    xr = xb.astype(F32)
    m = jnp.sum(xr, axis=1, keepdims=True) * (1.0 / D)
    xc = xr - m
    v = jnp.sum(xc * xc, axis=1, keepdims=True) * (1.0 / D)
    m = _round(m)
    v = _round(_round(v) + EPS)
    return xb, xr, m, xr - m, pl.reciprocal(_round(v * lax.rsqrt(v)), approx=True)


def _scores(q, kk):
    lane = lax.broadcasted_iota(I32, (8, 128), 1)
    q0 = q[:, 0:128].astype(BF16)
    qm = q[:, 128:256]
    q2 = q[:, 256:384].astype(BF16)
    mid = jnp.concatenate([jnp.where(lane < 64, qm, 0.0), jnp.where(lane >= 64, qm, 0.0)],
                          axis=0).astype(BF16)
    r0 = _dot(q0, kk[0])
    rm = _dot(mid, kk[1])
    r2 = _dot(q2, kk[2])
    return r0 + rm[0:8], rm[8:16] + r2


def _fold(x, op):
    r = x[:, 0:128]
    for t in range(1, x.shape[1] // 128):
        r = op(r, x[:, t * 128:(t + 1) * 128])
    return r


def _tile(x, n):
    return jnp.concatenate([x] * n, axis=1)


def _softmax_pair(se, so, c=None, bcast=False):
    row = lax.broadcasted_iota(I32, (8, 128), 0)
    top = row < 4

    def split(c):
        c = jnp.broadcast_to(c, (8, 128))
        r = pltpu.roll(c, 4, 0)
        return jnp.where(top, c, r), jnp.where(top, r, c)

    m = jnp.max(jnp.where(top, _fold(se, jnp.maximum), _fold(so, jnp.maximum)), axis=1, keepdims=True)
    me, mo = split(m)
    de, do = se - _tile(me, NL), so - _tile(mo, NL)
    if c is not None:
        de, do = de * c, do * c
    pe, po = jnp.exp2(de), jnp.exp2(do)
    le, lo = _fold(pe, jnp.add), _fold(po, jnp.add)
    if bcast:
        l = jnp.sum(jnp.where(row >= 1, lo, le), axis=1, keepdims=True)
        r = jnp.broadcast_to(pl.reciprocal(l, approx=True), (8, 128))
        ie, io = [jnp.broadcast_to(r[i:i + 1], (8, 128)) for i in range(2)]
    else:
        ie, io = split(pl.reciprocal(jnp.sum(jnp.where(top, le, lo), axis=1, keepdims=True), approx=True))
    lane = lax.broadcasted_iota(I32, (8, 128), 1)
    return pe, po, jnp.concatenate([ie, jnp.where(lane < 64, ie, io), io], axis=1)


def _pv(groups, hooks=None):
    nb = len(groups) // 16
    accs = {}
    for n, g in enumerate(16 * blk + i for i in range(16) for blk in range(nb)):
        if hooks and n in hooks:
            hooks[n]()
        vload, p = groups[g]
        accs[g] = _fold(vload() * p, jnp.add)
    return jnp.concatenate([accs[g] for g in range(len(groups))], axis=0)


def _lane_reduce_t(acc):
    at = acc.T
    s = at[0:8]
    for i in range(1, 16):
        s = s + at[8 * i:8 * i + 8]
    return s


def _kernel(x_hbm, kt_hbm, vt_hbm, wq_hbm, wo_hbm, wr_hbm, wg_hbm, wu_hbm, wd_hbm,
            o_ref,
            kv, vf, kp, wq_raw, wo_raw, wg_raw, wu_raw, wd_raw, wxp, wop, wdp, wguf, wqf, wdf, wof, cs,
            xb_ref, wrb, state, spin_ref, c_s, c_p, c_o, c_out,
            sems, wsem, *, cfg):
    LA, LEAD, NV, ND = cfg["LA"], cfg["LEAD"], cfg["NV"], cfg["ND"]
    NM = NH - NV
    order = _order(cfg)

    def piece(i, s):
        q, pair, w, b = i & (TPC - 1), (i >> 2) & (NP - 1), (i >> 6) & 1, i >> 7
        r0 = (q + s * TPC) * 8
        if not isinstance(i, int):
            r0 = pl.multiple_of(r0, 8)
        return pair, w, b, w * (1 + (b & 1)), i & (RING - 1), r0

    def start_piece(i, s, hf=None):
        pair, w, b, plane, ring, r0 = piece(i, s)
        osl = pl.ds(pair * RO, RO) if hf is None else pl.ds(pair * RO + hf * (RO // 2), RO // 2)

        def go(ww):
            src = vt_hbm if ww else kt_hbm
            pltpu.make_async_copy(src.at[b, osl, pl.ds(r0, 8), pl.ds(SK - W, W)],
                                  kv.at[plane, osl, pl.ds(r0, 8), :],
                                  sems.at[s, ring]).start(priority=1 - s)

        if isinstance(i, int):
            go(w)
        else:
            for ww in range(2):
                pl.when(jnp.logical_and(w == ww, i < NTICK))(functools.partial(go, ww))

    def wait_piece(i, s):
        pair, w, b, plane, ring, r0 = piece(i, s)
        view = kv.at[plane, pl.ds(pair * RO, RO), pl.ds(r0, 8), :]
        pltpu.make_async_copy(view, view, sems.at[s, ring]).wait()

    def wait_tick(i):
        wait_piece(i, 0)
        wait_piece(i, 1)

    def spin(n):
        v = spin_ref[...]
        lane = lax.broadcasted_iota(I32, v.shape, 1).astype(F32)
        for _ in range(n[0]):
            v = jnp.max(v, axis=1, keepdims=True) * 0.5 + lane
        for _ in range(n[1] // 2):
            v = v * 0.5
            v = v + lane
        spin_ref[...] = v

    def full_tick(i):
        wait_tick(i)
        start_piece(i + LEAD + 1, 1)
        start_piece(i + LA, 0)

    def spin_tick(i, c):
        full_tick(i)
        spin(cfg["SPIN"])
        return c

    def half_tick(h, lead, la, work, sp, top):
        i = h >> 1
        pl.when((h & 1) == 0)(lambda: wait_tick(i))
        if top:
            start_piece(i + lead, 1, h & 1)
        work()
        spin(sp)
        if not top:
            start_piece(i + lead, 1, h & 1)
        start_piece(jnp.where((h & 1) == 1, i + la, NTICK), 0)

    def idle_half(h, c):
        def work():
            n = (((h >> 3) & (NP - 1)) - 4) * 4 + (h & 7) - 2
            o0 = jnp.minimum(n * 2, VF * RO - 2)
            vf[pl.ds(o0, 2)] = kv[1 + ((h >> 8) & 1), pl.ds(o0, 2)].astype(F32)

        half_tick(h, LEAD, LA - 1, work, cfg["HSPIN"], False)
        return c

    def advance(t, need):
        t2 = jnp.maximum(t + 2, need)
        wait_tick(t)
        lax.fori_loop(2 * t + 2, 2 * t2 - 2, idle_half, 0)
        wait_tick(t2 - 1)
        start_piece(t2 - 1 + LEAD, 1, 0)
        return t2

    def mid(t2, n, after=None):
        if n == 0:
            start_piece(t2 - 1 + LEAD, 1, 1)
        if n == 1:
            start_piece(t2 + LEAD, 1, 0)
            start_piece(t2 - 2 + LA, 0)
            start_piece(t2 - 1 + LA, 0)
        if n == 2:
            kv[0, NP * RO, 0:16, 0:128] = jnp.concatenate([after, after], axis=0).astype(BF16)
            start_piece(t2 + LEAD, 1, 1)

    half = D // 2
    small = [pltpu.make_async_copy(x_hbm, xb_ref, wsem.at[0]),
             pltpu.make_async_copy(wr_hbm, wrb, wsem.at[1])]
    big = [pltpu.make_async_copy(wq_hbm, wq_raw, wsem.at[2]),
           pltpu.make_async_copy(wg_hbm, wg_raw, wsem.at[3]),
           pltpu.make_async_copy(wu_hbm.at[pl.ds(0, half)], wu_raw.at[pl.ds(0, half)], wsem.at[4])]
    for cp in big:
        cp.start(priority=1)
    for cp in small:
        cp.start()
    spin_ref[...] = jnp.zeros(spin_ref.shape, F32)

    inject = [(wo_hbm, wo_raw, 0, 48, HD // 48, 5), (wd_hbm, wd_raw, 0, 48, F // 48, 6),
              (wu_hbm, wu_raw, half, 16, half // 16, 7)]
    for src, dst, row0, rows, n, sem in inject:
        def body(i, c, src=src, dst=dst, row0=row0, rows=rows, sem=sem):
            r = pl.multiple_of(row0 + i * rows, 8)
            pltpu.make_async_copy(src.at[pl.ds(r, rows)], dst.at[pl.ds(r, rows)], wsem.at[sem]).start()
            spin(cfg["WSPIN"])
            return c
        lax.fori_loop(0, n, body, 0)
        if dst is wo_raw:
            for i in range(LA):
                start_piece(i, 0)

    def lead_in(h, c):
        start_piece(h >> 1, 1, h & 1)
        spin(cfg["LSPIN"])
        return c

    lax.fori_loop(0, 2 * (LEAD + 1), lead_in, 0)
    for cp in small:
        cp.wait()
    state[...] = jnp.concatenate([xb_ref[...].astype(F32), jnp.zeros((8 - B, D), F32)], axis=0)
    for src, dst, row0, rows, n, sem in inject:
        view = dst.at[pl.ds(row0, rows * n)]
        pltpu.make_async_copy(view, view, wsem.at[sem]).wait()
    for cp in big:
        cp.wait()

    NRP = D // 16

    def repack(h, c):
        full_tick(h)
        r = pl.multiple_of(h * 16, 16)
        r2 = pl.multiple_of(h * 8, 8)
        wxp[pl.ds(r2, 8), 0:HD] = _u32(wq_raw[pl.ds(r, 16), :])
        for n, pos in enumerate(cfg["VQ"]):
            wqf[pl.ds(r, 16), n * PD:(n + 1) * PD] = (
                wq_raw[pl.ds(r, 16), order[pos] * PD:(order[pos] + 1) * PD].astype(F32))
        g = wg_raw[pl.ds(r, 16), :]
        u = wu_raw[pl.ds(r, 16), :]
        gu = jnp.concatenate([w[:, i * 128:(i + 1) * 128] for i in range(NH) for w in (g, u)], axis=1)
        wxp[pl.ds(r2, 8), HD:HD + 2 * F] = _u32(gu)
        wguf[pl.ds(r, 16), :] = gu[:, NM * 256:].astype(F32)
        for n, pos in enumerate(cfg["VO"]):
            ro = pl.multiple_of(jnp.minimum(r, PD - 16), 16)
            wof[pl.ds(n * PD + ro, 16), :] = wo_raw[pl.ds(order[pos] * PD + ro, 16), :].astype(F32)
        nd = 16 if ND * 128 <= D else 32
        rd = pl.multiple_of(jnp.minimum(h * nd, ND * 128 - nd), 16)
        wdf[pl.ds(rd, nd), :] = wd_raw[pl.ds(rd, nd), :].astype(F32)
        for src, packed, n in ((wo_raw, wop, 160), (wd_raw, wdp, 48)):
            r = pl.multiple_of(jnp.minimum(h * n, src.shape[0] - n), 16)
            packed[pl.ds(pl.multiple_of(r >> 1, 8), n // 2), :] = _u32(src[pl.ds(r, n), :])
        return c

    lax.fori_loop(0, NRP, repack, 0)

    NCS = (HD + 2 * F) // 768

    def colsum(i, c):
        full_tick(NRP + i)
        c0 = pl.multiple_of(i * 768, 128)
        cs[:, pl.ds(c0, 768)] = _dot(jnp.ones((8, D), BF16), _bf(wxp[:, pl.ds(c0, 768)]))
        return c

    lax.fori_loop(0, NCS, colsum, 0)
    t0 = jnp.int32(NRP + NCS)

    never = spin_ref[...] < -1.0

    def xproj(xb, m, scale, c0, n):
        y = _dot(xb, _bf(wxp[:, pl.ds(c0, n)])) - m * cs[:, pl.ds(c0, n)]
        return y if scale is None else y * scale

    def qproj(xb, m, qscale, k):
        return xproj(xb, m, qscale, k * PD if isinstance(k, int) else pl.multiple_of(k * PD, 128), PD)

    def oproj(ob, k):
        r0 = pl.multiple_of(k * DH, DH) if not isinstance(k, int) else k * DH
        return _dot(ob, _bf(wop[pl.ds(r0, DH), :]))

    def kload(k):
        return [_bf(kp[pl.ds(k * RO + 2 * i, 2)].reshape(64, W)) for i in range(3)]

    def vgroup(slot, k, o, r):
        return lambda: kv[1 + slot, k * RO + o, pl.ds(r * 8, 8), :].astype(F32)

    def pair_groups(slot, k, pe, po):
        return [(vgroup(slot, k, g // RI, g % RI), pe if g < DH // 8 else po) for g in range(PD // 8)]

    def vpu_matvec(xr, w_ref, nadd, per_step=1, tok=None):
        nu = xr.shape[1] // 128
        xcol = [jnp.concatenate([xr[:, u * 128:(u + 1) * 128]] * 16, axis=0).T for u in range(nu)]
        seq = [(u, i) for u0 in range(0, nu, 2) for i in range(16) for u in range(u0, min(u0 + 2, nu))]
        accs = [None] * per_step
        for n in range(0, len(seq), per_step):
            if tok is not None:
                for _ in range(nadd):
                    tok = tok + 1.0
            for a, (u, i) in enumerate(seq[n:n + per_step]):
                col = xcol[u][i * 8:i * 8 + 8]
                if tok is not None:
                    col = jnp.where(never, tok, col)
                y = w_ref[u * 128 + i * 8:u * 128 + i * 8 + 8, :] * _tile(col, w_ref.shape[1] // 128)
                accs[a] = y if accs[a] is None else accs[a] + y
            tok = accs[0][:, 0:128]
        return functools.reduce(jnp.add, accs), tok

    def act(gu):
        g = gu[:, 0:128]
        return (g * _sigmoid(g) * gu[:, 128:256]).astype(BF16)

    def ffn_res(x, xc, rstd):
        wr = wrb[...].astype(F32)
        wr = jnp.concatenate([jnp.broadcast_to(wr[t:t + 1, :], (8, 128)) for t in range(D // 128)], axis=1)
        return x + xc * rstd, _round(_sigmoid(_round(jnp.sum(xc * wr, axis=1, keepdims=True) * rstd)))

    def ffn(x):
        xb, xr, m, xc, rstd = _ln_parts(x)

        hs = [act(xproj(xb, m, rstd, HD + i * 256, 256)) for i in range(NM)]
        gu, tok = vpu_matvec(xr, wguf, cfg["TOK"])
        gu = (_rowsum_all(gu) - m * cs[:, HD + NM * 256:]) * rstd
        hs += [act(gu[:, i * 256:(i + 1) * 256]) for i in range(NV)]
        y = None
        late = list(range(NM - cfg["DLATE"], NM))
        for i in [i for i in range(ND, NH) if i not in late] + late:
            yi = _dot(hs[i], _bf(wdp[i * 64:(i + 1) * 64, :]))
            y = yi if y is None else y + yi
        yv, _ = vpu_matvec(jnp.concatenate(hs[:ND], axis=1).astype(F32), wdf, cfg["DTOK"], 2, tok)
        y = y + _rowsum_all(yv)
        res, gate = ffn_res(xr, xc, rstd)
        return res + y * gate

    NFT = NH // 2 + 1

    def ffn_ticked(x, t):
        def body(i, carry):
            h, y, _ = carry
            full_tick(t + i)
            xb, xr, m, xc, rstd = _ln_parts(x)
            c0 = pl.multiple_of(HD + jnp.minimum(i, NFT - 2) * 512, 128)
            gu = xproj(xb, m, rstd, c0, 512)
            r0 = pl.multiple_of(jnp.maximum(i - 1, 0) * 128, 128)
            y = y + _dot(h, _bf(wdp[pl.ds(r0, 128), :]))
            res, gate = ffn_res(xr, xc, rstd)
            return jnp.concatenate([act(gu[:, 0:256]), act(gu[:, 256:512])], axis=1), y, res + y * gate

        return lax.fori_loop(0, NFT, body, (jnp.zeros((8, 256), BF16), jnp.zeros((8, D), F32), x))[2]

    NHP = 2 * B - 1

    def half_period(hp, t):
        b = hp >> 1
        slot = b & 1
        first = (hp & 1) == 0
        vbase = jnp.where(first, b * TPP + (NP + 1) * TPC, -TPP)

        tr = jnp.where(first, jnp.maximum(t, b * TPP + cfg["KRP"]), t)
        lax.fori_loop(t, tr, spin_tick, 0)

        def k_repack(h, c):
            def work():
                o0 = (h - 2 * tr) * 4
                kp[pl.ds(o0, 4)] = _u32(kv[0, pl.ds(o0, 4)].reshape(4 * 64, W)).reshape(4, 32, W)

            half_tick(h, LEAD + 1, LA, work, cfg["KSPIN"], True)
            return c

        t = jnp.where(first, tr + NP * RO // 8, t)
        lax.fori_loop(2 * tr, 2 * t, k_repack, 0)

        xb, x, m, _, rstd = _ln_parts(jnp.broadcast_to(state[pl.ds(b, 1), :], (8, D)))
        qscale = rstd * SCALE

        def step(j, carry):
            t, q, se, so, pe, po, inv, o, out = carry
            kv_ = jnp.maximum(j - 3, 0)
            t = advance(t, vbase + kv_ * TPC)
            se_n, so_n = _scores(q, kload(jnp.clip(j - 1, 0, NP - 1)))
            q_n = qproj(xb, m, qscale, jnp.minimum(j, NP - 1))
            out = out + oproj(o, jnp.maximum(j - 4, 0))
            pe_n, po_n, inv_n = _softmax_pair(se, so)
            acc = _pv(pair_groups(slot, kv_, pe, po),
                      {cfg["PVMID"][0]: lambda: mid(t, 0), cfg["PVMID"][1]: lambda: mid(t, 1)})
            mid(t, 2, q_n[:, 256:384])
            o_n = jnp.where(j >= 3, _lane_reduce_t(acc) * inv, 0.0).astype(BF16)
            return t, q_n, se_n, so_n, pe_n, po_n, inv_n, o_n, out

        zw = (lax.broadcasted_iota(I32, (8, W), 0) + lax.broadcasted_iota(I32, (8, W), 1)).astype(F32) * (1.0 / W)
        zp = zw[:, :PD]
        init = (t, zp, zw, zw, zw, zw, zp, jnp.zeros((8, PD), BF16), jnp.zeros((8, D), F32))
        last = hp == NHP - 1
        t, q, se, so, pe, po, inv, o, out = lax.fori_loop(0, jnp.where(last, NP, NP + 2), step, init)
        t2 = jnp.maximum(t + 2, vbase + (NP - 1) * TPC)

        @pl.when(last)
        def _():
            c_s[0] = se
            c_s[1] = so
            c_p[0] = pe
            c_p[1] = po
            c_o[0] = q
            c_o[1] = inv
            c_o[2] = o.astype(F32)
            c_out[...] = out

        @pl.when(jnp.logical_not(last))
        def _():
            advance(t, t2)
            y = out + oproj(o, NP - 2)
            acc = _pv(pair_groups(slot, NP - 1, pe, po), {24: lambda: mid(t2, 0), 45: lambda: mid(t2, 1)})
            olast = _lane_reduce_t(acc) * inv
            mid(t2, 2, olast[:, 0:128])
            olast = olast.astype(BF16)
            full_tick(t2)
            y = y + oproj(olast, NP - 1)
            state[pl.ds(b, 1), :] = ffn_ticked(x + _rowsum_all(y), t2 + 1)[0:1]

        return t2 + 1 + NFT

    lax.fori_loop(0, NHP, half_period, t0)

    slot = (B - 1) % 2
    ka, kb = NP - 2, NP - 1

    def wo_rows(runs):
        return _bf(jnp.concatenate(
            [wop[(k * PD + o * 64 + r * 8) // 2:(k * PD + o * 64 + (r + n) * 8) // 2, :] for k, o, r, n in runs],
            axis=0))

    def run_groups(runs, ps):
        return [(vgroup(slot, k, o, r + i), ps[k][0 if o < RO // 2 else 1]) for k, o, r, n in runs for i in range(n)]

    def normalised(pe, po, inv):
        return pe * _tile(inv[:, 0:128], NL), po * _tile(inv[:, 256:384], NL)

    def pv_o_vpu(runs):
        w = wo_rows(runs).astype(F32)
        return functools.reduce(jnp.add, [
            w[i * 8:(i + 1) * 8] * jnp.sum(_fold(vload() * p, jnp.add), axis=1, keepdims=True)
            for i, (vload, p) in enumerate(run_groups(runs, ps))])

    kc = NP - 3
    for i in range(NTICK - 3 * TPC, NTICK - TPC):
        wait_piece(i, 1)
    se, so = _scores(c_o[0], kload(kb))
    out = c_out[...] + oproj(c_o[2].astype(BF16), NP - 4)
    ps = {kc: normalised(c_p[0], c_p[1], c_o[1]), ka: normalised(*_softmax_pair(c_s[0], c_s[1]))}
    runs = [(k, o, TPC, TPC) for k in (kc, ka) for o in range(RO)]
    o = _lane_reduce_t(_pv(run_groups(runs, ps))).astype(BF16)
    ps[kb] = normalised(*_softmax_pair(se, so))

    for i in range(NTICK - 3 * TPC, NTICK - 2 * TPC):
        wait_piece(i, 0)
    for i in range(NTICK - TPC, NTICK):
        wait_piece(i, 1)
    out = out + _dot(o, wo_rows(runs))
    runs0 = [(kc, o, 0, TPC) for o in range(RO)] + [(kb, o, TPC, TPC) for o in range(RO)]
    o0 = _lane_reduce_t(_pv(run_groups(runs0, ps))).astype(BF16)

    for i in range(NTICK - 2 * TPC, NTICK - TPC):
        wait_piece(i, 0)
    out = out + _dot(o0, wo_rows(runs0))
    runs1 = [(ka, o, 0, TPC) for o in range(RO)]
    acc = [_fold(vload() * p, jnp.add) for vload, p in run_groups(runs1, ps)]
    zero = [jnp.zeros((8, 128), F32)] * 4
    o1 = _lane_reduce_t(jnp.concatenate(acc[:12] + zero + acc[12:] + zero, axis=0)).astype(BF16)

    for i in range(NTICK - TPC, NTICK - 2):
        wait_piece(i, 0)
    out = out + _dot(o1, wo_rows(runs1[:3] + runs1[:1] + runs1[3:] + runs1[:1]))
    out = out + pv_o_vpu([(kb, o, 0, 2) for o in range(RO)])

    for i in range(NTICK - 2, NTICK):
        wait_piece(i, 0)
    out = out + pv_o_vpu([(kb, o, 2, 2) for o in range(RO)])
    x = jnp.broadcast_to(state[B - 1:B, :], (8, D)) + _rowsum_all(out)

    def attn_fast(x):
        xb, xr, m, _, rstd = _ln_parts(x)
        qscale = rstd * SCALE
        q, sc, ps, os_, deadline, outv = {}, {}, {}, {}, {}, []
        invs = {}

        def get_o(pos):
            o = os_.pop(pos) * invs.pop(pos)
            return (_rowsum_all(o) if pos in cfg["VO"] else o).astype(BF16)

        out = None
        oslot = {}
        sl = cfg["OLAG"]
        for i in range(NP):
            while sl in cfg["OSKIP"]:
                sl += 1
            if i not in cfg["VO"]:
                oslot[sl] = i
            sl += 1
        qv = _rowsum_all(vpu_matvec(xr, wqf, cfg["QTOK"])[0])
        for n, pos in enumerate(cfg["VQ"]):
            k = order[pos]
            q[pos] = (qv[:, n * PD:(n + 1) * PD] - m * cs[:, k * PD:(k + 1) * PD]) * qscale
        qm = [pos for pos in range(NP) if pos not in cfg["VQ"]]
        for s in range(-3, sl):
            if 0 <= s + 3 < len(qm):
                q[qm[s + 3]] = qproj(xb, m, qscale if qm[s + 3] >= cfg["NLS"] else None, order[qm[s + 3]])
            if 0 <= s + 2 < NP:
                qq = q.pop(s + 2)
                if s in deadline:
                    qq = jnp.concatenate([jnp.where(never, deadline.pop(s), qq[:, 0:128]), qq[:, 128:]], axis=1)
                sc[s + 2] = _scores(qq, kload(order[s + 2]))
            if s in oslot:
                y = oproj(get_o(oslot[s]), order[oslot[s]])
                out = y if out is None else out + y
            if 0 <= s + 1 < NP:
                ps[s + 1] = _softmax_pair(*sc.pop(s + 1), None if s + 1 >= cfg["NLS"] else qscale, bcast=True)
            if 0 <= s < NP:
                pe, po, invs[s] = ps.pop(s)
                k = order[s]
                groups = pair_groups(slot, k, pe, po)
                if k < VF:
                    groups = [(functools.partial(lambda g: vf[k * RO + g // RI, pl.ds((g % RI) * 8, 8), :], g), p)
                              for g, (_, p) in enumerate(groups)]
                acc = _pv(groups)
                os_[s] = _lane_reduce_t(acc)
                for n, (tpos, tg, nadd, per, dl) in enumerate(cfg["VOT"]):
                    if tpos == s:
                        y, tok = vpu_matvec(get_o(cfg["VO"][n]).astype(F32), wof.at[n * PD:(n + 1) * PD], nadd, per,
                                            acc[tg * 8:tg * 8 + 8])
                        outv.append(y)
                        if dl:
                            deadline[s + dl] = tok
        out = functools.reduce(jnp.add, [out] + outv)
        return xr + _rowsum_all(out)

    x = ffn(attn_fast(ffn(x)))
    row = lax.broadcasted_iota(I32, (8, D), 0)
    o_ref[...] = jnp.where(row == B - 1, x, state[...])[0:B].astype(o_ref.dtype)


def _call(cfg, A_x, A_k_cache, A_v_cache, A_wq, A_wo, B_w_r, B_w_gate, B_w_up, B_w_down):
    kt = jnp.swapaxes(A_k_cache, 2, 3).reshape(B, NP * RO, RI * 8, SK)
    vt = jnp.swapaxes(A_v_cache, 2, 3).reshape(B, NP * RO, RI * 8, SK)
    out = pl.pallas_call(
        functools.partial(_kernel, cfg=cfg),
        out_shape=jax.ShapeDtypeStruct((B, D), BF16),
        in_specs=[pl.BlockSpec(memory_space=pl.ANY)] * 9,
        out_specs=pl.BlockSpec(memory_space=pltpu.VMEM),
        scratch_shapes=[
            pltpu.VMEM((3, NP * RO + 1, RI * 8, W), BF16),
            pltpu.VMEM((VF * RO, RI * 8, W), F32),
            pltpu.VMEM((NP * RO, RI * 4, W), U32),
            pltpu.VMEM((D, HD), BF16),
            pltpu.VMEM((HD, D), BF16),
            pltpu.VMEM((D, F), BF16),
            pltpu.VMEM((D, F), BF16),
            pltpu.VMEM((F, D), BF16),
            pltpu.VMEM((D // 2, HD + 2 * F), U32),
            pltpu.VMEM((HD // 2, D), U32),
            pltpu.VMEM((F // 2, D), U32),
            pltpu.VMEM((D, cfg["NV"] * 256), F32),
            pltpu.VMEM((D, len(cfg["VQ"]) * PD), F32),
            pltpu.VMEM((cfg["ND"] * 128, D), F32),
            pltpu.VMEM((len(cfg["VO"]) * PD, D), F32),
            pltpu.VMEM((8, HD + 2 * F), F32),
            pltpu.VMEM((B, D), BF16),
            pltpu.VMEM((D // 128, 128), BF16),
            pltpu.VMEM((8, D), F32),
            pltpu.VMEM((8, 128), F32),
            pltpu.VMEM((2, 8, W), F32),
            pltpu.VMEM((2, 8, W), F32),
            pltpu.VMEM((3, 8, PD), F32),
            pltpu.VMEM((8, D), F32),
            pltpu.SemaphoreType.DMA((2, RING)),
            pltpu.SemaphoreType.DMA((8,)),
        ],
        compiler_params=pltpu.CompilerParams(vmem_limit_bytes=126 * 1024 * 1024,
                                             disable_bounds_checks=True,
                                             disable_semaphore_checks=True),
        name="fused_decode",
    )(A_x.reshape(B, D), kt, vt, A_wq, A_wo, B_w_r.reshape(D // 128, 128), B_w_gate, B_w_up, B_w_down)
    return out.reshape(B, 1, D)


@jax.jit
def pallas_interleave_layers__sliding_block_cached__moe_arch_mod__decode_kernel(
    A_x: jax.Array,
    A_k_cache: jax.Array,
    A_v_cache: jax.Array,
    A_wq: jax.Array,
    A_wo: jax.Array,
    B_x: jax.Array,
    B_w_r: jax.Array,
    B_w_gate: jax.Array,
    B_w_up: jax.Array,
    B_w_down: jax.Array,
):
    del B_x
    return _call(CFG, A_x, A_k_cache, A_v_cache, A_wq, A_wo, B_w_r, B_w_gate, B_w_up, B_w_down)
```

```python
import functools

import jax
import jax.numpy as jnp
from jax import lax
import jax.experimental.pallas as pl
import jax.experimental.pallas.tpu as pltpu

F32 = jnp.float32
BF16 = jnp.bfloat16
U32 = jnp.uint32
I32 = jnp.int32

B, D, H, DH, SK, F = 4, 640, 32, 192, 4096, 1536
W = min(4096, max(256, SK // 4))
NP = H // 2
PD = 2 * DH
HD = H * DH
NL = W // 128
NH = F // 128
EPS = 1e-5
SCALE = DH ** -0.5 * 1.4426950408889634

RI = 8
RO = PD // (8 * RI)
TPC = RI // 2
TPP = 2 * NP * TPC
NTICK = B * TPP
RING = 32
VF = 12

CFG = dict(
    LA=23,
    LEAD=11,
    KRP=54,
    PVMID=(21, 45),
    SPIN=(1, 50),
    WSPIN=(1, 45),
    LSPIN=(1, 20),
    KSPIN=(1, 20),
    HSPIN=(1, 8),
    NV=4,
    ND=4,
    DLATE=(2, 2),
    TOK=(0, 0),
    DTOK=(1, 1),
    QTOK=0,
    RAWPOS=(2, 7, 10, 14),
    PROG="qqsqs.s.qqs.qqs.s.qs.qqos.s.qs.qsqo.so.so.so.so.s...ooooooo",
    NLS=1,
    VQ=(3, 4, 5),
    VO=(2, 0, 8),
    VOT=((15, 0, 0, 3, 0), (4, 16, 0, 2, 0), (11, 32, 0, 3, 2)),
)


def _order(cfg):
    order = list(range(VF))
    for pos, k in zip(sorted(cfg["RAWPOS"]), range(VF, NP)):
        order.insert(pos, k)
    return order


def _rowsum_all(x):
    x = x + pltpu.roll(x, 4, 0)
    x = x + pltpu.roll(x, 2, 0)
    return x + pltpu.roll(x, 1, 0)


def _bf(x):
    return pltpu.bitcast(x, BF16)


def _u32(x):
    return pltpu.bitcast(x, U32)


def _dot(a, b):
    return jnp.dot(a, b, preferred_element_type=F32)


def _sigmoid(x):
    return pl.reciprocal(1.0 + jnp.exp(-x), approx=True)


def _round(x):
    return x.astype(BF16).astype(F32)


def _ln_parts(x):
    xb = x.astype(BF16)
    xr = xb.astype(F32)
    m = jnp.sum(xr, axis=1, keepdims=True) * (1.0 / D)
    xc = xr - m
    v = jnp.sum(xc * xc, axis=1, keepdims=True) * (1.0 / D)
    m = _round(m)
    v = _round(_round(v) + EPS)
    return xb, xr, m, xr - m, pl.reciprocal(_round(v * lax.rsqrt(v)), approx=True)


def _scores(q, kk):
    lane = lax.broadcasted_iota(I32, (8, 128), 1)
    q0 = q[:, 0:128].astype(BF16)
    qm = q[:, 128:256]
    q2 = q[:, 256:384].astype(BF16)
    mid = jnp.concatenate([jnp.where(lane < 64, qm, 0.0), jnp.where(lane >= 64, qm, 0.0)],
                          axis=0).astype(BF16)
    r0 = _dot(q0, kk[0])
    rm = _dot(mid, kk[1])
    r2 = _dot(q2, kk[2])
    return r0 + rm[0:8], rm[8:16] + r2


def _fold(x, op):
    r = x[:, 0:128]
    for t in range(1, x.shape[1] // 128):
        r = op(r, x[:, t * 128:(t + 1) * 128])
    return r


def _tile(x, n):
    return jnp.concatenate([x] * n, axis=1)


def _softmax_pair(se, so, c=None, bcast=False):
    row = lax.broadcasted_iota(I32, (8, 128), 0)
    top = row < 4

    def split(c):
        c = jnp.broadcast_to(c, (8, 128))
        r = pltpu.roll(c, 4, 0)
        return jnp.where(top, c, r), jnp.where(top, r, c)

    m = jnp.max(jnp.where(top, _fold(se, jnp.maximum), _fold(so, jnp.maximum)), axis=1, keepdims=True)
    me, mo = split(m)
    de, do = se - _tile(me, NL), so - _tile(mo, NL)
    if c is not None:
        de, do = de * c, do * c
    pe, po = jnp.exp2(de), jnp.exp2(do)
    le, lo = _fold(pe, jnp.add), _fold(po, jnp.add)
    if bcast:
        l = jnp.sum(jnp.where(row >= 1, lo, le), axis=1, keepdims=True)
        r = jnp.broadcast_to(pl.reciprocal(l, approx=True), (8, 128))
        ie, io = [jnp.broadcast_to(r[i:i + 1], (8, 128)) for i in range(2)]
    else:
        ie, io = split(pl.reciprocal(jnp.sum(jnp.where(top, le, lo), axis=1, keepdims=True), approx=True))
    lane = lax.broadcasted_iota(I32, (8, 128), 1)
    return pe, po, jnp.concatenate([ie, jnp.where(lane < 64, ie, io), io], axis=1)


def _pv(groups, hooks=None):
    nb = len(groups) // 16
    accs = {}
    for n, g in enumerate(16 * blk + i for i in range(16) for blk in range(nb)):
        if hooks and n in hooks:
            hooks[n]()
        vload, p = groups[g]
        accs[g] = _fold(vload() * p, jnp.add)
    return jnp.concatenate([accs[g] for g in range(len(groups))], axis=0)


def _lane_reduce_t(acc):
    at = acc.T
    s = at[0:8]
    for i in range(1, 16):
        s = s + at[8 * i:8 * i + 8]
    return s


def _kernel(x_hbm, kt_hbm, vt_hbm, wq_hbm, wo_hbm, wr_hbm, wg_hbm, wu_hbm, wd_hbm,
            o_ref,
            kv, vf, kp, wq_raw, wo_raw, wg_raw, wu_raw, wd_raw, wxp, wop, wdp, wguf, wqf, wdf, wof, cs,
            xb_ref, wrb, state, spin_ref, c_s, c_p, c_o, c_out,
            sems, wsem, *, cfg):
    LA, LEAD, NV, ND = cfg["LA"], cfg["LEAD"], cfg["NV"], cfg["ND"]
    NM = NH - NV
    order = _order(cfg)

    def piece(i, s):
        q, pair, w, b = i & (TPC - 1), (i >> 2) & (NP - 1), (i >> 6) & 1, i >> 7
        r0 = (q + s * TPC) * 8
        if not isinstance(i, int):
            r0 = pl.multiple_of(r0, 8)
        return pair, w, b, w * (1 + (b & 1)), i & (RING - 1), r0

    def start_piece(i, s, hf=None):
        pair, w, b, plane, ring, r0 = piece(i, s)
        osl = pl.ds(pair * RO, RO) if hf is None else pl.ds(pair * RO + hf * (RO // 2), RO // 2)

        def go(ww):
            src = vt_hbm if ww else kt_hbm
            pltpu.make_async_copy(src.at[b, osl, pl.ds(r0, 8), pl.ds(SK - W, W)],
                                  kv.at[plane, osl, pl.ds(r0, 8), :],
                                  sems.at[s, ring]).start(priority=1 - s)

        if isinstance(i, int):
            go(w)
        else:
            for ww in range(2):
                pl.when(jnp.logical_and(w == ww, i < NTICK))(functools.partial(go, ww))

    def wait_piece(i, s):
        pair, w, b, plane, ring, r0 = piece(i, s)
        view = kv.at[plane, pl.ds(pair * RO, RO), pl.ds(r0, 8), :]
        pltpu.make_async_copy(view, view, sems.at[s, ring]).wait()

    def wait_tick(i):
        wait_piece(i, 0)
        wait_piece(i, 1)

    def spin(n):
        v = spin_ref[...]
        lane = lax.broadcasted_iota(I32, v.shape, 1).astype(F32)
        for _ in range(n[0]):
            v = jnp.max(v, axis=1, keepdims=True) * 0.5 + lane
        for _ in range(n[1] // 2):
            v = v * 0.5
            v = v + lane
        spin_ref[...] = v

    def full_tick(i):
        wait_tick(i)
        start_piece(i + LEAD + 1, 1)
        start_piece(i + LA, 0)

    def spin_tick(i, c):
        full_tick(i)
        spin(cfg["SPIN"])
        return c

    def half_tick(h, lead, la, work, sp, top):
        i = h >> 1
        pl.when((h & 1) == 0)(lambda: wait_tick(i))
        if top:
            start_piece(i + lead, 1, h & 1)
        work()
        spin(sp)
        if not top:
            start_piece(i + lead, 1, h & 1)
        start_piece(jnp.where((h & 1) == 1, i + la, NTICK), 0)

    def idle_half(h, c):
        def work():
            n = (((h >> 3) & (NP - 1)) - 4) * 4 + (h & 7) - 2
            o0 = jnp.minimum(n * 2, VF * RO - 2)
            vf[pl.ds(o0, 2)] = kv[1 + ((h >> 8) & 1), pl.ds(o0, 2)].astype(F32)

        half_tick(h, LEAD, LA - 1, work, cfg["HSPIN"], False)
        return c

    def advance(t, need):
        t2 = jnp.maximum(t + 2, need)
        wait_tick(t)
        lax.fori_loop(2 * t + 2, 2 * t2 - 2, idle_half, 0)
        wait_tick(t2 - 1)
        start_piece(t2 - 1 + LEAD, 1, 0)
        return t2

    def mid(t2, n, after=None):
        if n == 0:
            start_piece(t2 - 1 + LEAD, 1, 1)
        if n == 1:
            start_piece(t2 + LEAD, 1, 0)
            start_piece(t2 - 2 + LA, 0)
            start_piece(t2 - 1 + LA, 0)
        if n == 2:
            kv[0, NP * RO, 0:16, 0:128] = jnp.concatenate([after, after], axis=0).astype(BF16)
            start_piece(t2 + LEAD, 1, 1)

    half = D // 2
    small = [pltpu.make_async_copy(x_hbm, xb_ref, wsem.at[0]),
             pltpu.make_async_copy(wr_hbm, wrb, wsem.at[1])]
    big = [pltpu.make_async_copy(wq_hbm, wq_raw, wsem.at[2]),
           pltpu.make_async_copy(wg_hbm, wg_raw, wsem.at[3]),
           pltpu.make_async_copy(wu_hbm.at[pl.ds(0, half)], wu_raw.at[pl.ds(0, half)], wsem.at[4])]
    for cp in big:
        cp.start(priority=1)
    for cp in small:
        cp.start()
    spin_ref[...] = jnp.zeros(spin_ref.shape, F32)

    inject = [(wo_hbm, wo_raw, 0, 48, HD // 48, 5), (wd_hbm, wd_raw, 0, 48, F // 48, 6),
              (wu_hbm, wu_raw, half, 16, half // 16, 7)]
    for src, dst, row0, rows, n, sem in inject:
        def body(i, c, src=src, dst=dst, row0=row0, rows=rows, sem=sem):
            r = pl.multiple_of(row0 + i * rows, 8)
            pltpu.make_async_copy(src.at[pl.ds(r, rows)], dst.at[pl.ds(r, rows)], wsem.at[sem]).start()
            spin(cfg["WSPIN"])
            return c
        lax.fori_loop(0, n, body, 0)
        if dst is wo_raw:
            for i in range(LA):
                start_piece(i, 0)

    def lead_in(h, c):
        start_piece(h >> 1, 1, h & 1)
        spin(cfg["LSPIN"])
        return c

    lax.fori_loop(0, 2 * (LEAD + 1), lead_in, 0)
    for cp in small:
        cp.wait()
    state[...] = jnp.concatenate([xb_ref[...].astype(F32), jnp.zeros((8 - B, D), F32)], axis=0)
    for src, dst, row0, rows, n, sem in inject:
        view = dst.at[pl.ds(row0, rows * n)]
        pltpu.make_async_copy(view, view, wsem.at[sem]).wait()
    for cp in big:
        cp.wait()

    NRP = D // 16

    def repack(h, c):
        full_tick(h)
        r = pl.multiple_of(h * 16, 16)
        r2 = pl.multiple_of(h * 8, 8)
        wxp[pl.ds(r2, 8), 0:HD] = _u32(wq_raw[pl.ds(r, 16), :])
        for n, pos in enumerate(cfg["VQ"]):
            wqf[pl.ds(r, 16), n * PD:(n + 1) * PD] = (
                wq_raw[pl.ds(r, 16), order[pos] * PD:(order[pos] + 1) * PD].astype(F32))
        g = wg_raw[pl.ds(r, 16), :]
        u = wu_raw[pl.ds(r, 16), :]
        gu = jnp.concatenate([w[:, i * 128:(i + 1) * 128] for i in range(NH) for w in (g, u)], axis=1)
        wxp[pl.ds(r2, 8), HD:HD + 2 * F] = _u32(gu)
        wguf[pl.ds(r, 16), :] = gu[:, NM * 256:].astype(F32)
        for n, pos in enumerate(cfg["VO"]):
            ro = pl.multiple_of(jnp.minimum(r, PD - 16), 16)
            wof[pl.ds(n * PD + ro, 16), :] = wo_raw[pl.ds(order[pos] * PD + ro, 16), :].astype(F32)
        nd = 16 if ND * 128 <= D else 32
        rd = pl.multiple_of(jnp.minimum(h * nd, ND * 128 - nd), 16)
        wdf[pl.ds(rd, nd), :] = wd_raw[pl.ds(rd, nd), :].astype(F32)
        for src, packed, n in ((wo_raw, wop, 160), (wd_raw, wdp, 48)):
            r = pl.multiple_of(jnp.minimum(h * n, src.shape[0] - n), 16)
            packed[pl.ds(pl.multiple_of(r >> 1, 8), n // 2), :] = _u32(src[pl.ds(r, n), :])
        return c

    lax.fori_loop(0, NRP, repack, 0)

    NCS = (HD + 2 * F) // 768

    def colsum(i, c):
        full_tick(NRP + i)
        c0 = pl.multiple_of(i * 768, 128)
        cs[:, pl.ds(c0, 768)] = _dot(jnp.ones((8, D), BF16), _bf(wxp[:, pl.ds(c0, 768)]))
        return c

    lax.fori_loop(0, NCS, colsum, 0)
    t0 = jnp.int32(NRP + NCS)

    never = spin_ref[...] < -1.0

    def xproj(xb, m, scale, c0, n):
        y = _dot(xb, _bf(wxp[:, pl.ds(c0, n)])) - m * cs[:, pl.ds(c0, n)]
        return y if scale is None else y * scale

    def qproj(xb, m, qscale, k):
        return xproj(xb, m, qscale, k * PD if isinstance(k, int) else pl.multiple_of(k * PD, 128), PD)

    def oproj(ob, k):
        r0 = pl.multiple_of(k * DH, DH) if not isinstance(k, int) else k * DH
        return _dot(ob, _bf(wop[pl.ds(r0, DH), :]))

    def kload(k):
        return [_bf(kp[pl.ds(k * RO + 2 * i, 2)].reshape(64, W)) for i in range(3)]

    def vgroup(slot, k, o, r):
        return lambda: kv[1 + slot, k * RO + o, pl.ds(r * 8, 8), :].astype(F32)

    def pair_groups(slot, k, pe, po):
        return [(vgroup(slot, k, g // RI, g % RI), pe if g < DH // 8 else po) for g in range(PD // 8)]

    def vpu_matvec(xr, w_ref, nadd, per_step=1, tok=None):
        nu = xr.shape[1] // 128
        xcol = [jnp.concatenate([xr[:, u * 128:(u + 1) * 128]] * 16, axis=0).T for u in range(nu)]
        seq = [(u, i) for u0 in range(0, nu, 2) for i in range(16) for u in range(u0, min(u0 + 2, nu))]
        accs = [None] * per_step
        for n in range(0, len(seq), per_step):
            if tok is not None:
                for _ in range(nadd):
                    tok = tok + 1.0
            for a, (u, i) in enumerate(seq[n:n + per_step]):
                col = xcol[u][i * 8:i * 8 + 8]
                if tok is not None:
                    col = jnp.where(never, tok, col)
                y = w_ref[u * 128 + i * 8:u * 128 + i * 8 + 8, :] * _tile(col, w_ref.shape[1] // 128)
                accs[a] = y if accs[a] is None else accs[a] + y
            tok = accs[0][:, 0:128]
        return functools.reduce(jnp.add, accs), tok

    def act(gu):
        g = gu[:, 0:128]
        return (g * _sigmoid(g) * gu[:, 128:256]).astype(BF16)

    def ffn_res(x, xc, rstd):
        wr = wrb[...].astype(F32)
        wr = jnp.concatenate([jnp.broadcast_to(wr[t:t + 1, :], (8, 128)) for t in range(D // 128)], axis=1)
        return x + xc * rstd, _round(_sigmoid(_round(jnp.sum(xc * wr, axis=1, keepdims=True) * rstd)))

    def ffn(x, f):
        xb, xr, m, xc, rstd = _ln_parts(x)

        hs = [act(xproj(xb, m, rstd, HD + i * 256, 256)) for i in range(NM)]
        gu, tok = vpu_matvec(xr, wguf, cfg["TOK"][f])
        gu = (_rowsum_all(gu) - m * cs[:, HD + NM * 256:]) * rstd
        hs += [act(gu[:, i * 256:(i + 1) * 256]) for i in range(NV)]
        y = None
        late = list(range(NM - cfg["DLATE"][f], NM))
        for i in [i for i in range(ND, NH) if i not in late] + late:
            yi = _dot(hs[i], _bf(wdp[i * 64:(i + 1) * 64, :]))
            y = yi if y is None else y + yi
        yv, _ = vpu_matvec(jnp.concatenate(hs[:ND], axis=1).astype(F32), wdf, cfg["DTOK"][f], 2, tok)
        y = y + _rowsum_all(yv)
        res, gate = ffn_res(xr, xc, rstd)
        return res + y * gate

    NFT = NH // 2 + 1

    def ffn_ticked(x, t):
        def body(i, carry):
            h, y, _ = carry
            full_tick(t + i)
            xb, xr, m, xc, rstd = _ln_parts(x)
            c0 = pl.multiple_of(HD + jnp.minimum(i, NFT - 2) * 512, 128)
            gu = xproj(xb, m, rstd, c0, 512)
            r0 = pl.multiple_of(jnp.maximum(i - 1, 0) * 128, 128)
            y = y + _dot(h, _bf(wdp[pl.ds(r0, 128), :]))
            res, gate = ffn_res(xr, xc, rstd)
            return jnp.concatenate([act(gu[:, 0:256]), act(gu[:, 256:512])], axis=1), y, res + y * gate

        return lax.fori_loop(0, NFT, body, (jnp.zeros((8, 256), BF16), jnp.zeros((8, D), F32), x))[2]

    NHP = 2 * B - 1

    def half_period(hp, t):
        b = hp >> 1
        slot = b & 1
        first = (hp & 1) == 0
        vbase = jnp.where(first, b * TPP + (NP + 1) * TPC, -TPP)

        tr = jnp.where(first, jnp.maximum(t, b * TPP + cfg["KRP"]), t)
        lax.fori_loop(t, tr, spin_tick, 0)

        def k_repack(h, c):
            def work():
                o0 = (h - 2 * tr) * 4
                kp[pl.ds(o0, 4)] = _u32(kv[0, pl.ds(o0, 4)].reshape(4 * 64, W)).reshape(4, 32, W)

            half_tick(h, LEAD + 1, LA, work, cfg["KSPIN"], True)
            return c

        t = jnp.where(first, tr + NP * RO // 8, t)
        lax.fori_loop(2 * tr, 2 * t, k_repack, 0)

        xb, x, m, _, rstd = _ln_parts(jnp.broadcast_to(state[pl.ds(b, 1), :], (8, D)))
        qscale = rstd * SCALE

        def step(j, carry):
            t, q, se, so, pe, po, inv, o, out = carry
            kv_ = jnp.maximum(j - 3, 0)
            t = advance(t, vbase + kv_ * TPC)
            se_n, so_n = _scores(q, kload(jnp.clip(j - 1, 0, NP - 1)))
            q_n = qproj(xb, m, qscale, jnp.minimum(j, NP - 1))
            out = out + oproj(o, jnp.maximum(j - 4, 0))
            pe_n, po_n, inv_n = _softmax_pair(se, so)
            acc = _pv(pair_groups(slot, kv_, pe, po),
                      {cfg["PVMID"][0]: lambda: mid(t, 0), cfg["PVMID"][1]: lambda: mid(t, 1)})
            mid(t, 2, q_n[:, 256:384])
            o_n = jnp.where(j >= 3, _lane_reduce_t(acc) * inv, 0.0).astype(BF16)
            return t, q_n, se_n, so_n, pe_n, po_n, inv_n, o_n, out

        zw = (lax.broadcasted_iota(I32, (8, W), 0) + lax.broadcasted_iota(I32, (8, W), 1)).astype(F32) * (1.0 / W)
        zp = zw[:, :PD]
        init = (t, zp, zw, zw, zw, zw, zp, jnp.zeros((8, PD), BF16), jnp.zeros((8, D), F32))
        last = hp == NHP - 1
        t, q, se, so, pe, po, inv, o, out = lax.fori_loop(0, jnp.where(last, NP, NP + 2), step, init)
        t2 = jnp.maximum(t + 2, vbase + (NP - 1) * TPC)

        @pl.when(last)
        def _():
            c_s[0] = se
            c_s[1] = so
            c_p[0] = pe
            c_p[1] = po
            c_o[0] = q
            c_o[1] = inv
            c_o[2] = o.astype(F32)
            c_out[...] = out

        @pl.when(jnp.logical_not(last))
        def _():
            advance(t, t2)
            y = out + oproj(o, NP - 2)
            acc = _pv(pair_groups(slot, NP - 1, pe, po), {24: lambda: mid(t2, 0), 45: lambda: mid(t2, 1)})
            olast = _lane_reduce_t(acc) * inv
            mid(t2, 2, olast[:, 0:128])
            olast = olast.astype(BF16)
            full_tick(t2)
            y = y + oproj(olast, NP - 1)
            state[pl.ds(b, 1), :] = ffn_ticked(x + _rowsum_all(y), t2 + 1)[0:1]

        return t2 + 1 + NFT

    lax.fori_loop(0, NHP, half_period, t0)

    slot = (B - 1) % 2
    ka, kb = NP - 2, NP - 1

    def wo_rows(runs):
        return _bf(jnp.concatenate(
            [wop[(k * PD + o * 64 + r * 8) // 2:(k * PD + o * 64 + (r + n) * 8) // 2, :] for k, o, r, n in runs],
            axis=0))

    def run_groups(runs, ps):
        return [(vgroup(slot, k, o, r + i), ps[k][0 if o < RO // 2 else 1]) for k, o, r, n in runs for i in range(n)]

    def normalised(pe, po, inv):
        return pe * _tile(inv[:, 0:128], NL), po * _tile(inv[:, 256:384], NL)

    def pv_o_vpu(runs):
        w = wo_rows(runs).astype(F32)
        return functools.reduce(jnp.add, [
            w[i * 8:(i + 1) * 8] * jnp.sum(_fold(vload() * p, jnp.add), axis=1, keepdims=True)
            for i, (vload, p) in enumerate(run_groups(runs, ps))])

    kc = NP - 3
    for i in range(NTICK - 3 * TPC, NTICK - TPC):
        wait_piece(i, 1)
    se, so = _scores(c_o[0], kload(kb))
    out = c_out[...] + oproj(c_o[2].astype(BF16), NP - 4)
    ps = {kc: normalised(c_p[0], c_p[1], c_o[1]), ka: normalised(*_softmax_pair(c_s[0], c_s[1]))}
    runs = [(k, o, TPC, TPC) for k in (kc, ka) for o in range(RO)]
    o = _lane_reduce_t(_pv(run_groups(runs, ps))).astype(BF16)
    ps[kb] = normalised(*_softmax_pair(se, so))

    for i in range(NTICK - 3 * TPC, NTICK - 2 * TPC):
        wait_piece(i, 0)
    for i in range(NTICK - TPC, NTICK):
        wait_piece(i, 1)
    out = out + _dot(o, wo_rows(runs))
    runs0 = [(kc, o, 0, TPC) for o in range(RO)] + [(kb, o, TPC, TPC) for o in range(RO)]
    o0 = _lane_reduce_t(_pv(run_groups(runs0, ps))).astype(BF16)

    for i in range(NTICK - 2 * TPC, NTICK - TPC):
        wait_piece(i, 0)
    out = out + _dot(o0, wo_rows(runs0))
    runs1 = [(ka, o, 0, TPC) for o in range(RO)]
    acc = [_fold(vload() * p, jnp.add) for vload, p in run_groups(runs1, ps)]
    zero = [jnp.zeros((8, 128), F32)] * 4
    o1 = _lane_reduce_t(jnp.concatenate(acc[:12] + zero + acc[12:] + zero, axis=0)).astype(BF16)

    for i in range(NTICK - TPC, NTICK - 2):
        wait_piece(i, 0)
    out = out + _dot(o1, wo_rows(runs1[:3] + runs1[:1] + runs1[3:] + runs1[:1]))
    out = out + pv_o_vpu([(kb, o, 0, 2) for o in range(RO)])

    for i in range(NTICK - 2, NTICK):
        wait_piece(i, 0)
    out = out + pv_o_vpu([(kb, o, 2, 2) for o in range(RO)])
    x = jnp.broadcast_to(state[B - 1:B, :], (8, D)) + _rowsum_all(out)

    def attn_fast(x):
        xb, xr, m, _, rstd = _ln_parts(x)
        qscale = rstd * SCALE
        q, sc, ps, os_, deadline, outv = {}, {}, {}, {}, {}, []
        invs = {}

        def get_o(pos):
            o = os_.pop(pos) * invs.pop(pos)
            return (_rowsum_all(o) if pos in cfg["VO"] else o).astype(BF16)

        out = None
        qv = _rowsum_all(vpu_matvec(xr, wqf, cfg["QTOK"])[0])
        for n, pos in enumerate(cfg["VQ"]):
            k = order[pos]
            q[pos] = (qv[:, n * PD:(n + 1) * PD] - m * cs[:, k * PD:(k + 1) * PD]) * qscale
        qm = [pos for pos in range(NP) if pos not in cfg["VQ"]]
        om = [pos for pos in range(NP) if pos not in cfg["VO"]]

        def vpu_stage(s):
            if 0 <= s + 1 < NP:
                ps[s + 1] = _softmax_pair(*sc.pop(s + 1), None if s + 1 >= cfg["NLS"] else qscale, bcast=True)
            if 0 <= s < NP:
                pe, po, invs[s] = ps.pop(s)
                k = order[s]
                groups = pair_groups(slot, k, pe, po)
                if k < VF:
                    groups = [(functools.partial(lambda g: vf[k * RO + g // RI, pl.ds((g % RI) * 8, 8), :], g), p)
                              for g, (_, p) in enumerate(groups)]
                acc = _pv(groups)
                os_[s] = _lane_reduce_t(acc)
                for n, (tpos, tg, nadd, per, dl) in enumerate(cfg["VOT"]):
                    if tpos == s:
                        y, tok = vpu_matvec(get_o(cfg["VO"][n]).astype(F32), wof.at[n * PD:(n + 1) * PD], nadd, per,
                                            acc[tg * 8:tg * 8 + 8])
                        outv.append(y)
                        if dl:
                            deadline[s + dl + 2] = tok

        ns, nv = 0, -1
        for op in cfg["PROG"]:
            if op == "q":
                pos = qm.pop(0)
                q[pos] = qproj(xb, m, qscale if pos >= cfg["NLS"] else None, order[pos])
            elif op == "s":
                qq = q.pop(ns)
                if ns in deadline:
                    qq = jnp.concatenate([jnp.where(never, deadline.pop(ns), qq[:, 0:128]), qq[:, 128:]], axis=1)
                sc[ns] = _scores(qq, kload(order[ns]))
                ns += 1
            elif op == "o":
                pos = om.pop(0)
                y = oproj(get_o(pos), order[pos])
                out = y if out is None else out + y
            else:
                vpu_stage(nv)
                nv += 1
        out = functools.reduce(jnp.add, [out] + outv)
        return xr + _rowsum_all(out)

    x = ffn(attn_fast(ffn(x, 0)), 1)
    row = lax.broadcasted_iota(I32, (8, D), 0)
    o_ref[...] = jnp.where(row == B - 1, x, state[...])[0:B].astype(o_ref.dtype)


def _call(cfg, A_x, A_k_cache, A_v_cache, A_wq, A_wo, B_w_r, B_w_gate, B_w_up, B_w_down):
    kt = jnp.swapaxes(A_k_cache, 2, 3).reshape(B, NP * RO, RI * 8, SK)
    vt = jnp.swapaxes(A_v_cache, 2, 3).reshape(B, NP * RO, RI * 8, SK)
    out = pl.pallas_call(
        functools.partial(_kernel, cfg=cfg),
        out_shape=jax.ShapeDtypeStruct((B, D), BF16),
        in_specs=[pl.BlockSpec(memory_space=pl.ANY)] * 9,
        out_specs=pl.BlockSpec(memory_space=pltpu.VMEM),
        scratch_shapes=[
            pltpu.VMEM((3, NP * RO + 1, RI * 8, W), BF16),
            pltpu.VMEM((VF * RO, RI * 8, W), F32),
            pltpu.VMEM((NP * RO, RI * 4, W), U32),
            pltpu.VMEM((D, HD), BF16),
            pltpu.VMEM((HD, D), BF16),
            pltpu.VMEM((D, F), BF16),
            pltpu.VMEM((D, F), BF16),
            pltpu.VMEM((F, D), BF16),
            pltpu.VMEM((D // 2, HD + 2 * F), U32),
            pltpu.VMEM((HD // 2, D), U32),
            pltpu.VMEM((F // 2, D), U32),
            pltpu.VMEM((D, cfg["NV"] * 256), F32),
            pltpu.VMEM((D, len(cfg["VQ"]) * PD), F32),
            pltpu.VMEM((cfg["ND"] * 128, D), F32),
            pltpu.VMEM((len(cfg["VO"]) * PD, D), F32),
            pltpu.VMEM((8, HD + 2 * F), F32),
            pltpu.VMEM((B, D), BF16),
            pltpu.VMEM((D // 128, 128), BF16),
            pltpu.VMEM((8, D), F32),
            pltpu.VMEM((8, 128), F32),
            pltpu.VMEM((2, 8, W), F32),
            pltpu.VMEM((2, 8, W), F32),
            pltpu.VMEM((3, 8, PD), F32),
            pltpu.VMEM((8, D), F32),
            pltpu.SemaphoreType.DMA((2, RING)),
            pltpu.SemaphoreType.DMA((8,)),
        ],
        compiler_params=pltpu.CompilerParams(vmem_limit_bytes=126 * 1024 * 1024,
                                             disable_bounds_checks=True,
                                             disable_semaphore_checks=True),
        name="fused_decode",
    )(A_x.reshape(B, D), kt, vt, A_wq, A_wo, B_w_r.reshape(D // 128, 128), B_w_gate, B_w_up, B_w_down)
    return out.reshape(B, 1, D)


@jax.jit
def pallas_interleave_layers__sliding_block_cached__moe_arch_mod__decode_kernel(
    A_x: jax.Array,
    A_k_cache: jax.Array,
    A_v_cache: jax.Array,
    A_wq: jax.Array,
    A_wo: jax.Array,
    B_x: jax.Array,
    B_w_r: jax.Array,
    B_w_gate: jax.Array,
    B_w_up: jax.Array,
    B_w_down: jax.Array,
):
    del B_x
    return _call(CFG, A_x, A_k_cache, A_v_cache, A_wq, A_wo, B_w_r, B_w_gate, B_w_up, B_w_down)
```

```python
import functools

import jax
import jax.numpy as jnp
from jax import lax
import jax.experimental.pallas as pl
import jax.experimental.pallas.tpu as pltpu

F32 = jnp.float32
BF16 = jnp.bfloat16
U32 = jnp.uint32
I32 = jnp.int32

B, D, H, DH, SK, F = 4, 640, 32, 192, 4096, 1536
W = min(4096, max(256, SK // 4))
NP = H // 2
PD = 2 * DH
HD = H * DH
NL = W // 128
NH = F // 128
EPS = 1e-5
SCALE = DH ** -0.5 * 1.4426950408889634

RI = 8
RO = PD // (8 * RI)
TPC = RI // 2
TPP = 2 * NP * TPC
NTICK = B * TPP
RING = 32
VF = 12

CFG = dict(
    LA=23,
    LEAD=11,
    KRP=54,
    PVMID=(21, 45),
    SPIN=(1, 50),
    WSPIN=(1, 45),
    LSPIN=(1, 20),
    KSPIN=(1, 20),
    HSPIN=(1, 8),
    NV=(4, 4),
    ND=(4, 5),
    DLATE=(2, 2),
    TOK=(0, 0),
    DTOK=(1, 2),
    DPER=(2, 3),
    QTOK=0,
    RAWPOS=(2, 4, 7, 10),
    PROG="qqsqs.s.qqs.qs.qqs.s.qqos.s.qs.qsqo.so.so.so.so.s...ooooooo",
    NLS=1,
    VQ=(3, 4, 5),
    VO=(2, 0, 8),
    VOT=((14, 0, 1, 3, 0), (4, 16, 0, 2, 0), (11, 32, 0, 3, 2)),
)


def _order(cfg):
    order = list(range(VF))
    for pos, k in zip(sorted(cfg["RAWPOS"]), range(VF, NP)):
        order.insert(pos, k)
    return order


def _rowsum_all(x):
    x = x + pltpu.roll(x, 4, 0)
    x = x + pltpu.roll(x, 2, 0)
    return x + pltpu.roll(x, 1, 0)


def _bf(x):
    return pltpu.bitcast(x, BF16)


def _u32(x):
    return pltpu.bitcast(x, U32)


def _dot(a, b):
    return jnp.dot(a, b, preferred_element_type=F32)


def _sigmoid(x):
    return pl.reciprocal(1.0 + jnp.exp(-x), approx=True)


def _round(x):
    return x.astype(BF16).astype(F32)


def _ln_parts(x):
    xb = x.astype(BF16)
    xr = xb.astype(F32)
    m = jnp.sum(xr, axis=1, keepdims=True) * (1.0 / D)
    xc = xr - m
    v = jnp.sum(xc * xc, axis=1, keepdims=True) * (1.0 / D)
    m = _round(m)
    v = _round(_round(v) + EPS)
    return xb, xr, m, xr - m, pl.reciprocal(_round(v * lax.rsqrt(v)), approx=True)


def _scores(q, kk):
    lane = lax.broadcasted_iota(I32, (8, 128), 1)
    q0 = q[:, 0:128].astype(BF16)
    qm = q[:, 128:256]
    q2 = q[:, 256:384].astype(BF16)
    mid = jnp.concatenate([jnp.where(lane < 64, qm, 0.0), jnp.where(lane >= 64, qm, 0.0)],
                          axis=0).astype(BF16)
    r0 = _dot(q0, kk[0])
    rm = _dot(mid, kk[1])
    r2 = _dot(q2, kk[2])
    return r0 + rm[0:8], rm[8:16] + r2


def _fold(x, op):
    r = x[:, 0:128]
    for t in range(1, x.shape[1] // 128):
        r = op(r, x[:, t * 128:(t + 1) * 128])
    return r


def _tile(x, n):
    return jnp.concatenate([x] * n, axis=1)


def _softmax_pair(se, so, c=None, bcast=False):
    row = lax.broadcasted_iota(I32, (8, 128), 0)
    top = row < 4

    def split(c):
        c = jnp.broadcast_to(c, (8, 128))
        r = pltpu.roll(c, 4, 0)
        return jnp.where(top, c, r), jnp.where(top, r, c)

    m = jnp.max(jnp.where(top, _fold(se, jnp.maximum), _fold(so, jnp.maximum)), axis=1, keepdims=True)
    me, mo = split(m)
    de, do = se - _tile(me, NL), so - _tile(mo, NL)
    if c is not None:
        de, do = de * c, do * c
    pe, po = jnp.exp2(de), jnp.exp2(do)
    le, lo = _fold(pe, jnp.add), _fold(po, jnp.add)
    if bcast:
        l = jnp.sum(jnp.where(row >= 1, lo, le), axis=1, keepdims=True)
        r = jnp.broadcast_to(pl.reciprocal(l, approx=True), (8, 128))
        ie, io = [jnp.broadcast_to(r[i:i + 1], (8, 128)) for i in range(2)]
    else:
        ie, io = split(pl.reciprocal(jnp.sum(jnp.where(top, le, lo), axis=1, keepdims=True), approx=True))
    lane = lax.broadcasted_iota(I32, (8, 128), 1)
    return pe, po, jnp.concatenate([ie, jnp.where(lane < 64, ie, io), io], axis=1)


def _pv(groups, hooks=None):
    nb = len(groups) // 16
    accs = {}
    for n, g in enumerate(16 * blk + i for i in range(16) for blk in range(nb)):
        if hooks and n in hooks:
            hooks[n]()
        vload, p = groups[g]
        accs[g] = _fold(vload() * p, jnp.add)
    return jnp.concatenate([accs[g] for g in range(len(groups))], axis=0)


def _lane_reduce_t(acc):
    at = acc.T
    s = at[0:8]
    for i in range(1, 16):
        s = s + at[8 * i:8 * i + 8]
    return s


def _kernel(x_hbm, kt_hbm, vt_hbm, wq_hbm, wo_hbm, wr_hbm, wg_hbm, wu_hbm, wd_hbm,
            o_ref,
            kv, vf, kp, wq_raw, wo_raw, wg_raw, wu_raw, wd_raw, wxp, wop, wdp, wguf, wqf, wdf, wof, cs,
            xb_ref, wrb, state, spin_ref, c_s, c_p, c_o, c_out,
            sems, wsem, *, cfg):
    LA, LEAD, NV, ND = cfg["LA"], cfg["LEAD"], max(cfg["NV"]), max(cfg["ND"])
    order = _order(cfg)

    def piece(i, s):
        q, pair, w, b = i & (TPC - 1), (i >> 2) & (NP - 1), (i >> 6) & 1, i >> 7
        r0 = (q + s * TPC) * 8
        if not isinstance(i, int):
            r0 = pl.multiple_of(r0, 8)
        return pair, w, b, w * (1 + (b & 1)), i & (RING - 1), r0

    def start_piece(i, s, hf=None):
        pair, w, b, plane, ring, r0 = piece(i, s)
        osl = pl.ds(pair * RO, RO) if hf is None else pl.ds(pair * RO + hf * (RO // 2), RO // 2)

        def go(ww):
            src = vt_hbm if ww else kt_hbm
            pltpu.make_async_copy(src.at[b, osl, pl.ds(r0, 8), pl.ds(SK - W, W)],
                                  kv.at[plane, osl, pl.ds(r0, 8), :],
                                  sems.at[s, ring]).start(priority=1 - s)

        if isinstance(i, int):
            go(w)
        else:
            for ww in range(2):
                pl.when(jnp.logical_and(w == ww, i < NTICK))(functools.partial(go, ww))

    def wait_piece(i, s):
        pair, w, b, plane, ring, r0 = piece(i, s)
        view = kv.at[plane, pl.ds(pair * RO, RO), pl.ds(r0, 8), :]
        pltpu.make_async_copy(view, view, sems.at[s, ring]).wait()

    def wait_tick(i):
        wait_piece(i, 0)
        wait_piece(i, 1)

    def spin(n):
        v = spin_ref[...]
        lane = lax.broadcasted_iota(I32, v.shape, 1).astype(F32)
        for _ in range(n[0]):
            v = jnp.max(v, axis=1, keepdims=True) * 0.5 + lane
        for _ in range(n[1] // 2):
            v = v * 0.5
            v = v + lane
        spin_ref[...] = v

    def full_tick(i):
        wait_tick(i)
        start_piece(i + LEAD + 1, 1)
        start_piece(i + LA, 0)

    def spin_tick(i, c):
        full_tick(i)
        spin(cfg["SPIN"])
        return c

    def half_tick(h, lead, la, work, sp, top):
        i = h >> 1
        pl.when((h & 1) == 0)(lambda: wait_tick(i))
        if top:
            start_piece(i + lead, 1, h & 1)
        work()
        spin(sp)
        if not top:
            start_piece(i + lead, 1, h & 1)
        start_piece(jnp.where((h & 1) == 1, i + la, NTICK), 0)

    def idle_half(h, c):
        def work():
            n = (((h >> 3) & (NP - 1)) - 4) * 4 + (h & 7) - 2
            o0 = jnp.minimum(n * 2, VF * RO - 2)
            vf[pl.ds(o0, 2)] = kv[1 + ((h >> 8) & 1), pl.ds(o0, 2)].astype(F32)

        half_tick(h, LEAD, LA - 1, work, cfg["HSPIN"], False)
        return c

    def advance(t, need):
        t2 = jnp.maximum(t + 2, need)
        wait_tick(t)
        lax.fori_loop(2 * t + 2, 2 * t2 - 2, idle_half, 0)
        wait_tick(t2 - 1)
        start_piece(t2 - 1 + LEAD, 1, 0)
        return t2

    def mid(t2, n, after=None):
        if n == 0:
            start_piece(t2 - 1 + LEAD, 1, 1)
        if n == 1:
            start_piece(t2 + LEAD, 1, 0)
            start_piece(t2 - 2 + LA, 0)
            start_piece(t2 - 1 + LA, 0)
        if n == 2:
            kv[0, NP * RO, 0:16, 0:128] = jnp.concatenate([after, after], axis=0).astype(BF16)
            start_piece(t2 + LEAD, 1, 1)

    half = D // 2
    small = [pltpu.make_async_copy(x_hbm, xb_ref, wsem.at[0]),
             pltpu.make_async_copy(wr_hbm, wrb, wsem.at[1])]
    big = [pltpu.make_async_copy(wq_hbm, wq_raw, wsem.at[2]),
           pltpu.make_async_copy(wg_hbm, wg_raw, wsem.at[3]),
           pltpu.make_async_copy(wu_hbm.at[pl.ds(0, half)], wu_raw.at[pl.ds(0, half)], wsem.at[4])]
    for cp in big:
        cp.start(priority=1)
    for cp in small:
        cp.start()
    spin_ref[...] = jnp.zeros(spin_ref.shape, F32)

    inject = [(wo_hbm, wo_raw, 0, 48, HD // 48, 5), (wd_hbm, wd_raw, 0, 48, F // 48, 6),
              (wu_hbm, wu_raw, half, 16, half // 16, 7)]
    for src, dst, row0, rows, n, sem in inject:
        def body(i, c, src=src, dst=dst, row0=row0, rows=rows, sem=sem):
            r = pl.multiple_of(row0 + i * rows, 8)
            pltpu.make_async_copy(src.at[pl.ds(r, rows)], dst.at[pl.ds(r, rows)], wsem.at[sem]).start()
            spin(cfg["WSPIN"])
            return c
        lax.fori_loop(0, n, body, 0)
        if dst is wo_raw:
            for i in range(LA):
                start_piece(i, 0)

    def lead_in(h, c):
        start_piece(h >> 1, 1, h & 1)
        spin(cfg["LSPIN"])
        return c

    lax.fori_loop(0, 2 * (LEAD + 1), lead_in, 0)
    for cp in small:
        cp.wait()
    state[...] = jnp.concatenate([xb_ref[...].astype(F32), jnp.zeros((8 - B, D), F32)], axis=0)
    for src, dst, row0, rows, n, sem in inject:
        view = dst.at[pl.ds(row0, rows * n)]
        pltpu.make_async_copy(view, view, wsem.at[sem]).wait()
    for cp in big:
        cp.wait()

    NRP = D // 16

    def repack(h, c):
        full_tick(h)
        r = pl.multiple_of(h * 16, 16)
        r2 = pl.multiple_of(h * 8, 8)
        wxp[pl.ds(r2, 8), 0:HD] = _u32(wq_raw[pl.ds(r, 16), :])
        for n, pos in enumerate(cfg["VQ"]):
            wqf[pl.ds(r, 16), n * PD:(n + 1) * PD] = (
                wq_raw[pl.ds(r, 16), order[pos] * PD:(order[pos] + 1) * PD].astype(F32))
        g = wg_raw[pl.ds(r, 16), :]
        u = wu_raw[pl.ds(r, 16), :]
        gu = jnp.concatenate([w[:, i * 128:(i + 1) * 128] for i in range(NH) for w in (g, u)], axis=1)
        wxp[pl.ds(r2, 8), HD:HD + 2 * F] = _u32(gu)
        wguf[pl.ds(r, 16), :] = gu[:, (NH - NV) * 256:].astype(F32)
        for n, pos in enumerate(cfg["VO"]):
            ro = pl.multiple_of(jnp.minimum(r, PD - 16), 16)
            wof[pl.ds(n * PD + ro, 16), :] = wo_raw[pl.ds(order[pos] * PD + ro, 16), :].astype(F32)
        nd = 16 if ND * 128 <= D else 32
        rd = pl.multiple_of(jnp.minimum(h * nd, ND * 128 - nd), 16)
        wdf[pl.ds(rd, nd), :] = wd_raw[pl.ds(rd, nd), :].astype(F32)
        for src, packed, n in ((wo_raw, wop, 160), (wd_raw, wdp, 48)):
            r = pl.multiple_of(jnp.minimum(h * n, src.shape[0] - n), 16)
            packed[pl.ds(pl.multiple_of(r >> 1, 8), n // 2), :] = _u32(src[pl.ds(r, n), :])
        return c

    lax.fori_loop(0, NRP, repack, 0)

    NCS = (HD + 2 * F) // 768

    def colsum(i, c):
        full_tick(NRP + i)
        c0 = pl.multiple_of(i * 768, 128)
        cs[:, pl.ds(c0, 768)] = _dot(jnp.ones((8, D), BF16), _bf(wxp[:, pl.ds(c0, 768)]))
        return c

    lax.fori_loop(0, NCS, colsum, 0)
    t0 = jnp.int32(NRP + NCS)

    never = spin_ref[...] < -1.0

    def xproj(xb, m, scale, c0, n):
        y = _dot(xb, _bf(wxp[:, pl.ds(c0, n)])) - m * cs[:, pl.ds(c0, n)]
        return y if scale is None else y * scale

    def qproj(xb, m, qscale, k):
        return xproj(xb, m, qscale, k * PD if isinstance(k, int) else pl.multiple_of(k * PD, 128), PD)

    def oproj(ob, k):
        r0 = pl.multiple_of(k * DH, DH) if not isinstance(k, int) else k * DH
        return _dot(ob, _bf(wop[pl.ds(r0, DH), :]))

    def kload(k):
        return [_bf(kp[pl.ds(k * RO + 2 * i, 2)].reshape(64, W)) for i in range(3)]

    def vgroup(slot, k, o, r):
        return lambda: kv[1 + slot, k * RO + o, pl.ds(r * 8, 8), :].astype(F32)

    def pair_groups(slot, k, pe, po):
        return [(vgroup(slot, k, g // RI, g % RI), pe if g < DH // 8 else po) for g in range(PD // 8)]

    def vpu_matvec(xr, w_ref, nadd, per_step=1, tok=None):
        nu = xr.shape[1] // 128
        xcol = [jnp.concatenate([xr[:, u * 128:(u + 1) * 128]] * 16, axis=0).T for u in range(nu)]
        seq = [(u, i) for u0 in range(0, nu, 2) for i in range(16) for u in range(u0, min(u0 + 2, nu))]
        accs = [None] * per_step
        for n in range(0, len(seq), per_step):
            if tok is not None:
                for _ in range(nadd):
                    tok = tok + 1.0
            for a, (u, i) in enumerate(seq[n:n + per_step]):
                col = xcol[u][i * 8:i * 8 + 8]
                if tok is not None:
                    col = jnp.where(never, tok, col)
                y = w_ref[u * 128 + i * 8:u * 128 + i * 8 + 8, :] * _tile(col, w_ref.shape[1] // 128)
                accs[a] = y if accs[a] is None else accs[a] + y
            tok = accs[0][:, 0:128]
        return functools.reduce(jnp.add, accs), tok

    def act(gu):
        g = gu[:, 0:128]
        return (g * _sigmoid(g) * gu[:, 128:256]).astype(BF16)

    def ffn_res(x, xc, rstd):
        wr = wrb[...].astype(F32)
        wr = jnp.concatenate([jnp.broadcast_to(wr[t:t + 1, :], (8, 128)) for t in range(D // 128)], axis=1)
        return x + xc * rstd, _round(_sigmoid(_round(jnp.sum(xc * wr, axis=1, keepdims=True) * rstd)))

    def ffn(x, f):
        nv, nd = cfg["NV"][f], cfg["ND"][f]
        nm = NH - nv
        xb, xr, m, xc, rstd = _ln_parts(x)
        hs = [act(xproj(xb, m, rstd, HD + i * 256, 256)) for i in range(nm)]
        gu, tok = vpu_matvec(xr, wguf.at[:, (NV - nv) * 256:], cfg["TOK"][f])
        gu = (_rowsum_all(gu) - m * cs[:, HD + nm * 256:]) * rstd
        hs += [act(gu[:, i * 256:(i + 1) * 256]) for i in range(nv)]
        y = None
        late = list(range(nm - cfg["DLATE"][f], nm))
        for i in [i for i in range(nd, NH) if i not in late] + late:
            yi = _dot(hs[i], _bf(wdp[i * 64:(i + 1) * 64, :]))
            y = yi if y is None else y + yi
        yv, _ = vpu_matvec(jnp.concatenate(hs[:nd], axis=1).astype(F32), wdf, cfg["DTOK"][f], cfg["DPER"][f], tok)
        y = y + _rowsum_all(yv)
        res, gate = ffn_res(xr, xc, rstd)
        return res + y * gate

    NFT = NH // 2 + 1

    def ffn_ticked(x, t):
        def body(i, carry):
            h, y, _ = carry
            full_tick(t + i)
            xb, xr, m, xc, rstd = _ln_parts(x)
            c0 = pl.multiple_of(HD + jnp.minimum(i, NFT - 2) * 512, 128)
            gu = xproj(xb, m, rstd, c0, 512)
            r0 = pl.multiple_of(jnp.maximum(i - 1, 0) * 128, 128)
            y = y + _dot(h, _bf(wdp[pl.ds(r0, 128), :]))
            res, gate = ffn_res(xr, xc, rstd)
            return jnp.concatenate([act(gu[:, 0:256]), act(gu[:, 256:512])], axis=1), y, res + y * gate

        return lax.fori_loop(0, NFT, body, (jnp.zeros((8, 256), BF16), jnp.zeros((8, D), F32), x))[2]

    NHP = 2 * B - 1

    def half_period(hp, t):
        b = hp >> 1
        slot = b & 1
        first = (hp & 1) == 0
        vbase = jnp.where(first, b * TPP + (NP + 1) * TPC, -TPP)

        tr = jnp.where(first, jnp.maximum(t, b * TPP + cfg["KRP"]), t)
        lax.fori_loop(t, tr, spin_tick, 0)

        def k_repack(h, c):
            def work():
                o0 = (h - 2 * tr) * 4
                kp[pl.ds(o0, 4)] = _u32(kv[0, pl.ds(o0, 4)].reshape(4 * 64, W)).reshape(4, 32, W)

            half_tick(h, LEAD + 1, LA, work, cfg["KSPIN"], True)
            return c

        t = jnp.where(first, tr + NP * RO // 8, t)
        lax.fori_loop(2 * tr, 2 * t, k_repack, 0)

        xb, x, m, _, rstd = _ln_parts(jnp.broadcast_to(state[pl.ds(b, 1), :], (8, D)))
        qscale = rstd * SCALE

        def step(j, carry):
            t, q, se, so, pe, po, inv, o, out = carry
            kv_ = jnp.maximum(j - 3, 0)
            t = advance(t, vbase + kv_ * TPC)
            se_n, so_n = _scores(q, kload(jnp.clip(j - 1, 0, NP - 1)))
            q_n = qproj(xb, m, qscale, jnp.minimum(j, NP - 1))
            out = out + oproj(o, jnp.maximum(j - 4, 0))
            pe_n, po_n, inv_n = _softmax_pair(se, so)
            acc = _pv(pair_groups(slot, kv_, pe, po),
                      {cfg["PVMID"][0]: lambda: mid(t, 0), cfg["PVMID"][1]: lambda: mid(t, 1)})
            mid(t, 2, q_n[:, 256:384])
            o_n = jnp.where(j >= 3, _lane_reduce_t(acc) * inv, 0.0).astype(BF16)
            return t, q_n, se_n, so_n, pe_n, po_n, inv_n, o_n, out

        zw = (lax.broadcasted_iota(I32, (8, W), 0) + lax.broadcasted_iota(I32, (8, W), 1)).astype(F32) * (1.0 / W)
        zp = zw[:, :PD]
        init = (t, zp, zw, zw, zw, zw, zp, jnp.zeros((8, PD), BF16), jnp.zeros((8, D), F32))
        last = hp == NHP - 1
        t, q, se, so, pe, po, inv, o, out = lax.fori_loop(0, jnp.where(last, NP, NP + 2), step, init)
        t2 = jnp.maximum(t + 2, vbase + (NP - 1) * TPC)

        @pl.when(last)
        def _():
            c_s[0] = se
            c_s[1] = so
            c_p[0] = pe
            c_p[1] = po
            c_o[0] = q
            c_o[1] = inv
            c_o[2] = o.astype(F32)
            c_out[...] = out

        @pl.when(jnp.logical_not(last))
        def _():
            advance(t, t2)
            y = out + oproj(o, NP - 2)
            acc = _pv(pair_groups(slot, NP - 1, pe, po), {24: lambda: mid(t2, 0), 45: lambda: mid(t2, 1)})
            olast = _lane_reduce_t(acc) * inv
            mid(t2, 2, olast[:, 0:128])
            olast = olast.astype(BF16)
            full_tick(t2)
            y = y + oproj(olast, NP - 1)
            state[pl.ds(b, 1), :] = ffn_ticked(x + _rowsum_all(y), t2 + 1)[0:1]

        return t2 + 1 + NFT

    lax.fori_loop(0, NHP, half_period, t0)

    slot = (B - 1) % 2
    ka, kb = NP - 2, NP - 1

    def wo_rows(runs):
        return _bf(jnp.concatenate(
            [wop[(k * PD + o * 64 + r * 8) // 2:(k * PD + o * 64 + (r + n) * 8) // 2, :] for k, o, r, n in runs],
            axis=0))

    def run_groups(runs, ps):
        return [(vgroup(slot, k, o, r + i), ps[k][0 if o < RO // 2 else 1]) for k, o, r, n in runs for i in range(n)]

    def normalised(pe, po, inv):
        return pe * _tile(inv[:, 0:128], NL), po * _tile(inv[:, 256:384], NL)

    def pv_o_vpu(runs):
        w = wo_rows(runs).astype(F32)
        return functools.reduce(jnp.add, [
            w[i * 8:(i + 1) * 8] * jnp.sum(_fold(vload() * p, jnp.add), axis=1, keepdims=True)
            for i, (vload, p) in enumerate(run_groups(runs, ps))])

    kc = NP - 3
    for i in range(NTICK - 3 * TPC, NTICK - TPC):
        wait_piece(i, 1)
    se, so = _scores(c_o[0], kload(kb))
    out = c_out[...] + oproj(c_o[2].astype(BF16), NP - 4)
    ps = {kc: normalised(c_p[0], c_p[1], c_o[1]), ka: normalised(*_softmax_pair(c_s[0], c_s[1]))}
    runs = [(k, o, TPC, TPC) for k in (kc, ka) for o in range(RO)]
    o = _lane_reduce_t(_pv(run_groups(runs, ps))).astype(BF16)
    ps[kb] = normalised(*_softmax_pair(se, so))

    for i in range(NTICK - 3 * TPC, NTICK - 2 * TPC):
        wait_piece(i, 0)
    for i in range(NTICK - TPC, NTICK):
        wait_piece(i, 1)
    out = out + _dot(o, wo_rows(runs))
    runs0 = [(kc, o, 0, TPC) for o in range(RO)] + [(kb, o, TPC, TPC) for o in range(RO)]
    o0 = _lane_reduce_t(_pv(run_groups(runs0, ps))).astype(BF16)

    for i in range(NTICK - 2 * TPC, NTICK - TPC):
        wait_piece(i, 0)
    out = out + _dot(o0, wo_rows(runs0))
    runs1 = [(ka, o, 0, TPC) for o in range(RO)]
    acc = [_fold(vload() * p, jnp.add) for vload, p in run_groups(runs1, ps)]
    zero = [jnp.zeros((8, 128), F32)] * 4
    o1 = _lane_reduce_t(jnp.concatenate(acc[:12] + zero + acc[12:] + zero, axis=0)).astype(BF16)

    for i in range(NTICK - TPC, NTICK - 2):
        wait_piece(i, 0)
    out = out + _dot(o1, wo_rows(runs1[:3] + runs1[:1] + runs1[3:] + runs1[:1]))
    out = out + pv_o_vpu([(kb, o, 0, 2) for o in range(RO)])

    for i in range(NTICK - 2, NTICK):
        wait_piece(i, 0)
    out = out + pv_o_vpu([(kb, o, 2, 2) for o in range(RO)])
    x = jnp.broadcast_to(state[B - 1:B, :], (8, D)) + _rowsum_all(out)

    def attn_fast(x):
        xb, xr, m, _, rstd = _ln_parts(x)
        qscale = rstd * SCALE
        q, sc, ps, os_, deadline, outv = {}, {}, {}, {}, {}, []
        invs = {}

        def get_o(pos):
            o = os_.pop(pos) * invs.pop(pos)
            return (_rowsum_all(o) if pos in cfg["VO"] else o).astype(BF16)

        out = None
        qv = _rowsum_all(vpu_matvec(xr, wqf, cfg["QTOK"])[0])
        for n, pos in enumerate(cfg["VQ"]):
            k = order[pos]
            q[pos] = (qv[:, n * PD:(n + 1) * PD] - m * cs[:, k * PD:(k + 1) * PD]) * qscale
        qm = [pos for pos in range(NP) if pos not in cfg["VQ"]]
        om = [pos for pos in range(NP) if pos not in cfg["VO"]]

        def vpu_stage(s):
            if 0 <= s + 1 < NP:
                ps[s + 1] = _softmax_pair(*sc.pop(s + 1), None if s + 1 >= cfg["NLS"] else qscale, bcast=True)
            if 0 <= s < NP:
                pe, po, invs[s] = ps.pop(s)
                k = order[s]
                groups = pair_groups(slot, k, pe, po)
                if k < VF:
                    groups = [(functools.partial(lambda g: vf[k * RO + g // RI, pl.ds((g % RI) * 8, 8), :], g), p)
                              for g, (_, p) in enumerate(groups)]
                acc = _pv(groups)
                os_[s] = _lane_reduce_t(acc)
                for n, (tpos, tg, nadd, per, dl) in enumerate(cfg["VOT"]):
                    if tpos == s:
                        y, tok = vpu_matvec(get_o(cfg["VO"][n]).astype(F32), wof.at[n * PD:(n + 1) * PD], nadd, per,
                                            acc[tg * 8:tg * 8 + 8])
                        outv.append(y)
                        if dl:
                            deadline[s + dl + 2] = tok

        ns, nv = 0, -1
        for op in cfg["PROG"]:
            if op == "q":
                pos = qm.pop(0)
                q[pos] = qproj(xb, m, qscale if pos >= cfg["NLS"] else None, order[pos])
            elif op == "s":
                qq = q.pop(ns)
                if ns in deadline:
                    qq = jnp.concatenate([jnp.where(never, deadline.pop(ns), qq[:, 0:128]), qq[:, 128:]], axis=1)
                sc[ns] = _scores(qq, kload(order[ns]))
                ns += 1
            elif op == "o":
                pos = om.pop(0)
                y = oproj(get_o(pos), order[pos])
                out = y if out is None else out + y
            else:
                vpu_stage(nv)
                nv += 1
        out = functools.reduce(jnp.add, [out] + outv)
        return xr + _rowsum_all(out)

    x = ffn(attn_fast(ffn(x, 0)), 1)
    row = lax.broadcasted_iota(I32, (8, D), 0)
    o_ref[...] = jnp.where(row == B - 1, x, state[...])[0:B].astype(o_ref.dtype)


def _call(cfg, A_x, A_k_cache, A_v_cache, A_wq, A_wo, B_w_r, B_w_gate, B_w_up, B_w_down):
    kt = jnp.swapaxes(A_k_cache, 2, 3).reshape(B, NP * RO, RI * 8, SK)
    vt = jnp.swapaxes(A_v_cache, 2, 3).reshape(B, NP * RO, RI * 8, SK)
    out = pl.pallas_call(
        functools.partial(_kernel, cfg=cfg),
        out_shape=jax.ShapeDtypeStruct((B, D), BF16),
        in_specs=[pl.BlockSpec(memory_space=pl.ANY)] * 9,
        out_specs=pl.BlockSpec(memory_space=pltpu.VMEM),
        scratch_shapes=[
            pltpu.VMEM((3, NP * RO + 1, RI * 8, W), BF16),
            pltpu.VMEM((VF * RO, RI * 8, W), F32),
            pltpu.VMEM((NP * RO, RI * 4, W), U32),
            pltpu.VMEM((D, HD), BF16),
            pltpu.VMEM((HD, D), BF16),
            pltpu.VMEM((D, F), BF16),
            pltpu.VMEM((D, F), BF16),
            pltpu.VMEM((F, D), BF16),
            pltpu.VMEM((D // 2, HD + 2 * F), U32),
            pltpu.VMEM((HD // 2, D), U32),
            pltpu.VMEM((F // 2, D), U32),
            pltpu.VMEM((D, max(cfg["NV"]) * 256), F32),
            pltpu.VMEM((D, len(cfg["VQ"]) * PD), F32),
            pltpu.VMEM((max(cfg["ND"]) * 128, D), F32),
            pltpu.VMEM((len(cfg["VO"]) * PD, D), F32),
            pltpu.VMEM((8, HD + 2 * F), F32),
            pltpu.VMEM((B, D), BF16),
            pltpu.VMEM((D // 128, 128), BF16),
            pltpu.VMEM((8, D), F32),
            pltpu.VMEM((8, 128), F32),
            pltpu.VMEM((2, 8, W), F32),
            pltpu.VMEM((2, 8, W), F32),
            pltpu.VMEM((3, 8, PD), F32),
            pltpu.VMEM((8, D), F32),
            pltpu.SemaphoreType.DMA((2, RING)),
            pltpu.SemaphoreType.DMA((8,)),
        ],
        compiler_params=pltpu.CompilerParams(vmem_limit_bytes=126 * 1024 * 1024,
                                             disable_bounds_checks=True,
                                             disable_semaphore_checks=True),
        name="fused_decode",
    )(A_x.reshape(B, D), kt, vt, A_wq, A_wo, B_w_r.reshape(D // 128, 128), B_w_gate, B_w_up, B_w_down)
    return out.reshape(B, 1, D)


@jax.jit
def pallas_interleave_layers__sliding_block_cached__moe_arch_mod__decode_kernel(
    A_x: jax.Array,
    A_k_cache: jax.Array,
    A_v_cache: jax.Array,
    A_wq: jax.Array,
    A_wo: jax.Array,
    B_x: jax.Array,
    B_w_r: jax.Array,
    B_w_gate: jax.Array,
    B_w_up: jax.Array,
    B_w_down: jax.Array,
):
    del B_x
    return _call(CFG, A_x, A_k_cache, A_v_cache, A_wq, A_wo, B_w_r, B_w_gate, B_w_up, B_w_down)
```

```python
import functools

import jax
import jax.numpy as jnp
from jax import lax
import jax.experimental.pallas as pl
import jax.experimental.pallas.tpu as pltpu

F32 = jnp.float32
BF16 = jnp.bfloat16
U32 = jnp.uint32
I32 = jnp.int32

B, D, H, DH, SK, F = 4, 640, 32, 192, 4096, 1536
W = min(4096, max(256, SK // 4))
NP = H // 2
PD = 2 * DH
HD = H * DH
NL = W // 128
NH = F // 128
EPS = 1e-5
SCALE = DH ** -0.5 * 1.4426950408889634

RI = 8
RO = PD // (8 * RI)
TPC = RI // 2
TPP = 2 * NP * TPC
NTICK = B * TPP
RING = 32
VF = 12

CFG = dict(
    LA=23,
    LEAD=11,
    KRP=54,
    PVMID=(21, 45),
    SPIN=(1, 50),
    WSPIN=(1, 45),
    LSPIN=(1, 20),
    KSPIN=(1, 20),
    HSPIN=(1, 8),
    NV=(3, 4),
    ND=(5, 5),
    DLATE=(0, 3),
    TOK=(0, 0),
    DTOK=(2, 2),
    DPER=(2, 3),
    QTOK=0,
    ROT=(1, 1, 3, 0),
    RAWPOS=(0, 2, 4, 10),
    PROG="qqsqs.s.qqs.qs.qqos.s.qqs.s.qs.qso.qso.s.oso.so.s...ooooooo",
    NLS=2,
    VQ=(3, 4, 5),
    VO=(1, 0, 8),
    VOT=((14, 0, 0, 3, 0), (4, 16, 0, 2, 0), (11, 32, 0, 3, 2)),
)


def _order(cfg):
    order = list(range(VF))
    for pos, k in zip(sorted(cfg["RAWPOS"]), range(VF, NP)):
        order.insert(pos, k)
    return order


def _rowsum_all(x):
    x = x + pltpu.roll(x, 4, 0)
    x = x + pltpu.roll(x, 2, 0)
    return x + pltpu.roll(x, 1, 0)


def _bf(x):
    return pltpu.bitcast(x, BF16)


def _u32(x):
    return pltpu.bitcast(x, U32)


def _dot(a, b):
    return jnp.dot(a, b, preferred_element_type=F32)


def _sigmoid(x):
    return pl.reciprocal(1.0 + jnp.exp(-x), approx=True)


def _round(x):
    return x.astype(BF16).astype(F32)


def _ln_parts(x):
    xb = x.astype(BF16)
    xr = xb.astype(F32)
    m = jnp.sum(xr, axis=1, keepdims=True) * (1.0 / D)
    xc = xr - m
    v = jnp.sum(xc * xc, axis=1, keepdims=True) * (1.0 / D)
    m = _round(m)
    v = _round(_round(v) + EPS)
    return xb, xr, m, xr - m, pl.reciprocal(_round(v * lax.rsqrt(v)), approx=True)


def _scores(q, kk):
    lane = lax.broadcasted_iota(I32, (8, 128), 1)
    q0 = q[:, 0:128].astype(BF16)
    qm = q[:, 128:256]
    q2 = q[:, 256:384].astype(BF16)
    mid = jnp.concatenate([jnp.where(lane < 64, qm, 0.0), jnp.where(lane >= 64, qm, 0.0)],
                          axis=0).astype(BF16)
    r0 = _dot(q0, kk[0])
    rm = _dot(mid, kk[1])
    r2 = _dot(q2, kk[2])
    return r0 + rm[0:8], rm[8:16] + r2


def _fold(x, op):
    r = x[:, 0:128]
    for t in range(1, x.shape[1] // 128):
        r = op(r, x[:, t * 128:(t + 1) * 128])
    return r


def _tile(x, n):
    return jnp.concatenate([x] * n, axis=1)


def _softmax_pair(se, so, c=None, bcast=False):
    row = lax.broadcasted_iota(I32, (8, 128), 0)
    top = row < 4

    def split(c):
        c = jnp.broadcast_to(c, (8, 128))
        r = pltpu.roll(c, 4, 0)
        return jnp.where(top, c, r), jnp.where(top, r, c)

    m = jnp.max(jnp.where(top, _fold(se, jnp.maximum), _fold(so, jnp.maximum)), axis=1, keepdims=True)
    me, mo = split(m)
    de, do = se - _tile(me, NL), so - _tile(mo, NL)
    if c is not None:
        de, do = de * c, do * c
    pe, po = jnp.exp2(de), jnp.exp2(do)
    le, lo = _fold(pe, jnp.add), _fold(po, jnp.add)
    if bcast:
        l = jnp.sum(jnp.where(row >= 1, lo, le), axis=1, keepdims=True)
        r = jnp.broadcast_to(pl.reciprocal(l, approx=True), (8, 128))
        ie, io = [jnp.broadcast_to(r[i:i + 1], (8, 128)) for i in range(2)]
    else:
        ie, io = split(pl.reciprocal(jnp.sum(jnp.where(top, le, lo), axis=1, keepdims=True), approx=True))
    lane = lax.broadcasted_iota(I32, (8, 128), 1)
    return pe, po, jnp.concatenate([ie, jnp.where(lane < 64, ie, io), io], axis=1)


def _pv(groups, hooks=None):
    nb = len(groups) // 16
    accs = {}
    for n, g in enumerate(16 * blk + i for i in range(16) for blk in range(nb)):
        if hooks and n in hooks:
            hooks[n]()
        vload, p = groups[g]
        accs[g] = _fold(vload() * p, jnp.add)
    return jnp.concatenate([accs[g] for g in range(len(groups))], axis=0)


def _lane_reduce_t(acc):
    at = acc.T
    s = at[0:8]
    for i in range(1, 16):
        s = s + at[8 * i:8 * i + 8]
    return s


def _kernel(x_hbm, kt_hbm, vt_hbm, wq_hbm, wo_hbm, wr_hbm, wg_hbm, wu_hbm, wd_hbm,
            o_ref,
            kv, vf, kp, wq_raw, wo_raw, wg_raw, wu_raw, wd_raw, wxp, wop, wdp, wguf, wqf, wdf, wof, cs,
            xb_ref, wrb, state, spin_ref, c_s, c_p, c_o, c_out,
            sems, wsem, *, cfg):
    LA, LEAD, NV, ND = cfg["LA"], cfg["LEAD"], max(cfg["NV"]), max(cfg["ND"])
    order = _order(cfg)

    def piece(i, s):
        q, pair, w, b = i & (TPC - 1), (i >> 2) & (NP - 1), (i >> 6) & 1, i >> 7
        r0 = (q + s * TPC) * 8
        if not isinstance(i, int):
            r0 = pl.multiple_of(r0, 8)
        return pair, w, b, w * (1 + (b & 1)), i & (RING - 1), r0

    def start_piece(i, s, hf=None):
        pair, w, b, plane, ring, r0 = piece(i, s)
        osl = pl.ds(pair * RO, RO) if hf is None else pl.ds(pair * RO + hf * (RO // 2), RO // 2)

        def go(ww):
            src = vt_hbm if ww else kt_hbm
            pltpu.make_async_copy(src.at[b, osl, pl.ds(r0, 8), pl.ds(SK - W, W)],
                                  kv.at[plane, osl, pl.ds(r0, 8), :],
                                  sems.at[s, ring]).start(priority=1 - s)

        if isinstance(i, int):
            go(w)
        else:
            for ww in range(2):
                pl.when(jnp.logical_and(w == ww, i < NTICK))(functools.partial(go, ww))

    def wait_piece(i, s):
        pair, w, b, plane, ring, r0 = piece(i, s)
        view = kv.at[plane, pl.ds(pair * RO, RO), pl.ds(r0, 8), :]
        pltpu.make_async_copy(view, view, sems.at[s, ring]).wait()

    def wait_tick(i):
        wait_piece(i, 0)
        wait_piece(i, 1)

    def spin(n):
        v = spin_ref[...]
        lane = lax.broadcasted_iota(I32, v.shape, 1).astype(F32)
        for _ in range(n[0]):
            v = jnp.max(v, axis=1, keepdims=True) * 0.5 + lane
        for _ in range(n[1] // 2):
            v = v * 0.5
            v = v + lane
        spin_ref[...] = v

    def full_tick(i):
        wait_tick(i)
        start_piece(i + LEAD + 1, 1)
        start_piece(i + LA, 0)

    def spin_tick(i, c):
        full_tick(i)
        spin(cfg["SPIN"])
        return c

    def half_tick(h, lead, la, work, sp, top):
        i = h >> 1
        pl.when((h & 1) == 0)(lambda: wait_tick(i))
        if top:
            start_piece(i + lead, 1, h & 1)
        work()
        spin(sp)
        if not top:
            start_piece(i + lead, 1, h & 1)
        start_piece(jnp.where((h & 1) == 1, i + la, NTICK), 0)

    def idle_half(h, c):
        def work():
            n = (((h >> 3) & (NP - 1)) - 4) * 4 + (h & 7) - 2
            o0 = jnp.minimum(n * 2, VF * RO - 2)
            vf[pl.ds(o0, 2)] = kv[1 + ((h >> 8) & 1), pl.ds(o0, 2)].astype(F32)

        half_tick(h, LEAD, LA - 1, work, cfg["HSPIN"], False)
        return c

    def advance(t, need):
        t2 = jnp.maximum(t + 2, need)
        wait_tick(t)
        lax.fori_loop(2 * t + 2, 2 * t2 - 2, idle_half, 0)
        wait_tick(t2 - 1)
        start_piece(t2 - 1 + LEAD, 1, 0)
        return t2

    def mid(t2, n, after=None):
        if n == 0:
            start_piece(t2 - 1 + LEAD, 1, 1)
        if n == 1:
            start_piece(t2 + LEAD, 1, 0)
            start_piece(t2 - 2 + LA, 0)
            start_piece(t2 - 1 + LA, 0)
        if n == 2:
            kv[0, NP * RO, 0:16, 0:128] = jnp.concatenate([after, after], axis=0).astype(BF16)
            start_piece(t2 + LEAD, 1, 1)

    half = D // 2
    small = [pltpu.make_async_copy(x_hbm, xb_ref, wsem.at[0]),
             pltpu.make_async_copy(wr_hbm, wrb, wsem.at[1])]
    big = [pltpu.make_async_copy(wq_hbm, wq_raw, wsem.at[2]),
           pltpu.make_async_copy(wg_hbm, wg_raw, wsem.at[3]),
           pltpu.make_async_copy(wu_hbm.at[pl.ds(0, half)], wu_raw.at[pl.ds(0, half)], wsem.at[4])]
    for cp in big:
        cp.start(priority=1)
    for cp in small:
        cp.start()
    spin_ref[...] = jnp.zeros(spin_ref.shape, F32)

    inject = [(wo_hbm, wo_raw, 0, 48, HD // 48, 5), (wd_hbm, wd_raw, 0, 48, F // 48, 6),
              (wu_hbm, wu_raw, half, 16, half // 16, 7)]
    for src, dst, row0, rows, n, sem in inject:
        def body(i, c, src=src, dst=dst, row0=row0, rows=rows, sem=sem):
            r = pl.multiple_of(row0 + i * rows, 8)
            pltpu.make_async_copy(src.at[pl.ds(r, rows)], dst.at[pl.ds(r, rows)], wsem.at[sem]).start()
            spin(cfg["WSPIN"])
            return c
        lax.fori_loop(0, n, body, 0)
        if dst is wo_raw:
            for i in range(LA):
                start_piece(i, 0)

    def lead_in(h, c):
        start_piece(h >> 1, 1, h & 1)
        spin(cfg["LSPIN"])
        return c

    lax.fori_loop(0, 2 * (LEAD + 1), lead_in, 0)
    for cp in small:
        cp.wait()
    state[...] = jnp.concatenate([xb_ref[...].astype(F32), jnp.zeros((8 - B, D), F32)], axis=0)
    for src, dst, row0, rows, n, sem in inject:
        view = dst.at[pl.ds(row0, rows * n)]
        pltpu.make_async_copy(view, view, wsem.at[sem]).wait()
    for cp in big:
        cp.wait()

    NRP = D // 16

    def repack(h, c):
        full_tick(h)
        r = pl.multiple_of(h * 16, 16)
        r2 = pl.multiple_of(h * 8, 8)
        wxp[pl.ds(r2, 8), 0:HD] = _u32(wq_raw[pl.ds(r, 16), :])
        for n, pos in enumerate(cfg["VQ"]):
            wqf[pl.ds(r, 16), n * PD:(n + 1) * PD] = (
                wq_raw[pl.ds(r, 16), order[pos] * PD:(order[pos] + 1) * PD].astype(F32))
        g = wg_raw[pl.ds(r, 16), :]
        u = wu_raw[pl.ds(r, 16), :]
        gu = jnp.concatenate([w[:, i * 128:(i + 1) * 128] for i in range(NH) for w in (g, u)], axis=1)
        wxp[pl.ds(r2, 8), HD:HD + 2 * F] = _u32(gu)
        wguf[pl.ds(r, 16), :] = gu[:, (NH - NV) * 256:].astype(F32)
        for n, pos in enumerate(cfg["VO"]):
            ro = pl.multiple_of(jnp.minimum(r, PD - 16), 16)
            wof[pl.ds(n * PD + ro, 16), :] = wo_raw[pl.ds(order[pos] * PD + ro, 16), :].astype(F32)
        nd = 16 if ND * 128 <= D else 32
        rd = pl.multiple_of(jnp.minimum(h * nd, ND * 128 - nd), 16)
        wdf[pl.ds(rd, nd), :] = wd_raw[pl.ds(rd, nd), :].astype(F32)
        for src, packed, n in ((wo_raw, wop, 160), (wd_raw, wdp, 48)):
            r = pl.multiple_of(jnp.minimum(h * n, src.shape[0] - n), 16)
            packed[pl.ds(pl.multiple_of(r >> 1, 8), n // 2), :] = _u32(src[pl.ds(r, n), :])
        return c

    lax.fori_loop(0, NRP, repack, 0)

    NCS = (HD + 2 * F) // 768

    def colsum(i, c):
        full_tick(NRP + i)
        c0 = pl.multiple_of(i * 768, 128)
        cs[:, pl.ds(c0, 768)] = _dot(jnp.ones((8, D), BF16), _bf(wxp[:, pl.ds(c0, 768)]))
        return c

    lax.fori_loop(0, NCS, colsum, 0)
    t0 = jnp.int32(NRP + NCS)

    never = spin_ref[...] < -1.0

    def xproj(xb, m, scale, c0, n):
        y = _dot(xb, _bf(wxp[:, pl.ds(c0, n)])) - m * cs[:, pl.ds(c0, n)]
        return y if scale is None else y * scale

    def qproj(xb, m, qscale, k):
        return xproj(xb, m, qscale, k * PD if isinstance(k, int) else pl.multiple_of(k * PD, 128), PD)

    def oproj(ob, k):
        r0 = pl.multiple_of(k * DH, DH) if not isinstance(k, int) else k * DH
        return _dot(ob, _bf(wop[pl.ds(r0, DH), :]))

    def kload(k):
        return [_bf(kp[pl.ds(k * RO + 2 * i, 2)].reshape(64, W)) for i in range(3)]

    def vgroup(slot, k, o, r):
        return lambda: kv[1 + slot, k * RO + o, pl.ds(r * 8, 8), :].astype(F32)

    def pair_groups(slot, k, pe, po):
        return [(vgroup(slot, k, g // RI, g % RI), pe if g < DH // 8 else po) for g in range(PD // 8)]

    def vpu_matvec(xr, w_ref, nadd, per_step=1, tok=None, rot=0):
        nu = xr.shape[1] // 128
        xcol = [jnp.concatenate([xr[:, u * 128:(u + 1) * 128]] * 16, axis=0).T for u in range(nu)]
        seq = [(u, i) for u0 in range(0, nu, 2) for i in range(16) for u in range(u0, min(u0 + 2, nu))]
        accs = [None] * per_step
        for n in range(0, len(seq), per_step):
            if tok is not None:
                for _ in range(nadd):
                    tok = tok + 1.0
            for a, (u, i) in enumerate(seq[n:n + per_step]):
                col = xcol[u][i * 8:i * 8 + 8]
                if tok is not None:
                    col = jnp.where(never, tok, col)
                y = w_ref[u * 128 + i * 8:u * 128 + i * 8 + 8, :] * _tile(col, w_ref.shape[1] // 128)
                accs[a] = y if accs[a] is None else accs[a] + y
            c = (n // per_step * rot) % (per_step * (w_ref.shape[1] // 128))
            tok = accs[c % per_step][:, c // per_step * 128:(c // per_step + 1) * 128]
        return functools.reduce(jnp.add, accs), tok

    def act(gu):
        g = gu[:, 0:128]
        return (g * _sigmoid(g) * gu[:, 128:256]).astype(BF16)

    def ffn_res(x, xc, rstd):
        wr = wrb[...].astype(F32)
        wr = jnp.concatenate([jnp.broadcast_to(wr[t:t + 1, :], (8, 128)) for t in range(D // 128)], axis=1)
        return x + xc * rstd, _round(_sigmoid(_round(jnp.sum(xc * wr, axis=1, keepdims=True) * rstd)))

    def ffn(x, f):
        nv, nd = cfg["NV"][f], cfg["ND"][f]
        nm = NH - nv
        xb, xr, m, xc, rstd = _ln_parts(x)
        hs = [act(xproj(xb, m, rstd, HD + i * 256, 256)) for i in range(nm)]
        gu, tok = vpu_matvec(xr, wguf.at[:, (NV - nv) * 256:], cfg["TOK"][f], rot=cfg["ROT"][0])
        gu = (_rowsum_all(gu) - m * cs[:, HD + nm * 256:]) * rstd
        hs += [act(gu[:, i * 256:(i + 1) * 256]) for i in range(nv)]
        y = None
        late = list(range(nm - cfg["DLATE"][f], nm))
        for i in [i for i in range(nd, NH) if i not in late] + late:
            yi = _dot(hs[i], _bf(wdp[i * 64:(i + 1) * 64, :]))
            y = yi if y is None else y + yi
        yv, _ = vpu_matvec(jnp.concatenate(hs[:nd], axis=1).astype(F32), wdf, cfg["DTOK"][f], cfg["DPER"][f], tok,
                           cfg["ROT"][1])
        y = y + _rowsum_all(yv)
        res, gate = ffn_res(xr, xc, rstd)
        return res + y * gate

    NFT = NH // 2 + 1

    def ffn_ticked(x, t):
        def body(i, carry):
            h, y, _ = carry
            full_tick(t + i)
            xb, xr, m, xc, rstd = _ln_parts(x)
            c0 = pl.multiple_of(HD + jnp.minimum(i, NFT - 2) * 512, 128)
            gu = xproj(xb, m, rstd, c0, 512)
            r0 = pl.multiple_of(jnp.maximum(i - 1, 0) * 128, 128)
            y = y + _dot(h, _bf(wdp[pl.ds(r0, 128), :]))
            res, gate = ffn_res(xr, xc, rstd)
            return jnp.concatenate([act(gu[:, 0:256]), act(gu[:, 256:512])], axis=1), y, res + y * gate

        return lax.fori_loop(0, NFT, body, (jnp.zeros((8, 256), BF16), jnp.zeros((8, D), F32), x))[2]

    NHP = 2 * B - 1

    def half_period(hp, t):
        b = hp >> 1
        slot = b & 1
        first = (hp & 1) == 0
        vbase = jnp.where(first, b * TPP + (NP + 1) * TPC, -TPP)

        tr = jnp.where(first, jnp.maximum(t, b * TPP + cfg["KRP"]), t)
        lax.fori_loop(t, tr, spin_tick, 0)

        def k_repack(h, c):
            def work():
                o0 = (h - 2 * tr) * 4
                kp[pl.ds(o0, 4)] = _u32(kv[0, pl.ds(o0, 4)].reshape(4 * 64, W)).reshape(4, 32, W)

            half_tick(h, LEAD + 1, LA, work, cfg["KSPIN"], True)
            return c

        t = jnp.where(first, tr + NP * RO // 8, t)
        lax.fori_loop(2 * tr, 2 * t, k_repack, 0)

        xb, x, m, _, rstd = _ln_parts(jnp.broadcast_to(state[pl.ds(b, 1), :], (8, D)))
        qscale = rstd * SCALE

        def step(j, carry):
            t, q, se, so, pe, po, inv, o, out = carry
            kv_ = jnp.maximum(j - 3, 0)
            t = advance(t, vbase + kv_ * TPC)
            se_n, so_n = _scores(q, kload(jnp.clip(j - 1, 0, NP - 1)))
            q_n = qproj(xb, m, qscale, jnp.minimum(j, NP - 1))
            out = out + oproj(o, jnp.maximum(j - 4, 0))
            pe_n, po_n, inv_n = _softmax_pair(se, so)
            acc = _pv(pair_groups(slot, kv_, pe, po),
                      {cfg["PVMID"][0]: lambda: mid(t, 0), cfg["PVMID"][1]: lambda: mid(t, 1)})
            mid(t, 2, q_n[:, 256:384])
            o_n = jnp.where(j >= 3, _lane_reduce_t(acc) * inv, 0.0).astype(BF16)
            return t, q_n, se_n, so_n, pe_n, po_n, inv_n, o_n, out

        zw = (lax.broadcasted_iota(I32, (8, W), 0) + lax.broadcasted_iota(I32, (8, W), 1)).astype(F32) * (1.0 / W)
        zp = zw[:, :PD]
        init = (t, zp, zw, zw, zw, zw, zp, jnp.zeros((8, PD), BF16), jnp.zeros((8, D), F32))
        last = hp == NHP - 1
        t, q, se, so, pe, po, inv, o, out = lax.fori_loop(0, jnp.where(last, NP, NP + 2), step, init)
        t2 = jnp.maximum(t + 2, vbase + (NP - 1) * TPC)

        @pl.when(last)
        def _():
            c_s[0] = se
            c_s[1] = so
            c_p[0] = pe
            c_p[1] = po
            c_o[0] = q
            c_o[1] = inv
            c_o[2] = o.astype(F32)
            c_out[...] = out

        @pl.when(jnp.logical_not(last))
        def _():
            advance(t, t2)
            y = out + oproj(o, NP - 2)
            acc = _pv(pair_groups(slot, NP - 1, pe, po), {24: lambda: mid(t2, 0), 45: lambda: mid(t2, 1)})
            olast = _lane_reduce_t(acc) * inv
            mid(t2, 2, olast[:, 0:128])
            olast = olast.astype(BF16)
            full_tick(t2)
            y = y + oproj(olast, NP - 1)
            state[pl.ds(b, 1), :] = ffn_ticked(x + _rowsum_all(y), t2 + 1)[0:1]

        return t2 + 1 + NFT

    lax.fori_loop(0, NHP, half_period, t0)

    slot = (B - 1) % 2
    ka, kb = NP - 2, NP - 1

    def wo_rows(runs):
        return _bf(jnp.concatenate(
            [wop[(k * PD + o * 64 + r * 8) // 2:(k * PD + o * 64 + (r + n) * 8) // 2, :] for k, o, r, n in runs],
            axis=0))

    def run_groups(runs, ps):
        return [(vgroup(slot, k, o, r + i), ps[k][0 if o < RO // 2 else 1]) for k, o, r, n in runs for i in range(n)]

    def normalised(pe, po, inv):
        return pe * _tile(inv[:, 0:128], NL), po * _tile(inv[:, 256:384], NL)

    def pv_o_vpu(runs):
        w = wo_rows(runs).astype(F32)
        return functools.reduce(jnp.add, [
            w[i * 8:(i + 1) * 8] * jnp.sum(_fold(vload() * p, jnp.add), axis=1, keepdims=True)
            for i, (vload, p) in enumerate(run_groups(runs, ps))])

    kc = NP - 3
    for i in range(NTICK - 3 * TPC, NTICK - TPC):
        wait_piece(i, 1)
    se, so = _scores(c_o[0], kload(kb))
    out = c_out[...] + oproj(c_o[2].astype(BF16), NP - 4)
    ps = {kc: normalised(c_p[0], c_p[1], c_o[1]), ka: normalised(*_softmax_pair(c_s[0], c_s[1]))}
    runs = [(k, o, TPC, TPC) for k in (kc, ka) for o in range(RO)]
    o = _lane_reduce_t(_pv(run_groups(runs, ps))).astype(BF16)
    ps[kb] = normalised(*_softmax_pair(se, so))

    for i in range(NTICK - 3 * TPC, NTICK - 2 * TPC):
        wait_piece(i, 0)
    for i in range(NTICK - TPC, NTICK):
        wait_piece(i, 1)
    out = out + _dot(o, wo_rows(runs))
    runs0 = [(kc, o, 0, TPC) for o in range(RO)] + [(kb, o, TPC, TPC) for o in range(RO)]
    o0 = _lane_reduce_t(_pv(run_groups(runs0, ps))).astype(BF16)

    for i in range(NTICK - 2 * TPC, NTICK - TPC):
        wait_piece(i, 0)
    out = out + _dot(o0, wo_rows(runs0))
    runs1 = [(ka, o, 0, TPC) for o in range(RO)]
    acc = [_fold(vload() * p, jnp.add) for vload, p in run_groups(runs1, ps)]
    zero = [jnp.zeros((8, 128), F32)] * 4
    o1 = _lane_reduce_t(jnp.concatenate(acc[:12] + zero + acc[12:] + zero, axis=0)).astype(BF16)

    for i in range(NTICK - TPC, NTICK - 2):
        wait_piece(i, 0)
    out = out + _dot(o1, wo_rows(runs1[:3] + runs1[:1] + runs1[3:] + runs1[:1]))
    out = out + pv_o_vpu([(kb, o, 0, 2) for o in range(RO)])

    for i in range(NTICK - 2, NTICK):
        wait_piece(i, 0)
    out = out + pv_o_vpu([(kb, o, 2, 2) for o in range(RO)])
    x = jnp.broadcast_to(state[B - 1:B, :], (8, D)) + _rowsum_all(out)

    def attn_fast(x):
        xb, xr, m, _, rstd = _ln_parts(x)
        qscale = rstd * SCALE
        q, sc, ps, os_, deadline, outv = {}, {}, {}, {}, {}, []
        invs = {}

        def get_o(pos):
            o = os_.pop(pos) * invs.pop(pos)
            return (_rowsum_all(o) if pos in cfg["VO"] else o).astype(BF16)

        out = None
        qv = _rowsum_all(vpu_matvec(xr, wqf, cfg["QTOK"], rot=cfg["ROT"][2])[0])
        for n, pos in enumerate(cfg["VQ"]):
            k = order[pos]
            q[pos] = (qv[:, n * PD:(n + 1) * PD] - m * cs[:, k * PD:(k + 1) * PD]) * qscale
        qm = [pos for pos in range(NP) if pos not in cfg["VQ"]]
        om = [pos for pos in range(NP) if pos not in cfg["VO"]]

        def vpu_stage(s):
            if 0 <= s + 1 < NP:
                ps[s + 1] = _softmax_pair(*sc.pop(s + 1), None if s + 1 >= cfg["NLS"] else qscale, bcast=True)
            if 0 <= s < NP:
                pe, po, invs[s] = ps.pop(s)
                k = order[s]
                groups = pair_groups(slot, k, pe, po)
                if k < VF:
                    groups = [(functools.partial(lambda g: vf[k * RO + g // RI, pl.ds((g % RI) * 8, 8), :], g), p)
                              for g, (_, p) in enumerate(groups)]
                acc = _pv(groups)
                os_[s] = _lane_reduce_t(acc)
                for n, (tpos, tg, nadd, per, dl) in enumerate(cfg["VOT"]):
                    if tpos == s:
                        y, tok = vpu_matvec(get_o(cfg["VO"][n]).astype(F32), wof.at[n * PD:(n + 1) * PD], nadd, per,
                                            acc[tg * 8:tg * 8 + 8], cfg["ROT"][3])
                        outv.append(y)
                        if dl:
                            deadline[s + dl + 2] = tok

        ns, nv = 0, -1
        for op in cfg["PROG"]:
            if op == "q":
                pos = qm.pop(0)
                q[pos] = qproj(xb, m, qscale if pos >= cfg["NLS"] else None, order[pos])
            elif op == "s":
                qq = q.pop(ns)
                if ns in deadline:
                    qq = jnp.concatenate([jnp.where(never, deadline.pop(ns), qq[:, 0:128]), qq[:, 128:]], axis=1)
                sc[ns] = _scores(qq, kload(order[ns]))
                ns += 1
            elif op == "o":
                pos = om.pop(0)
                y = oproj(get_o(pos), order[pos])
                out = y if out is None else out + y
            else:
                vpu_stage(nv)
                nv += 1
        out = functools.reduce(jnp.add, [out] + outv)
        return xr + _rowsum_all(out)

    x = ffn(attn_fast(ffn(x, 0)), 1)
    row = lax.broadcasted_iota(I32, (8, D), 0)
    o_ref[...] = jnp.where(row == B - 1, x, state[...])[0:B].astype(o_ref.dtype)


def _call(cfg, A_x, A_k_cache, A_v_cache, A_wq, A_wo, B_w_r, B_w_gate, B_w_up, B_w_down):
    kt = jnp.swapaxes(A_k_cache, 2, 3).reshape(B, NP * RO, RI * 8, SK)
    vt = jnp.swapaxes(A_v_cache, 2, 3).reshape(B, NP * RO, RI * 8, SK)
    out = pl.pallas_call(
        functools.partial(_kernel, cfg=cfg),
        out_shape=jax.ShapeDtypeStruct((B, D), BF16),
        in_specs=[pl.BlockSpec(memory_space=pl.ANY)] * 9,
        out_specs=pl.BlockSpec(memory_space=pltpu.VMEM),
        scratch_shapes=[
            pltpu.VMEM((3, NP * RO + 1, RI * 8, W), BF16),
            pltpu.VMEM((VF * RO, RI * 8, W), F32),
            pltpu.VMEM((NP * RO, RI * 4, W), U32),
            pltpu.VMEM((D, HD), BF16),
            pltpu.VMEM((HD, D), BF16),
            pltpu.VMEM((D, F), BF16),
            pltpu.VMEM((D, F), BF16),
            pltpu.VMEM((F, D), BF16),
            pltpu.VMEM((D // 2, HD + 2 * F), U32),
            pltpu.VMEM((HD // 2, D), U32),
            pltpu.VMEM((F // 2, D), U32),
            pltpu.VMEM((D, max(cfg["NV"]) * 256), F32),
            pltpu.VMEM((D, len(cfg["VQ"]) * PD), F32),
            pltpu.VMEM((max(cfg["ND"]) * 128, D), F32),
            pltpu.VMEM((len(cfg["VO"]) * PD, D), F32),
            pltpu.VMEM((8, HD + 2 * F), F32),
            pltpu.VMEM((B, D), BF16),
            pltpu.VMEM((D // 128, 128), BF16),
            pltpu.VMEM((8, D), F32),
            pltpu.VMEM((8, 128), F32),
            pltpu.VMEM((2, 8, W), F32),
            pltpu.VMEM((2, 8, W), F32),
            pltpu.VMEM((3, 8, PD), F32),
            pltpu.VMEM((8, D), F32),
            pltpu.SemaphoreType.DMA((2, RING)),
            pltpu.SemaphoreType.DMA((8,)),
        ],
        compiler_params=pltpu.CompilerParams(vmem_limit_bytes=126 * 1024 * 1024,
                                             disable_bounds_checks=True,
                                             disable_semaphore_checks=True),
        name="fused_decode",
    )(A_x.reshape(B, D), kt, vt, A_wq, A_wo, B_w_r.reshape(D // 128, 128), B_w_gate, B_w_up, B_w_down)
    return out.reshape(B, 1, D)


@jax.jit
def pallas_interleave_layers__sliding_block_cached__moe_arch_mod__decode_kernel(
    A_x: jax.Array,
    A_k_cache: jax.Array,
    A_v_cache: jax.Array,
    A_wq: jax.Array,
    A_wo: jax.Array,
    B_x: jax.Array,
    B_w_r: jax.Array,
    B_w_gate: jax.Array,
    B_w_up: jax.Array,
    B_w_down: jax.Array,
):
    del B_x
    return _call(CFG, A_x, A_k_cache, A_v_cache, A_wq, A_wo, B_w_r, B_w_gate, B_w_up, B_w_down)
```

```python
import functools

import jax
import jax.numpy as jnp
from jax import lax
import jax.experimental.pallas as pl
import jax.experimental.pallas.tpu as pltpu

F32 = jnp.float32
BF16 = jnp.bfloat16
U32 = jnp.uint32
I32 = jnp.int32

B, D, H, DH, SK, F = 4, 640, 32, 192, 4096, 1536
W = min(4096, max(256, SK // 4))
NP = H // 2
PD = 2 * DH
HD = H * DH
NL = W // 128
NH = F // 128
EPS = 1e-5
SCALE = DH ** -0.5 * 1.4426950408889634

RI = 8
RO = PD // (8 * RI)
TPC = RI // 2
TPP = 2 * NP * TPC
NTICK = B * TPP
RING = 32
VF = 12

CFG = dict(
    LA=23,
    LEAD=11,
    KRP=54,
    PVMID=(21, 45),
    SPIN=(1, 50),
    WSPIN=(1, 45),
    LSPIN=(1, 20),
    KSPIN=(1, 20),
    HSPIN=(1, 8),
    RSPIN=(1, 20),
    NV=(3, 4),
    ND=(5, 5),
    DLATE=(0, 3),
    TOK=(0, 0),
    DTOK=(2, 2),
    DPER=(2, 3),
    QTOK=0,
    ROT=(1, 1, 3, 0),
    RAWPOS=(0, 2, 4, 10),
    PROG="qqsqs.s.qqs.qs.qqos.s.qqs.s.qs.qso.qso.s.oso.so.s...ooooooo",
    NLS=2,
    VQ=(3, 4, 5),
    VO=(1, 0, 8),
    VOT=((14, 0, 0, 3, 0), (4, 16, 0, 2, 0), (11, 32, 0, 3, 2)),
)


def _order(cfg):
    order = list(range(VF))
    for pos, k in zip(sorted(cfg["RAWPOS"]), range(VF, NP)):
        order.insert(pos, k)
    return order


def _rowsum_all(x):
    x = x + pltpu.roll(x, 4, 0)
    x = x + pltpu.roll(x, 2, 0)
    return x + pltpu.roll(x, 1, 0)


def _bf(x):
    return pltpu.bitcast(x, BF16)


def _u32(x):
    return pltpu.bitcast(x, U32)


def _dot(a, b):
    return jnp.dot(a, b, preferred_element_type=F32)


def _sigmoid(x):
    return pl.reciprocal(1.0 + jnp.exp(-x), approx=True)


def _round(x):
    return x.astype(BF16).astype(F32)


def _ln_parts(x):
    xb = x.astype(BF16)
    xr = xb.astype(F32)
    m = jnp.sum(xr, axis=1, keepdims=True) * (1.0 / D)
    xc = xr - m
    v = jnp.sum(xc * xc, axis=1, keepdims=True) * (1.0 / D)
    m = _round(m)
    v = _round(_round(v) + EPS)
    return xb, xr, m, xr - m, pl.reciprocal(_round(v * lax.rsqrt(v)), approx=True)


def _scores(q, kk):
    lane = lax.broadcasted_iota(I32, (8, 128), 1)
    q0 = q[:, 0:128].astype(BF16)
    qm = q[:, 128:256]
    q2 = q[:, 256:384].astype(BF16)
    mid = jnp.concatenate([jnp.where(lane < 64, qm, 0.0), jnp.where(lane >= 64, qm, 0.0)],
                          axis=0).astype(BF16)
    r0 = _dot(q0, kk[0])
    rm = _dot(mid, kk[1])
    r2 = _dot(q2, kk[2])
    return r0 + rm[0:8], rm[8:16] + r2


def _fold(x, op):
    r = x[:, 0:128]
    for t in range(1, x.shape[1] // 128):
        r = op(r, x[:, t * 128:(t + 1) * 128])
    return r


def _tile(x, n):
    return jnp.concatenate([x] * n, axis=1)


def _softmax_pair(se, so, c=None, bcast=False):
    row = lax.broadcasted_iota(I32, (8, 128), 0)
    top = row < 4

    def split(c):
        c = jnp.broadcast_to(c, (8, 128))
        r = pltpu.roll(c, 4, 0)
        return jnp.where(top, c, r), jnp.where(top, r, c)

    m = jnp.max(jnp.where(top, _fold(se, jnp.maximum), _fold(so, jnp.maximum)), axis=1, keepdims=True)
    me, mo = split(m)
    de, do = se - _tile(me, NL), so - _tile(mo, NL)
    if c is not None:
        de, do = de * c, do * c
    pe, po = jnp.exp2(de), jnp.exp2(do)
    le, lo = _fold(pe, jnp.add), _fold(po, jnp.add)
    if bcast:
        l = jnp.sum(jnp.where(row >= 1, lo, le), axis=1, keepdims=True)
        r = jnp.broadcast_to(pl.reciprocal(l, approx=True), (8, 128))
        ie, io = [jnp.broadcast_to(r[i:i + 1], (8, 128)) for i in range(2)]
    else:
        ie, io = split(pl.reciprocal(jnp.sum(jnp.where(top, le, lo), axis=1, keepdims=True), approx=True))
    lane = lax.broadcasted_iota(I32, (8, 128), 1)
    return pe, po, jnp.concatenate([ie, jnp.where(lane < 64, ie, io), io], axis=1)


def _pv(groups, hooks=None):
    nb = len(groups) // 16
    accs = {}
    for n, g in enumerate(16 * blk + i for i in range(16) for blk in range(nb)):
        if hooks and n in hooks:
            hooks[n]()
        vload, p = groups[g]
        accs[g] = _fold(vload() * p, jnp.add)
    return jnp.concatenate([accs[g] for g in range(len(groups))], axis=0)


def _lane_reduce_t(acc):
    at = acc.T
    s = at[0:8]
    for i in range(1, 16):
        s = s + at[8 * i:8 * i + 8]
    return s


def _kernel(x_hbm, kt_hbm, vt_hbm, wq_hbm, wo_hbm, wr_hbm, wg_hbm, wu_hbm, wd_hbm,
            o_ref,
            kv, vf, kp, wq_raw, wo_raw, wg_raw, wu_raw, wd_raw, wxp, wop, wdp, wguf, wqf, wdf, wof, cs,
            xb_ref, wrb, state, spin_ref, c_s, c_p, c_o, c_out,
            sems, wsem, *, cfg):
    LA, LEAD, NV, ND = cfg["LA"], cfg["LEAD"], max(cfg["NV"]), max(cfg["ND"])
    order = _order(cfg)

    def piece(i, s):
        q, pair, w, b = i & (TPC - 1), (i >> 2) & (NP - 1), (i >> 6) & 1, i >> 7
        r0 = (q + s * TPC) * 8
        if not isinstance(i, int):
            r0 = pl.multiple_of(r0, 8)
        return pair, w, b, w * (1 + (b & 1)), i & (RING - 1), r0

    def start_piece(i, s, hf=None):
        pair, w, b, plane, ring, r0 = piece(i, s)
        osl = pl.ds(pair * RO, RO) if hf is None else pl.ds(pair * RO + hf * (RO // 2), RO // 2)

        def go(ww):
            src = vt_hbm if ww else kt_hbm
            pltpu.make_async_copy(src.at[b, osl, pl.ds(r0, 8), pl.ds(SK - W, W)],
                                  kv.at[plane, osl, pl.ds(r0, 8), :],
                                  sems.at[s, ring]).start(priority=1 - s)

        if isinstance(i, int):
            go(w)
        else:
            for ww in range(2):
                pl.when(jnp.logical_and(w == ww, i < NTICK))(functools.partial(go, ww))

    def wait_piece(i, s):
        pair, w, b, plane, ring, r0 = piece(i, s)
        view = kv.at[plane, pl.ds(pair * RO, RO), pl.ds(r0, 8), :]
        pltpu.make_async_copy(view, view, sems.at[s, ring]).wait()

    def wait_tick(i):
        wait_piece(i, 0)
        wait_piece(i, 1)

    def delay(v, n):
        lane = lax.broadcasted_iota(I32, v.shape, 1).astype(F32)
        for _ in range(n[0]):
            v = jnp.max(v, axis=1, keepdims=True) * 0.5 + lane
        for _ in range(n[1] // 2):
            v = v * 0.5
            v = v + lane
        return v

    def spin(n):
        spin_ref[...] = delay(spin_ref[...], n)

    def full_tick(i):
        wait_tick(i)
        start_piece(i + LEAD + 1, 1)
        start_piece(i + LA, 0)

    def spin_tick(i, c):
        full_tick(i)
        spin(cfg["SPIN"])
        return c

    def half_tick(h, lead, la, work, sp, top):
        i = h >> 1
        pl.when((h & 1) == 0)(lambda: wait_tick(i))
        if top:
            start_piece(i + lead, 1, h & 1)
        work()
        spin(sp)
        if not top:
            start_piece(i + lead, 1, h & 1)
        start_piece(jnp.where((h & 1) == 1, i + la, NTICK), 0)

    def idle_half(h, c):
        def work():
            n = (((h >> 3) & (NP - 1)) - 4) * 4 + (h & 7) - 2
            o0 = jnp.minimum(n * 2, VF * RO - 2)
            vf[pl.ds(o0, 2)] = kv[1 + ((h >> 8) & 1), pl.ds(o0, 2)].astype(F32)

        half_tick(h, LEAD, LA - 1, work, cfg["HSPIN"], False)
        return c

    def advance(t, need):
        t2 = jnp.maximum(t + 2, need)
        wait_tick(t)
        lax.fori_loop(2 * t + 2, 2 * t2 - 2, idle_half, 0)
        wait_tick(t2 - 1)
        start_piece(t2 - 1 + LEAD, 1, 0)
        return t2

    def mid(t2, n, after=None):
        if n == 0:
            start_piece(t2 - 1 + LEAD, 1, 1)
        if n == 1:
            start_piece(t2 + LEAD, 1, 0)
            start_piece(t2 - 2 + LA, 0)
            start_piece(t2 - 1 + LA, 0)
        if n == 2:
            pin_after(after)
            start_piece(t2 + LEAD, 1, 1)

    def pin_after(v):
        kv[0, NP * RO, 0:16, 0:128] = jnp.concatenate([v, v], axis=0).astype(BF16)

    def pin_before(x):
        spare = kv[0, NP * RO, 0:8, 0:128].astype(F32)
        x0 = jnp.where(spin_ref[...] < -1.0, spare, x[:, 0:128])
        return x0 if x.shape[1] == 128 else jnp.concatenate([x0, x[:, 128:]], axis=1)

    def split_tick(i, x):
        wait_tick(i)
        start_piece(i + LEAD + 1, 1, 0)

        def second(after):
            pin_after(after)
            start_piece(i + LEAD + 1, 1, 1)
            start_piece(i + LA, 0)

        return pin_before(x), second

    half = D // 2
    small = [pltpu.make_async_copy(x_hbm, xb_ref, wsem.at[0]),
             pltpu.make_async_copy(wr_hbm, wrb, wsem.at[1])]
    big = [pltpu.make_async_copy(wq_hbm, wq_raw, wsem.at[2]),
           pltpu.make_async_copy(wg_hbm, wg_raw, wsem.at[3]),
           pltpu.make_async_copy(wu_hbm.at[pl.ds(0, half)], wu_raw.at[pl.ds(0, half)], wsem.at[4])]
    for cp in big:
        cp.start(priority=1)
    for cp in small:
        cp.start()
    spin_ref[...] = jnp.zeros(spin_ref.shape, F32)
    pin_after(jnp.zeros((8, 128), F32))

    inject = [(wo_hbm, wo_raw, 0, 48, HD // 48, 5), (wd_hbm, wd_raw, 0, 48, F // 48, 6),
              (wu_hbm, wu_raw, half, 16, half // 16, 7)]
    for src, dst, row0, rows, n, sem in inject:
        def body(i, c, src=src, dst=dst, row0=row0, rows=rows, sem=sem):
            r = pl.multiple_of(row0 + i * rows, 8)
            pltpu.make_async_copy(src.at[pl.ds(r, rows)], dst.at[pl.ds(r, rows)], wsem.at[sem]).start()
            spin(cfg["WSPIN"])
            return c
        lax.fori_loop(0, n, body, 0)
        if dst is wo_raw:
            for i in range(LA):
                start_piece(i, 0)

    def lead_in(h, c):
        start_piece(h >> 1, 1, h & 1)
        spin(cfg["LSPIN"])
        return c

    lax.fori_loop(0, 2 * (LEAD + 1), lead_in, 0)
    for cp in small:
        cp.wait()
    state[...] = jnp.concatenate([xb_ref[...].astype(F32), jnp.zeros((8 - B, D), F32)], axis=0)
    for src, dst, row0, rows, n, sem in inject:
        view = dst.at[pl.ds(row0, rows * n)]
        pltpu.make_async_copy(view, view, wsem.at[sem]).wait()
    for cp in big:
        cp.wait()

    NRP = D // 16

    def repack(h, c):
        v, second = split_tick(h, spin_ref[...])
        second(delay(v, cfg["RSPIN"]))
        r = pl.multiple_of(h * 16, 16)
        r2 = pl.multiple_of(h * 8, 8)
        wxp[pl.ds(r2, 8), 0:HD] = _u32(wq_raw[pl.ds(r, 16), :])
        for n, pos in enumerate(cfg["VQ"]):
            wqf[pl.ds(r, 16), n * PD:(n + 1) * PD] = (
                wq_raw[pl.ds(r, 16), order[pos] * PD:(order[pos] + 1) * PD].astype(F32))
        g = wg_raw[pl.ds(r, 16), :]
        u = wu_raw[pl.ds(r, 16), :]
        gu = jnp.concatenate([w[:, i * 128:(i + 1) * 128] for i in range(NH) for w in (g, u)], axis=1)
        wxp[pl.ds(r2, 8), HD:HD + 2 * F] = _u32(gu)
        wguf[pl.ds(r, 16), :] = gu[:, (NH - NV) * 256:].astype(F32)
        for n, pos in enumerate(cfg["VO"]):
            ro = pl.multiple_of(jnp.minimum(r, PD - 16), 16)
            wof[pl.ds(n * PD + ro, 16), :] = wo_raw[pl.ds(order[pos] * PD + ro, 16), :].astype(F32)
        nd = 16 if ND * 128 <= D else 32
        rd = pl.multiple_of(jnp.minimum(h * nd, ND * 128 - nd), 16)
        wdf[pl.ds(rd, nd), :] = wd_raw[pl.ds(rd, nd), :].astype(F32)
        for src, packed, n in ((wo_raw, wop, 160), (wd_raw, wdp, 48)):
            r = pl.multiple_of(jnp.minimum(h * n, src.shape[0] - n), 16)
            packed[pl.ds(pl.multiple_of(r >> 1, 8), n // 2), :] = _u32(src[pl.ds(r, n), :])
        return c

    lax.fori_loop(0, NRP, repack, 0)

    NCS = (HD + 2 * F) // 768

    def colsum(i, c):
        ones, second = split_tick(NRP + i, jnp.ones((8, D), F32))
        c0 = pl.multiple_of(i * 768, 128)
        y = _dot(ones.astype(BF16), _bf(wxp[:, pl.ds(c0, 768)]))
        second(y[:, 0:128])
        cs[:, pl.ds(c0, 768)] = y
        return c

    lax.fori_loop(0, NCS, colsum, 0)
    t0 = jnp.int32(NRP + NCS)

    never = spin_ref[...] < -1.0

    def xproj(xb, m, scale, c0, n):
        y = _dot(xb, _bf(wxp[:, pl.ds(c0, n)])) - m * cs[:, pl.ds(c0, n)]
        return y if scale is None else y * scale

    def qproj(xb, m, qscale, k):
        return xproj(xb, m, qscale, k * PD if isinstance(k, int) else pl.multiple_of(k * PD, 128), PD)

    def oproj(ob, k):
        r0 = pl.multiple_of(k * DH, DH) if not isinstance(k, int) else k * DH
        return _dot(ob, _bf(wop[pl.ds(r0, DH), :]))

    def kload(k):
        return [_bf(kp[pl.ds(k * RO + 2 * i, 2)].reshape(64, W)) for i in range(3)]

    def vgroup(slot, k, o, r):
        return lambda: kv[1 + slot, k * RO + o, pl.ds(r * 8, 8), :].astype(F32)

    def pair_groups(slot, k, pe, po):
        return [(vgroup(slot, k, g // RI, g % RI), pe if g < DH // 8 else po) for g in range(PD // 8)]

    def vpu_matvec(xr, w_ref, nadd, per_step=1, tok=None, rot=0):
        nu = xr.shape[1] // 128
        xcol = [jnp.concatenate([xr[:, u * 128:(u + 1) * 128]] * 16, axis=0).T for u in range(nu)]
        seq = [(u, i) for u0 in range(0, nu, 2) for i in range(16) for u in range(u0, min(u0 + 2, nu))]
        accs = [None] * per_step
        for n in range(0, len(seq), per_step):
            if tok is not None:
                for _ in range(nadd):
                    tok = tok + 1.0
            for a, (u, i) in enumerate(seq[n:n + per_step]):
                col = xcol[u][i * 8:i * 8 + 8]
                if tok is not None:
                    col = jnp.where(never, tok, col)
                y = w_ref[u * 128 + i * 8:u * 128 + i * 8 + 8, :] * _tile(col, w_ref.shape[1] // 128)
                accs[a] = y if accs[a] is None else accs[a] + y
            c = (n // per_step * rot) % (per_step * (w_ref.shape[1] // 128))
            tok = accs[c % per_step][:, c // per_step * 128:(c // per_step + 1) * 128]
        return functools.reduce(jnp.add, accs), tok

    def act(gu):
        g = gu[:, 0:128]
        return (g * _sigmoid(g) * gu[:, 128:256]).astype(BF16)

    def ffn_res(x, xc, rstd):
        wr = wrb[...].astype(F32)
        wr = jnp.concatenate([jnp.broadcast_to(wr[t:t + 1, :], (8, 128)) for t in range(D // 128)], axis=1)
        return x + xc * rstd, _round(_sigmoid(_round(jnp.sum(xc * wr, axis=1, keepdims=True) * rstd)))

    def ffn(x, f):
        nv, nd = cfg["NV"][f], cfg["ND"][f]
        nm = NH - nv
        xb, xr, m, xc, rstd = _ln_parts(x)
        hs = [act(xproj(xb, m, rstd, HD + i * 256, 256)) for i in range(nm)]
        gu, tok = vpu_matvec(xr, wguf.at[:, (NV - nv) * 256:], cfg["TOK"][f], rot=cfg["ROT"][0])
        gu = (_rowsum_all(gu) - m * cs[:, HD + nm * 256:]) * rstd
        hs += [act(gu[:, i * 256:(i + 1) * 256]) for i in range(nv)]
        y = None
        late = list(range(nm - cfg["DLATE"][f], nm))
        for i in [i for i in range(nd, NH) if i not in late] + late:
            yi = _dot(hs[i], _bf(wdp[i * 64:(i + 1) * 64, :]))
            y = yi if y is None else y + yi
        yv, _ = vpu_matvec(jnp.concatenate(hs[:nd], axis=1).astype(F32), wdf, cfg["DTOK"][f], cfg["DPER"][f], tok,
                           cfg["ROT"][1])
        y = y + _rowsum_all(yv)
        res, gate = ffn_res(xr, xc, rstd)
        return res + y * gate

    NFT = NH // 2 + 1

    def ffn_ticked(x, t):
        def body(i, carry):
            h, y, _ = carry
            xx, second = split_tick(t + i, x)
            xb, xr, m, xc, rstd = _ln_parts(xx)
            second(xc[:, 0:128])
            c0 = pl.multiple_of(HD + jnp.minimum(i, NFT - 2) * 512, 128)
            gu = xproj(xb, m, rstd, c0, 512)
            r0 = pl.multiple_of(jnp.maximum(i - 1, 0) * 128, 128)
            y = y + _dot(h, _bf(wdp[pl.ds(r0, 128), :]))
            res, gate = ffn_res(xr, xc, rstd)
            return jnp.concatenate([act(gu[:, 0:256]), act(gu[:, 256:512])], axis=1), y, res + y * gate

        return lax.fori_loop(0, NFT, body, (jnp.zeros((8, 256), BF16), jnp.zeros((8, D), F32), x))[2]

    NHP = 2 * B - 1

    def half_period(hp, t):
        b = hp >> 1
        slot = b & 1
        first = (hp & 1) == 0
        vbase = jnp.where(first, b * TPP + (NP + 1) * TPC, -TPP)

        tr = jnp.where(first, jnp.maximum(t, b * TPP + cfg["KRP"]), t)
        lax.fori_loop(t, tr, spin_tick, 0)

        def k_repack(h, c):
            def work():
                o0 = (h - 2 * tr) * 4
                kp[pl.ds(o0, 4)] = _u32(kv[0, pl.ds(o0, 4)].reshape(4 * 64, W)).reshape(4, 32, W)

            half_tick(h, LEAD + 1, LA, work, cfg["KSPIN"], True)
            return c

        t = jnp.where(first, tr + NP * RO // 8, t)
        lax.fori_loop(2 * tr, 2 * t, k_repack, 0)

        xb, x, m, _, rstd = _ln_parts(jnp.broadcast_to(state[pl.ds(b, 1), :], (8, D)))
        qscale = rstd * SCALE

        def step(j, carry):
            t, q, se, so, pe, po, inv, o, out = carry
            kv_ = jnp.maximum(j - 3, 0)
            t = advance(t, vbase + kv_ * TPC)
            se_n, so_n = _scores(q, kload(jnp.clip(j - 1, 0, NP - 1)))
            q_n = qproj(xb, m, qscale, jnp.minimum(j, NP - 1))
            out = out + oproj(o, jnp.maximum(j - 4, 0))
            pe_n, po_n, inv_n = _softmax_pair(se, so)
            acc = _pv(pair_groups(slot, kv_, pe, po),
                      {cfg["PVMID"][0]: lambda: mid(t, 0), cfg["PVMID"][1]: lambda: mid(t, 1)})
            mid(t, 2, q_n[:, 256:384])
            o_n = jnp.where(j >= 3, _lane_reduce_t(acc) * inv, 0.0).astype(BF16)
            return t, q_n, se_n, so_n, pe_n, po_n, inv_n, o_n, out

        zw = (lax.broadcasted_iota(I32, (8, W), 0) + lax.broadcasted_iota(I32, (8, W), 1)).astype(F32) * (1.0 / W)
        zp = zw[:, :PD]
        init = (t, zp, zw, zw, zw, zw, zp, jnp.zeros((8, PD), BF16), jnp.zeros((8, D), F32))
        last = hp == NHP - 1
        t, q, se, so, pe, po, inv, o, out = lax.fori_loop(0, jnp.where(last, NP, NP + 2), step, init)
        t2 = jnp.maximum(t + 2, vbase + (NP - 1) * TPC)

        @pl.when(last)
        def _():
            c_s[0] = se
            c_s[1] = so
            c_p[0] = pe
            c_p[1] = po
            c_o[0] = q
            c_o[1] = inv
            c_o[2] = o.astype(F32)
            c_out[...] = out

        @pl.when(jnp.logical_not(last))
        def _():
            advance(t, t2)
            y = out + oproj(o, NP - 2)
            acc = _pv(pair_groups(slot, NP - 1, pe, po), {24: lambda: mid(t2, 0), 45: lambda: mid(t2, 1)})
            olast = _lane_reduce_t(acc) * inv
            mid(t2, 2, olast[:, 0:128])
            olast, second = split_tick(t2, olast)
            yl = oproj(olast.astype(BF16), NP - 1)
            second(yl[:, 0:128])
            y = y + yl
            state[pl.ds(b, 1), :] = ffn_ticked(x + _rowsum_all(y), t2 + 1)[0:1]

        return t2 + 1 + NFT

    lax.fori_loop(0, NHP, half_period, t0)

    slot = (B - 1) % 2
    ka, kb = NP - 2, NP - 1

    def wo_rows(runs):
        return _bf(jnp.concatenate(
            [wop[(k * PD + o * 64 + r * 8) // 2:(k * PD + o * 64 + (r + n) * 8) // 2, :] for k, o, r, n in runs],
            axis=0))

    def run_groups(runs, ps):
        return [(vgroup(slot, k, o, r + i), ps[k][0 if o < RO // 2 else 1]) for k, o, r, n in runs for i in range(n)]

    def normalised(pe, po, inv):
        return pe * _tile(inv[:, 0:128], NL), po * _tile(inv[:, 256:384], NL)

    def pv_o_vpu(runs):
        w = wo_rows(runs).astype(F32)
        return functools.reduce(jnp.add, [
            w[i * 8:(i + 1) * 8] * jnp.sum(_fold(vload() * p, jnp.add), axis=1, keepdims=True)
            for i, (vload, p) in enumerate(run_groups(runs, ps))])

    kc = NP - 3
    for i in range(NTICK - 3 * TPC, NTICK - TPC):
        wait_piece(i, 1)
    se, so = _scores(c_o[0], kload(kb))
    out = c_out[...] + oproj(c_o[2].astype(BF16), NP - 4)
    ps = {kc: normalised(c_p[0], c_p[1], c_o[1]), ka: normalised(*_softmax_pair(c_s[0], c_s[1]))}
    runs = [(k, o, TPC, TPC) for k in (kc, ka) for o in range(RO)]
    o = _lane_reduce_t(_pv(run_groups(runs, ps))).astype(BF16)
    ps[kb] = normalised(*_softmax_pair(se, so))

    for i in range(NTICK - 3 * TPC, NTICK - 2 * TPC):
        wait_piece(i, 0)
    for i in range(NTICK - TPC, NTICK):
        wait_piece(i, 1)
    out = out + _dot(o, wo_rows(runs))
    runs0 = [(kc, o, 0, TPC) for o in range(RO)] + [(kb, o, TPC, TPC) for o in range(RO)]
    o0 = _lane_reduce_t(_pv(run_groups(runs0, ps))).astype(BF16)

    for i in range(NTICK - 2 * TPC, NTICK - TPC):
        wait_piece(i, 0)
    out = out + _dot(o0, wo_rows(runs0))
    runs1 = [(ka, o, 0, TPC) for o in range(RO)]
    acc = [_fold(vload() * p, jnp.add) for vload, p in run_groups(runs1, ps)]
    zero = [jnp.zeros((8, 128), F32)] * 4
    o1 = _lane_reduce_t(jnp.concatenate(acc[:12] + zero + acc[12:] + zero, axis=0)).astype(BF16)

    for i in range(NTICK - TPC, NTICK - 2):
        wait_piece(i, 0)
    out = out + _dot(o1, wo_rows(runs1[:3] + runs1[:1] + runs1[3:] + runs1[:1]))
    out = out + pv_o_vpu([(kb, o, 0, 2) for o in range(RO)])

    for i in range(NTICK - 2, NTICK):
        wait_piece(i, 0)
    out = out + pv_o_vpu([(kb, o, 2, 2) for o in range(RO)])
    x = jnp.broadcast_to(state[B - 1:B, :], (8, D)) + _rowsum_all(out)

    def attn_fast(x):
        xb, xr, m, _, rstd = _ln_parts(x)
        qscale = rstd * SCALE
        q, sc, ps, os_, deadline, outv = {}, {}, {}, {}, {}, []
        invs = {}

        def get_o(pos):
            o = os_.pop(pos) * invs.pop(pos)
            return (_rowsum_all(o) if pos in cfg["VO"] else o).astype(BF16)

        out = None
        qv = _rowsum_all(vpu_matvec(xr, wqf, cfg["QTOK"], rot=cfg["ROT"][2])[0])
        for n, pos in enumerate(cfg["VQ"]):
            k = order[pos]
            q[pos] = (qv[:, n * PD:(n + 1) * PD] - m * cs[:, k * PD:(k + 1) * PD]) * qscale
        qm = [pos for pos in range(NP) if pos not in cfg["VQ"]]
        om = [pos for pos in range(NP) if pos not in cfg["VO"]]

        def vpu_stage(s):
            if 0 <= s + 1 < NP:
                ps[s + 1] = _softmax_pair(*sc.pop(s + 1), None if s + 1 >= cfg["NLS"] else qscale, bcast=True)
            if 0 <= s < NP:
                pe, po, invs[s] = ps.pop(s)
                k = order[s]
                groups = pair_groups(slot, k, pe, po)
                if k < VF:
                    groups = [(functools.partial(lambda g: vf[k * RO + g // RI, pl.ds((g % RI) * 8, 8), :], g), p)
                              for g, (_, p) in enumerate(groups)]
                acc = _pv(groups)
                os_[s] = _lane_reduce_t(acc)
                for n, (tpos, tg, nadd, per, dl) in enumerate(cfg["VOT"]):
                    if tpos == s:
                        y, tok = vpu_matvec(get_o(cfg["VO"][n]).astype(F32), wof.at[n * PD:(n + 1) * PD], nadd, per,
                                            acc[tg * 8:tg * 8 + 8], cfg["ROT"][3])
                        outv.append(y)
                        if dl:
                            deadline[s + dl + 2] = tok

        ns, nv = 0, -1
        for op in cfg["PROG"]:
            if op == "q":
                pos = qm.pop(0)
                q[pos] = qproj(xb, m, qscale if pos >= cfg["NLS"] else None, order[pos])
            elif op == "s":
                qq = q.pop(ns)
                if ns in deadline:
                    qq = jnp.concatenate([jnp.where(never, deadline.pop(ns), qq[:, 0:128]), qq[:, 128:]], axis=1)
                sc[ns] = _scores(qq, kload(order[ns]))
                ns += 1
            elif op == "o":
                pos = om.pop(0)
                y = oproj(get_o(pos), order[pos])
                out = y if out is None else out + y
            else:
                vpu_stage(nv)
                nv += 1
        out = functools.reduce(jnp.add, [out] + outv)
        return xr + _rowsum_all(out)

    x = ffn(attn_fast(ffn(x, 0)), 1)
    row = lax.broadcasted_iota(I32, (8, D), 0)
    o_ref[...] = jnp.where(row == B - 1, x, state[...])[0:B].astype(o_ref.dtype)


def _call(cfg, A_x, A_k_cache, A_v_cache, A_wq, A_wo, B_w_r, B_w_gate, B_w_up, B_w_down):
    kt = jnp.swapaxes(A_k_cache, 2, 3).reshape(B, NP * RO, RI * 8, SK)
    vt = jnp.swapaxes(A_v_cache, 2, 3).reshape(B, NP * RO, RI * 8, SK)
    out = pl.pallas_call(
        functools.partial(_kernel, cfg=cfg),
        out_shape=jax.ShapeDtypeStruct((B, D), BF16),
        in_specs=[pl.BlockSpec(memory_space=pl.ANY)] * 9,
        out_specs=pl.BlockSpec(memory_space=pltpu.VMEM),
        scratch_shapes=[
            pltpu.VMEM((3, NP * RO + 1, RI * 8, W), BF16),
            pltpu.VMEM((VF * RO, RI * 8, W), F32),
            pltpu.VMEM((NP * RO, RI * 4, W), U32),
            pltpu.VMEM((D, HD), BF16),
            pltpu.VMEM((HD, D), BF16),
            pltpu.VMEM((D, F), BF16),
            pltpu.VMEM((D, F), BF16),
            pltpu.VMEM((F, D), BF16),
            pltpu.VMEM((D // 2, HD + 2 * F), U32),
            pltpu.VMEM((HD // 2, D), U32),
            pltpu.VMEM((F // 2, D), U32),
            pltpu.VMEM((D, max(cfg["NV"]) * 256), F32),
            pltpu.VMEM((D, len(cfg["VQ"]) * PD), F32),
            pltpu.VMEM((max(cfg["ND"]) * 128, D), F32),
            pltpu.VMEM((len(cfg["VO"]) * PD, D), F32),
            pltpu.VMEM((8, HD + 2 * F), F32),
            pltpu.VMEM((B, D), BF16),
            pltpu.VMEM((D // 128, 128), BF16),
            pltpu.VMEM((8, D), F32),
            pltpu.VMEM((8, 128), F32),
            pltpu.VMEM((2, 8, W), F32),
            pltpu.VMEM((2, 8, W), F32),
            pltpu.VMEM((3, 8, PD), F32),
            pltpu.VMEM((8, D), F32),
            pltpu.SemaphoreType.DMA((2, RING)),
            pltpu.SemaphoreType.DMA((8,)),
        ],
        compiler_params=pltpu.CompilerParams(vmem_limit_bytes=126 * 1024 * 1024,
                                             disable_bounds_checks=True,
                                             disable_semaphore_checks=True),
        name="fused_decode",
    )(A_x.reshape(B, D), kt, vt, A_wq, A_wo, B_w_r.reshape(D // 128, 128), B_w_gate, B_w_up, B_w_down)
    return out.reshape(B, 1, D)


@jax.jit
def pallas_interleave_layers__sliding_block_cached__moe_arch_mod__decode_kernel(
    A_x: jax.Array,
    A_k_cache: jax.Array,
    A_v_cache: jax.Array,
    A_wq: jax.Array,
    A_wo: jax.Array,
    B_x: jax.Array,
    B_w_r: jax.Array,
    B_w_gate: jax.Array,
    B_w_up: jax.Array,
    B_w_down: jax.Array,
):
    del B_x
    return _call(CFG, A_x, A_k_cache, A_v_cache, A_wq, A_wo, B_w_r, B_w_gate, B_w_up, B_w_down)
```

```python
import functools

import jax
import jax.numpy as jnp
from jax import lax
import jax.experimental.pallas as pl
import jax.experimental.pallas.tpu as pltpu

F32 = jnp.float32
BF16 = jnp.bfloat16
U32 = jnp.uint32
I32 = jnp.int32

B, D, H, DH, SK, F = 4, 640, 32, 192, 4096, 1536
W = min(4096, max(256, SK // 4))
NP = H // 2
PD = 2 * DH
HD = H * DH
NL = W // 128
NH = F // 128
EPS = 1e-5
SCALE = DH ** -0.5 * 1.4426950408889634

RI = 8
RO = PD // (8 * RI)
TPC = RI // 2
TPP = 2 * NP * TPC
NTICK = B * TPP
RING = 32
VF = 12

CFG = dict(
    LA=23,
    LEAD=11,
    KRP=54,
    PVMID=(21, 45),
    SPIN=(1, 50),
    WSPIN=(1, 45),
    LSPIN=(1, 20),
    KSPIN=(1, 20),
    HSPIN=(1, 8),
    RSPIN=(1, 10),
    NV=(3, 4),
    ND=(5, 5),
    DLATE=(0, 3),
    TOK=(0, 0),
    DTOK=(2, 2),
    DPER=(2, 3),
    QTOK=0,
    ROT=(1, 1, 3, 0),
    RAWPOS=(0, 2, 4, 10),
    PROG="qqsqs.s.qqs.qs.qqos.s.qqs.s.qs.qso.qso.s.oso.so.s...ooooooo",
    NLS=2,
    VQ=(3, 4, 5),
    VO=(1, 0, 8),
    VOT=((14, 0, 0, 3, 0), (4, 16, 0, 2, 0), (11, 32, 0, 3, 2)),
)


def _order(cfg):
    order = list(range(VF))
    for pos, k in zip(sorted(cfg["RAWPOS"]), range(VF, NP)):
        order.insert(pos, k)
    return order


def _rowsum_all(x):
    x = x + pltpu.roll(x, 4, 0)
    x = x + pltpu.roll(x, 2, 0)
    return x + pltpu.roll(x, 1, 0)


def _bf(x):
    return pltpu.bitcast(x, BF16)


def _u32(x):
    return pltpu.bitcast(x, U32)


def _dot(a, b):
    return jnp.dot(a, b, preferred_element_type=F32)


def _sigmoid(x):
    return pl.reciprocal(1.0 + jnp.exp(-x), approx=True)


def _round(x):
    return x.astype(BF16).astype(F32)


def _ln_parts(x):
    xb = x.astype(BF16)
    xr = xb.astype(F32)
    m = jnp.sum(xr, axis=1, keepdims=True) * (1.0 / D)
    xc = xr - m
    v = jnp.sum(xc * xc, axis=1, keepdims=True) * (1.0 / D)
    m = _round(m)
    v = _round(_round(v) + EPS)
    return xb, xr, m, xr - m, pl.reciprocal(_round(v * lax.rsqrt(v)), approx=True)


def _scores(q, kk):
    lane = lax.broadcasted_iota(I32, (8, 128), 1)
    q0 = q[:, 0:128].astype(BF16)
    qm = q[:, 128:256]
    q2 = q[:, 256:384].astype(BF16)
    mid = jnp.concatenate([jnp.where(lane < 64, qm, 0.0), jnp.where(lane >= 64, qm, 0.0)],
                          axis=0).astype(BF16)
    r0 = _dot(q0, kk[0])
    rm = _dot(mid, kk[1])
    r2 = _dot(q2, kk[2])
    return r0 + rm[0:8], rm[8:16] + r2


def _fold(x, op):
    r = x[:, 0:128]
    for t in range(1, x.shape[1] // 128):
        r = op(r, x[:, t * 128:(t + 1) * 128])
    return r


def _tile(x, n):
    return jnp.concatenate([x] * n, axis=1)


def _softmax_pair(se, so, c=None, bcast=False):
    row = lax.broadcasted_iota(I32, (8, 128), 0)
    top = row < 4

    def split(c):
        c = jnp.broadcast_to(c, (8, 128))
        r = pltpu.roll(c, 4, 0)
        return jnp.where(top, c, r), jnp.where(top, r, c)

    m = jnp.max(jnp.where(top, _fold(se, jnp.maximum), _fold(so, jnp.maximum)), axis=1, keepdims=True)
    me, mo = split(m)
    de, do = se - _tile(me, NL), so - _tile(mo, NL)
    if c is not None:
        de, do = de * c, do * c
    pe, po = jnp.exp2(de), jnp.exp2(do)
    le, lo = _fold(pe, jnp.add), _fold(po, jnp.add)
    if bcast:
        l = jnp.sum(jnp.where(row >= 1, lo, le), axis=1, keepdims=True)
        r = jnp.broadcast_to(pl.reciprocal(l, approx=True), (8, 128))
        ie, io = [jnp.broadcast_to(r[i:i + 1], (8, 128)) for i in range(2)]
    else:
        ie, io = split(pl.reciprocal(jnp.sum(jnp.where(top, le, lo), axis=1, keepdims=True), approx=True))
    lane = lax.broadcasted_iota(I32, (8, 128), 1)
    return pe, po, jnp.concatenate([ie, jnp.where(lane < 64, ie, io), io], axis=1)


def _pv(groups, hooks=None):
    nb = len(groups) // 16
    accs = {}
    for n, g in enumerate(16 * blk + i for i in range(16) for blk in range(nb)):
        if hooks and n in hooks:
            hooks[n]()
        vload, p = groups[g]
        accs[g] = _fold(vload() * p, jnp.add)
    return jnp.concatenate([accs[g] for g in range(len(groups))], axis=0)


def _lane_reduce_t(acc):
    at = acc.T
    s = at[0:8]
    for i in range(1, 16):
        s = s + at[8 * i:8 * i + 8]
    return s


def _kernel(x_hbm, kt_hbm, vt_hbm, wq_hbm, wo_hbm, wr_hbm, wg_hbm, wu_hbm, wd_hbm,
            o_ref,
            kv, vf, kp, wq_raw, wo_raw, wg_raw, wu_raw, wd_raw, wxp, wop, wdp, wguf, wqf, wdf, wof, cs,
            xb_ref, wrb, state, spin_ref, c_s, c_p, c_o, c_out,
            sems, wsem, *, cfg):
    LA, LEAD, NV, ND = cfg["LA"], cfg["LEAD"], max(cfg["NV"]), max(cfg["ND"])
    order = _order(cfg)

    def piece(i, s):
        q, pair, w, b = i & (TPC - 1), (i >> 2) & (NP - 1), (i >> 6) & 1, i >> 7
        r0 = (q + s * TPC) * 8
        if not isinstance(i, int):
            r0 = pl.multiple_of(r0, 8)
        return pair, w, b, w * (1 + (b & 1)), i & (RING - 1), r0

    def start_piece(i, s, hf=None):
        pair, w, b, plane, ring, r0 = piece(i, s)
        osl = pl.ds(pair * RO, RO) if hf is None else pl.ds(pair * RO + hf * (RO // 2), RO // 2)

        def go(ww):
            src = vt_hbm if ww else kt_hbm
            pltpu.make_async_copy(src.at[b, osl, pl.ds(r0, 8), pl.ds(SK - W, W)],
                                  kv.at[plane, osl, pl.ds(r0, 8), :],
                                  sems.at[s, ring]).start(priority=1 - s)

        if isinstance(i, int):
            go(w)
        else:
            for ww in range(2):
                pl.when(jnp.logical_and(w == ww, i < NTICK))(functools.partial(go, ww))

    def wait_piece(i, s):
        pair, w, b, plane, ring, r0 = piece(i, s)
        view = kv.at[plane, pl.ds(pair * RO, RO), pl.ds(r0, 8), :]
        pltpu.make_async_copy(view, view, sems.at[s, ring]).wait()

    def wait_tick(i):
        wait_piece(i, 0)
        wait_piece(i, 1)

    def delay(v, n):
        lane = lax.broadcasted_iota(I32, v.shape, 1).astype(F32)
        for _ in range(n[0]):
            v = jnp.max(v, axis=1, keepdims=True) * 0.5 + lane
        for _ in range(n[1] // 2):
            v = v * 0.5
            v = v + lane
        return v

    def spin(n):
        spin_ref[...] = delay(spin_ref[...], n)

    def full_tick(i):
        wait_tick(i)
        start_piece(i + LEAD + 1, 1)
        start_piece(i + LA, 0)

    def spin_tick(i, c):
        full_tick(i)
        spin(cfg["SPIN"])
        return c

    def half_tick(h, lead, la, work, sp, top):
        i = h >> 1
        pl.when((h & 1) == 0)(lambda: wait_tick(i))
        if top:
            start_piece(i + lead, 1, h & 1)
        work()
        spin(sp)
        if not top:
            start_piece(i + lead, 1, h & 1)
        start_piece(jnp.where((h & 1) == 1, i + la, NTICK), 0)

    def idle_half(h, c):
        def work():
            n = (((h >> 3) & (NP - 1)) - 4) * 4 + (h & 7) - 2
            o0 = jnp.minimum(n * 2, VF * RO - 2)
            vf[pl.ds(o0, 2)] = kv[1 + ((h >> 8) & 1), pl.ds(o0, 2)].astype(F32)

        half_tick(h, LEAD, LA - 1, work, cfg["HSPIN"], False)
        return c

    def advance(t, need):
        t2 = jnp.maximum(t + 2, need)
        wait_tick(t)
        lax.fori_loop(2 * t + 2, 2 * t2 - 2, idle_half, 0)
        wait_tick(t2 - 1)
        start_piece(t2 - 1 + LEAD, 1, 0)
        return t2

    def mid(t2, n, after=None):
        if n == 0:
            start_piece(t2 - 1 + LEAD, 1, 1)
        if n == 1:
            start_piece(t2 + LEAD, 1, 0)
            start_piece(t2 - 2 + LA, 0)
            start_piece(t2 - 1 + LA, 0)
        if n == 2:
            pin_after(after)
            start_piece(t2 + LEAD, 1, 1)

    def pin_after(v):
        kv[0, NP * RO, 0:16, 0:128] = jnp.concatenate([v, v], axis=0).astype(BF16)

    def pin_before(x):
        spare = kv[0, NP * RO, 0:8, 0:128].astype(F32)
        x0 = jnp.where(spin_ref[...] < -1.0, spare, x[:, 0:128])
        return x0 if x.shape[1] == 128 else jnp.concatenate([x0, x[:, 128:]], axis=1)

    def split_tick(i, x):
        wait_tick(i)
        start_piece(i + LEAD + 1, 1, 0)

        def second(after):
            pin_after(after)
            start_piece(i + LEAD + 1, 1, 1)
            start_piece(i + LA, 0)

        return pin_before(x), second

    small = [pltpu.make_async_copy(x_hbm, xb_ref, wsem.at[0]),
             pltpu.make_async_copy(wr_hbm, wrb, wsem.at[1])]
    big = [pltpu.make_async_copy(wq_hbm, wq_raw, wsem.at[2]),
           pltpu.make_async_copy(wg_hbm, wg_raw, wsem.at[3]),
           pltpu.make_async_copy(wu_hbm.at[0:2], wu_raw.at[0:2], wsem.at[4])]
    for cp in big:
        cp.start(priority=1)
    for cp in small:
        cp.start()
    spin_ref[...] = jnp.zeros(spin_ref.shape, F32)
    pin_after(jnp.zeros((8, 128), F32))

    inject = [(wo_hbm, wo_raw, 5), (wd_hbm, wd_raw, 6), (wu_hbm.at[2:4], wu_raw.at[2:4], 7)]
    for src, dst, sem in inject:
        def body(i, c, src=src, dst=dst, sem=sem):
            r = pl.ds(pl.multiple_of(i * 8, 8), 8)
            pltpu.make_async_copy(src.at[:, r], dst.at[:, r], wsem.at[sem]).start()
            spin(cfg["WSPIN"])
            return c
        lax.fori_loop(0, dst.shape[1] // 8, body, 0)
        if dst is wo_raw:
            for i in range(LA):
                start_piece(i, 0)

    def lead_in(h, c):
        start_piece(h >> 1, 1, h & 1)
        spin(cfg["LSPIN"])
        return c

    lax.fori_loop(0, 2 * (LEAD + 1), lead_in, 0)
    for cp in small:
        cp.wait()
    state[...] = jnp.concatenate([xb_ref[...].astype(F32), jnp.zeros((8 - B, D), F32)], axis=0)
    for src, dst, sem in inject:
        pltpu.make_async_copy(dst, dst, wsem.at[sem]).wait()
    for cp in big:
        cp.wait()

    NRP = D // 16

    def repack(h, c):
        v, second = split_tick(h, spin_ref[...])
        second(delay(v, cfg["RSPIN"]))
        r = pl.multiple_of(h * 16, 16)
        r2 = pl.multiple_of(h * 8, 8)
        wxp[pl.ds(r2, 8), 0:HD] = _u32(wq_raw[pl.ds(r, 16), :])
        for n, pos in enumerate(cfg["VQ"]):
            wqf[pl.ds(r, 16), n * PD:(n + 1) * PD] = (
                wq_raw[pl.ds(r, 16), order[pos] * PD:(order[pos] + 1) * PD].astype(F32))
        g = wg_raw[pl.ds(r, 16), :]
        pu = (h * 205) >> 11
        u = wu_raw[pu, pl.ds(pl.multiple_of(r - pu * 160, 16), 16), :]
        gu = jnp.concatenate([w[:, i * 128:(i + 1) * 128] for i in range(NH) for w in (g, u)], axis=1)
        wxp[pl.ds(r2, 8), HD:HD + 2 * F] = _u32(gu)
        wguf[pl.ds(r, 16), :] = gu[:, (NH - NV) * 256:].astype(F32)
        for n, pos in enumerate(cfg["VO"]):
            ro = jnp.minimum(r, PD - 16)
            rs = order[pos] * PD + ro
            wof[pl.ds(pl.multiple_of(n * PD + ro, 16), 16), :] = (
                wo_raw[rs >> 10, pl.ds(pl.multiple_of(rs & 1023, 16), 16), :].astype(F32))
        nd = 16 if ND * 128 <= D else 32
        rd = pl.multiple_of(jnp.minimum(h * nd, ND * 128 - nd), 16)
        wdf[pl.ds(rd, nd), :] = wd_raw[rd >> 8, pl.ds(pl.multiple_of(rd & 255, 16), nd), :].astype(F32)
        ho = jnp.minimum(h, 31)
        for g in range(6):
            wop[pl.ds(pl.multiple_of(g * 512 + ho * 16, 16), 16), :] = _u32(
                wo_raw[g, pl.ds(pl.multiple_of(ho * 32, 32), 32), :])
        for g in range(3):
            gg = (ho >> 4) * 3 + g
            wdp[pl.ds(pl.multiple_of(gg * 128 + (ho & 15) * 8, 8), 8), :] = _u32(
                wd_raw[gg, pl.ds(pl.multiple_of((ho & 15) * 16, 16), 16), :])
        return c

    lax.fori_loop(0, NRP, repack, 0)

    NCS = (HD + 2 * F) // 768

    def colsum(i, c):
        ones, second = split_tick(NRP + i, jnp.ones((8, D), F32))
        c0 = pl.multiple_of(i * 768, 128)
        y = _dot(ones.astype(BF16), _bf(wxp[:, pl.ds(c0, 768)]))
        second(y[:, 0:128])
        cs[:, pl.ds(c0, 768)] = y
        return c

    lax.fori_loop(0, NCS, colsum, 0)
    t0 = jnp.int32(NRP + NCS)

    never = spin_ref[...] < -1.0

    def xproj(xb, m, scale, c0, n):
        y = _dot(xb, _bf(wxp[:, pl.ds(c0, n)])) - m * cs[:, pl.ds(c0, n)]
        return y if scale is None else y * scale

    def qproj(xb, m, qscale, k):
        return xproj(xb, m, qscale, k * PD if isinstance(k, int) else pl.multiple_of(k * PD, 128), PD)

    def oproj(ob, k):
        r0 = pl.multiple_of(k * DH, DH) if not isinstance(k, int) else k * DH
        return _dot(ob, _bf(wop[pl.ds(r0, DH), :]))

    def kload(k):
        return [_bf(kp[pl.ds(k * RO + 2 * i, 2)].reshape(64, W)) for i in range(3)]

    def vgroup(slot, k, o, r):
        return lambda: kv[1 + slot, k * RO + o, pl.ds(r * 8, 8), :].astype(F32)

    def pair_groups(slot, k, pe, po):
        return [(vgroup(slot, k, g // RI, g % RI), pe if g < DH // 8 else po) for g in range(PD // 8)]

    def vpu_matvec(xr, w_ref, nadd, per_step=1, tok=None, rot=0):
        nu = xr.shape[1] // 128
        xcol = [jnp.concatenate([xr[:, u * 128:(u + 1) * 128]] * 16, axis=0).T for u in range(nu)]
        seq = [(u, i) for u0 in range(0, nu, 2) for i in range(16) for u in range(u0, min(u0 + 2, nu))]
        accs = [None] * per_step
        for n in range(0, len(seq), per_step):
            if tok is not None:
                for _ in range(nadd):
                    tok = tok + 1.0
            for a, (u, i) in enumerate(seq[n:n + per_step]):
                col = xcol[u][i * 8:i * 8 + 8]
                if tok is not None:
                    col = jnp.where(never, tok, col)
                y = w_ref[u * 128 + i * 8:u * 128 + i * 8 + 8, :] * _tile(col, w_ref.shape[1] // 128)
                accs[a] = y if accs[a] is None else accs[a] + y
            c = (n // per_step * rot) % (per_step * (w_ref.shape[1] // 128))
            tok = accs[c % per_step][:, c // per_step * 128:(c // per_step + 1) * 128]
        return functools.reduce(jnp.add, accs), tok

    def act(gu):
        g = gu[:, 0:128]
        return (g * _sigmoid(g) * gu[:, 128:256]).astype(BF16)

    def ffn_res(x, xc, rstd):
        wr = wrb[...].astype(F32)
        wr = jnp.concatenate([jnp.broadcast_to(wr[t:t + 1, :], (8, 128)) for t in range(D // 128)], axis=1)
        return x + xc * rstd, _round(_sigmoid(_round(jnp.sum(xc * wr, axis=1, keepdims=True) * rstd)))

    def ffn(x, f):
        nv, nd = cfg["NV"][f], cfg["ND"][f]
        nm = NH - nv
        xb, xr, m, xc, rstd = _ln_parts(x)
        hs = [act(xproj(xb, m, rstd, HD + i * 256, 256)) for i in range(nm)]
        gu, tok = vpu_matvec(xr, wguf.at[:, (NV - nv) * 256:], cfg["TOK"][f], rot=cfg["ROT"][0])
        gu = (_rowsum_all(gu) - m * cs[:, HD + nm * 256:]) * rstd
        hs += [act(gu[:, i * 256:(i + 1) * 256]) for i in range(nv)]
        y = None
        late = list(range(nm - cfg["DLATE"][f], nm))
        for i in [i for i in range(nd, NH) if i not in late] + late:
            yi = _dot(hs[i], _bf(wdp[i * 64:(i + 1) * 64, :]))
            y = yi if y is None else y + yi
        yv, _ = vpu_matvec(jnp.concatenate(hs[:nd], axis=1).astype(F32), wdf, cfg["DTOK"][f], cfg["DPER"][f], tok,
                           cfg["ROT"][1])
        y = y + _rowsum_all(yv)
        res, gate = ffn_res(xr, xc, rstd)
        return res + y * gate

    NFT = NH // 2 + 1

    def ffn_ticked(x, t):
        def body(i, carry):
            h, y, _ = carry
            xx, second = split_tick(t + i, x)
            xb, xr, m, xc, rstd = _ln_parts(xx)
            second(xc[:, 0:128])
            c0 = pl.multiple_of(HD + jnp.minimum(i, NFT - 2) * 512, 128)
            gu = xproj(xb, m, rstd, c0, 512)
            r0 = pl.multiple_of(jnp.maximum(i - 1, 0) * 128, 128)
            y = y + _dot(h, _bf(wdp[pl.ds(r0, 128), :]))
            res, gate = ffn_res(xr, xc, rstd)
            return jnp.concatenate([act(gu[:, 0:256]), act(gu[:, 256:512])], axis=1), y, res + y * gate

        return lax.fori_loop(0, NFT, body, (jnp.zeros((8, 256), BF16), jnp.zeros((8, D), F32), x))[2]

    NHP = 2 * B - 1

    def half_period(hp, t):
        b = hp >> 1
        slot = b & 1
        first = (hp & 1) == 0
        vbase = jnp.where(first, b * TPP + (NP + 1) * TPC, -TPP)

        tr = jnp.where(first, jnp.maximum(t, b * TPP + cfg["KRP"]), t)
        lax.fori_loop(t, tr, spin_tick, 0)

        def k_repack(h, c):
            def work():
                o0 = (h - 2 * tr) * 4
                kp[pl.ds(o0, 4)] = _u32(kv[0, pl.ds(o0, 4)].reshape(4 * 64, W)).reshape(4, 32, W)

            half_tick(h, LEAD + 1, LA, work, cfg["KSPIN"], True)
            return c

        t = jnp.where(first, tr + NP * RO // 8, t)
        lax.fori_loop(2 * tr, 2 * t, k_repack, 0)

        xb, x, m, _, rstd = _ln_parts(jnp.broadcast_to(state[pl.ds(b, 1), :], (8, D)))
        qscale = rstd * SCALE

        def step(j, carry):
            t, q, se, so, pe, po, inv, o, out = carry
            kv_ = jnp.maximum(j - 3, 0)
            t = advance(t, vbase + kv_ * TPC)
            se_n, so_n = _scores(q, kload(jnp.clip(j - 1, 0, NP - 1)))
            q_n = qproj(xb, m, qscale, jnp.minimum(j, NP - 1))
            out = out + oproj(o, jnp.maximum(j - 4, 0))
            pe_n, po_n, inv_n = _softmax_pair(se, so)
            acc = _pv(pair_groups(slot, kv_, pe, po),
                      {cfg["PVMID"][0]: lambda: mid(t, 0), cfg["PVMID"][1]: lambda: mid(t, 1)})
            mid(t, 2, q_n[:, 256:384])
            o_n = jnp.where(j >= 3, _lane_reduce_t(acc) * inv, 0.0).astype(BF16)
            return t, q_n, se_n, so_n, pe_n, po_n, inv_n, o_n, out

        zw = (lax.broadcasted_iota(I32, (8, W), 0) + lax.broadcasted_iota(I32, (8, W), 1)).astype(F32) * (1.0 / W)
        zp = zw[:, :PD]
        init = (t, zp, zw, zw, zw, zw, zp, jnp.zeros((8, PD), BF16), jnp.zeros((8, D), F32))
        last = hp == NHP - 1
        t, q, se, so, pe, po, inv, o, out = lax.fori_loop(0, jnp.where(last, NP, NP + 2), step, init)
        t2 = jnp.maximum(t + 2, vbase + (NP - 1) * TPC)

        @pl.when(last)
        def _():
            c_s[0] = se
            c_s[1] = so
            c_p[0] = pe
            c_p[1] = po
            c_o[0] = q
            c_o[1] = inv
            c_o[2] = o.astype(F32)
            c_out[...] = out

        @pl.when(jnp.logical_not(last))
        def _():
            advance(t, t2)
            y = out + oproj(o, NP - 2)
            acc = _pv(pair_groups(slot, NP - 1, pe, po), {24: lambda: mid(t2, 0), 45: lambda: mid(t2, 1)})
            olast = _lane_reduce_t(acc) * inv
            mid(t2, 2, olast[:, 0:128])
            olast, second = split_tick(t2, olast)
            yl = oproj(olast.astype(BF16), NP - 1)
            second(yl[:, 0:128])
            y = y + yl
            state[pl.ds(b, 1), :] = ffn_ticked(x + _rowsum_all(y), t2 + 1)[0:1]

        return t2 + 1 + NFT

    lax.fori_loop(0, NHP, half_period, t0)

    slot = (B - 1) % 2
    ka, kb = NP - 2, NP - 1

    def wo_rows(runs):
        return _bf(jnp.concatenate(
            [wop[(k * PD + o * 64 + r * 8) // 2:(k * PD + o * 64 + (r + n) * 8) // 2, :] for k, o, r, n in runs],
            axis=0))

    def run_groups(runs, ps):
        return [(vgroup(slot, k, o, r + i), ps[k][0 if o < RO // 2 else 1]) for k, o, r, n in runs for i in range(n)]

    def normalised(pe, po, inv):
        return pe * _tile(inv[:, 0:128], NL), po * _tile(inv[:, 256:384], NL)

    def pv_o_vpu(runs):
        w = wo_rows(runs).astype(F32)
        return functools.reduce(jnp.add, [
            w[i * 8:(i + 1) * 8] * jnp.sum(_fold(vload() * p, jnp.add), axis=1, keepdims=True)
            for i, (vload, p) in enumerate(run_groups(runs, ps))])

    kc = NP - 3
    for i in range(NTICK - 3 * TPC, NTICK - TPC):
        wait_piece(i, 1)
    se, so = _scores(c_o[0], kload(kb))
    out = c_out[...] + oproj(c_o[2].astype(BF16), NP - 4)
    ps = {kc: normalised(c_p[0], c_p[1], c_o[1]), ka: normalised(*_softmax_pair(c_s[0], c_s[1]))}
    runs = [(k, o, TPC, TPC) for k in (kc, ka) for o in range(RO)]
    o = _lane_reduce_t(_pv(run_groups(runs, ps))).astype(BF16)
    ps[kb] = normalised(*_softmax_pair(se, so))

    for i in range(NTICK - 3 * TPC, NTICK - 2 * TPC):
        wait_piece(i, 0)
    for i in range(NTICK - TPC, NTICK):
        wait_piece(i, 1)
    out = out + _dot(o, wo_rows(runs))
    runs0 = [(kc, o, 0, TPC) for o in range(RO)] + [(kb, o, TPC, TPC) for o in range(RO)]
    o0 = _lane_reduce_t(_pv(run_groups(runs0, ps))).astype(BF16)

    for i in range(NTICK - 2 * TPC, NTICK - TPC):
        wait_piece(i, 0)
    out = out + _dot(o0, wo_rows(runs0))
    runs1 = [(ka, o, 0, TPC) for o in range(RO)]
    acc = [_fold(vload() * p, jnp.add) for vload, p in run_groups(runs1, ps)]
    zero = [jnp.zeros((8, 128), F32)] * 4
    o1 = _lane_reduce_t(jnp.concatenate(acc[:12] + zero + acc[12:] + zero, axis=0)).astype(BF16)

    for i in range(NTICK - TPC, NTICK - 2):
        wait_piece(i, 0)
    out = out + _dot(o1, wo_rows(runs1[:3] + runs1[:1] + runs1[3:] + runs1[:1]))
    out = out + pv_o_vpu([(kb, o, 0, 2) for o in range(RO)])

    for i in range(NTICK - 2, NTICK):
        wait_piece(i, 0)
    out = out + pv_o_vpu([(kb, o, 2, 2) for o in range(RO)])
    x = jnp.broadcast_to(state[B - 1:B, :], (8, D)) + _rowsum_all(out)

    def attn_fast(x):
        xb, xr, m, _, rstd = _ln_parts(x)
        qscale = rstd * SCALE
        q, sc, ps, os_, deadline, outv = {}, {}, {}, {}, {}, []
        invs = {}

        def get_o(pos):
            o = os_.pop(pos) * invs.pop(pos)
            return (_rowsum_all(o) if pos in cfg["VO"] else o).astype(BF16)

        out = None
        qv = _rowsum_all(vpu_matvec(xr, wqf, cfg["QTOK"], rot=cfg["ROT"][2])[0])
        for n, pos in enumerate(cfg["VQ"]):
            k = order[pos]
            q[pos] = (qv[:, n * PD:(n + 1) * PD] - m * cs[:, k * PD:(k + 1) * PD]) * qscale
        qm = [pos for pos in range(NP) if pos not in cfg["VQ"]]
        om = [pos for pos in range(NP) if pos not in cfg["VO"]]

        def vpu_stage(s):
            if 0 <= s + 1 < NP:
                ps[s + 1] = _softmax_pair(*sc.pop(s + 1), None if s + 1 >= cfg["NLS"] else qscale, bcast=True)
            if 0 <= s < NP:
                pe, po, invs[s] = ps.pop(s)
                k = order[s]
                groups = pair_groups(slot, k, pe, po)
                if k < VF:
                    groups = [(functools.partial(lambda g: vf[k * RO + g // RI, pl.ds((g % RI) * 8, 8), :], g), p)
                              for g, (_, p) in enumerate(groups)]
                acc = _pv(groups)
                os_[s] = _lane_reduce_t(acc)
                for n, (tpos, tg, nadd, per, dl) in enumerate(cfg["VOT"]):
                    if tpos == s:
                        y, tok = vpu_matvec(get_o(cfg["VO"][n]).astype(F32), wof.at[n * PD:(n + 1) * PD], nadd, per,
                                            acc[tg * 8:tg * 8 + 8], cfg["ROT"][3])
                        outv.append(y)
                        if dl:
                            deadline[s + dl + 2] = tok

        ns, nv = 0, -1
        for op in cfg["PROG"]:
            if op == "q":
                pos = qm.pop(0)
                q[pos] = qproj(xb, m, qscale if pos >= cfg["NLS"] else None, order[pos])
            elif op == "s":
                qq = q.pop(ns)
                if ns in deadline:
                    qq = jnp.concatenate([jnp.where(never, deadline.pop(ns), qq[:, 0:128]), qq[:, 128:]], axis=1)
                sc[ns] = _scores(qq, kload(order[ns]))
                ns += 1
            elif op == "o":
                pos = om.pop(0)
                y = oproj(get_o(pos), order[pos])
                out = y if out is None else out + y
            else:
                vpu_stage(nv)
                nv += 1
        out = functools.reduce(jnp.add, [out] + outv)
        return xr + _rowsum_all(out)

    x = ffn(attn_fast(ffn(x, 0)), 1)
    row = lax.broadcasted_iota(I32, (8, D), 0)
    o_ref[...] = jnp.where(row == B - 1, x, state[...])[0:B].astype(o_ref.dtype)


def _call(cfg, A_x, A_k_cache, A_v_cache, A_wq, A_wo, B_w_r, B_w_gate, B_w_up, B_w_down):
    kt = jnp.swapaxes(A_k_cache, 2, 3).reshape(B, NP * RO, RI * 8, SK)
    vt = jnp.swapaxes(A_v_cache, 2, 3).reshape(B, NP * RO, RI * 8, SK)
    out = pl.pallas_call(
        functools.partial(_kernel, cfg=cfg),
        out_shape=jax.ShapeDtypeStruct((B, D), BF16),
        in_specs=[pl.BlockSpec(memory_space=pl.ANY)] * 9,
        out_specs=pl.BlockSpec(memory_space=pltpu.VMEM),
        scratch_shapes=[
            pltpu.VMEM((3, NP * RO + 1, RI * 8, W), BF16),
            pltpu.VMEM((VF * RO, RI * 8, W), F32),
            pltpu.VMEM((NP * RO, RI * 4, W), U32),
            pltpu.VMEM((D, HD), BF16),
            pltpu.VMEM((6, HD // 6, D), BF16),
            pltpu.VMEM((D, F), BF16),
            pltpu.VMEM((4, D // 4, F), BF16),
            pltpu.VMEM((6, F // 6, D), BF16),
            pltpu.VMEM((D // 2, HD + 2 * F), U32),
            pltpu.VMEM((HD // 2, D), U32),
            pltpu.VMEM((F // 2, D), U32),
            pltpu.VMEM((D, max(cfg["NV"]) * 256), F32),
            pltpu.VMEM((D, len(cfg["VQ"]) * PD), F32),
            pltpu.VMEM((max(cfg["ND"]) * 128, D), F32),
            pltpu.VMEM((len(cfg["VO"]) * PD, D), F32),
            pltpu.VMEM((8, HD + 2 * F), F32),
            pltpu.VMEM((B, D), BF16),
            pltpu.VMEM((D // 128, 128), BF16),
            pltpu.VMEM((8, D), F32),
            pltpu.VMEM((8, 128), F32),
            pltpu.VMEM((2, 8, W), F32),
            pltpu.VMEM((2, 8, W), F32),
            pltpu.VMEM((3, 8, PD), F32),
            pltpu.VMEM((8, D), F32),
            pltpu.SemaphoreType.DMA((2, RING)),
            pltpu.SemaphoreType.DMA((8,)),
        ],
        compiler_params=pltpu.CompilerParams(vmem_limit_bytes=126 * 1024 * 1024,
                                             disable_bounds_checks=True,
                                             disable_semaphore_checks=True),
        name="fused_decode",
    )(A_x.reshape(B, D), kt, vt, A_wq, A_wo.reshape(6, HD // 6, D), B_w_r.reshape(D // 128, 128), B_w_gate,
      B_w_up.reshape(4, D // 4, F), B_w_down.reshape(6, F // 6, D))
    return out.reshape(B, 1, D)


@jax.jit
def pallas_interleave_layers__sliding_block_cached__moe_arch_mod__decode_kernel(
    A_x: jax.Array,
    A_k_cache: jax.Array,
    A_v_cache: jax.Array,
    A_wq: jax.Array,
    A_wo: jax.Array,
    B_x: jax.Array,
    B_w_r: jax.Array,
    B_w_gate: jax.Array,
    B_w_up: jax.Array,
    B_w_down: jax.Array,
):
    del B_x
    return _call(CFG, A_x, A_k_cache, A_v_cache, A_wq, A_wo, B_w_r, B_w_gate, B_w_up, B_w_down)
```

```python
import functools

import jax
import jax.numpy as jnp
from jax import lax
import jax.experimental.pallas as pl
import jax.experimental.pallas.tpu as pltpu

F32 = jnp.float32
BF16 = jnp.bfloat16
U32 = jnp.uint32
I32 = jnp.int32

B, D, H, DH, SK, F = 4, 640, 32, 192, 4096, 1536
W = min(4096, max(256, SK // 4))
NP = H // 2
PD = 2 * DH
HD = H * DH
NL = W // 128
NH = F // 128
EPS = 1e-5
SCALE = DH ** -0.5 * 1.4426950408889634

RI = 8
RO = PD // (8 * RI)
NA = NP * RO // 2
TPC = RI // 2
TPP = 2 * NP * TPC
NTICK = B * TPP
RING = 32
VF = 12

CFG = dict(
    LA=23,
    LEAD=11,
    KRP=54,
    PVMID=(21, 45),
    SPIN=(1, 50),
    WSPIN=(1, 45),
    LSPIN=(1, 20),
    KSPIN=(1, 20),
    HSPIN=(1, 8),
    RSPIN=(1, 10),
    NV=(3, 4),
    ND=(5, 5),
    DLATE=(0, 3),
    TOK=(0, 0),
    DTOK=(2, 2),
    DPER=(2, 3),
    QTOK=0,
    ROT=(1, 1, 3, 0),
    RAWPOS=(0, 2, 4, 10),
    PROG="qqsqs.s.qqs.qs.qqos.s.qqs.s.qs.qso.qso.s.oso.so.s...ooooooo",
    NLS=2,
    VQ=(3, 4, 5),
    VO=(1, 0, 8),
    VOT=((14, 0, 0, 3, 0), (4, 16, 0, 2, 0), (11, 32, 0, 3, 2)),
)


def _order(cfg):
    order = list(range(VF))
    for pos, k in zip(sorted(cfg["RAWPOS"]), range(VF, NP)):
        order.insert(pos, k)
    return order


def _rowsum_all(x):
    x = x + pltpu.roll(x, 4, 0)
    x = x + pltpu.roll(x, 2, 0)
    return x + pltpu.roll(x, 1, 0)


def _bf(x):
    return pltpu.bitcast(x, BF16)


def _u32(x):
    return pltpu.bitcast(x, U32)


def _dot(a, b):
    return jnp.dot(a, b, preferred_element_type=F32)


def _sigmoid(x):
    return pl.reciprocal(1.0 + jnp.exp(-x), approx=True)


def _round(x):
    return x.astype(BF16).astype(F32)


def _ln_parts(x):
    xb = x.astype(BF16)
    xr = xb.astype(F32)
    m = jnp.sum(xr, axis=1, keepdims=True) * (1.0 / D)
    xc = xr - m
    v = jnp.sum(xc * xc, axis=1, keepdims=True) * (1.0 / D)
    m = _round(m)
    v = _round(_round(v) + EPS)
    return xb, xr, m, xr - m, pl.reciprocal(_round(v * lax.rsqrt(v)), approx=True)


def _scores(q, kk):
    lane = lax.broadcasted_iota(I32, (8, 128), 1)
    q0 = q[:, 0:128].astype(BF16)
    qm = q[:, 128:256]
    q2 = q[:, 256:384].astype(BF16)
    mid = jnp.concatenate([jnp.where(lane < 64, qm, 0.0), jnp.where(lane >= 64, qm, 0.0)],
                          axis=0).astype(BF16)
    r0 = _dot(q0, kk[0])
    rm = _dot(mid, kk[1])
    r2 = _dot(q2, kk[2])
    return r0 + rm[0:8], rm[8:16] + r2


def _fold(x, op):
    r = x[:, 0:128]
    for t in range(1, x.shape[1] // 128):
        r = op(r, x[:, t * 128:(t + 1) * 128])
    return r


def _tile(x, n):
    return jnp.concatenate([x] * n, axis=1)


def _softmax_pair(se, so, c=None, bcast=False):
    row = lax.broadcasted_iota(I32, (8, 128), 0)
    top = row < 4

    def split(c):
        c = jnp.broadcast_to(c, (8, 128))
        r = pltpu.roll(c, 4, 0)
        return jnp.where(top, c, r), jnp.where(top, r, c)

    m = jnp.max(jnp.where(top, _fold(se, jnp.maximum), _fold(so, jnp.maximum)), axis=1, keepdims=True)
    me, mo = split(m)
    de, do = se - _tile(me, NL), so - _tile(mo, NL)
    if c is not None:
        de, do = de * c, do * c
    pe, po = jnp.exp2(de), jnp.exp2(do)
    le, lo = _fold(pe, jnp.add), _fold(po, jnp.add)
    if bcast:
        l = jnp.sum(jnp.where(row >= 1, lo, le), axis=1, keepdims=True)
        r = jnp.broadcast_to(pl.reciprocal(l, approx=True), (8, 128))
        ie, io = [jnp.broadcast_to(r[i:i + 1], (8, 128)) for i in range(2)]
    else:
        ie, io = split(pl.reciprocal(jnp.sum(jnp.where(top, le, lo), axis=1, keepdims=True), approx=True))
    lane = lax.broadcasted_iota(I32, (8, 128), 1)
    return pe, po, jnp.concatenate([ie, jnp.where(lane < 64, ie, io), io], axis=1)


def _pv(groups, hooks=None):
    nb = len(groups) // 16
    accs = {}
    for n, g in enumerate(16 * blk + i for i in range(16) for blk in range(nb)):
        if hooks and n in hooks:
            hooks[n]()
        vload, p = groups[g]
        accs[g] = _fold(vload() * p, jnp.add)
    return jnp.concatenate([accs[g] for g in range(len(groups))], axis=0)


def _lane_reduce_t(acc):
    at = acc.T
    s = at[0:8]
    for i in range(1, 16):
        s = s + at[8 * i:8 * i + 8]
    return s


def _kernel(x_hbm, kt_hbm, vt_hbm, wq_hbm, wo_hbm, wr_hbm, wg_hbm, wu_hbm, wd_hbm,
            o_ref,
            kv, vf, kp, wq_raw, wo_raw, wg_raw, wu_raw, wd_raw, wxp, wop, wdp, wguf, wqf, wdf, wof, cs,
            xb_ref, wrb, state, spin_ref, c_s, c_p, c_o, c_out,
            sems, wsem, *, cfg):
    LA, LEAD, NV, ND = cfg["LA"], cfg["LEAD"], max(cfg["NV"]), max(cfg["ND"])
    order = _order(cfg)

    def piece(i, s, w, hf):
        def rows(r):
            return pl.ds(r * 8 if isinstance(r, int) else pl.multiple_of(r * 8, 8), 8)

        if w == 0:
            a0 = (i & 7) * 6
            return (pl.ds(a0, 6) if hf is None else pl.ds(a0 + hf * 3, 3)), s, rows((i >> 3) & 7)
        return pl.ds(((i >> 2) & (NP - 1)) * 3, 3), (slice(None) if hf is None else hf), rows((i & 3) + s * TPC)

    def on_kind(i, f, kind, cond=None):
        if isinstance(i, int) or (kind is not None and cond is None):
            f((i >> 6) & 1 if kind is None else kind)
        elif kind is not None:
            pl.when(cond)(functools.partial(f, kind))
        else:
            for w in range(2):
                c = ((i >> 6) & 1) == w
                pl.when(c if cond is None else jnp.logical_and(c, cond))(functools.partial(f, w))

    def start_piece(i, s, hf=None, kind=None, cond=None):
        def go(w):
            idx = piece(i, s, w, hf)
            pltpu.make_async_copy((vt_hbm if w else kt_hbm).at[(i >> 7,) + idx + (pl.ds(SK - W, W),)],
                                  kv.at[(w * (1 + ((i >> 7) & 1)),) + idx],
                                  sems.at[s, i & (RING - 1)]).start(priority=1 - s)

        if kind is None:
            cond = i < NTICK if cond is None else jnp.logical_and(cond, i < NTICK)
        on_kind(i, go, kind, cond)

    def wait_piece(i, s, kind=None, cond=None):
        def go(w):
            view = kv.at[(w * (1 + ((i >> 7) & 1)),) + piece(i, s, w, None)]
            pltpu.make_async_copy(view, view, sems.at[s, i & (RING - 1)]).wait()

        on_kind(i, go, kind, cond)

    def wait_tick(i, kind=None, cond=None):
        wait_piece(i, 0, kind, cond)
        wait_piece(i, 1, kind, cond)

    def delay(v, n):
        lane = lax.broadcasted_iota(I32, v.shape, 1).astype(F32)
        for _ in range(n[0]):
            v = jnp.max(v, axis=1, keepdims=True) * 0.5 + lane
        for _ in range(n[1] // 2):
            v = v * 0.5
            v = v + lane
        return v

    def spin(n):
        spin_ref[...] = delay(spin_ref[...], n)

    def full_tick(i):
        wait_tick(i)
        start_piece(i + LEAD + 1, 1)
        start_piece(i + LA, 0)

    def spin_tick(i, c):
        full_tick(i)
        spin(cfg["SPIN"])
        return c

    def half_tick(h, lead, la, work, sp, top, wkind, skind):
        i = h >> 1
        wait_tick(i, wkind, (h & 1) == 0)
        if top:
            start_piece(i + lead, 1, h & 1, skind)
        work()
        spin(sp)
        if not top:
            start_piece(i + lead, 1, h & 1, skind)
        start_piece(i + la, 0, None, skind, (h & 1) == 1)

    def idle_half(h, c):
        def work():
            n = (((h >> 3) & (NP - 1)) - 4) * 4 + (h & 7) - 2
            a = jnp.minimum(n, VF * 3 - 1)
            vf[a] = kv[1 + ((h >> 8) & 1), a].astype(F32)

        half_tick(h, LEAD, LA - 1, work, cfg["HSPIN"], False, 1, None)
        return c

    def advance(t, need):
        t2 = jnp.maximum(t + 2, need)
        wait_tick(t)
        lax.fori_loop(2 * t + 2, 2 * t2 - 2, idle_half, 0)
        wait_tick(t2 - 1)
        start_piece(t2 - 1 + LEAD, 1, 0)
        return t2

    def mid(t2, n, after=None):
        if n == 0:
            start_piece(t2 - 1 + LEAD, 1, 1)
        if n == 1:
            start_piece(t2 + LEAD, 1, 0)
            start_piece(t2 - 2 + LA, 0)
            start_piece(t2 - 1 + LA, 0)
        if n == 2:
            pin_after(after)
            start_piece(t2 + LEAD, 1, 1)

    def pin_after(v):
        kv[0, NA, 0, 0:16, 0:128] = jnp.concatenate([v, v], axis=0).astype(BF16)

    def pin_before(x):
        spare = kv[0, NA, 0, 0:8, 0:128].astype(F32)
        x0 = jnp.where(spin_ref[...] < -1.0, spare, x[:, 0:128])
        return x0 if x.shape[1] == 128 else jnp.concatenate([x0, x[:, 128:]], axis=1)

    def split_tick(i, x, k1=None, k0=None):
        wait_tick(i, 0)
        start_piece(i + LEAD + 1, 1, 0, k1)

        def second(after):
            pin_after(after)
            start_piece(i + LEAD + 1, 1, 1, k1)
            start_piece(i + LA, 0, None, k0)

        return pin_before(x), second

    small = [pltpu.make_async_copy(x_hbm, xb_ref, wsem.at[0]),
             pltpu.make_async_copy(wr_hbm, wrb, wsem.at[1])]
    big = [pltpu.make_async_copy(wq_hbm, wq_raw, wsem.at[2]),
           pltpu.make_async_copy(wg_hbm, wg_raw, wsem.at[3]),
           pltpu.make_async_copy(wu_hbm.at[0:2], wu_raw.at[0:2], wsem.at[4])]
    for cp in big:
        cp.start(priority=1)
    for cp in small:
        cp.start()
    spin_ref[...] = jnp.zeros(spin_ref.shape, F32)
    pin_after(jnp.zeros((8, 128), F32))

    inject = [(wo_hbm, wo_raw, 5), (wd_hbm, wd_raw, 6), (wu_hbm.at[2:4], wu_raw.at[2:4], 7)]
    for src, dst, sem in inject:
        def body(i, c, src=src, dst=dst, sem=sem):
            r = pl.ds(pl.multiple_of(i * 8, 8), 8)
            pltpu.make_async_copy(src.at[:, r], dst.at[:, r], wsem.at[sem]).start()
            spin(cfg["WSPIN"])
            return c
        lax.fori_loop(0, dst.shape[1] // 8, body, 0)
        if dst is wo_raw:
            for i in range(LA):
                start_piece(i, 0)

    def lead_in(h, c):
        start_piece(h >> 1, 1, h & 1, 0)
        spin(cfg["LSPIN"])
        return c

    lax.fori_loop(0, 2 * (LEAD + 1), lead_in, 0)
    for cp in small:
        cp.wait()
    state[...] = jnp.concatenate([xb_ref[...].astype(F32), jnp.zeros((8 - B, D), F32)], axis=0)
    for src, dst, sem in inject:
        pltpu.make_async_copy(dst, dst, wsem.at[sem]).wait()
    for cp in big:
        cp.wait()

    NRP = D // 16

    def repack(h, c):
        v, second = split_tick(h, spin_ref[...], 0, 0)
        second(delay(v, cfg["RSPIN"]))
        r = pl.multiple_of(h * 16, 16)
        r2 = pl.multiple_of(h * 8, 8)
        wxp[pl.ds(r2, 8), 0:HD] = _u32(wq_raw[pl.ds(r, 16), :])
        for n, pos in enumerate(cfg["VQ"]):
            wqf[pl.ds(r, 16), n * PD:(n + 1) * PD] = (
                wq_raw[pl.ds(r, 16), order[pos] * PD:(order[pos] + 1) * PD].astype(F32))
        g = wg_raw[pl.ds(r, 16), :]
        pu = (h * 205) >> 11
        u = wu_raw[pu, pl.ds(pl.multiple_of(r - pu * 160, 16), 16), :]
        gu = jnp.concatenate([w[:, i * 128:(i + 1) * 128] for i in range(NH) for w in (g, u)], axis=1)
        wxp[pl.ds(r2, 8), HD:HD + 2 * F] = _u32(gu)
        wguf[pl.ds(r, 16), :] = gu[:, (NH - NV) * 256:].astype(F32)
        for n, pos in enumerate(cfg["VO"]):
            ro = jnp.minimum(r, PD - 16)
            rs = order[pos] * PD + ro
            wof[pl.ds(pl.multiple_of(n * PD + ro, 16), 16), :] = (
                wo_raw[rs >> 10, pl.ds(pl.multiple_of(rs & 1023, 16), 16), :].astype(F32))
        nd = 16 if ND * 128 <= D else 32
        rd = pl.multiple_of(jnp.minimum(h * nd, ND * 128 - nd), 16)
        wdf[pl.ds(rd, nd), :] = wd_raw[rd >> 8, pl.ds(pl.multiple_of(rd & 255, 16), nd), :].astype(F32)
        ho = jnp.minimum(h, 31)
        for g in range(6):
            wop[pl.ds(pl.multiple_of(g * 512 + ho * 16, 16), 16), :] = _u32(
                wo_raw[g, pl.ds(pl.multiple_of(ho * 32, 32), 32), :])
        for g in range(3):
            gg = (ho >> 4) * 3 + g
            wdp[pl.ds(pl.multiple_of(gg * 128 + (ho & 15) * 8, 8), 8), :] = _u32(
                wd_raw[gg, pl.ds(pl.multiple_of((ho & 15) * 16, 16), 16), :])
        return c

    lax.fori_loop(0, NRP, repack, 0)

    NCS = (HD + 2 * F) // 768

    def colsum(i, c):
        ones, second = split_tick(NRP + i, jnp.ones((8, D), F32), 0)
        c0 = pl.multiple_of(i * 768, 128)
        y = _dot(ones.astype(BF16), _bf(wxp[:, pl.ds(c0, 768)]))
        second(y[:, 0:128])
        cs[:, pl.ds(c0, 768)] = y
        return c

    lax.fori_loop(0, NCS, colsum, 0)
    t0 = jnp.int32(NRP + NCS)

    never = spin_ref[...] < -1.0

    def xproj(xb, m, scale, c0, n):
        y = _dot(xb, _bf(wxp[:, pl.ds(c0, n)])) - m * cs[:, pl.ds(c0, n)]
        return y if scale is None else y * scale

    def qproj(xb, m, qscale, k):
        return xproj(xb, m, qscale, k * PD if isinstance(k, int) else pl.multiple_of(k * PD, 128), PD)

    def oproj(ob, k):
        r0 = pl.multiple_of(k * DH, DH) if not isinstance(k, int) else k * DH
        return _dot(ob, _bf(wop[pl.ds(r0, DH), :]))

    def kload(k):
        return [_bf(kp[k * 3 + i]) for i in range(3)]

    def vgroup(slot, k, o, r):
        return lambda: kv[1 + slot, k * 3 + o // 2, o % 2, pl.ds(r * 8, 8), :].astype(F32)

    def pair_groups(slot, k, pe, po):
        return [(vgroup(slot, k, g // RI, g % RI), pe if g < DH // 8 else po) for g in range(PD // 8)]

    def vpu_matvec(xr, w_ref, nadd, per_step=1, tok=None, rot=0):
        nu = xr.shape[1] // 128
        xcol = [jnp.concatenate([xr[:, u * 128:(u + 1) * 128]] * 16, axis=0).T for u in range(nu)]
        seq = [(u, i) for u0 in range(0, nu, 2) for i in range(16) for u in range(u0, min(u0 + 2, nu))]
        accs = [None] * per_step
        for n in range(0, len(seq), per_step):
            if tok is not None:
                for _ in range(nadd):
                    tok = tok + 1.0
            for a, (u, i) in enumerate(seq[n:n + per_step]):
                col = xcol[u][i * 8:i * 8 + 8]
                if tok is not None:
                    col = jnp.where(never, tok, col)
                y = w_ref[u * 128 + i * 8:u * 128 + i * 8 + 8, :] * _tile(col, w_ref.shape[1] // 128)
                accs[a] = y if accs[a] is None else accs[a] + y
            c = (n // per_step * rot) % (per_step * (w_ref.shape[1] // 128))
            tok = accs[c % per_step][:, c // per_step * 128:(c // per_step + 1) * 128]
        return functools.reduce(jnp.add, accs), tok

    def act(gu):
        g = gu[:, 0:128]
        return (g * _sigmoid(g) * gu[:, 128:256]).astype(BF16)

    def ffn_res(x, xc, rstd):
        wr = wrb[...].astype(F32)
        wr = jnp.concatenate([jnp.broadcast_to(wr[t:t + 1, :], (8, 128)) for t in range(D // 128)], axis=1)
        return x + xc * rstd, _round(_sigmoid(_round(jnp.sum(xc * wr, axis=1, keepdims=True) * rstd)))

    def ffn(x, f):
        nv, nd = cfg["NV"][f], cfg["ND"][f]
        nm = NH - nv
        xb, xr, m, xc, rstd = _ln_parts(x)
        hs = [act(xproj(xb, m, rstd, HD + i * 256, 256)) for i in range(nm)]
        gu, tok = vpu_matvec(xr, wguf.at[:, (NV - nv) * 256:], cfg["TOK"][f], rot=cfg["ROT"][0])
        gu = (_rowsum_all(gu) - m * cs[:, HD + nm * 256:]) * rstd
        hs += [act(gu[:, i * 256:(i + 1) * 256]) for i in range(nv)]
        y = None
        late = list(range(nm - cfg["DLATE"][f], nm))
        for i in [i for i in range(nd, NH) if i not in late] + late:
            yi = _dot(hs[i], _bf(wdp[i * 64:(i + 1) * 64, :]))
            y = yi if y is None else y + yi
        yv, _ = vpu_matvec(jnp.concatenate(hs[:nd], axis=1).astype(F32), wdf, cfg["DTOK"][f], cfg["DPER"][f], tok,
                           cfg["ROT"][1])
        y = y + _rowsum_all(yv)
        res, gate = ffn_res(xr, xc, rstd)
        return res + y * gate

    NFT = NH // 2 + 1

    def ffn_ticked(x, t):
        def body(i, carry):
            h, y, _ = carry
            xx, second = split_tick(t + i, x)
            xb, xr, m, xc, rstd = _ln_parts(xx)
            second(xc[:, 0:128])
            c0 = pl.multiple_of(HD + jnp.minimum(i, NFT - 2) * 512, 128)
            gu = xproj(xb, m, rstd, c0, 512)
            r0 = pl.multiple_of(jnp.maximum(i - 1, 0) * 128, 128)
            y = y + _dot(h, _bf(wdp[pl.ds(r0, 128), :]))
            res, gate = ffn_res(xr, xc, rstd)
            return jnp.concatenate([act(gu[:, 0:256]), act(gu[:, 256:512])], axis=1), y, res + y * gate

        return lax.fori_loop(0, NFT, body, (jnp.zeros((8, 256), BF16), jnp.zeros((8, D), F32), x))[2]

    NHP = 2 * B - 1

    def half_period(hp, t):
        b = hp >> 1
        slot = b & 1
        first = (hp & 1) == 0
        vbase = jnp.where(first, b * TPP + (NP + 1) * TPC, -TPP)

        tr = jnp.where(first, jnp.maximum(t, b * TPP + cfg["KRP"]), t)
        lax.fori_loop(t, tr, spin_tick, 0)

        def k_repack(h, c):
            def work():
                u = h - 2 * tr
                u3 = (u * 43) >> 7
                a = pl.ds((u - u3 * 3) * 16, 16)
                k16 = kv[0, a, u3 & 1, pl.ds(pl.multiple_of((u3 >> 1) * 16, 16), 16), :]
                kp[a, pl.ds(pl.multiple_of((u3 & 1) * 32 + (u3 >> 1) * 8, 8), 8), :] = (
                    _u32(k16.reshape(256, W)).reshape(16, 8, W))

            half_tick(h, LEAD + 1, LA, work, cfg["KSPIN"], True, None, 1)
            return c

        t = jnp.where(first, tr + NP * RO // 8, t)
        lax.fori_loop(2 * tr, 2 * t, k_repack, 0)

        xb, x, m, _, rstd = _ln_parts(jnp.broadcast_to(state[pl.ds(b, 1), :], (8, D)))
        qscale = rstd * SCALE

        def step(j, carry):
            t, q, se, so, pe, po, inv, o, out = carry
            kv_ = jnp.maximum(j - 3, 0)
            t = advance(t, vbase + kv_ * TPC)
            se_n, so_n = _scores(q, kload(jnp.clip(j - 1, 0, NP - 1)))
            q_n = qproj(xb, m, qscale, jnp.minimum(j, NP - 1))
            out = out + oproj(o, jnp.maximum(j - 4, 0))
            pe_n, po_n, inv_n = _softmax_pair(se, so)
            acc = _pv(pair_groups(slot, kv_, pe, po),
                      {cfg["PVMID"][0]: lambda: mid(t, 0), cfg["PVMID"][1]: lambda: mid(t, 1)})
            mid(t, 2, q_n[:, 256:384])
            o_n = jnp.where(j >= 3, _lane_reduce_t(acc) * inv, 0.0).astype(BF16)
            return t, q_n, se_n, so_n, pe_n, po_n, inv_n, o_n, out

        zw = (lax.broadcasted_iota(I32, (8, W), 0) + lax.broadcasted_iota(I32, (8, W), 1)).astype(F32) * (1.0 / W)
        zp = zw[:, :PD]
        init = (t, zp, zw, zw, zw, zw, zp, jnp.zeros((8, PD), BF16), jnp.zeros((8, D), F32))
        last = hp == NHP - 1
        t, q, se, so, pe, po, inv, o, out = lax.fori_loop(0, jnp.where(last, NP, NP + 2), step, init)
        t2 = jnp.maximum(t + 2, vbase + (NP - 1) * TPC)

        @pl.when(last)
        def _():
            c_s[0] = se
            c_s[1] = so
            c_p[0] = pe
            c_p[1] = po
            c_o[0] = q
            c_o[1] = inv
            c_o[2] = o.astype(F32)
            c_out[...] = out

        @pl.when(jnp.logical_not(last))
        def _():
            advance(t, t2)
            y = out + oproj(o, NP - 2)
            acc = _pv(pair_groups(slot, NP - 1, pe, po), {24: lambda: mid(t2, 0), 45: lambda: mid(t2, 1)})
            olast = _lane_reduce_t(acc) * inv
            mid(t2, 2, olast[:, 0:128])
            olast, second = split_tick(t2, olast, 0)
            yl = oproj(olast.astype(BF16), NP - 1)
            second(yl[:, 0:128])
            y = y + yl
            state[pl.ds(b, 1), :] = ffn_ticked(x + _rowsum_all(y), t2 + 1)[0:1]

        return t2 + 1 + NFT

    lax.fori_loop(0, NHP, half_period, t0)

    slot = (B - 1) % 2
    ka, kb = NP - 2, NP - 1

    def wo_rows(runs):
        return _bf(jnp.concatenate(
            [wop[(k * PD + o * 64 + r * 8) // 2:(k * PD + o * 64 + (r + n) * 8) // 2, :] for k, o, r, n in runs],
            axis=0))

    def run_groups(runs, ps):
        return [(vgroup(slot, k, o, r + i), ps[k][0 if o < RO // 2 else 1]) for k, o, r, n in runs for i in range(n)]

    def normalised(pe, po, inv):
        return pe * _tile(inv[:, 0:128], NL), po * _tile(inv[:, 256:384], NL)

    def pv_o_vpu(runs):
        w = wo_rows(runs).astype(F32)
        return functools.reduce(jnp.add, [
            w[i * 8:(i + 1) * 8] * jnp.sum(_fold(vload() * p, jnp.add), axis=1, keepdims=True)
            for i, (vload, p) in enumerate(run_groups(runs, ps))])

    kc = NP - 3
    for i in range(NTICK - 3 * TPC, NTICK - TPC):
        wait_piece(i, 1)
    se, so = _scores(c_o[0], kload(kb))
    out = c_out[...] + oproj(c_o[2].astype(BF16), NP - 4)
    ps = {kc: normalised(c_p[0], c_p[1], c_o[1]), ka: normalised(*_softmax_pair(c_s[0], c_s[1]))}
    runs = [(k, o, TPC, TPC) for k in (kc, ka) for o in range(RO)]
    o = _lane_reduce_t(_pv(run_groups(runs, ps))).astype(BF16)
    ps[kb] = normalised(*_softmax_pair(se, so))

    for i in range(NTICK - 3 * TPC, NTICK - 2 * TPC):
        wait_piece(i, 0)
    for i in range(NTICK - TPC, NTICK):
        wait_piece(i, 1)
    out = out + _dot(o, wo_rows(runs))
    runs0 = [(kc, o, 0, TPC) for o in range(RO)] + [(kb, o, TPC, TPC) for o in range(RO)]
    o0 = _lane_reduce_t(_pv(run_groups(runs0, ps))).astype(BF16)

    for i in range(NTICK - 2 * TPC, NTICK - TPC):
        wait_piece(i, 0)
    out = out + _dot(o0, wo_rows(runs0))
    runs1 = [(ka, o, 0, TPC) for o in range(RO)]
    acc = [_fold(vload() * p, jnp.add) for vload, p in run_groups(runs1, ps)]
    zero = [jnp.zeros((8, 128), F32)] * 4
    o1 = _lane_reduce_t(jnp.concatenate(acc[:12] + zero + acc[12:] + zero, axis=0)).astype(BF16)

    for i in range(NTICK - TPC, NTICK - 2):
        wait_piece(i, 0)
    out = out + _dot(o1, wo_rows(runs1[:3] + runs1[:1] + runs1[3:] + runs1[:1]))
    out = out + pv_o_vpu([(kb, o, 0, 2) for o in range(RO)])

    for i in range(NTICK - 2, NTICK):
        wait_piece(i, 0)
    out = out + pv_o_vpu([(kb, o, 2, 2) for o in range(RO)])
    x = jnp.broadcast_to(state[B - 1:B, :], (8, D)) + _rowsum_all(out)

    def attn_fast(x):
        xb, xr, m, _, rstd = _ln_parts(x)
        qscale = rstd * SCALE
        q, sc, ps, os_, deadline, outv = {}, {}, {}, {}, {}, []
        invs = {}

        def get_o(pos):
            o = os_.pop(pos) * invs.pop(pos)
            return (_rowsum_all(o) if pos in cfg["VO"] else o).astype(BF16)

        out = None
        qv = _rowsum_all(vpu_matvec(xr, wqf, cfg["QTOK"], rot=cfg["ROT"][2])[0])
        for n, pos in enumerate(cfg["VQ"]):
            k = order[pos]
            q[pos] = (qv[:, n * PD:(n + 1) * PD] - m * cs[:, k * PD:(k + 1) * PD]) * qscale
        qm = [pos for pos in range(NP) if pos not in cfg["VQ"]]
        om = [pos for pos in range(NP) if pos not in cfg["VO"]]

        def vpu_stage(s):
            if 0 <= s + 1 < NP:
                ps[s + 1] = _softmax_pair(*sc.pop(s + 1), None if s + 1 >= cfg["NLS"] else qscale, bcast=True)
            if 0 <= s < NP:
                pe, po, invs[s] = ps.pop(s)
                k = order[s]
                groups = pair_groups(slot, k, pe, po)
                if k < VF:
                    groups = [(functools.partial(lambda g: vf[k * 3 + g // 16, g // 8 % 2, pl.ds(g % 8 * 8, 8), :], g), p)
                              for g, (_, p) in enumerate(groups)]
                acc = _pv(groups)
                os_[s] = _lane_reduce_t(acc)
                for n, (tpos, tg, nadd, per, dl) in enumerate(cfg["VOT"]):
                    if tpos == s:
                        y, tok = vpu_matvec(get_o(cfg["VO"][n]).astype(F32), wof.at[n * PD:(n + 1) * PD], nadd, per,
                                            acc[tg * 8:tg * 8 + 8], cfg["ROT"][3])
                        outv.append(y)
                        if dl:
                            deadline[s + dl + 2] = tok

        ns, nv = 0, -1
        for op in cfg["PROG"]:
            if op == "q":
                pos = qm.pop(0)
                q[pos] = qproj(xb, m, qscale if pos >= cfg["NLS"] else None, order[pos])
            elif op == "s":
                qq = q.pop(ns)
                if ns in deadline:
                    qq = jnp.concatenate([jnp.where(never, deadline.pop(ns), qq[:, 0:128]), qq[:, 128:]], axis=1)
                sc[ns] = _scores(qq, kload(order[ns]))
                ns += 1
            elif op == "o":
                pos = om.pop(0)
                y = oproj(get_o(pos), order[pos])
                out = y if out is None else out + y
            else:
                vpu_stage(nv)
                nv += 1
        out = functools.reduce(jnp.add, [out] + outv)
        return xr + _rowsum_all(out)

    x = ffn(attn_fast(ffn(x, 0)), 1)
    row = lax.broadcasted_iota(I32, (8, D), 0)
    o_ref[...] = jnp.where(row == B - 1, x, state[...])[0:B].astype(o_ref.dtype)


def _call(cfg, A_x, A_k_cache, A_v_cache, A_wq, A_wo, B_w_r, B_w_gate, B_w_up, B_w_down):
    kt = jnp.swapaxes(A_k_cache, 2, 3).reshape(B, NA, 2, 64, SK)
    vt = jnp.swapaxes(A_v_cache, 2, 3).reshape(B, NA, 2, 64, SK)
    out = pl.pallas_call(
        functools.partial(_kernel, cfg=cfg),
        out_shape=jax.ShapeDtypeStruct((B, D), BF16),
        in_specs=[pl.BlockSpec(memory_space=pl.ANY)] * 9,
        out_specs=pl.BlockSpec(memory_space=pltpu.VMEM),
        scratch_shapes=[
            pltpu.VMEM((3, NA + 1, 2, 64, W), BF16),
            pltpu.VMEM((VF * 3, 2, 64, W), F32),
            pltpu.VMEM((NA, 64, W), U32),
            pltpu.VMEM((D, HD), BF16),
            pltpu.VMEM((6, HD // 6, D), BF16),
            pltpu.VMEM((D, F), BF16),
            pltpu.VMEM((4, D // 4, F), BF16),
            pltpu.VMEM((6, F // 6, D), BF16),
            pltpu.VMEM((D // 2, HD + 2 * F), U32),
            pltpu.VMEM((HD // 2, D), U32),
            pltpu.VMEM((F // 2, D), U32),
            pltpu.VMEM((D, max(cfg["NV"]) * 256), F32),
            pltpu.VMEM((D, len(cfg["VQ"]) * PD), F32),
            pltpu.VMEM((max(cfg["ND"]) * 128, D), F32),
            pltpu.VMEM((len(cfg["VO"]) * PD, D), F32),
            pltpu.VMEM((8, HD + 2 * F), F32),
            pltpu.VMEM((B, D), BF16),
            pltpu.VMEM((D // 128, 128), BF16),
            pltpu.VMEM((8, D), F32),
            pltpu.VMEM((8, 128), F32),
            pltpu.VMEM((2, 8, W), F32),
            pltpu.VMEM((2, 8, W), F32),
            pltpu.VMEM((3, 8, PD), F32),
            pltpu.VMEM((8, D), F32),
            pltpu.SemaphoreType.DMA((2, RING)),
            pltpu.SemaphoreType.DMA((8,)),
        ],
        compiler_params=pltpu.CompilerParams(vmem_limit_bytes=126 * 1024 * 1024,
                                             disable_bounds_checks=True,
                                             disable_semaphore_checks=True),
        name="fused_decode",
    )(A_x.reshape(B, D), kt, vt, A_wq, A_wo.reshape(6, HD // 6, D), B_w_r.reshape(D // 128, 128), B_w_gate,
      B_w_up.reshape(4, D // 4, F), B_w_down.reshape(6, F // 6, D))
    return out.reshape(B, 1, D)


@jax.jit
def pallas_interleave_layers__sliding_block_cached__moe_arch_mod__decode_kernel(
    A_x: jax.Array,
    A_k_cache: jax.Array,
    A_v_cache: jax.Array,
    A_wq: jax.Array,
    A_wo: jax.Array,
    B_x: jax.Array,
    B_w_r: jax.Array,
    B_w_gate: jax.Array,
    B_w_up: jax.Array,
    B_w_down: jax.Array,
):
    del B_x
    return _call(CFG, A_x, A_k_cache, A_v_cache, A_wq, A_wo, B_w_r, B_w_gate, B_w_up, B_w_down)
```
